```python
import jax
import jax.numpy as jnp

def _softmax(x, axis=-1):
    return jax.nn.softmax(x, axis=axis)
def _gelu(x):
    return jax.nn.gelu(x, approximate=True)
def _silu(x):
    return jax.nn.silu(x)
def _sigmoid(x):
    return jax.nn.sigmoid(x)
def _layernorm(x, axis=-1, eps=1e-5):
    m = jnp.mean(x, axis=axis, keepdims=True)
    v = jnp.var(x, axis=axis, keepdims=True)
    return (x - m) / jnp.sqrt(v + eps)
def _scatter_add(tgt, idx, src, axis=0):
    return tgt.at[idx].add(src)
def _segment_sum(src, seg, n):
    return jax.ops.segment_sum(src, seg, n)
class _Rng:
    def __init__(self, key):
        self._k = key
    def _next(self):
        self._k, sub = jax.random.split(self._k)
        return sub
    def normal(self, shape):
        return jax.random.normal(self._next(), shape, dtype=jnp.bfloat16)
    def randint(self, lo, hi, shape):
        return jax.random.randint(self._next(), shape, lo, hi, dtype=jnp.int32)
    def uniform(self, shape, lo=0.0, hi=1.0):
        return jax.random.uniform(self._next(), shape, jnp.bfloat16, lo, hi)
    def permutation(self, n):
        return jax.random.permutation(self._next(), n)


kernel_name = 'standalone__adm_resblock__diffusion'

def setup_inputs():
    _rng = _Rng(jax.random.key(int.from_bytes(__import__("os").urandom(4), "little")))
    _w = (lambda a: (lambda t: t.astype(jnp.bfloat16) if jnp.issubdtype(t.dtype, jnp.floating) else t)(jnp.asarray(a)))
    B, C, HW, E = 2, 512, 64, 1152
    sc = (9.0 * C) ** -0.5
    return {
        "x": _w((lambda *s: _rng.normal(s) * 0.05)(B, C, HW, HW)),
        "t_emb": _w((lambda *s: _rng.normal(s) * 0.05)(B, E)),
        "g1": _w(1.0 + 0.1 * (lambda *s: _rng.normal(s) * 0.05)(C)),
        "be1": _w(0.1 * (lambda *s: _rng.normal(s) * 0.05)(C)),
        "w1": _w((lambda *s: _rng.normal(s) * 0.05)(C, C, 3, 3) * sc),
        "w_emb": _w((lambda *s: _rng.normal(s) * 0.05)(E, C) * (E ** -0.5)),
        "g2": _w(1.0 + 0.1 * (lambda *s: _rng.normal(s) * 0.05)(C)),
        "be2": _w(0.1 * (lambda *s: _rng.normal(s) * 0.05)(C)),
        "w2": _w((lambda *s: _rng.normal(s) * 0.05)(C, C, 3, 3) * sc),
    }

def reference(x, t_emb, g1, be1, w1, w_emb, g2, be2, w2):
    B, C, H, W = x.shape
    G, eps = 4, 1e-5
    def gn(z, gamma, beta):
        zr = z.reshape(B, G, (C // G) * H * W)
        mu = zr.mean(-1).reshape(B, G, 1)
        var = ((zr - mu) ** 2).mean(-1).reshape(B, G, 1)
        zn = ((zr - mu) / jnp.sqrt(var + eps)).reshape(B, C, H, W)
        return zn * gamma.reshape(1, C, 1, 1) + beta.reshape(1, C, 1, 1)
    def conv3(z, w):
        zp = jnp.pad(z, ((0, 0), (0, 0), (1, 1), (1, 1)))
        taps = [jnp.einsum("bchw,oc->bohw", zp[:, :, i:i+H, j:j+W], w[:, :, i, j]) for i in range(3) for j in range(3)]
        out = taps[0]
        for t in taps[1:]:
            out = out + t
        return out
    h = conv3(_silu(gn(x, g1, be1)), w1)
    emb = _silu(t_emb) @ w_emb
    h = h + emb.reshape(B, C, 1, 1)
    h = conv3(_silu(gn(h, g2, be2)), w2)
    return x + h
```

```python
import jax
import jax.numpy as jnp
from jax import lax
from jax.experimental import pallas as pl
from jax.experimental.pallas import tpu as pltpu

f32 = jnp.float32
bf16 = jnp.bfloat16
u32 = jnp.uint32
NT = (((1,), (1,)), ((), ()))


def build(B, C, H, W, E, TM=512, opts=None):
    opts = opts or {}
    HW = H * W
    G = 4
    CG = C // G
    assert CG == 128 and B == 2
    EPS = 1e-5
    T = HW // TM
    R = TM + 2 * W
    NCH = R // W
    NCB = C // 128
    NSTEP = 4 * T
    ER = opts.get('er', 32)
    NER = TM // ER
    XT = 2
    use_dep = opts.get('dep', 1)
    last_slot = opts.get('last_slot', 34)
    scope = jax.named_scope

    PW = opts.get('pw', 256)
    NPW = C // PW
    SUB = opts.get('sub', 4)
    XR = opts.get('xr', 64)
    NXR = TM // XR

    def marker_of(d, n, sub=0):
        rp = sub * (TM // SUB)
        m = d[rp:rp + 8, n * 128:(n + 1) * 128]
        b = pltpu.bitcast(m, u32)
        z = pltpu.bitcast((b >> 16) >> 16, f32)
        if PW > 128:
            z = jnp.concatenate([z] * (PW // 128), axis=1)
        return z

    def act(s_ref, p_ref, q, rc, nrows, cs, marker):
        v = s_ref[q, pl.ds(rc, nrows), cs].astype(f32)
        mu = p_ref[q, 0, :, cs]
        sc = p_ref[q, 1, :, cs]
        bt = p_ref[q, 2, :, cs]
        if marker is not None:
            mu = mu + marker
        v3 = v.reshape(nrows // 8, 8, PW)
        hz = ((v3 - mu[None]) * sc[None] + bt[None]).reshape(nrows, PW)
        return hz * jnp.tanh(hz) + hz

    HR = W // 2

    def produce_sub(s_ref, p_ref, z_ref, q, row0, k, cb, part, carry, marker, edge):
        r = row0 + W * k
        rc = pl.multiple_of(jnp.clip(r, 0, HW - W) + part * HR, HR)
        cs = slice(cb * PW, (cb + 1) * PW)
        a = act(s_ref, p_ref, q, rc, HR, cs, marker)
        if edge:
            valid = jnp.logical_and(r >= 0, r < HW)
            a = jnp.where(valid, a, 0.0)
        zb = W * k if isinstance(k, int) else pl.multiple_of(W * k, W)
        if part == 0:
            row = lax.broadcasted_iota(jnp.int32, (HR, PW), 0)
            am = jnp.where(row == 0, 0.0, pltpu.roll(a, 1, 0))
            ap = pltpu.roll(a, HR - 1, 0)[0:HR - 8]
            z_ref[0, pl.ds(zb, HR), cs] = am.astype(bf16)
            z_ref[1, pl.ds(zb, HR), cs] = a.astype(bf16)
            z_ref[2, pl.ds(zb, HR - 8), cs] = ap.astype(bf16)
            return a[HR - 8:HR]
        else:
            ext = jnp.concatenate([carry, a], axis=0)
            am = pltpu.roll(ext, 1, 0)[8:HR + 8]
            row = lax.broadcasted_iota(jnp.int32, (HR + 8, PW), 0)
            ap = jnp.where(row == HR + 7, 0.0, pltpu.roll(ext, HR + 7, 0))
            z_ref[0, pl.ds(zb + HR, HR), cs] = am.astype(bf16)
            z_ref[1, pl.ds(zb + HR, HR), cs] = a.astype(bf16)
            z_ref[2, pl.ds(zb + HR - 8, HR + 8), cs] = ap.astype(bf16)
            return None

    def stat_acc(v, state, marker=None):
        n = v.shape[0] // 8
        wd = v.shape[1]
        if state is None:
            K = v[0:1, :]
            if marker is not None:
                K = K + marker[0:1, :]
            d = v - K
            return (K, d.reshape(n, 8, wd).sum(axis=0), (d * d).reshape(n, 8, wd).sum(axis=0))
        K, s1, s2 = state
        Kd = K if marker is None else K + marker[0:1, :]
        d = v - Kd
        return (K, s1 + d.reshape(n, 8, wd).sum(axis=0), s2 + (d * d).reshape(n, 8, wd).sum(axis=0))

    def store_stats(st_ref, q, t, cb, state):
        K, s1, s2 = state
        cs = slice(cb * PW, (cb + 1) * PW)
        st_ref[q, t, 0, :, cs] = jnp.broadcast_to(K, (8, PW))
        st_ref[q, t, 1, :, cs] = jnp.broadcast_to(s1.sum(axis=0, keepdims=True), (8, PW))
        st_ref[q, t, 2, :, cs] = jnp.broadcast_to(s2.sum(axis=0, keepdims=True), (8, PW))

    def finalize(st_ref, p_ref, gb_ref, e_ref, q):
        cv = q // 2
        for g in range(G):
            cs = slice(g * 128, (g + 1) * 128)
            K = st_ref[q, :, 0, :, cs]
            s1 = st_ref[q, :, 1, :, cs]
            s2 = st_ref[q, :, 2, :, cs]
            e = e_ref[q, :, cs]
            mean_t = K + s1 * (1.0 / TM) + e[None]
            m2_t = s2 - s1 * s1 * (1.0 / TM)
            mu = jnp.sum(jnp.sum(mean_t, axis=0), axis=1, keepdims=True) * (1.0 / (T * 128))
            dev = mean_t - mu[None]
            tot = m2_t + dev * dev * float(TM)
            var = jnp.sum(jnp.sum(tot, axis=0), axis=1, keepdims=True) * (1.0 / (HW * 128))
            rstd = lax.rsqrt(var + EPS)
            p_ref[q, 0, :, cs] = mu - e
            p_ref[q, 1, :, cs] = gb_ref[cv, 0, :, cs] * (rstd * 0.5)
            p_ref[q, 2, :, cs] = gb_ref[cv, 1, :, cs] * 0.5

    def kern(x_hbm, te_hbm, g1_hbm, b1_hbm, w1_hbm, we_hbm, g2_hbm, b2_hbm, w2_hbm, o_hbm,
             s_ref, w_ref, za_ref, zb_ref, acca_ref, accb_ref, st_ref, p_ref, gb_ref, e_ref,
             te_ref, we_ref, gsm_ref, sem_x, sem_w, sem_s, sem_o):

        def x_copy(b, c):
            r0 = c * TM if isinstance(c, int) else pl.multiple_of(c * TM, TM)
            return pltpu.make_async_copy(x_hbm.at[b, pl.ds(r0, TM), :],
                                         s_ref.at[b, pl.ds(r0, TM), :], sem_x.at[b, c])

        def w_copy(cv, tap):
            src = w1_hbm if cv == 0 else w2_hbm
            return pltpu.make_async_copy(src.at[tap], w_ref.at[cv * 9 + tap], sem_w.at[cv, tap])

        def small_copies():
            return [pltpu.make_async_copy(g1_hbm, gsm_ref.at[0], sem_s.at[0]),
                    pltpu.make_async_copy(b1_hbm, gsm_ref.at[1], sem_s.at[1]),
                    pltpu.make_async_copy(g2_hbm, gsm_ref.at[2], sem_s.at[2]),
                    pltpu.make_async_copy(b2_hbm, gsm_ref.at[3], sem_s.at[3]),
                    pltpu.make_async_copy(te_hbm, te_ref, sem_s.at[4])]

        def we_copy():
            return pltpu.make_async_copy(we_hbm, we_ref, sem_s.at[5])

        def o_copy(s):
            b = s // T - 2
            t = s % T
            r0 = t * TM if isinstance(t, int) else pl.multiple_of(t * TM, TM)
            return pltpu.make_async_copy(s_ref.at[b, pl.ds(r0, TM), :], o_hbm.at[b, pl.ds(r0, TM), :], sem_o.at[0])

        def epi_piece(acc_ref, s_prev, cb, ri, state, marker):
            p = s_prev // T
            t = s_prev % T
            is2 = p >= 2
            dst = jnp.where(is2, p - 2, p + 2)
            cs = slice(cb * PW, (cb + 1) * PW)
            r0 = pl.multiple_of(t * TM + ri * ER, ER)
            a = acc_ref[ri * ER:(ri + 1) * ER, cs]
            if marker is not None:
                a = (a.reshape(ER // 8, 8, PW) + marker[None]).reshape(ER, PW)
            xr = s_ref[dst, pl.ds(r0, ER), cs].astype(f32)
            res = a + jnp.where(is2, xr, 0.0)
            state = stat_acc(res, state)
            s_ref[dst, pl.ds(r0, ER), cs] = res.astype(bf16)
            if ri == NER - 1:
                store_stats(st_ref, jnp.where(is2, 0, p + 2), t, cb, state)
                state = None
            return state

        def xstat_piece(q, tile, cb, ri, state, marker):
            cs = slice(cb * PW, (cb + 1) * PW)
            r0 = tile * TM + ri * XR
            if not isinstance(r0, int):
                r0 = pl.multiple_of(r0, XR)
            v = s_ref[q, pl.ds(r0, XR), cs].astype(f32)
            state = stat_acc(v, state, marker)
            if ri == NXR - 1:
                store_stats(st_ref, q, tile, cb, state)
                state = None
            return state

        def merge(lists):
            items = []
            for li, l in enumerate(lists):
                for i, it in enumerate(l):
                    items.append(((i + 0.5) / len(l), li, it))
            items.sort(key=lambda z: (z[0], z[1]))
            return [it for _, _, it in items]

        def half(s, zc_ref, zn_ref, accc_ref, accp_ref, do_prod, do_epi, do_x, do_fin):
            conv = s // (2 * T)
            if opts.get('staticw') == 1:
                conv = 1
            sn = s + 1
            pn = sn // T
            tn = sn % T
            lists = []
            if do_prod:
                lists.append([('p', k, cb, part) for k in range(NCH) for cb in range(NPW) for part in range(2)])
            if do_epi:
                lists.append([('e', cb, ri) for cb in range(NPW) for ri in range(NER)])
            if do_x:
                lists.append([('x', tl, cb, ri) for tl in range(XT) for cb in range(NPW) for ri in range(NXR)])
            pieces = merge(lists)
            npc = len(pieces)
            if do_fin:
                finalize(st_ref, p_ref, gb_ref, e_ref, jnp.minimum(s // T + 1, 3))
            xj = jnp.clip(s - 1, 0, T // XT - 1) * XT
            done = 0
            acc = None
            est = None
            xst = None
            pcar = None
            nslots = last_slot * SUB
            for i in range(3):
                for j in range(3):
                    tap = i * 3 + j
                    wv = w_ref[conv * 9 + tap]
                    d = lax.dot_general(zc_ref[j, pl.ds(W * i, TM), :], wv, NT,
                                        preferred_element_type=f32)
                    for nn in range(4 * SUB):
                        n, sub = nn // SUB, nn % SUB
                        slot = tap * 4 * SUB + nn
                        hi_ = min(npc, ((slot + 1) * npc) // nslots)
                        while done < hi_:
                            pc = pieces[done]
                            marker = marker_of(d, n, sub) if use_dep else None
                            if pc[0] == 'p':
                                pcar = produce_sub(s_ref, p_ref, zn_ref, pn, tn * TM - W, pc[1], pc[2], pc[3], pcar,
                                                   marker, pc[1] == 0 or pc[1] == NCH - 1)
                            elif pc[0] == 'e':
                                est = epi_piece(accp_ref, s - 1, pc[1], pc[2], est, marker)
                            else:
                                xst = xstat_piece(1, xj + pc[1], pc[2], pc[3], xst, marker)
                            done += 1
                    acc = d if acc is None else acc + d
            accc_ref[...] = acc

        with scope('prologue'):
            for c in small_copies():
                c.start()
            lax.fori_loop(0, T, lambda c, _: (x_copy(0, c).start(), 0)[1], 0)
            lax.fori_loop(0, 9, lambda c, _: (w_copy(0, c).start(), 0)[1], 0)
            lax.fori_loop(0, T, lambda c, _: (x_copy(1, c).start(), 0)[1], 0)
            we_copy().start()
            lax.fori_loop(0, 9, lambda c, _: (w_copy(1, c).start(), 0)[1], 0)

            for c in small_copies():
                c.wait()
            for cv in range(2):
                for k in range(2):
                    v = gsm_ref[2 * cv + k].astype(f32)
                    for g in range(G):
                        gb_ref[cv, k, :, g * 128:(g + 1) * 128] = jnp.broadcast_to(v[g:g + 1, :], (8, 128))
            e_ref[...] = jnp.zeros(e_ref.shape, f32)
            st_ref[...] = jnp.zeros(st_ref.shape, f32)

            def xs0(c, _):
                x_copy(0, c).wait()
                for cb in range(NPW):
                    st = None
                    for ri in range(NXR):
                        st = xstat_piece(0, c, cb, ri, st, None)
                return 0
            lax.fori_loop(0, T, xs0, 0)
            finalize(st_ref, p_ref, gb_ref, e_ref, 0)

            def prod0(k, _):
                for cb in range(NPW):
                    car = None
                    for part in range(2):
                        car = produce_sub(s_ref, p_ref, za_ref, 0, -W, k, cb, part, car, None, True)
                return 0
            lax.fori_loop(0, NCH, prod0, 0)

        KPER = -(-NCH // 3)

        def first(i, _):
            for j in range(3):
                w_copy(0, 3 * i + j).wait()
            acc = None
            pieces = [(kk, cb, part) for kk in range(KPER) for cb in range(NPW) for part in range(2)]
            done = 0
            car = None
            r0 = pl.multiple_of(W * i, W)
            for j in range(3):
                wv = w_ref[3 * i + j]
                d = lax.dot_general(za_ref[j, pl.ds(r0, TM), :], wv, NT,
                                    preferred_element_type=f32)
                for nn in range(4 * SUB):
                    n, sub = nn // SUB, nn % SUB
                    slot = j * 4 * SUB + nn
                    hi_ = min(len(pieces), ((slot + 1) * len(pieces)) // (11 * SUB))
                    while done < hi_:
                        kk, cb, part = pieces[done]
                        k = jnp.minimum(i * KPER + kk, NCH - 1)
                        car = produce_sub(s_ref, p_ref, zb_ref, 0, TM - W, k, cb, part, car,
                                          marker_of(d, n, sub) if use_dep else None, True)
                        done += 1
                acc = d if acc is None else acc + d
            prev = jnp.where(i == 0, 0.0, acca_ref[...])
            acca_ref[...] = prev + acc
            return 0

        acca_ref[...] = jnp.zeros(acca_ref.shape, f32)
        with scope('first'):
            if opts.get('nofirst'):
                for tap in range(9):
                    w_copy(0, tap).wait()
            else:
                lax.fori_loop(0, 3, first, 0)

        with scope('mid'):
            for c in range(T):
                x_copy(1, c).wait()
            we_copy().wait()
            te = te_ref[...].astype(f32)
            sl = te * jax.nn.sigmoid(te)
            emb = jnp.dot(sl.astype(bf16), we_ref[...], preferred_element_type=f32)
            e_ref[2] = jnp.broadcast_to(emb[0:1, :], (8, C))
            e_ref[3] = jnp.broadcast_to(emb[1:2, :], (8, C))

        NIT = (NSTEP - 2) // 2

        def body(it, carry):
            s0 = 2 * it + 1
            s1 = s0 + 1

            if not opts.get('w2early'):
                @pl.when(it == 2)
                def _():
                    for tap in range(9):
                        w_copy(1, tap).wait()

            with scope('iter'):
                half(s0, zb_ref, za_ref, accb_ref, acca_ref, not opts.get('nop'), not opts.get('noe'), not opts.get('nox'), False)
                half(s1, za_ref, zb_ref, acca_ref, accb_ref, not opts.get('nop'), not opts.get('noe'), not opts.get('nox'), not opts.get('nof'))

            if not opts.get('noo'):
                @pl.when(s0 - 1 >= 2 * T)
                def _():
                    o_copy(s0 - 1).start()

                @pl.when(s1 - 1 >= 2 * T)
                def _():
                    o_copy(s1 - 1).start()
            return carry

        if opts.get('w2early'):
            for tap in range(9):
                w_copy(1, tap).wait()
        with scope('main'):
            lax.fori_loop(0, NIT, body, 0)

        with scope('last'):
            sl_ = NSTEP - 1
            if not opts.get('nolast'):
                half(sl_, zb_ref, za_ref, accb_ref, acca_ref, False, True, False, False)
            o_copy(sl_ - 1).start()
        with scope('final'):
            for cb in range(NPW):
                st = None
                for ri in range(NER):
                    st = epi_piece(accb_ref, sl_, cb, ri, st, None)
            o_copy(sl_).start()
        with scope('owait'):
            for s in range(2 * T if not opts.get('noo') else NSTEP - 2, NSTEP):
                o_copy(s).wait()

    def fn(x, t_emb, g1, be1, w1, w_emb, g2, be2, w2):
        xn = jnp.transpose(x, (0, 2, 3, 1)).reshape(B, HW, C)
        w1t = jnp.transpose(w1, (2, 3, 0, 1)).reshape(9, C, C)
        w2t = jnp.transpose(w2, (2, 3, 0, 1)).reshape(9, C, C)
        any_spec = pl.BlockSpec(memory_space=pl.ANY)
        out = pl.pallas_call(
            kern,
            in_specs=[any_spec] * 9,
            out_specs=any_spec,
            out_shape=jax.ShapeDtypeStruct((B, HW, C), bf16),
            scratch_shapes=[
                pltpu.VMEM((4, HW, C), bf16),
                pltpu.VMEM((18, C, C), bf16),
                pltpu.VMEM((3, R, C), bf16),
                pltpu.VMEM((3, R, C), bf16),
                pltpu.VMEM((TM, C), f32),
                pltpu.VMEM((TM, C), f32),
                pltpu.VMEM((4, T, 3, 8, C), f32),
                pltpu.VMEM((4, 3, 8, C), f32),
                pltpu.VMEM((2, 2, 8, C), f32),
                pltpu.VMEM((4, 8, C), f32),
                pltpu.VMEM((B, E), bf16),
                pltpu.VMEM((E, C), bf16),
                pltpu.VMEM((4, G, 128), bf16),
                pltpu.SemaphoreType.DMA((2, T)),
                pltpu.SemaphoreType.DMA((2, 9)),
                pltpu.SemaphoreType.DMA((6,)),
                pltpu.SemaphoreType.DMA((1,)),
            ],
            compiler_params=pltpu.CompilerParams(vmem_limit_bytes=100 * 1024 * 1024, disable_bounds_checks=bool(opts.get('nobc', 0))),
        )(xn, t_emb, g1.reshape(G, 128), be1.reshape(G, 128), w1t, w_emb,
          g2.reshape(G, 128), be2.reshape(G, 128), w2t)
        return jnp.transpose(out.reshape(B, H, W, C), (0, 3, 1, 2))
    return fn


_OPTS = {'nobc': 1}


@jax.jit
def pallas_standalone__adm_resblock__diffusion_kernel(x, t_emb, g1, be1, w1, w_emb, g2, be2, w2):
    B, C, H, W = x.shape
    E = t_emb.shape[1]
    return build(B, C, H, W, E, TM=512, opts=_OPTS)(x, t_emb, g1, be1, w1, w_emb, g2, be2, w2)
```

```python
import jax
import jax.numpy as jnp
from jax import lax
from jax.experimental import pallas as pl
from jax.experimental.pallas import tpu as pltpu

f32 = jnp.float32
bf16 = jnp.bfloat16
u32 = jnp.uint32
NT = (((1,), (1,)), ((), ()))


def build(B, C, H, W, E, TM=512, opts=None):
    opts = opts or {}
    HW = H * W
    G = 4
    CG = C // G
    assert CG == 128 and B == 2
    EPS = 1e-5
    T = HW // TM
    R = TM + 2 * W
    NCH = R // W
    NCB = C // 128
    NSTEP = 4 * T
    ER = opts.get('er', 32)
    NER = TM // ER
    XT = 2
    use_dep = opts.get('dep', 1)
    last_slot = opts.get('last_slot', 34)
    scope = jax.named_scope

    PW = opts.get('pw', 256)
    NPW = C // PW
    SUB = opts.get('sub', 4)
    XR = opts.get('xr', 64)
    NXR = TM // XR

    assert T == 8
    def divT(v):
        return v // T if isinstance(v, int) else lax.shift_right_logical(v, 3)

    def modT(v):
        return v % T if isinstance(v, int) else jnp.bitwise_and(v, T - 1)

    def marker_of(d, n, sub=0):
        rp = sub * (TM // SUB)
        m = d[rp:rp + 8, n * 128:(n + 1) * 128]
        b = pltpu.bitcast(m, u32)
        z = pltpu.bitcast((b >> 16) >> 16, f32)
        if PW > 128:
            z = jnp.concatenate([z] * (PW // 128), axis=1)
        return z

    def act(s_ref, pv, q, rc, nrows, cs, marker):
        v = s_ref[q, pl.ds(rc, nrows), cs].astype(f32)
        mu = pv[0][:, cs]
        sc = pv[1][:, cs]
        bt = pv[2][:, cs]
        if marker is not None:
            mu = mu + marker
        v3 = v.reshape(nrows // 8, 8, PW)
        hz = ((v3 - mu[None]) * sc[None] + bt[None]).reshape(nrows, PW)
        return hz * jnp.tanh(hz) + hz

    def load_p(p_ref, q):
        return tuple(p_ref[q, k] for k in range(3))

    HR = W // 2
    ZU = opts.get('zu', 0)

    def produce_sub(s_ref, pv, z_ref, q, row0, k, cb, part, carry, marker, edge):
        r = row0 + W * k
        rc = pl.multiple_of(jnp.clip(r, 0, HW - W) + part * HR, HR)
        cs = slice(cb * PW, (cb + 1) * PW)
        a = act(s_ref, pv, q, rc, HR, cs, marker)
        if edge:
            valid = jnp.logical_and(r >= 0, r < HW)
            a = jnp.where(valid, a, 0.0)
        zb = W * k if isinstance(k, int) else pl.multiple_of(W * k, W)
        if ZU:
            zh = zb // 2 if isinstance(zb, int) else pl.multiple_of(zb // 2, W // 2)
            pk = lambda t: pltpu.bitcast(t.astype(bf16), u32)
            HH = HR // 2
            if part == 0:
                row = lax.broadcasted_iota(jnp.int32, (HR, PW), 0)
                am = jnp.where(row == 0, 0.0, pltpu.roll(a, 1, 0))
                ap = pltpu.roll(a, HR - 1, 0)[0:HR - 16]
                z_ref[0, pl.ds(zh, HH), cs] = pk(am)
                z_ref[1, pl.ds(zh, HH), cs] = pk(a)
                z_ref[2, pl.ds(zh, HH - 8), cs] = pk(ap)
                return a[HR - 16:HR]
            else:
                ext = jnp.concatenate([carry, a], axis=0)
                am = pltpu.roll(ext, 1, 0)[16:HR + 16]
                row = lax.broadcasted_iota(jnp.int32, (HR + 16, PW), 0)
                ap = jnp.where(row == HR + 15, 0.0, pltpu.roll(ext, HR + 15, 0))
                z_ref[0, pl.ds(zh + HH, HH), cs] = pk(am)
                z_ref[1, pl.ds(zh + HH, HH), cs] = pk(a)
                z_ref[2, pl.ds(zh + HH - 8, HH + 8), cs] = pk(ap)
                return None
        if part == 0:
            row = lax.broadcasted_iota(jnp.int32, (HR, PW), 0)
            am = jnp.where(row == 0, 0.0, pltpu.roll(a, 1, 0))
            ap = pltpu.roll(a, HR - 1, 0)[0:HR - 8]
            z_ref[0, pl.ds(zb, HR), cs] = am.astype(bf16)
            z_ref[1, pl.ds(zb, HR), cs] = a.astype(bf16)
            z_ref[2, pl.ds(zb, HR - 8), cs] = ap.astype(bf16)
            return a[HR - 8:HR]
        else:
            ext = jnp.concatenate([carry, a], axis=0)
            am = pltpu.roll(ext, 1, 0)[8:HR + 8]
            row = lax.broadcasted_iota(jnp.int32, (HR + 8, PW), 0)
            ap = jnp.where(row == HR + 7, 0.0, pltpu.roll(ext, HR + 7, 0))
            z_ref[0, pl.ds(zb + HR, HR), cs] = am.astype(bf16)
            z_ref[1, pl.ds(zb + HR, HR), cs] = a.astype(bf16)
            z_ref[2, pl.ds(zb + HR - 8, HR + 8), cs] = ap.astype(bf16)
            return None

    def zload(z_ref, j, r0):
        if ZU:
            rh = r0 // 2 if isinstance(r0, int) else pl.multiple_of(r0 // 2, W // 2)
            return pltpu.bitcast(z_ref[j, pl.ds(rh, TM // 2), :], bf16)
        return z_ref[j, pl.ds(r0, TM), :]

    def stat_acc(v, state, marker=None):
        n = v.shape[0] // 8
        wd = v.shape[1]
        if state is None:
            K = v[0:1, :]
            if marker is not None:
                K = K + marker[0:1, :]
            d = v - K
            return (K, d.reshape(n, 8, wd).sum(axis=0), (d * d).reshape(n, 8, wd).sum(axis=0))
        K, s1, s2 = state
        Kd = K if marker is None else K + marker[0:1, :]
        d = v - Kd
        return (K, s1 + d.reshape(n, 8, wd).sum(axis=0), s2 + (d * d).reshape(n, 8, wd).sum(axis=0))

    def store_stats(st_ref, q, t, cb, state):
        K, s1, s2 = state
        cs = slice(cb * PW, (cb + 1) * PW)
        st_ref[q, t, 0, :, cs] = jnp.broadcast_to(K, (8, PW))
        st_ref[q, t, 1, :, cs] = jnp.broadcast_to(s1.sum(axis=0, keepdims=True), (8, PW))
        st_ref[q, t, 2, :, cs] = jnp.broadcast_to(s2.sum(axis=0, keepdims=True), (8, PW))

    def finalize(st_ref, p_ref, gb_ref, e_ref, q):
        cv = q // 2
        for g in range(G):
            cs = slice(g * 128, (g + 1) * 128)
            K = st_ref[q, :, 0, :, cs]
            s1 = st_ref[q, :, 1, :, cs]
            s2 = st_ref[q, :, 2, :, cs]
            e = e_ref[q, :, cs]
            mean_t = K + s1 * (1.0 / TM) + e[None]
            m2_t = s2 - s1 * s1 * (1.0 / TM)
            mu = jnp.sum(jnp.sum(mean_t, axis=0), axis=1, keepdims=True) * (1.0 / (T * 128))
            dev = mean_t - mu[None]
            tot = m2_t + dev * dev * float(TM)
            var = jnp.sum(jnp.sum(tot, axis=0), axis=1, keepdims=True) * (1.0 / (HW * 128))
            rstd = lax.rsqrt(var + EPS)
            p_ref[q, 0, :, cs] = mu - e
            p_ref[q, 1, :, cs] = gb_ref[cv, 0, :, cs] * (rstd * 0.5)
            p_ref[q, 2, :, cs] = gb_ref[cv, 1, :, cs] * 0.5

    def kern(x_hbm, te_hbm, g1_hbm, b1_hbm, w1_hbm, we_hbm, g2_hbm, b2_hbm, w2_hbm, o_hbm,
             s_ref, w_ref, za_ref, zb_ref, acca_ref, accb_ref, st_ref, p_ref, gb_ref, e_ref,
             te_ref, we_ref, gsm_ref, sem_x, sem_w, sem_s, sem_o):

        def x_copy(c):
            r0 = c * TM if isinstance(c, int) else pl.multiple_of(c * TM, TM)
            return pltpu.make_async_copy(x_hbm.at[0, pl.ds(r0, TM), :],
                                         s_ref.at[0, pl.ds(r0, TM), :], sem_x.at[c])

        def x1_copy():
            return pltpu.make_async_copy(x_hbm.at[1], s_ref.at[1], sem_s.at[6])

        def w1_copy(i):
            return pltpu.make_async_copy(w1_hbm.at[pl.ds(3 * i, 3)], w_ref.at[pl.ds(3 * i, 3)], sem_w.at[i])

        def w2_copy():
            return pltpu.make_async_copy(w2_hbm, w_ref.at[pl.ds(9, 9)], sem_s.at[7])

        def small_copies():
            return [pltpu.make_async_copy(g1_hbm, gsm_ref.at[0], sem_s.at[0]),
                    pltpu.make_async_copy(b1_hbm, gsm_ref.at[1], sem_s.at[1]),
                    pltpu.make_async_copy(g2_hbm, gsm_ref.at[2], sem_s.at[2]),
                    pltpu.make_async_copy(b2_hbm, gsm_ref.at[3], sem_s.at[3]),
                    pltpu.make_async_copy(te_hbm, te_ref, sem_s.at[4])]

        def we_copy():
            return pltpu.make_async_copy(we_hbm, we_ref, sem_s.at[5])

        def o_copy(s):
            b = divT(s) - 2
            t = modT(s)
            r0 = t * TM if isinstance(t, int) else pl.multiple_of(t * TM, TM)
            return pltpu.make_async_copy(s_ref.at[b, pl.ds(r0, TM), :], o_hbm.at[b, pl.ds(r0, TM), :], sem_o.at[0])

        def epi_piece(acc_ref, s_prev, cb, ri, state, marker):
            p = divT(s_prev)
            t = modT(s_prev)
            is2 = p >= 2
            dst = jnp.where(is2, p - 2, p + 2)
            cs = slice(cb * PW, (cb + 1) * PW)
            r0 = pl.multiple_of(t * TM + ri * ER, ER)
            a = acc_ref[ri * ER:(ri + 1) * ER, cs]
            if marker is not None:
                a = (a.reshape(ER // 8, 8, PW) + marker[None]).reshape(ER, PW)
            xr = s_ref[dst, pl.ds(r0, ER), cs].astype(f32)
            res = a + jnp.where(is2, xr, 0.0)
            state = stat_acc(res, state)
            s_ref[dst, pl.ds(r0, ER), cs] = res.astype(bf16)
            if ri == NER - 1:
                store_stats(st_ref, jnp.where(is2, 0, p + 2), t, cb, state)
                state = None
            return state

        def xstat_piece(q, tile, cb, ri, state, marker):
            cs = slice(cb * PW, (cb + 1) * PW)
            r0 = tile * TM + ri * XR
            if not isinstance(r0, int):
                r0 = pl.multiple_of(r0, XR)
            v = s_ref[q, pl.ds(r0, XR), cs].astype(f32)
            state = stat_acc(v, state, marker)
            if ri == NXR - 1:
                store_stats(st_ref, q, tile, cb, state)
                state = None
            return state

        def merge(lists):
            items = []
            for li, l in enumerate(lists):
                for i, it in enumerate(l):
                    items.append(((i + 0.5) / len(l), li, it))
            items.sort(key=lambda z: (z[0], z[1]))
            return [it for _, _, it in items]

        def half(s, zc_ref, zn_ref, accc_ref, accp_ref, do_prod, do_epi, do_x, do_fin, wstat=None):
            is_c2 = s >= 2 * T
            sn = s + 1
            pn = divT(sn)
            tn = modT(sn)
            lists = []
            if do_prod:
                lists.append([('p', k, cb, part) for k in range(NCH) for cb in range(NPW) for part in range(2)])
            if do_epi:
                lists.append([('e', cb, ri) for cb in range(NPW) for ri in range(NER)])
            if do_x:
                lists.append([('x', tl, cb, ri) for tl in range(XT) for cb in range(NPW) for ri in range(NXR)])
            pieces = merge(lists)
            npc = len(pieces)
            if do_fin:
                finalize(st_ref, p_ref, gb_ref, e_ref, jnp.minimum(divT(s - 1) + 1, 3))
            pv = load_p(p_ref, pn) if do_prod else None
            xj = jnp.clip(s - 3, 0, T // XT - 1) * XT
            xq = jnp.where(s < 3, 0, 1)
            done = 0
            acc = None
            est = None
            xst = None
            pcar = None
            nslots = last_slot * SUB
            for i in range(3):
                for j in range(3):
                    tap = i * 3 + j
                    if wstat is not None:
                        wv = w_ref[wstat * 9 + tap]
                    elif opts.get('dynw'):
                        wv = w_ref[jnp.where(is_c2, 9, 0) + tap]
                    else:
                        wv = pltpu.bitcast(jnp.where(is_c2, pltpu.bitcast(w_ref[9 + tap], u32),
                                                     pltpu.bitcast(w_ref[tap], u32)), bf16)
                    d = lax.dot_general(zload(zc_ref, j, W * i), wv, NT,
                                        preferred_element_type=f32)
                    for nn in range(4 * SUB):
                        n, sub = nn // SUB, nn % SUB
                        slot = tap * 4 * SUB + nn
                        hi_ = min(npc, ((slot + 1) * npc) // nslots)
                        while done < hi_:
                            pc = pieces[done]
                            marker = marker_of(d, n, sub) if use_dep else None
                            if pc[0] == 'p':
                                pcar = produce_sub(s_ref, pv, zn_ref, pn, tn * TM - W, pc[1], pc[2], pc[3], pcar,
                                                   marker, pc[1] == 0 or pc[1] == NCH - 1)
                            elif pc[0] == 'e':
                                est = epi_piece(accp_ref, s - 1, pc[1], pc[2], est, marker)
                            else:
                                xst = xstat_piece(xq, xj + pc[1], pc[2], pc[3], xst, marker)
                            done += 1
                    acc = d if acc is None else acc + d
            accc_ref[...] = acc

        with scope('prologue'):
            for c in small_copies():
                c.start()
            lax.fori_loop(0, T, lambda c, _: (x_copy(c).start(), 0)[1], 0)
            lax.fori_loop(0, 3, lambda c, _: (w1_copy(c).start(), 0)[1], 0)

            def rest(c, _):
                @pl.when(c == 0)
                def _():
                    w2_copy().start()

                @pl.when(c == 1)
                def _():
                    x1_copy().start()

                @pl.when(c == 2)
                def _():
                    we_copy().start()
                return 0
            lax.fori_loop(0, 3, rest, 0)

            for c in small_copies():
                c.wait()
            for cv in range(2):
                for k in range(2):
                    v = gsm_ref[2 * cv + k].astype(f32)
                    for g in range(G):
                        gb_ref[cv, k, :, g * 128:(g + 1) * 128] = jnp.broadcast_to(v[g:g + 1, :], (8, 128))
            e_ref[...] = jnp.zeros(e_ref.shape, f32)
            st_ref[...] = jnp.zeros(st_ref.shape, f32)

            def xs0(c, _):
                x_copy(c).wait()
                for cb in range(NPW):
                    st = None
                    for ri in range(NXR):
                        st = xstat_piece(0, c, cb, ri, st, None)
                return 0
            lax.fori_loop(0, T, xs0, 0)
            finalize(st_ref, p_ref, gb_ref, e_ref, 0)

            def prod0(k, _):
                for cb in range(NPW):
                    car = None
                    for part in range(2):
                        car = produce_sub(s_ref, load_p(p_ref, 0), za_ref, 0, -W, k, cb, part, car, None, True)
                return 0
            lax.fori_loop(0, NCH, prod0, 0)

        KPER = -(-NCH // 3)

        def first(i, _):
            w1_copy(i).wait()
            acc = None
            pieces = [(kk, cb, part) for kk in range(KPER) for cb in range(NPW) for part in range(2)]
            done = 0
            car = None
            pv = load_p(p_ref, 0)
            r0 = pl.multiple_of(W * i, W)
            for j in range(3):
                wv = w_ref[3 * i + j]
                d = lax.dot_general(zload(za_ref, j, r0), wv, NT,
                                    preferred_element_type=f32)
                for nn in range(4 * SUB):
                    n, sub = nn // SUB, nn % SUB
                    slot = j * 4 * SUB + nn
                    hi_ = min(len(pieces), ((slot + 1) * len(pieces)) // (11 * SUB))
                    while done < hi_:
                        kk, cb, part = pieces[done]
                        k = jnp.minimum(i * KPER + kk, NCH - 1)
                        car = produce_sub(s_ref, pv, zb_ref, 0, TM - W, k, cb, part, car,
                                          marker_of(d, n, sub) if use_dep else None, True)
                        done += 1
                acc = d if acc is None else acc + d
            prev = jnp.where(i == 0, 0.0, acca_ref[...])
            acca_ref[...] = prev + acc
            return 0

        acca_ref[...] = jnp.zeros(acca_ref.shape, f32)
        with scope('first'):
            if opts.get('nofirst'):
                for i in range(3):
                    w1_copy(i).wait()
            else:
                lax.fori_loop(0, 3, first, 0)

        with scope('mid'):
            w2_copy().wait()

        NIT = (NSTEP - 2) // 2

        def body(it, carry):
            s0 = 2 * it + 1
            s1 = s0 + 1

            @pl.when(it == 1)
            def _():
                x1_copy().wait()
                we_copy().wait()
                te = te_ref[...].astype(f32)
                sl = te * jax.nn.sigmoid(te)
                emb = jnp.dot(sl.astype(bf16), we_ref[...], preferred_element_type=f32)
                e_ref[2] = jnp.broadcast_to(emb[0:1, :], (8, C))
                e_ref[3] = jnp.broadcast_to(emb[1:2, :], (8, C))

            with scope('iter'):
                half(s0, zb_ref, za_ref, accb_ref, acca_ref, not opts.get('nop'), not opts.get('noe'), not opts.get('nox'), not opts.get('nof'))
                half(s1, za_ref, zb_ref, acca_ref, accb_ref, not opts.get('nop'), not opts.get('noe'), not opts.get('nox'), False)

            if not opts.get('noo'):
                @pl.when(s0 - 1 >= 2 * T)
                def _():
                    o_copy(s0 - 1).start()

                @pl.when(s1 - 1 >= 2 * T)
                def _():
                    o_copy(s1 - 1).start()
            return carry

        with scope('main'):
            lax.fori_loop(0, NIT, body, 0)

        with scope('last'):
            sl_ = NSTEP - 1
            if not opts.get('nolast'):
                half(sl_, zb_ref, za_ref, accb_ref, acca_ref, False, True, False, False, wstat=1)
            o_copy(sl_ - 1).start()
        with scope('final'):
            for cb in range(NPW):
                st = None
                for ri in range(NER):
                    st = epi_piece(accb_ref, sl_, cb, ri, st, None)
            o_copy(sl_).start()
        with scope('owait'):
            for s in range(2 * T if not opts.get('noo') else NSTEP - 2, NSTEP):
                o_copy(s).wait()

    def fn(x, t_emb, g1, be1, w1, w_emb, g2, be2, w2):
        xn = jnp.transpose(x, (0, 2, 3, 1)).reshape(B, HW, C)
        w1t = jnp.transpose(w1, (2, 3, 0, 1)).reshape(9, C, C)
        w2t = jnp.transpose(w2, (2, 3, 0, 1)).reshape(9, C, C)
        any_spec = pl.BlockSpec(memory_space=pl.ANY)
        out = pl.pallas_call(
            kern,
            in_specs=[any_spec] * 9,
            out_specs=any_spec,
            out_shape=jax.ShapeDtypeStruct((B, HW, C), bf16),
            scratch_shapes=[
                pltpu.VMEM((4, HW, C), bf16),
                pltpu.VMEM((18, C, C), bf16),
                pltpu.VMEM((3, R // 2, C), u32) if ZU else pltpu.VMEM((3, R, C), bf16),
                pltpu.VMEM((3, R // 2, C), u32) if ZU else pltpu.VMEM((3, R, C), bf16),
                pltpu.VMEM((TM, C), f32),
                pltpu.VMEM((TM, C), f32),
                pltpu.VMEM((4, T, 3, 8, C), f32),
                pltpu.VMEM((4, 3, 8, C), f32),
                pltpu.VMEM((2, 2, 8, C), f32),
                pltpu.VMEM((4, 8, C), f32),
                pltpu.VMEM((B, E), bf16),
                pltpu.VMEM((E, C), bf16),
                pltpu.VMEM((4, G, 128), bf16),
                pltpu.SemaphoreType.DMA((T,)),
                pltpu.SemaphoreType.DMA((3,)),
                pltpu.SemaphoreType.DMA((8,)),
                pltpu.SemaphoreType.DMA((1,)),
            ],
            compiler_params=pltpu.CompilerParams(vmem_limit_bytes=100 * 1024 * 1024, disable_bounds_checks=bool(opts.get('nobc', 0))),
        )(xn, t_emb, g1.reshape(G, 128), be1.reshape(G, 128), w1t, w_emb,
          g2.reshape(G, 128), be2.reshape(G, 128), w2t)
        return jnp.transpose(out.reshape(B, H, W, C), (0, 3, 1, 2))
    return fn


_OPTS = {'nobc': 1, 'zu': 1}


@jax.jit
def pallas_standalone__adm_resblock__diffusion_kernel(x, t_emb, g1, be1, w1, w_emb, g2, be2, w2):
    B, C, H, W = x.shape
    E = t_emb.shape[1]
    return build(B, C, H, W, E, TM=512, opts=_OPTS)(x, t_emb, g1, be1, w1, w_emb, g2, be2, w2)
```

```python
import jax
import jax.numpy as jnp
from jax import lax
from jax.experimental import pallas as pl
from jax.experimental.pallas import tpu as pltpu

f32 = jnp.float32
bf16 = jnp.bfloat16
u32 = jnp.uint32
NT = (((1,), (1,)), ((), ()))


def build(B, C, H, W, E, TM=512, opts=None):
    opts = opts or {}
    HW = H * W
    G = 4
    CG = C // G
    EPS = 1e-5
    T = HW // TM
    assert CG == 128 and B == 2 and T == 8 and W == 64
    R = TM + 2 * W
    NCH = R // W
    NSTEP = 4 * T
    ER = opts.get('er', 32)
    NER = TM // ER
    XT = 2
    last_slot = opts.get('last_slot', 34)
    scope = jax.named_scope

    PW = opts.get('pw', 256)
    NPW = C // PW
    SUB = opts.get('sub', 4)
    XR = opts.get('xr', 64)
    NXR = TM // XR
    HR = W // 2
    HH = HR // 2

    def divT(v):
        return v // T if isinstance(v, int) else lax.shift_right_logical(v, 3)

    def modT(v):
        return v % T if isinstance(v, int) else jnp.bitwise_and(v, T - 1)

    def mult(v, m):
        return v if isinstance(v, int) else pl.multiple_of(v, m)

    def marker_of(d, n, sub, width):
        rp = sub * (TM // SUB)
        m = d[rp:rp + 8, n * 128:(n + 1) * 128]
        b = pltpu.bitcast(m, u32)
        z = pltpu.bitcast((b >> 16) >> 16, f32)
        if width > 128:
            z = jnp.concatenate([z] * (width // 128), axis=1)
        return z

    def pack(t):
        return pltpu.bitcast(t.astype(bf16), u32)

    def act(v, pv, marker):
        n, wd = v.shape
        mu, sc, bt = pv
        if marker is not None:
            mu = mu + marker
        v3 = v.reshape(n // 8, 8, wd)
        hz = ((v3 - mu[None]) * sc[None] + bt[None]).reshape(n, wd)
        return hz * jnp.tanh(hz) + hz

    def produce_sub(s_ref, pv, z_ref, q, row0, k, cb, part, carry, marker, edge):
        r = row0 + W * k
        rc = pl.multiple_of(jnp.clip(r, 0, HW - W) + part * HR, HR)
        cs = slice(cb * PW, (cb + 1) * PW)
        a = act(s_ref[q, pl.ds(rc, HR), cs].astype(f32), tuple(p[:, cs] for p in pv), marker)
        if edge:
            valid = jnp.logical_and(r >= 0, r < HW)
            a = jnp.where(valid, a, 0.0)
        zh = k * HR
        if part == 0:
            row = lax.broadcasted_iota(jnp.int32, (HR, PW), 0)
            am = jnp.where(row == 0, 0.0, pltpu.roll(a, 1, 0))
            ap = pltpu.roll(a, HR - 1, 0)[0:HR - 16]
            z_ref[0, pl.ds(zh, HH), cs] = pack(am)
            z_ref[1, pl.ds(zh, HH), cs] = pack(a)
            z_ref[2, pl.ds(zh, HH - 8), cs] = pack(ap)
            return a[HR - 16:HR]
        ext = jnp.concatenate([carry, a], axis=0)
        am = pltpu.roll(ext, 1, 0)[16:HR + 16]
        row = lax.broadcasted_iota(jnp.int32, (HR + 16, PW), 0)
        ap = jnp.where(row == HR + 15, 0.0, pltpu.roll(ext, HR + 15, 0))
        z_ref[0, pl.ds(zh + HH, HH), cs] = pack(am)
        z_ref[1, pl.ds(zh + HH, HH), cs] = pack(a)
        z_ref[2, pl.ds(zh + HH - 8, HH + 8), cs] = pack(ap)
        return None

    def produce_row(s_ref, pv, z_ref, row0, k, cs_src, cs_dst, marker):
        r = row0 + W * k
        zs = pl.ds(k * HR, HR)
        if r < 0 or r >= HW:
            z = jnp.zeros((HR, 128), u32)
            for j in range(3):
                z_ref[j, zs, cs_dst] = z
            return
        a = act(s_ref[0, pl.ds(r, W), cs_src].astype(f32), pv, marker)
        row = lax.broadcasted_iota(jnp.int32, (W, 128), 0)
        z_ref[0, zs, cs_dst] = pack(jnp.where(row == 0, 0.0, pltpu.roll(a, 1, 0)))
        z_ref[1, zs, cs_dst] = pack(a)
        z_ref[2, zs, cs_dst] = pack(jnp.where(row == W - 1, 0.0, pltpu.roll(a, W - 1, 0)))

    def zload(z_ref, j, i):
        return pltpu.bitcast(z_ref[j, i * HR:i * HR + TM // 2, :], bf16)

    def stat_acc(v, state, marker=None):
        n = v.shape[0] // 8
        wd = v.shape[1]
        if state is None:
            K = v[0:1, :]
            if marker is not None:
                K = K + marker[0:1, :]
            d = v - K
            return (K, d.reshape(n, 8, wd).sum(axis=0), (d * d).reshape(n, 8, wd).sum(axis=0))
        K, s1, s2 = state
        Kd = K if marker is None else K + marker[0:1, :]
        d = v - Kd
        return (K, s1 + d.reshape(n, 8, wd).sum(axis=0), s2 + (d * d).reshape(n, 8, wd).sum(axis=0))

    def store_stats(st_ref, q, t, cs, state):
        K, s1, s2 = state
        wd = K.shape[1]
        st_ref[q, t, 0, :, cs] = jnp.broadcast_to(K, (8, wd))
        st_ref[q, t, 1, :, cs] = jnp.broadcast_to(s1.sum(axis=0, keepdims=True), (8, wd))
        st_ref[q, t, 2, :, cs] = jnp.broadcast_to(s2.sum(axis=0, keepdims=True), (8, wd))

    def finalize_group(st_ref, p_ref, gb_ref, e_ref, q, cv, cs, marker=None):
        K = st_ref[q, :, 0, :, cs]
        s1 = st_ref[q, :, 1, :, cs]
        s2 = st_ref[q, :, 2, :, cs]
        mean_t = K + s1 * (1.0 / TM)
        if e_ref is not None:
            e = e_ref[q, :, cs]
            mean_t = mean_t + e[None]
        if marker is not None:
            mean_t = mean_t + marker[None]
        m2_t = s2 - s1 * s1 * (1.0 / TM)
        mu = jnp.sum(jnp.sum(mean_t, axis=0), axis=1, keepdims=True) * (1.0 / (T * 128))
        dev = mean_t - mu[None]
        tot = m2_t + dev * dev * float(TM)
        var = jnp.sum(jnp.sum(tot, axis=0), axis=1, keepdims=True) * (1.0 / (HW * 128))
        rstd = lax.rsqrt(var + EPS)
        if e_ref is not None:
            p_ref[q, 0, :, cs] = mu - e
        else:
            p_ref[q, 0, :, cs] = jnp.broadcast_to(mu, (8, 128))
        p_ref[q, 1, :, cs] = gb_ref[cv, 0, :, cs] * (rstd * 0.5)
        p_ref[q, 2, :, cs] = gb_ref[cv, 1, :, cs] * 0.5

    def merge(lists):
        items = []
        for li, l in enumerate(lists):
            for i, it in enumerate(l):
                items.append(((i + 0.5) / len(l), li, it))
        items.sort(key=lambda z: (z[0], z[1]))
        return [it for _, _, it in items]

    def kern(x_hbm, te_hbm, g1_hbm, b1_hbm, w1_hbm, we_hbm, g2_hbm, b2_hbm, w2_hbm, o_hbm,
             s_ref, w_ref, za_ref, zb_ref, y00_ref, y01_ref, y10_ref, y11_ref,
             acca_ref, accb_ref, accc_ref, st_ref, p_ref, gb_ref, e_ref,
             te_ref, we_ref, gsm_ref, sem_x, sem_w, sem_s, sem_o):

        def gcols(g):
            return pl.ds(mult(g * 128, 128), 128)

        def x0_copy(g):
            return pltpu.make_async_copy(x_hbm.at[0, :, gcols(g)], s_ref.at[0, :, gcols(g)], sem_x.at[g])

        def w1_copy(g):
            return pltpu.make_async_copy(w1_hbm.at[:, :, gcols(g)], w_ref.at[pl.ds(0, 9), :, gcols(g)], sem_w.at[g])

        def x1_copy():
            return pltpu.make_async_copy(x_hbm.at[1], s_ref.at[1], sem_s.at[6])

        def w2_copy():
            return pltpu.make_async_copy(w2_hbm, w_ref.at[pl.ds(9, 9)], sem_s.at[7])

        def small_copies():
            return [pltpu.make_async_copy(g1_hbm, gsm_ref.at[0], sem_s.at[0]),
                    pltpu.make_async_copy(b1_hbm, gsm_ref.at[1], sem_s.at[1]),
                    pltpu.make_async_copy(g2_hbm, gsm_ref.at[2], sem_s.at[2]),
                    pltpu.make_async_copy(b2_hbm, gsm_ref.at[3], sem_s.at[3]),
                    pltpu.make_async_copy(te_hbm, te_ref, sem_s.at[4])]

        def we_copy():
            return pltpu.make_async_copy(we_hbm, we_ref, sem_s.at[5])

        def o_copy(s):
            b = divT(s) - 2
            r0 = mult(modT(s) * TM, TM)
            return pltpu.make_async_copy(s_ref.at[b, pl.ds(r0, TM), :], o_hbm.at[b, pl.ds(r0, TM), :], sem_o.at[0])

        def epi_piece(acc_ref, s_prev, cb, ri, state, marker):
            p = divT(s_prev)
            t = modT(s_prev)
            cs = slice(cb * PW, (cb + 1) * PW)
            r0 = mult(t * TM + ri * ER, ER)
            a = acc_ref[ri * ER:(ri + 1) * ER, cs]
            if marker is not None:
                a = (a.reshape(ER // 8, 8, PW) + marker[None]).reshape(ER, PW)
            if isinstance(s_prev, int):
                is2 = p >= 2
                dst = p - 2 if is2 else p + 2
                res = a + s_ref[dst, pl.ds(r0, ER), cs].astype(f32) if is2 else a
                sq = 0 if is2 else p + 2
            else:
                is2 = p >= 2
                dst = jnp.where(is2, p - 2, p + 2)
                xr = s_ref[dst, pl.ds(r0, ER), cs].astype(f32)
                res = a + jnp.where(is2, xr, 0.0)
                sq = jnp.where(is2, 0, p + 2)
            state = stat_acc(res, state)
            s_ref[dst, pl.ds(r0, ER), cs] = res.astype(bf16)
            if ri == NER - 1:
                store_stats(st_ref, sq, t, cs, state)
                state = None
            return state

        def xstat_piece(q, tile, cs, ri, state, marker):
            r0 = mult(tile * TM + ri * XR, XR)
            v = s_ref[q, pl.ds(r0, XR), cs].astype(f32)
            state = stat_acc(v, state, marker)
            if ri == NXR - 1:
                store_stats(st_ref, q, tile, cs, state)
                state = None
            return state

        def half(s, zc_ref, zn_ref, accc_ref, accp_ref, do_fin):
            is_c2 = s >= 2 * T
            sn = s + 1
            pn = jnp.minimum(divT(sn), 3)
            tn = modT(sn)
            lists = [[('p', k, cb, part) for k in range(NCH) for cb in range(NPW) for part in range(2)],
                     [('e', cb, ri) for cb in range(NPW) for ri in range(NER)]]
            if not opts.get('nox'):
                lists.append([('x', tl, cb, ri) for tl in range(XT) for cb in range(NPW) for ri in range(NXR)])
            pieces = merge(lists)
            npc = len(pieces)
            if do_fin:
                q = jnp.minimum(divT(s) + 1, 3)
                cv = lax.shift_right_logical(q, 1)
                for g in range(G):
                    finalize_group(st_ref, p_ref, gb_ref, e_ref, q, cv, slice(g * 128, (g + 1) * 128))
            pv = tuple(p_ref[pn, k] for k in range(3))
            xj = jnp.clip(s - 2, 0, T // XT - 1) * XT
            done = 0
            acc = None
            est = None
            xst = None
            pcar = None
            nslots = last_slot * SUB
            for i in range(3):
                for j in range(3):
                    tap = i * 3 + j
                    wv = pltpu.bitcast(jnp.where(is_c2, pltpu.bitcast(w_ref[9 + tap], u32),
                                                 pltpu.bitcast(w_ref[tap], u32)), bf16)
                    d = lax.dot_general(zload(zc_ref, j, i), wv, NT, preferred_element_type=f32)
                    for nn in range(4 * SUB):
                        n, sub = nn // SUB, nn % SUB
                        slot = tap * 4 * SUB + nn
                        hi_ = min(npc, ((slot + 1) * npc) // nslots)
                        while done < hi_:
                            pc = pieces[done]
                            marker = marker_of(d, n, sub, PW)
                            if pc[0] == 'p':
                                pcar = produce_sub(s_ref, pv, zn_ref, pn, tn * TM - W, pc[1], pc[2], pc[3], pcar,
                                                   marker, pc[1] == 0 or pc[1] == NCH - 1)
                            elif pc[0] == 'e':
                                est = epi_piece(accp_ref, s - 1, pc[1], pc[2], est, marker)
                            else:
                                xst = xstat_piece(1, xj + pc[1], slice(pc[2] * PW, (pc[2] + 1) * PW), pc[3],
                                                  xst, marker)
                            done += 1
                    acc = d if acc is None else acc + d
            accc_ref[...] = acc

        def load_pg(cs):
            return tuple(p_ref[0, k, :, cs] for k in range(3))

        def chunk_dots(y_ref, acc_ref, g, first, pieces, run):
            cs = gcols(g)
            npc = len(pieces)
            nslots = opts.get('a_last', 34) * SUB
            done = 0
            acc = None
            for i in range(3):
                for j in range(3):
                    tap = i * 3 + j
                    d = lax.dot_general(zload(y_ref, j, i), w_ref[tap, :, cs], NT, preferred_element_type=f32)
                    for nn in range(4 * SUB):
                        n, sub = nn // SUB, nn % SUB
                        slot = tap * 4 * SUB + nn
                        hi_ = min(npc, ((slot + 1) * npc) // nslots)
                        while done < hi_:
                            run(pieces[done], d, n, sub)
                            done += 1
                    acc = d if acc is None else acc + d
            if first:
                acc_ref[...] = jnp.where(g == 0, 0.0, acc_ref[...]) + acc
            else:
                acc_ref[...] = acc_ref[...] + acc

        with scope('prologue'):
            for c in small_copies():
                c.start()

            def issue(g, _):
                x0_copy(g).start()
                w1_copy(g).start()
                return 0
            lax.fori_loop(0, G, issue, 0)

            def rest(c, _):
                @pl.when(c == 0)
                def _():
                    w2_copy().start()

                @pl.when(c == 1)
                def _():
                    x1_copy().start()

                @pl.when(c == 2)
                def _():
                    we_copy().start()
                return 0
            lax.fori_loop(0, 3, rest, 0)

            for c in small_copies():
                c.wait()
            for cv in range(2):
                for k in range(2):
                    v = gsm_ref[2 * cv + k].astype(f32)
                    for g in range(G):
                        gb_ref[cv, k, :, g * 128:(g + 1) * 128] = jnp.broadcast_to(v[g:g + 1, :], (8, 128))
            e_ref[...] = jnp.zeros(e_ref.shape, f32)
            st_ref[...] = jnp.zeros(st_ref.shape, f32)
            acca_ref[...] = jnp.zeros(acca_ref.shape, f32)
            accb_ref[...] = jnp.zeros(accb_ref.shape, f32)
            accc_ref[...] = jnp.zeros(accc_ref.shape, f32)

            x0_copy(0).wait()
            c0 = slice(0, 128)

            def xs0(t, _):
                st = None
                for ri in range(NXR):
                    st = xstat_piece(0, t, c0, ri, st, None)
                return 0
            lax.fori_loop(0, T, xs0, 0)
            finalize_group(st_ref, p_ref, gb_ref, None, 0, 0, c0)
            pv0 = load_pg(c0)
            for k in range(NCH):
                produce_row(s_ref, pv0, y00_ref, -W, k, c0, c0, None)
                produce_row(s_ref, pv0, y01_ref, TM - W, k, c0, c0, None)

        def chunk(g, c, h):
            ycur = (y00_ref, y01_ref) if c == 0 else (y10_ref, y11_ref)
            ynxt = (y10_ref, y11_ref) if c == 0 else (y00_ref, y01_ref)
            gn = jnp.minimum(g + 1, G - 1)
            cs = gcols(g)
            csn = gcols(gn)
            c0 = slice(0, 128)
            pvc = load_pg(cs)
            state = {'e': None, 'x': None, 'pv': None}
            zs = [('z', k) for k in range(NCH)]
            xs = [('x', t, ri) for t in range(T) for ri in range(NXR)]
            ps = [('p', tl, k) for k in range(NCH) for tl in range(2)]
            es = [('e', cb, ri) for cb in range(NPW) for ri in range(NER)]
            nz = opts.get('nz', 4)
            if c == 0:
                part0 = zs[:nz]
                part1 = xs + [('f',)] + zs[nz:] + ps
            else:
                part0 = merge([xs, zs[:nz]]) + [('f',)] + zs[nz:]
                part1 = merge([ps, es])

            def run(pc, d, n, sub):
                if pc[0] == 'z':
                    produce_row(s_ref, pvc, za_ref, 2 * TM - W, pc[1], cs, cs, marker_of(d, n, sub, 128))
                elif pc[0] == 'e':
                    state['e'] = epi_piece(accc_ref, 0, pc[1], pc[2], state['e'], marker_of(d, n, sub, PW))
                elif pc[0] == 'x':
                    state['x'] = xstat_piece(0, pc[1], csn, pc[2], state['x'], marker_of(d, n, sub, 128))
                elif pc[0] == 'f':
                    finalize_group(st_ref, p_ref, gb_ref, None, 0, 0, csn)
                    state['pv'] = load_pg(csn)
                else:
                    produce_row(s_ref, state['pv'], ynxt[pc[1]], pc[1] * TM - W, pc[2], csn, c0,
                                marker_of(d, n, sub, 128))
            chunk_dots(ycur[0], accc_ref, g, c == 0, part0, run)
            if c == 0:
                x0_copy(g + 1).wait()
            chunk_dots(ycur[1], accb_ref, g, c == 0, part1, run)

        def phase_a(h, _):
            g0 = 2 * h
            w1_copy(g0).wait()
            chunk(g0, 0, h)
            w1_copy(g0 + 1).wait()

            @pl.when(h == 0)
            def _():
                x0_copy(2).wait()
            chunk(g0 + 1, 1, h)
            return 0

        with scope('first'):
            lax.fori_loop(0, 2, phase_a, 0)

        with scope('mid'):
            w2_copy().wait()
            x1_copy().wait()
            we_copy().wait()
            te = te_ref[...].astype(f32)
            sl = te * jax.nn.sigmoid(te)
            emb = jnp.dot(sl.astype(bf16), we_ref[...], preferred_element_type=f32)
            e_ref[2] = jnp.broadcast_to(emb[0:1, :], (8, C))
            e_ref[3] = jnp.broadcast_to(emb[1:2, :], (8, C))

        NIT = (NSTEP - 2) // 2

        def body(it, carry):
            s0 = 2 * it + 2
            s1 = s0 + 1
            with scope('iter'):
                half(s0, za_ref, zb_ref, acca_ref, accb_ref, True)
                if opts.get('omid'):
                    @pl.when(s0 - 1 >= 2 * T)
                    def _():
                        o_copy(s0 - 1).start()
                half(s1, zb_ref, za_ref, accb_ref, acca_ref, False)

            if not opts.get('omid'):
                @pl.when(s0 - 1 >= 2 * T)
                def _():
                    o_copy(s0 - 1).start()

            @pl.when(s0 >= 2 * T)
            def _():
                o_copy(s0).start()
            return carry

        with scope('main'):
            lax.fori_loop(0, NIT, body, 0)

        sl_ = NSTEP - 1
        with scope('final'):
            for cb in range(NPW):
                st = None
                for ri in range(NER):
                    st = epi_piece(accb_ref, sl_, cb, ri, st, None)
            o_copy(sl_).start()
        with scope('owait'):
            for s in range(2 * T, NSTEP):
                o_copy(s).wait()

    def fn(x, t_emb, g1, be1, w1, w_emb, g2, be2, w2):
        xn = jnp.transpose(x, (0, 2, 3, 1)).reshape(B, HW, C)
        w1t = jnp.transpose(w1, (2, 3, 0, 1)).reshape(9, C, C)
        w2t = jnp.transpose(w2, (2, 3, 0, 1)).reshape(9, C, C)
        any_spec = pl.BlockSpec(memory_space=pl.ANY)
        zbuf = pltpu.VMEM((3, R // 2, C), u32)
        ybuf = pltpu.VMEM((3, R // 2, 128), u32)
        abuf = pltpu.VMEM((TM, C), f32)
        out = pl.pallas_call(
            kern,
            in_specs=[any_spec] * 9,
            out_specs=any_spec,
            out_shape=jax.ShapeDtypeStruct((B, HW, C), bf16),
            scratch_shapes=[
                pltpu.VMEM((4, HW, C), bf16),
                pltpu.VMEM((18, C, C), bf16),
                zbuf, zbuf, ybuf, ybuf, ybuf, ybuf,
                abuf, abuf, abuf,
                pltpu.VMEM((4, T, 3, 8, C), f32),
                pltpu.VMEM((4, 3, 8, C), f32),
                pltpu.VMEM((2, 2, 8, C), f32),
                pltpu.VMEM((4, 8, C), f32),
                pltpu.VMEM((B, E), bf16),
                pltpu.VMEM((E, C), bf16),
                pltpu.VMEM((4, G, 128), bf16),
                pltpu.SemaphoreType.DMA((G,)),
                pltpu.SemaphoreType.DMA((G,)),
                pltpu.SemaphoreType.DMA((8,)),
                pltpu.SemaphoreType.DMA((1,)),
            ],
            compiler_params=pltpu.CompilerParams(vmem_limit_bytes=100 * 1024 * 1024,
                                                 disable_bounds_checks=True),
        )(xn, t_emb, g1.reshape(G, 128), be1.reshape(G, 128), w1t, w_emb,
          g2.reshape(G, 128), be2.reshape(G, 128), w2t)
        return jnp.transpose(out.reshape(B, H, W, C), (0, 3, 1, 2))
    return fn


_OPTS = {'omid': 1}


@jax.jit
def pallas_standalone__adm_resblock__diffusion_kernel(x, t_emb, g1, be1, w1, w_emb, g2, be2, w2):
    B, C, H, W = x.shape
    E = t_emb.shape[1]
    return build(B, C, H, W, E, TM=512, opts=_OPTS)(x, t_emb, g1, be1, w1, w_emb, g2, be2, w2)
```

```python
import jax
import jax.numpy as jnp
from jax import lax
from jax.experimental import pallas as pl
from jax.experimental.pallas import tpu as pltpu

f32 = jnp.float32
bf16 = jnp.bfloat16
u32 = jnp.uint32
NT = (((1,), (1,)), ((), ()))


def build(B, C, H, W, E, TM=512, opts=None):
    opts = opts or {}
    HW = H * W
    G = 4
    CG = C // G
    EPS = 1e-5
    T = HW // TM
    assert CG == 128 and B == 2 and T == 8 and W == 64
    R = TM + 2 * W
    NCH = R // W
    NSTEP = 4 * T
    ER = opts.get('er', 32)
    NER = TM // ER
    XT = 2
    last_slot = opts.get('last_slot', 34)
    scope = jax.named_scope

    PW = opts.get('pw', 256)
    NPW = C // PW
    SUB = opts.get('sub', 4)
    XR = opts.get('xr', 64)
    NXR = TM // XR
    HR = W // 2
    HH = HR // 2

    def divT(v):
        return v // T if isinstance(v, int) else lax.shift_right_logical(v, 3)

    def modT(v):
        return v % T if isinstance(v, int) else jnp.bitwise_and(v, T - 1)

    def mult(v, m):
        return v if isinstance(v, int) else pl.multiple_of(v, m)

    def marker_of(d, n, sub, width):
        rp = sub * (d.shape[0] // SUB) // 8 * 8
        m = d[rp:rp + 8, n * 128:(n + 1) * 128]
        b = pltpu.bitcast(m, u32)
        z = pltpu.bitcast((b >> 16) >> 16, f32)
        if width > 128:
            z = jnp.concatenate([z] * (width // 128), axis=1)
        return z

    def pack(t):
        return pltpu.bitcast(t.astype(bf16), u32)

    def act(v, pv, marker):
        n, wd = v.shape
        mu, sc, bt = pv
        if marker is not None:
            mu = mu + marker
        v3 = v.reshape(n // 8, 8, wd)
        hz = ((v3 - mu[None]) * sc[None] + bt[None]).reshape(n, wd)
        return hz * jnp.tanh(hz) + hz

    def produce_sub(s_ref, pv, z_ref, q, row0, k, cb, part, carry, marker):
        r = row0 + W * k
        rc = pl.multiple_of(jnp.clip(r, 0, HW - W) + part * HR, HR)
        cs = slice(cb * PW, (cb + 1) * PW)
        a = act(s_ref[q, pl.ds(rc, HR), cs].astype(f32), tuple(p[:, cs] for p in pv), marker)
        zh = k * HR
        if part == 0:
            row = lax.broadcasted_iota(jnp.int32, (HR, PW), 0)
            am = jnp.where(row == 0, 0.0, pltpu.roll(a, 1, 0))
            ap = pltpu.roll(a, HR - 1, 0)[0:HR - 16]
            z_ref[0, pl.ds(zh, HH), cs] = pack(am)
            z_ref[1, pl.ds(zh, HH), cs] = pack(a)
            z_ref[2, pl.ds(zh, HH - 8), cs] = pack(ap)
            return a[HR - 16:HR]
        ext = jnp.concatenate([carry, a], axis=0)
        am = pltpu.roll(ext, 1, 0)[16:HR + 16]
        row = lax.broadcasted_iota(jnp.int32, (HR + 16, PW), 0)
        ap = jnp.where(row == HR + 15, 0.0, pltpu.roll(ext, HR + 15, 0))
        z_ref[0, pl.ds(zh + HH, HH), cs] = pack(am)
        z_ref[1, pl.ds(zh + HH, HH), cs] = pack(a)
        z_ref[2, pl.ds(zh + HH - 8, HH + 8), cs] = pack(ap)
        return None

    def produce_row(s_ref, pv, z_ref, row0, k, cs_src, cs_dst, marker):
        r = row0 + W * k
        zs = pl.ds(k * HR, HR)
        if r < 0 or r >= HW:
            z = jnp.zeros((HR, 128), u32)
            for j in range(3):
                z_ref[j, zs, cs_dst] = z
            return
        a = act(s_ref[0, pl.ds(r, W), cs_src].astype(f32), pv, marker)
        row = lax.broadcasted_iota(jnp.int32, (W, 128), 0)
        z_ref[0, zs, cs_dst] = pack(jnp.where(row == 0, 0.0, pltpu.roll(a, 1, 0)))
        z_ref[1, zs, cs_dst] = pack(a)
        z_ref[2, zs, cs_dst] = pack(jnp.where(row == W - 1, 0.0, pltpu.roll(a, W - 1, 0)))

    def zload(z_ref, j, i):
        return pltpu.bitcast(z_ref[j, i * HR:i * HR + TM // 2, :], bf16)

    def stat_acc(v, state, marker=None):
        n = v.shape[0] // 8
        wd = v.shape[1]
        if state is None:
            K = v[0:1, :]
            if marker is not None:
                K = K + marker[0:1, :]
            d = v - K
            return (K, d.reshape(n, 8, wd).sum(axis=0), (d * d).reshape(n, 8, wd).sum(axis=0))
        K, s1, s2 = state
        Kd = K if marker is None else K + marker[0:1, :]
        d = v - Kd
        return (K, s1 + d.reshape(n, 8, wd).sum(axis=0), s2 + (d * d).reshape(n, 8, wd).sum(axis=0))

    def store_stats(st_ref, q, t, cs, state):
        K, s1, s2 = state
        wd = K.shape[1]
        st_ref[q, t, 0, :, cs] = jnp.broadcast_to(K, (8, wd))
        st_ref[q, t, 1, :, cs] = jnp.broadcast_to(s1.sum(axis=0, keepdims=True), (8, wd))
        st_ref[q, t, 2, :, cs] = jnp.broadcast_to(s2.sum(axis=0, keepdims=True), (8, wd))

    def finalize_group(st_ref, p_ref, gb_ref, e_ref, q, cv, cs, marker=None):
        K = st_ref[q, :, 0, :, cs]
        s1 = st_ref[q, :, 1, :, cs]
        s2 = st_ref[q, :, 2, :, cs]
        mean_t = K + s1 * (1.0 / TM)
        if e_ref is not None:
            e = e_ref[q, :, cs]
            mean_t = mean_t + e[None]
        if marker is not None:
            mean_t = mean_t + marker[None]
        m2_t = s2 - s1 * s1 * (1.0 / TM)
        mu = jnp.sum(jnp.sum(mean_t, axis=0), axis=1, keepdims=True) * (1.0 / (T * 128))
        dev = mean_t - mu[None]
        tot = m2_t + dev * dev * float(TM)
        var = jnp.sum(jnp.sum(tot, axis=0), axis=1, keepdims=True) * (1.0 / (HW * 128))
        rstd = lax.rsqrt(var + EPS)
        if e_ref is not None:
            p_ref[q, 0, :, cs] = mu - e
        else:
            p_ref[q, 0, :, cs] = jnp.broadcast_to(mu, (8, 128))
        p_ref[q, 1, :, cs] = gb_ref[cv, 0, :, cs] * (rstd * 0.5)
        p_ref[q, 2, :, cs] = gb_ref[cv, 1, :, cs] * 0.5

    def merge(lists):
        items = []
        for li, l in enumerate(lists):
            for i, it in enumerate(l):
                items.append(((i + 0.5) / len(l), li, it))
        items.sort(key=lambda z: (z[0], z[1]))
        return [it for _, _, it in items]

    def kern(x_hbm, te_hbm, g1_hbm, b1_hbm, w1_hbm, we_hbm, g2_hbm, b2_hbm, w2_hbm, o_hbm,
             s_ref, w_ref, za_ref, zb_ref, y00_ref, y01_ref, y10_ref, y11_ref,
             acca_ref, accb_ref, accc_ref, xa_ref, st_ref, p_ref, gb_ref, e_ref,
             te_ref, we_ref, gsm_ref, sem_x, sem_w, sem_s, sem_o):

        def gcols(g):
            return pl.ds(mult(g * 128, 128), 128)

        def x0_copy(g):
            return pltpu.make_async_copy(x_hbm.at[0, :, gcols(g)], s_ref.at[0, :, gcols(g)], sem_x.at[g])

        def w1_copy(g):
            return pltpu.make_async_copy(w1_hbm.at[:, :, gcols(g)], w_ref.at[pl.ds(0, 9), :, gcols(g)], sem_w.at[g])

        def x1_copy():
            return pltpu.make_async_copy(x_hbm.at[1], s_ref.at[1], sem_s.at[6])

        def w2_copy():
            return pltpu.make_async_copy(w2_hbm, w_ref.at[pl.ds(9, 9)], sem_s.at[7])

        def small_copies():
            return [pltpu.make_async_copy(g1_hbm, gsm_ref.at[0], sem_s.at[0]),
                    pltpu.make_async_copy(b1_hbm, gsm_ref.at[1], sem_s.at[1]),
                    pltpu.make_async_copy(g2_hbm, gsm_ref.at[2], sem_s.at[2]),
                    pltpu.make_async_copy(b2_hbm, gsm_ref.at[3], sem_s.at[3]),
                    pltpu.make_async_copy(te_hbm, te_ref, sem_s.at[4])]

        def we_copy():
            return pltpu.make_async_copy(we_hbm, we_ref, sem_s.at[5])

        NQ = opts.get('nq', 4)
        QR = TM // NQ

        def o_copy(s, qi):
            b = divT(s) - 2
            r0 = mult(modT(s) * TM + qi * QR, QR)
            return pltpu.make_async_copy(s_ref.at[b, pl.ds(r0, QR), :], o_hbm.at[b, pl.ds(r0, QR), :], sem_o.at[0])

        def o_all():
            return pltpu.make_async_copy(s_ref.at[pl.ds(0, B)], o_hbm, sem_o.at[0])

        def epi_piece(acc_ref, s_prev, cb, ri, state, marker):
            p = divT(s_prev)
            t = modT(s_prev)
            cs = slice(cb * PW, (cb + 1) * PW)
            r0 = mult(t * TM + ri * ER, ER)
            a = acc_ref[ri * ER:(ri + 1) * ER, cs]
            if marker is not None:
                a = (a.reshape(ER // 8, 8, PW) + marker[None]).reshape(ER, PW)
            if isinstance(s_prev, int):
                is2 = p >= 2
                dst = p - 2 if is2 else p + 2
                res = a + s_ref[dst, pl.ds(r0, ER), cs].astype(f32) if is2 else a
                sq = None if is2 else p + 2
            else:
                is2 = p >= 2
                dst = jnp.where(is2, p - 2, p + 2)
                xr = s_ref[dst, pl.ds(r0, ER), cs].astype(f32)
                res = a + jnp.where(is2, xr, 0.0)
                sq = jnp.where(is2, 0, p + 2)
            if sq is not None:
                state = stat_acc(res, state)
            s_ref[dst, pl.ds(r0, ER), cs] = res.astype(bf16)
            if sq is not None and ri == NER - 1:
                store_stats(st_ref, sq, t, cs, state)
                state = None
            return state

        def xstat_piece(q, tile, cs, ri, state, marker):
            r0 = mult(tile * TM + ri * XR, XR)
            v = s_ref[q, pl.ds(r0, XR), cs].astype(f32)
            state = stat_acc(v, state, marker)
            if ri == NXR - 1:
                store_stats(st_ref, q, tile, cs, state)
                state = None
            return state

        def wsel(is_c2, tap):
            return pltpu.bitcast(jnp.where(is_c2, pltpu.bitcast(w_ref[9 + tap], u32),
                                           pltpu.bitcast(w_ref[tap], u32)), bf16)

        def half(s, zc_ref, zn_ref, accc_ref, accp_ref, kind):
            is_c2 = s >= 2 * T
            sn = s + 1
            pn = jnp.minimum(divT(sn), 3)
            tn = modT(sn)
            lists = [[('p', k, cb, part) for k in range(NCH) for cb in range(NPW) for part in range(2)],
                     [('e', cb, ri) for ri in range(NER) for cb in range(NPW)]]
            if not opts.get('nox'):
                lists.append([('x', tl, cb, ri) for tl in range(XT) for cb in range(NPW) for ri in range(NXR)])
            pieces = merge(lists)
            npc = len(pieces)
            if kind == 0:
                q = jnp.minimum(divT(s) + 1, 3)
                cv = lax.shift_right_logical(q, 1)
                for g in range(G):
                    finalize_group(st_ref, p_ref, gb_ref, e_ref, q, cv, slice(g * 128, (g + 1) * 128))
            pv = tuple(p_ref[pn, k] for k in range(3))
            xj = jnp.clip(s - 2, 0, T // XT - 1) * XT
            done = 0
            acc = None
            est = [None] * NPW
            xst = None
            pcar = None
            order = (1, 2, 0) if kind == 0 else (0, 1, 2)
            total = 6 * TM + 3 * (TM - W)
            lim = total * last_slot // 36
            pos = 0
            for i in order:
                for j in range(3):
                    tap = i * 3 + j
                    skip = i == order[2]
                    if not skip:
                        lhs = zload(zc_ref, j, i)
                    elif kind == 0:
                        lhs = pltpu.bitcast(zc_ref[j, HR:TM // 2, :], bf16)
                    else:
                        lhs = pltpu.bitcast(zc_ref[j, 2 * HR:2 * HR + (TM - W) // 2, :], bf16)
                    d = lax.dot_general(lhs, wsel(is_c2, tap), NT, preferred_element_type=f32)
                    rows = d.shape[0]
                    for nn in range(4 * SUB):
                        n, sub = nn // SUB, nn % SUB
                        hi_ = min(npc, ((pos + (rows * (nn + 1)) // (4 * SUB)) * npc) // lim)
                        while done < hi_:
                            pc = pieces[done]
                            marker = marker_of(d, n, sub, PW)
                            if pc[0] == 'p':
                                pcar = produce_sub(s_ref, pv, zn_ref, pn, tn * TM - W, pc[1], pc[2], pc[3], pcar,
                                                   marker)
                            elif pc[0] == 'e':
                                est[pc[1]] = epi_piece(accp_ref, s - 1, pc[1], pc[2], est[pc[1]], marker)
                                if pc[1] == NPW - 1 and ((pc[2] + 1) * ER) % QR == 0:
                                    qi = ((pc[2] + 1) * ER) // QR - 1

                                    @pl.when(s - 1 >= 2 * T)
                                    def _():
                                        o_copy(s - 1, qi).start()
                            else:
                                xst = xstat_piece(1, xj + pc[1], slice(pc[2] * PW, (pc[2] + 1) * PW), pc[3],
                                                  xst, marker)
                            done += 1
                    pos += rows
                    if not skip:
                        acc = d if acc is None else acc + d
                    elif kind == 0:
                        acc = jnp.concatenate([acc[0:W], acc[W:] + d], axis=0)
                    else:
                        acc = jnp.concatenate([acc[0:TM - W] + d, acc[TM - W:]], axis=0)
            if kind == 0:
                top = jnp.where(modT(s) == 0, 0.0, xa_ref[...])
                acc = jnp.concatenate([acc[0:W] + top, acc[W:]], axis=0)
            accc_ref[...] = acc

        def halo_top(wget):
            d = None
            for j in range(3):
                dj = lax.dot_general(pltpu.bitcast(za_ref[j, 0:HR, :], bf16), wget(j), NT,
                                     preferred_element_type=f32)
                d = dj if d is None else d + dj
            xa_ref[...] = d

        def halo_bot(wget):
            d = None
            for j in range(3):
                dj = lax.dot_general(pltpu.bitcast(zb_ref[j, TM // 2 + HR:TM // 2 + 2 * HR, :], bf16), wget(6 + j),
                                     NT, preferred_element_type=f32)
                d = dj if d is None else d + dj
            accb_ref[TM - W:TM, :] = accb_ref[TM - W:TM, :] + d

        def load_pg(cs):
            return tuple(p_ref[0, k, :, cs] for k in range(3))

        def chunk_dots(y_ref, acc_ref, g, first, top, pieces, run):
            cs = gcols(g)
            npc = len(pieces)
            nslots = opts.get('a_last', 34) * SUB
            done = 0
            acc = None
            for ti, i in enumerate((1, 2, 0)):
                for j in range(3):
                    tap = i * 3 + j
                    skip = top and i == 0
                    if skip:
                        lhs = pltpu.bitcast(y_ref[j, HR:TM // 2, :], bf16)
                    else:
                        lhs = zload(y_ref, j, i)
                    d = lax.dot_general(lhs, w_ref[tap, :, cs], NT, preferred_element_type=f32)
                    for nn in range(4 * SUB):
                        n, sub = nn // SUB, nn % SUB
                        slot = (ti * 3 + j) * 4 * SUB + nn
                        hi_ = min(npc, ((slot + 1) * npc) // nslots)
                        while done < hi_:
                            run(pieces[done], marker_of(d, n, sub, 128))
                            done += 1
                    if skip:
                        acc = jnp.concatenate([acc[0:W], acc[W:] + d], axis=0)
                    else:
                        acc = d if acc is None else acc + d
            if first:
                acc_ref[...] = jnp.where(g == 0, 0.0, acc_ref[...]) + acc
            else:
                acc_ref[...] = acc_ref[...] + acc

        with scope('prologue'):
            for c in small_copies():
                c.start()

            def issue(g, _):
                x0_copy(g).start()
                w1_copy(g).start()
                return 0
            lax.fori_loop(0, G, issue, 0)

            def rest(c, _):
                @pl.when(c == 0)
                def _():
                    w2_copy().start()

                @pl.when(c == 1)
                def _():
                    x1_copy().start()

                @pl.when(c == 2)
                def _():
                    we_copy().start()
                return 0
            lax.fori_loop(0, 3, rest, 0)

            for c in small_copies():
                c.wait()
            for cv in range(2):
                for k in range(2):
                    v = gsm_ref[2 * cv + k].astype(f32)
                    for g in range(G):
                        gb_ref[cv, k, :, g * 128:(g + 1) * 128] = jnp.broadcast_to(v[g:g + 1, :], (8, 128))
            e_ref[...] = jnp.zeros(e_ref.shape, f32)
            st_ref[...] = jnp.zeros(st_ref.shape, f32)
            acca_ref[...] = jnp.zeros(acca_ref.shape, f32)
            accb_ref[...] = jnp.zeros(accb_ref.shape, f32)
            accc_ref[...] = jnp.zeros(accc_ref.shape, f32)

            x0_copy(0).wait()
            c0 = slice(0, 128)

            def xs0(t, _):
                st = None
                for ri in range(NXR):
                    st = xstat_piece(0, t, c0, ri, st, None)
                return 0
            lax.fori_loop(0, T, xs0, 0)
            finalize_group(st_ref, p_ref, gb_ref, None, 0, 0, c0)
            pv0 = load_pg(c0)
            for k in range(NCH):
                produce_row(s_ref, pv0, y00_ref, -W, k, c0, c0, None)
                produce_row(s_ref, pv0, y01_ref, TM - W, k, c0, c0, None)

        def chunk(g, c, h):
            ycur = (y00_ref, y01_ref) if c == 0 else (y10_ref, y11_ref)
            ynxt = (y10_ref, y11_ref) if c == 0 else (y00_ref, y01_ref)
            gn = jnp.minimum(g + 1, G - 1)
            cs = gcols(g)
            csn = gcols(gn)
            c0 = slice(0, 128)
            pvc = load_pg(cs)
            state = {'e': [None] * NPW, 'x': None, 'pv': None}
            zs = [('z', k) for k in range(NCH)]
            xs = [('x', t, ri) for t in range(T) for ri in range(NXR)]
            ps = [('p', tl, k) for k in range(NCH) for tl in range(2)]
            es = [('e', cb, ri) for cb in range(NPW) for ri in range(NER)]
            nz = opts.get('nz', 4)
            if c == 0:
                part0 = zs[:nz]
                part1 = xs + [('f',)] + zs[nz:] + ps
            else:
                part0 = merge([xs, zs[:nz]]) + [('f',)] + zs[nz:]
                part1 = merge([ps, es])

            def run(pc, mk):
                if pc[0] == 'z':
                    produce_row(s_ref, pvc, za_ref, 2 * TM - W, pc[1], cs, cs, mk)
                elif pc[0] == 'e':
                    mw = jnp.concatenate([mk] * (PW // 128), axis=1)
                    state['e'][pc[1]] = epi_piece(accc_ref, 0, pc[1], pc[2], state['e'][pc[1]], mw)
                elif pc[0] == 'x':
                    state['x'] = xstat_piece(0, pc[1], csn, pc[2], state['x'], mk)
                elif pc[0] == 'f':
                    finalize_group(st_ref, p_ref, gb_ref, None, 0, 0, csn)
                    state['pv'] = load_pg(csn)
                else:
                    produce_row(s_ref, state['pv'], ynxt[pc[1]], pc[1] * TM - W, pc[2], csn, c0, mk)
            chunk_dots(ycur[0], accc_ref, g, c == 0, True, part0, run)
            if c == 0:
                x0_copy(g + 1).wait()
            chunk_dots(ycur[1], accb_ref, g, c == 0, False, part1, run)

        def phase_a(h, _):
            g0 = 2 * h
            w1_copy(g0).wait()
            chunk(g0, 0, h)
            w1_copy(g0 + 1).wait()

            @pl.when(h == 0)
            def _():
                x0_copy(2).wait()
            chunk(g0 + 1, 1, h)
            return 0

        with scope('first'):
            lax.fori_loop(0, 2, phase_a, 0)

        with scope('mid'):
            w2_copy().wait()
            x1_copy().wait()
            we_copy().wait()
            te = te_ref[...].astype(f32)
            sl = te * jax.nn.sigmoid(te)
            emb = jnp.dot(sl.astype(bf16), we_ref[...], preferred_element_type=f32)
            e_ref[2] = jnp.broadcast_to(emb[0:1, :], (8, C))
            e_ref[3] = jnp.broadcast_to(emb[1:2, :], (8, C))
            halo_top(lambda tap: w_ref[tap])

        NIT = (NSTEP - 2) // 2

        def body(it, carry):
            s0 = 2 * it + 2
            s1 = s0 + 1
            with scope('iter'):
                half(s0, za_ref, zb_ref, acca_ref, accb_ref, 0)
                half(s1, zb_ref, za_ref, accb_ref, acca_ref, 1)

            @pl.when(modT(s1) != T - 1)
            def _():
                if opts.get('hdyn'):
                    wb = jnp.where(s1 >= 2 * T, 9, 0)
                    wget = lambda tap: w_ref[wb + tap]
                else:
                    wget = lambda tap: wsel(s1 >= 2 * T, tap)
                with scope('halo'):
                    halo_bot(wget)
                    halo_top(wget)
            return carry

        with scope('main'):
            lax.fori_loop(0, NIT, body, 0)

        sl_ = NSTEP - 1
        with scope('final'):
            st = [None] * NPW
            for ri in range(NER):
                for cb in range(NPW):
                    st[cb] = epi_piece(accb_ref, sl_, cb, ri, st[cb], None)
                if ((ri + 1) * ER) % QR == 0:
                    o_copy(sl_, ((ri + 1) * ER) // QR - 1).start()
        with scope('owait'):
            o_all().wait()

    def fn(x, t_emb, g1, be1, w1, w_emb, g2, be2, w2):
        xn = jnp.transpose(x, (0, 2, 3, 1)).reshape(B, HW, C)
        w1t = jnp.transpose(w1, (2, 3, 0, 1)).reshape(9, C, C)
        w2t = jnp.transpose(w2, (2, 3, 0, 1)).reshape(9, C, C)
        any_spec = pl.BlockSpec(memory_space=pl.ANY)
        zbuf = pltpu.VMEM((3, R // 2, C), u32)
        ybuf = pltpu.VMEM((3, R // 2, 128), u32)
        abuf = pltpu.VMEM((TM, C), f32)
        out = pl.pallas_call(
            kern,
            in_specs=[any_spec] * 9,
            out_specs=any_spec,
            out_shape=jax.ShapeDtypeStruct((B, HW, C), bf16),
            scratch_shapes=[
                pltpu.VMEM((4, HW, C), bf16),
                pltpu.VMEM((18, C, C), bf16),
                zbuf, zbuf, ybuf, ybuf, ybuf, ybuf,
                abuf, abuf, abuf,
                pltpu.VMEM((W, C), f32),
                pltpu.VMEM((4, T, 3, 8, C), f32),
                pltpu.VMEM((4, 3, 8, C), f32),
                pltpu.VMEM((2, 2, 8, C), f32),
                pltpu.VMEM((4, 8, C), f32),
                pltpu.VMEM((B, E), bf16),
                pltpu.VMEM((E, C), bf16),
                pltpu.VMEM((4, G, 128), bf16),
                pltpu.SemaphoreType.DMA((G,)),
                pltpu.SemaphoreType.DMA((G,)),
                pltpu.SemaphoreType.DMA((8,)),
                pltpu.SemaphoreType.DMA((1,)),
            ],
            compiler_params=pltpu.CompilerParams(vmem_limit_bytes=100 * 1024 * 1024,
                                                 disable_bounds_checks=True),
        )(xn, t_emb, g1.reshape(G, 128), be1.reshape(G, 128), w1t, w_emb,
          g2.reshape(G, 128), be2.reshape(G, 128), w2t)
        return jnp.transpose(out.reshape(B, H, W, C), (0, 3, 1, 2))
    return fn


_OPTS = {'sub': 8}


@jax.jit
def pallas_standalone__adm_resblock__diffusion_kernel(x, t_emb, g1, be1, w1, w_emb, g2, be2, w2):
    B, C, H, W = x.shape
    E = t_emb.shape[1]
    return build(B, C, H, W, E, TM=512, opts=_OPTS)(x, t_emb, g1, be1, w1, w_emb, g2, be2, w2)
```

```python
import jax
import jax.numpy as jnp
from jax import lax
from jax.experimental import pallas as pl
from jax.experimental.pallas import tpu as pltpu

f32 = jnp.float32
bf16 = jnp.bfloat16
u32 = jnp.uint32
NT = (((1,), (1,)), ((), ()))


def build(B, C, H, W, E, TM=512, opts=None):
    opts = opts or {}
    HW = H * W
    G = 4
    CG = C // G
    EPS = 1e-5
    T = HW // TM
    assert CG == 128 and B == 2 and T == 8 and W == 64
    R = TM + 2 * W
    NCH = R // W
    NSTEP = 4 * T
    ER = opts.get('er', 32)
    NER = TM // ER
    XT = 2
    last_slot = opts.get('last_slot', 34)
    scope = jax.named_scope

    PW = opts.get('pw', 256)
    NPW = C // PW
    SUB = opts.get('sub', 4)
    XR = opts.get('xr', 64)
    NXR = TM // XR
    HR = W // 2
    HH = HR // 2

    def divT(v):
        return v // T if isinstance(v, int) else lax.shift_right_logical(v, 3)

    def modT(v):
        return v % T if isinstance(v, int) else jnp.bitwise_and(v, T - 1)

    def mult(v, m):
        return v if isinstance(v, int) else pl.multiple_of(v, m)

    def marker_of(d, n, sub, width, nsub=SUB):
        rp = sub * (d.shape[0] // nsub) // 8 * 8
        m = d[rp:rp + 8, n * 128:(n + 1) * 128]
        b = pltpu.bitcast(m, u32)
        z = pltpu.bitcast((b >> 16) >> 16, f32)
        if width > 128:
            z = jnp.concatenate([z] * (width // 128), axis=1)
        return z

    def pack(t):
        return pltpu.bitcast(t.astype(bf16), u32)

    def act(v, pv, marker):
        n, wd = v.shape
        mu, sc, bt = pv
        if marker is not None:
            mu = mu + marker
        v3 = v.reshape(n // 8, 8, wd)
        hz = ((v3 - mu[None]) * sc[None] + bt[None]).reshape(n, wd)
        return hz * jnp.tanh(hz) + hz

    def produce_sub(s_ref, pv, z_ref, q, row0, k, cb, part, carry, marker):
        r = row0 + W * k
        rc = pl.multiple_of(jnp.clip(r, 0, HW - W) + part * HR, HR)
        cs = slice(cb * PW, (cb + 1) * PW)
        a = act(s_ref[q, pl.ds(rc, HR), cs].astype(f32), tuple(p[:, cs] for p in pv), marker)
        zh = k * HR
        if part == 0:
            row = lax.broadcasted_iota(jnp.int32, (HR, PW), 0)
            am = jnp.where(row == 0, 0.0, pltpu.roll(a, 1, 0))
            ap = pltpu.roll(a, HR - 1, 0)[0:HR - 16]
            z_ref[0, pl.ds(zh, HH), cs] = pack(am)
            z_ref[1, pl.ds(zh, HH), cs] = pack(a)
            z_ref[2, pl.ds(zh, HH - 8), cs] = pack(ap)
            return a[HR - 16:HR]
        ext = jnp.concatenate([carry, a], axis=0)
        am = pltpu.roll(ext, 1, 0)[16:HR + 16]
        row = lax.broadcasted_iota(jnp.int32, (HR + 16, PW), 0)
        ap = jnp.where(row == HR + 15, 0.0, pltpu.roll(ext, HR + 15, 0))
        z_ref[0, pl.ds(zh + HH, HH), cs] = pack(am)
        z_ref[1, pl.ds(zh + HH, HH), cs] = pack(a)
        z_ref[2, pl.ds(zh + HH - 8, HH + 8), cs] = pack(ap)
        return None

    def produce_row(s_ref, pv, z_ref, row0, k, cs_src, cs_dst, marker):
        r = row0 + W * k
        zs = pl.ds(k * HR, HR)
        if r < 0 or r >= HW:
            z = jnp.zeros((HR, 128), u32)
            for j in range(3):
                z_ref[j, zs, cs_dst] = z
            return
        a = act(s_ref[0, pl.ds(r, W), cs_src].astype(f32), pv, marker)
        row = lax.broadcasted_iota(jnp.int32, (W, 128), 0)
        z_ref[0, zs, cs_dst] = pack(jnp.where(row == 0, 0.0, pltpu.roll(a, 1, 0)))
        z_ref[1, zs, cs_dst] = pack(a)
        z_ref[2, zs, cs_dst] = pack(jnp.where(row == W - 1, 0.0, pltpu.roll(a, W - 1, 0)))

    def zload(z_ref, j, i):
        return pltpu.bitcast(z_ref[j, i * HR:i * HR + TM // 2, :], bf16)

    def stat_acc(v, state, marker=None):
        n = v.shape[0] // 8
        wd = v.shape[1]
        if state is None:
            K = v[0:1, :]
            if marker is not None:
                K = K + marker[0:1, :]
            d = v - K
            return (K, d.reshape(n, 8, wd).sum(axis=0), (d * d).reshape(n, 8, wd).sum(axis=0))
        K, s1, s2 = state
        Kd = K if marker is None else K + marker[0:1, :]
        d = v - Kd
        return (K, s1 + d.reshape(n, 8, wd).sum(axis=0), s2 + (d * d).reshape(n, 8, wd).sum(axis=0))

    def store_stats(st_ref, q, t, cs, state):
        K, s1, s2 = state
        wd = K.shape[1]
        st_ref[q, t, 0, :, cs] = jnp.broadcast_to(K, (8, wd))
        st_ref[q, t, 1, :, cs] = jnp.broadcast_to(s1.sum(axis=0, keepdims=True), (8, wd))
        st_ref[q, t, 2, :, cs] = jnp.broadcast_to(s2.sum(axis=0, keepdims=True), (8, wd))

    def finalize_group(st_ref, p_ref, gb_ref, e_ref, q, cv, cs, marker=None):
        K = st_ref[q, :, 0, :, cs]
        s1 = st_ref[q, :, 1, :, cs]
        s2 = st_ref[q, :, 2, :, cs]
        mean_t = K + s1 * (1.0 / TM)
        if e_ref is not None:
            e = e_ref[q, :, cs]
            mean_t = mean_t + e[None]
        if marker is not None:
            mean_t = mean_t + marker[None]
        m2_t = s2 - s1 * s1 * (1.0 / TM)
        mu = jnp.sum(jnp.sum(mean_t, axis=0), axis=1, keepdims=True) * (1.0 / (T * 128))
        dev = mean_t - mu[None]
        tot = m2_t + dev * dev * float(TM)
        var = jnp.sum(jnp.sum(tot, axis=0), axis=1, keepdims=True) * (1.0 / (HW * 128))
        rstd = lax.rsqrt(var + EPS)
        if e_ref is not None:
            p_ref[q, 0, :, cs] = mu - e
        else:
            p_ref[q, 0, :, cs] = jnp.broadcast_to(mu, (8, 128))
        p_ref[q, 1, :, cs] = gb_ref[cv, 0, :, cs] * (rstd * 0.5)
        p_ref[q, 2, :, cs] = gb_ref[cv, 1, :, cs] * 0.5

    def merge(lists):
        items = []
        for li, l in enumerate(lists):
            for i, it in enumerate(l):
                items.append(((i + 0.5) / len(l), li, it))
        items.sort(key=lambda z: (z[0], z[1]))
        return [it for _, _, it in items]

    def kern(x_hbm, te_hbm, g1_hbm, b1_hbm, w1_hbm, we_hbm, g2_hbm, b2_hbm, w2_hbm, o_hbm,
             s_ref, w_ref, za_ref, zb_ref, y00_ref, y01_ref, y10_ref, y11_ref,
             acca_ref, accb_ref, accc_ref, xa_ref, pca_ref, pcb_ref, st_ref, p_ref, gb_ref, e_ref,
             te_ref, we_ref, gsm_ref, sem_x, sem_w, sem_s, sem_o):

        def gcols(g):
            return pl.ds(mult(g * 128, 128), 128)

        def x0_copy(g):
            return pltpu.make_async_copy(x_hbm.at[0, :, gcols(g)], s_ref.at[0, :, gcols(g)], sem_x.at[g])

        NXP = 4
        XPR = HW // NXP

        def x00_copy(k):
            rows = pl.ds(mult(k * XPR, XPR), XPR)
            return pltpu.make_async_copy(x_hbm.at[0, rows, pl.ds(0, 128)], s_ref.at[0, rows, pl.ds(0, 128)],
                                         sem_x.at[G + k])

        def w1_copy(g, i):
            taps = pl.ds(3 * i, 3)
            return pltpu.make_async_copy(w1_hbm.at[taps, :, gcols(g)], w_ref.at[taps, :, gcols(g)], sem_w.at[g, i])

        def x1_copy():
            return pltpu.make_async_copy(x_hbm.at[1], s_ref.at[1], sem_s.at[6])

        def w2_copy():
            return pltpu.make_async_copy(w2_hbm, w_ref.at[pl.ds(9, 9)], sem_s.at[7])

        def small_copies():
            return [pltpu.make_async_copy(g1_hbm, gsm_ref.at[0], sem_s.at[0]),
                    pltpu.make_async_copy(b1_hbm, gsm_ref.at[1], sem_s.at[1]),
                    pltpu.make_async_copy(g2_hbm, gsm_ref.at[2], sem_s.at[2]),
                    pltpu.make_async_copy(b2_hbm, gsm_ref.at[3], sem_s.at[3]),
                    pltpu.make_async_copy(te_hbm, te_ref, sem_s.at[4])]

        def we_copy():
            return pltpu.make_async_copy(we_hbm, we_ref, sem_s.at[5])

        NQ = opts.get('nq', 4)
        QR = TM // NQ

        def o_copy(s, qi):
            b = divT(s) - 2
            r0 = mult(modT(s) * TM + qi * QR, QR)
            return pltpu.make_async_copy(s_ref.at[b, pl.ds(r0, QR), :], o_hbm.at[b, pl.ds(r0, QR), :], sem_o.at[0])

        def o_all():
            return pltpu.make_async_copy(s_ref.at[pl.ds(0, B)], o_hbm, sem_o.at[0])

        def epi_piece(acc_ref, s_prev, cb, ri, state, marker):
            p = divT(s_prev)
            t = modT(s_prev)
            cs = slice(cb * PW, (cb + 1) * PW)
            r0 = mult(t * TM + ri * ER, ER)
            a = acc_ref[ri * ER:(ri + 1) * ER, cs]
            if marker is not None:
                a = (a.reshape(ER // 8, 8, PW) + marker[None]).reshape(ER, PW)
            if isinstance(s_prev, int):
                is2 = p >= 2
                dst = p - 2 if is2 else p + 2
                res = a + s_ref[dst, pl.ds(r0, ER), cs].astype(f32) if is2 else a
                sq = None if is2 else p + 2
            else:
                is2 = p >= 2
                dst = jnp.where(is2, p - 2, p + 2)
                xr = s_ref[dst, pl.ds(r0, ER), cs].astype(f32)
                res = a + jnp.where(is2, xr, 0.0)
                sq = jnp.where(is2, 0, p + 2)
            if sq is not None:
                state = stat_acc(res, state)
            s_ref[dst, pl.ds(r0, ER), cs] = res.astype(bf16)
            if sq is not None and ri == NER - 1:
                store_stats(st_ref, sq, t, cs, state)
                state = None
            return state

        def xstat_piece(q, tile, cs, ri, state, marker):
            r0 = mult(tile * TM + ri * XR, XR)
            v = s_ref[q, pl.ds(r0, XR), cs].astype(f32)
            state = stat_acc(v, state, marker)
            if ri == NXR - 1:
                store_stats(st_ref, q, tile, cs, state)
                state = None
            return state

        def wsel(is_c2, tap):
            return pltpu.bitcast(jnp.where(is_c2, pltpu.bitcast(w_ref[9 + tap], u32),
                                           pltpu.bitcast(w_ref[tap], u32)), bf16)

        def half(s, zc_ref, zn_ref, accc_ref, accp_ref, kind):
            is_c2 = s >= 2 * T
            sn = s + 1
            pn = jnp.minimum(divT(sn), 3)
            tn = modT(sn)
            lists = [[('p', k, cb, part) for k in range(NCH) for cb in range(NPW) for part in range(2)],
                     [('e', cb, ri) for ri in range(NER) for cb in range(NPW)]]
            if not opts.get('nox'):
                lists.append([('x', tl, cb, ri) for tl in range(XT) for cb in range(NPW) for ri in range(NXR)])
            pieces = merge(lists)
            npc = len(pieces)
            if kind == 0:
                q = jnp.minimum(divT(s) + 1, 3)
                cv = lax.shift_right_logical(q, 1)
                for g in range(G):
                    finalize_group(st_ref, p_ref, gb_ref, e_ref, q, cv, slice(g * 128, (g + 1) * 128))
            if opts.get('pstat'):
                pc_ref = pca_ref if kind == 0 else pcb_ref
                pc_ref[...] = p_ref[pn]
                pv = tuple(pc_ref[k] for k in range(3))
            else:
                pv = tuple(p_ref[pn, k] for k in range(3))
            xj = jnp.clip(s - 2, 0, T // XT - 1) * XT
            done = 0
            acc = None
            est = [None] * NPW
            xst = None
            pcar = None
            order = (1, 2, 0) if kind == 0 else (0, 1, 2)
            total = 6 * TM + 3 * (TM - W)
            lim = total * last_slot // 36
            pos = 0
            for i in order:
                for j in range(3):
                    tap = i * 3 + j
                    skip = i == order[2]
                    if not skip:
                        lhs = zload(zc_ref, j, i)
                    elif kind == 0:
                        lhs = pltpu.bitcast(zc_ref[j, HR:TM // 2, :], bf16)
                    else:
                        lhs = pltpu.bitcast(zc_ref[j, 2 * HR:2 * HR + (TM - W) // 2, :], bf16)
                    if opts.get('fdyn') and acc is None and (kind == 0 or opts.get('fdyn') == 2):
                        wv = w_ref[jnp.where(is_c2, 9, 0) + tap]
                    else:
                        wv = wsel(is_c2, tap)
                    d = lax.dot_general(lhs, wv, NT, preferred_element_type=f32)
                    rows = d.shape[0]
                    for nn in range(4 * SUB):
                        n, sub = nn // SUB, nn % SUB
                        hi_ = min(npc, ((pos + (rows * (nn + 1)) // (4 * SUB)) * npc) // lim)
                        while done < hi_:
                            pc = pieces[done]
                            marker = marker_of(d, n, sub, PW)
                            if pc[0] == 'p':
                                pcar = produce_sub(s_ref, pv, zn_ref, pn, tn * TM - W, pc[1], pc[2], pc[3], pcar,
                                                   marker)
                            elif pc[0] == 'e':
                                est[pc[1]] = epi_piece(accp_ref, s - 1, pc[1], pc[2], est[pc[1]], marker)
                                if pc[1] == NPW - 1 and ((pc[2] + 1) * ER) % QR == 0:
                                    qi = ((pc[2] + 1) * ER) // QR - 1

                                    @pl.when(s - 1 >= 2 * T)
                                    def _():
                                        o_copy(s - 1, qi).start()
                            else:
                                xst = xstat_piece(1, xj + pc[1], slice(pc[2] * PW, (pc[2] + 1) * PW), pc[3],
                                                  xst, marker)
                            done += 1
                    pos += rows
                    if not skip:
                        acc = d if acc is None else acc + d
                    elif kind == 0:
                        acc = jnp.concatenate([acc[0:W], acc[W:] + d], axis=0)
                    else:
                        acc = jnp.concatenate([acc[0:TM - W] + d, acc[TM - W:]], axis=0)
            if kind == 0:
                top = jnp.where(modT(s) == 0, 0.0, xa_ref[...])
                acc = jnp.concatenate([acc[0:W] + top, acc[W:]], axis=0)
            accc_ref[...] = acc

        def halo_top(wget):
            d = None
            for j in range(3):
                dj = lax.dot_general(pltpu.bitcast(za_ref[j, 0:HR, :], bf16), wget(j), NT,
                                     preferred_element_type=f32)
                d = dj if d is None else d + dj
            xa_ref[...] = d

        def halo_bot(wget):
            d = None
            for j in range(3):
                dj = lax.dot_general(pltpu.bitcast(zb_ref[j, TM // 2 + HR:TM // 2 + 2 * HR, :], bf16), wget(6 + j),
                                     NT, preferred_element_type=f32)
                d = dj if d is None else d + dj
            accb_ref[TM - W:TM, :] = accb_ref[TM - W:TM, :] + d

        def load_pg(cs):
            return tuple(p_ref[0, k, :, cs] for k in range(3))

        def chunk_dots(y_ref, acc_ref, g, first, top, pieces, run, hook=None):
            cs = gcols(g)
            npc = len(pieces)
            KC = opts.get('kc', 1)
            ASUB = opts.get('asub', SUB * KC)
            ndot = 9 // KC
            nslots = (opts.get('a_last', 34) * ndot * 4 * ASUB) // 36
            done = 0
            acc = None
            di = 0
            for ti, i in enumerate((1, 2, 0)):
                if ti == 1 and hook is not None:
                    hook()
                skip = top and i == 0
                for j0 in range(0, 3, KC):
                    js = range(j0, j0 + KC)
                    if skip:
                        lhs = [pltpu.bitcast(y_ref[j, HR:TM // 2, :], bf16) for j in js]
                    else:
                        lhs = [zload(y_ref, j, i) for j in js]
                    rhs = [w_ref[i * 3 + j, :, cs] for j in js]
                    lhs = lhs[0] if KC == 1 else jnp.concatenate(lhs, axis=1)
                    rhs = rhs[0] if KC == 1 else jnp.concatenate(rhs, axis=1)
                    d = lax.dot_general(lhs, rhs, NT, preferred_element_type=f32)
                    for nn in range(4 * ASUB):
                        n, sub = nn // ASUB, nn % ASUB
                        slot = di * 4 * ASUB + nn
                        hi_ = min(npc, ((slot + 1) * npc) // nslots)
                        while done < hi_:
                            run(pieces[done], marker_of(d, n, sub, 128, ASUB))
                            done += 1
                    di += 1
                    if skip:
                        acc = jnp.concatenate([acc[0:W], acc[W:] + d], axis=0)
                    else:
                        acc = d if acc is None else acc + d
            if first:
                acc_ref[...] = jnp.where(g == 0, 0.0, acc_ref[...]) + acc
            else:
                acc_ref[...] = acc_ref[...] + acc

        with scope('prologue'):
            if opts.get('smallfirst', 1):
                for c in small_copies():
                    c.start()
            lax.fori_loop(0, NXP, lambda k, _: (x00_copy(k).start(), 0)[1], 0)
            if not opts.get('smallfirst', 1):
                def smalls(k, _):
                    for c in small_copies():
                        c.start()
                    return 0
                lax.fori_loop(0, 1, smalls, 0)

            def issue(g, _):
                @pl.when(g > 0)
                def _():
                    x0_copy(g).start()

                def wi(i, _):
                    w1_copy(g, jnp.where(i == 2, 0, i + 1)).start()
                    return 0
                lax.fori_loop(0, 3, wi, 0)
                return 0
            lax.fori_loop(0, G, issue, 0)

            def rest(c, _):
                @pl.when(c == 0)
                def _():
                    w2_copy().start()

                @pl.when(c == 1)
                def _():
                    x1_copy().start()

                @pl.when(c == 2)
                def _():
                    we_copy().start()
                return 0
            lax.fori_loop(0, 3, rest, 0)

            for c in small_copies():
                c.wait()
            for cv in range(2):
                for k in range(2):
                    v = gsm_ref[2 * cv + k].astype(f32)
                    for g in range(G):
                        gb_ref[cv, k, :, g * 128:(g + 1) * 128] = jnp.broadcast_to(v[g:g + 1, :], (8, 128))
            e_ref[...] = jnp.zeros(e_ref.shape, f32)
            st_ref[...] = jnp.zeros(st_ref.shape, f32)
            acca_ref[...] = jnp.zeros(acca_ref.shape, f32)
            accb_ref[...] = jnp.zeros(accb_ref.shape, f32)
            accc_ref[...] = jnp.zeros(accc_ref.shape, f32)

            c0 = slice(0, 128)

            def xs0(k, _):
                x00_copy(k).wait()
                for tt in range(T // NXP):
                    st = None
                    for ri in range(NXR):
                        st = xstat_piece(0, k * (T // NXP) + tt, c0, ri, st, None)
                return 0
            lax.fori_loop(0, NXP, xs0, 0)
            finalize_group(st_ref, p_ref, gb_ref, None, 0, 0, c0)
            pv0 = load_pg(c0)
            for k in range(NCH):
                produce_row(s_ref, pv0, y00_ref, -W, k, c0, c0, None)
                produce_row(s_ref, pv0, y01_ref, TM - W, k, c0, c0, None)

        def chunk(g, c, h):
            ycur = (y00_ref, y01_ref) if c == 0 else (y10_ref, y11_ref)
            ynxt = (y10_ref, y11_ref) if c == 0 else (y00_ref, y01_ref)
            gn = jnp.minimum(g + 1, G - 1)
            cs = gcols(g)
            csn = gcols(gn)
            c0 = slice(0, 128)
            pvc = load_pg(cs)
            state = {'e': [None] * NPW, 'x': None, 'pv': None}
            zs = [('z', k) for k in range(NCH)]
            xs = [('x', t, ri) for t in range(T) for ri in range(NXR)]
            ps = [('p', tl, k) for k in range(NCH) for tl in range(2)]
            es = [('e', cb, ri) for cb in range(NPW) for ri in range(NER)]
            nz = opts.get('nz', 4)
            if c == 0:
                part0 = zs[:nz]
                part1 = xs + [('f',)] + zs[nz:] + ps
            else:
                part0 = merge([xs, zs[:nz]]) + [('f',)] + zs[nz:]
                part1 = merge([ps, es])

            def run(pc, mk):
                if pc[0] == 'z':
                    produce_row(s_ref, pvc, za_ref, 2 * TM - W, pc[1], cs, cs, mk)
                elif pc[0] == 'e':
                    mw = jnp.concatenate([mk] * (PW // 128), axis=1)
                    state['e'][pc[1]] = epi_piece(accc_ref, 0, pc[1], pc[2], state['e'][pc[1]], mw)
                elif pc[0] == 'x':
                    state['x'] = xstat_piece(0, pc[1], csn, pc[2], state['x'], mk)
                elif pc[0] == 'f':
                    finalize_group(st_ref, p_ref, gb_ref, None, 0, 0, csn)
                    state['pv'] = load_pg(csn)
                else:
                    produce_row(s_ref, state['pv'], ynxt[pc[1]], pc[1] * TM - W, pc[2], csn, c0, mk)
            def hook():
                w1_copy(g, 2).wait()
                w1_copy(g, 0).wait()
            chunk_dots(ycur[0], accc_ref, g, c == 0, True, part0, run, hook if c == 0 else None)
            if c == 0:
                x0_copy(g + 1).wait()
            chunk_dots(ycur[1], accb_ref, g, c == 0, False, part1, run)

        def phase_a(h, _):
            g0 = 2 * h
            w1_copy(g0, 1).wait()
            chunk(g0, 0, h)
            for i in range(3):
                w1_copy(g0 + 1, i).wait()

            @pl.when(h == 0)
            def _():
                x0_copy(2).wait()
            chunk(g0 + 1, 1, h)
            return 0

        with scope('first'):
            lax.fori_loop(0, 2, phase_a, 0)

        with scope('mid'):
            w2_copy().wait()
            x1_copy().wait()
            we_copy().wait()
            te = te_ref[...].astype(f32)
            sl = te * jax.nn.sigmoid(te)
            emb = jnp.dot(sl.astype(bf16), we_ref[...], preferred_element_type=f32)
            e_ref[2] = jnp.broadcast_to(emb[0:1, :], (8, C))
            e_ref[3] = jnp.broadcast_to(emb[1:2, :], (8, C))
            halo_top(lambda tap: w_ref[tap])

        NIT = (NSTEP - 2) // 2

        def body(it, carry):
            s0 = 2 * it + 2
            s1 = s0 + 1
            with scope('iter'):
                half(s0, za_ref, zb_ref, acca_ref, accb_ref, 0)
                half(s1, zb_ref, za_ref, accb_ref, acca_ref, 1)

            @pl.when(modT(s1) != T - 1)
            def _():
                if opts.get('hdyn') == 1:
                    wb = jnp.where(s1 >= 2 * T, 9, 0)
                    wget = lambda tap: w_ref[wb + tap]
                elif opts.get('hdyn') == 2:
                    wb = jnp.where(s1 >= 2 * T, 9, 0)
                    wget = lambda tap: w_ref[wb + tap] if tap == 6 else wsel(s1 >= 2 * T, tap)
                else:
                    wget = lambda tap: wsel(s1 >= 2 * T, tap)
                with scope('halo'):
                    halo_bot(wget)
                    halo_top(wget)
            return carry

        with scope('main'):
            lax.fori_loop(0, NIT, body, 0)

        sl_ = NSTEP - 1
        with scope('final'):
            st = [None] * NPW
            for ri in range(NER):
                for cb in range(NPW):
                    st[cb] = epi_piece(accb_ref, sl_, cb, ri, st[cb], None)
                if ((ri + 1) * ER) % QR == 0:
                    o_copy(sl_, ((ri + 1) * ER) // QR - 1).start()
        with scope('owait'):
            o_all().wait()

    def fn(x, t_emb, g1, be1, w1, w_emb, g2, be2, w2):
        xn = jnp.transpose(x, (0, 2, 3, 1)).reshape(B, HW, C)
        w1t = jnp.transpose(w1, (2, 3, 0, 1)).reshape(9, C, C)
        w2t = jnp.transpose(w2, (2, 3, 0, 1)).reshape(9, C, C)
        any_spec = pl.BlockSpec(memory_space=pl.ANY)
        zbuf = pltpu.VMEM((3, R // 2, C), u32)
        ybuf = pltpu.VMEM((3, R // 2, 128), u32)
        abuf = pltpu.VMEM((TM, C), f32)
        out = pl.pallas_call(
            kern,
            in_specs=[any_spec] * 9,
            out_specs=any_spec,
            out_shape=jax.ShapeDtypeStruct((B, HW, C), bf16),
            scratch_shapes=[
                pltpu.VMEM((4, HW, C), bf16),
                pltpu.VMEM((18, C, C), bf16),
                zbuf, zbuf, ybuf, ybuf, ybuf, ybuf,
                abuf, abuf, abuf,
                pltpu.VMEM((W, C), f32),
                pltpu.VMEM((3, 8, C), f32),
                pltpu.VMEM((3, 8, C), f32),
                pltpu.VMEM((4, T, 3, 8, C), f32),
                pltpu.VMEM((4, 3, 8, C), f32),
                pltpu.VMEM((2, 2, 8, C), f32),
                pltpu.VMEM((4, 8, C), f32),
                pltpu.VMEM((B, E), bf16),
                pltpu.VMEM((E, C), bf16),
                pltpu.VMEM((4, G, 128), bf16),
                pltpu.SemaphoreType.DMA((G + 4,)),
                pltpu.SemaphoreType.DMA((G, 3)),
                pltpu.SemaphoreType.DMA((8,)),
                pltpu.SemaphoreType.DMA((1,)),
            ],
            compiler_params=pltpu.CompilerParams(vmem_limit_bytes=100 * 1024 * 1024,
                                                 disable_bounds_checks=True),
        )(xn, t_emb, g1.reshape(G, 128), be1.reshape(G, 128), w1t, w_emb,
          g2.reshape(G, 128), be2.reshape(G, 128), w2t)
        return jnp.transpose(out.reshape(B, H, W, C), (0, 3, 1, 2))
    return fn


_OPTS = {'sub': 8, 'kc': 3}


@jax.jit
def pallas_standalone__adm_resblock__diffusion_kernel(x, t_emb, g1, be1, w1, w_emb, g2, be2, w2):
    B, C, H, W = x.shape
    E = t_emb.shape[1]
    return build(B, C, H, W, E, TM=512, opts=_OPTS)(x, t_emb, g1, be1, w1, w_emb, g2, be2, w2)
```

```python
import jax
import jax.numpy as jnp
from jax import lax
from jax.experimental import pallas as pl
from jax.experimental.pallas import tpu as pltpu

f32 = jnp.float32
bf16 = jnp.bfloat16
u32 = jnp.uint32
NT = (((1,), (1,)), ((), ()))


def build(B, C, H, W, E, TM=512, opts=None):
    opts = opts or {}
    HW = H * W
    G = 4
    CG = C // G
    EPS = 1e-5
    T = HW // TM
    assert CG == 128 and B == 2 and T == 8 and W == 64
    R = TM + 2 * W
    NCH = R // W
    NSTEP = 4 * T
    ER = opts.get('er', 32)
    NER = TM // ER
    XT = 2
    last_slot = opts.get('last_slot', 34)
    scope = jax.named_scope

    PW = opts.get('pw', 256)
    NPW = C // PW
    SUB = opts.get('sub', 4)
    XR = opts.get('xr', 64)
    NXR = TM // XR
    HR = W // 2
    HH = HR // 2

    def divT(v):
        return v // T if isinstance(v, int) else lax.shift_right_logical(v, 3)

    def modT(v):
        return v % T if isinstance(v, int) else jnp.bitwise_and(v, T - 1)

    def mult(v, m):
        return v if isinstance(v, int) else pl.multiple_of(v, m)

    def marker_of(d, n, sub, width, nsub=SUB):
        rp = sub * (d.shape[0] // nsub) // 8 * 8
        m = d[rp:rp + 8, n * 128:(n + 1) * 128]
        b = pltpu.bitcast(m, u32)
        z = pltpu.bitcast((b >> 16) >> 16, f32)
        if width > 128:
            z = jnp.concatenate([z] * (width // 128), axis=1)
        return z

    def pack(t):
        return pltpu.bitcast(t.astype(bf16), u32)

    def act(v, pv, marker):
        n, wd = v.shape
        mu, sc, bt = pv
        if marker is not None:
            mu = mu + marker
        v3 = v.reshape(n // 8, 8, wd)
        hz = ((v3 - mu[None]) * sc[None] + bt[None]).reshape(n, wd)
        return hz * jnp.tanh(hz) + hz

    def produce_sub(s_ref, pv, z_ref, q, row0, k, cb, part, carry, marker):
        r = row0 + W * k
        rc = pl.multiple_of(jnp.clip(r, 0, HW - W) + part * HR, HR)
        cs = slice(cb * PW, (cb + 1) * PW)
        a = act(s_ref[q, pl.ds(rc, HR), cs].astype(f32), tuple(p[:, cs] for p in pv), marker)
        zh = k * HR
        if part == 0:
            row = lax.broadcasted_iota(jnp.int32, (HR, PW), 0)
            am = jnp.where(row == 0, 0.0, pltpu.roll(a, 1, 0))
            ap = pltpu.roll(a, HR - 1, 0)[0:HR - 16]
            z_ref[0, pl.ds(zh, HH), cs] = pack(am)
            z_ref[1, pl.ds(zh, HH), cs] = pack(a)
            z_ref[2, pl.ds(zh, HH - 8), cs] = pack(ap)
            return a[HR - 16:HR]
        ext = jnp.concatenate([carry, a], axis=0)
        am = pltpu.roll(ext, 1, 0)[16:HR + 16]
        row = lax.broadcasted_iota(jnp.int32, (HR + 16, PW), 0)
        ap = jnp.where(row == HR + 15, 0.0, pltpu.roll(ext, HR + 15, 0))
        z_ref[0, pl.ds(zh + HH, HH), cs] = pack(am)
        z_ref[1, pl.ds(zh + HH, HH), cs] = pack(a)
        z_ref[2, pl.ds(zh + HH - 8, HH + 8), cs] = pack(ap)
        return None

    def produce_row(s_ref, pv, z_ref, row0, k, cs_src, cs_dst, marker):
        r = row0 + W * k
        zs = pl.ds(k * HR, HR)
        if r < 0 or r >= HW:
            z = jnp.zeros((HR, 128), u32)
            for j in range(3):
                z_ref[j, zs, cs_dst] = z
            return
        a = act(s_ref[0, pl.ds(r, W), cs_src].astype(f32), pv, marker)
        row = lax.broadcasted_iota(jnp.int32, (W, 128), 0)
        z_ref[0, zs, cs_dst] = pack(jnp.where(row == 0, 0.0, pltpu.roll(a, 1, 0)))
        z_ref[1, zs, cs_dst] = pack(a)
        z_ref[2, zs, cs_dst] = pack(jnp.where(row == W - 1, 0.0, pltpu.roll(a, W - 1, 0)))

    def zload(z_ref, j, i):
        return pltpu.bitcast(z_ref[j, i * HR:i * HR + TM // 2, :], bf16)

    def stat_acc(v, state, marker=None):
        n = v.shape[0] // 8
        wd = v.shape[1]
        if state is None:
            K = v[0:1, :]
            if marker is not None:
                K = K + marker[0:1, :]
            d = v - K
            return (K, d.reshape(n, 8, wd).sum(axis=0), (d * d).reshape(n, 8, wd).sum(axis=0))
        K, s1, s2 = state
        Kd = K if marker is None else K + marker[0:1, :]
        d = v - Kd
        return (K, s1 + d.reshape(n, 8, wd).sum(axis=0), s2 + (d * d).reshape(n, 8, wd).sum(axis=0))

    def store_stats(st_ref, q, t, cs, state):
        K, s1, s2 = state
        wd = K.shape[1]
        st_ref[q, t, 0, :, cs] = jnp.broadcast_to(K, (8, wd))
        st_ref[q, t, 1, :, cs] = jnp.broadcast_to(s1.sum(axis=0, keepdims=True), (8, wd))
        st_ref[q, t, 2, :, cs] = jnp.broadcast_to(s2.sum(axis=0, keepdims=True), (8, wd))

    def finalize_group(st_ref, p_ref, gb_ref, e_ref, q, cv, cs, marker=None):
        K = st_ref[q, :, 0, :, cs]
        s1 = st_ref[q, :, 1, :, cs]
        s2 = st_ref[q, :, 2, :, cs]
        mean_t = K + s1 * (1.0 / TM)
        if e_ref is not None:
            e = e_ref[q, :, cs]
            mean_t = mean_t + e[None]
        if marker is not None:
            mean_t = mean_t + marker[None]
        m2_t = s2 - s1 * s1 * (1.0 / TM)
        mu = jnp.sum(jnp.sum(mean_t, axis=0), axis=1, keepdims=True) * (1.0 / (T * 128))
        dev = mean_t - mu[None]
        tot = m2_t + dev * dev * float(TM)
        var = jnp.sum(jnp.sum(tot, axis=0), axis=1, keepdims=True) * (1.0 / (HW * 128))
        rstd = lax.rsqrt(var + EPS)
        if e_ref is not None:
            p_ref[q, 0, :, cs] = mu - e
        else:
            p_ref[q, 0, :, cs] = jnp.broadcast_to(mu, (8, 128))
        p_ref[q, 1, :, cs] = gb_ref[cv, 0, :, cs] * (rstd * 0.5)
        p_ref[q, 2, :, cs] = gb_ref[cv, 1, :, cs] * 0.5

    def merge(lists):
        items = []
        for li, l in enumerate(lists):
            for i, it in enumerate(l):
                items.append(((i + 0.5) / len(l), li, it))
        items.sort(key=lambda z: (z[0], z[1]))
        return [it for _, _, it in items]

    def kern(x_hbm, te_hbm, g1_hbm, b1_hbm, w1_hbm, we_hbm, g2_hbm, b2_hbm, w2_hbm, o_hbm,
             s_ref, w_ref, w32_ref, za_ref, zb_ref, y00_ref, y01_ref, y10_ref, y11_ref,
             acca_ref, accb_ref, accc_ref, xa_ref, pca_ref, pcb_ref, st_ref, p_ref, gb_ref, e_ref,
             te_ref, we_ref, gsm_ref, sem_x, sem_w, sem_s, sem_o):

        def gcols(g):
            return pl.ds(mult(g * 128, 128), 128)

        def x0_copy(g):
            return pltpu.make_async_copy(x_hbm.at[0, :, gcols(g)], s_ref.at[0, :, gcols(g)], sem_x.at[g])

        NXP = 4
        XPR = HW // NXP

        def x00_copy(k):
            rows = pl.ds(mult(k * XPR, XPR), XPR)
            return pltpu.make_async_copy(x_hbm.at[0, rows, pl.ds(0, 128)], s_ref.at[0, rows, pl.ds(0, 128)],
                                         sem_x.at[G + k])

        def w1_copy(g, i):
            taps = pl.ds(3 * i, 3)
            return pltpu.make_async_copy(w1_hbm.at[taps, :, gcols(g)], w_ref.at[taps, :, gcols(g)], sem_w.at[g, i])

        def x1_copy():
            return pltpu.make_async_copy(x_hbm.at[1], s_ref.at[1], sem_s.at[6])

        def w2_copy():
            return pltpu.make_async_copy(w2_hbm, w_ref.at[pl.ds(9, 9)], sem_s.at[7])

        def small_copies():
            return [pltpu.make_async_copy(g1_hbm, gsm_ref.at[0], sem_s.at[0]),
                    pltpu.make_async_copy(b1_hbm, gsm_ref.at[1], sem_s.at[1]),
                    pltpu.make_async_copy(g2_hbm, gsm_ref.at[2], sem_s.at[2]),
                    pltpu.make_async_copy(b2_hbm, gsm_ref.at[3], sem_s.at[3]),
                    pltpu.make_async_copy(te_hbm, te_ref, sem_s.at[4])]

        def we_copy():
            return pltpu.make_async_copy(we_hbm, we_ref, sem_s.at[5])

        NQ = opts.get('nq', 4)
        QR = TM // NQ

        def o_copy(s, qi):
            b = divT(s) - 2
            r0 = mult(modT(s) * TM + qi * QR, QR)
            return pltpu.make_async_copy(s_ref.at[b, pl.ds(r0, QR), :], o_hbm.at[b, pl.ds(r0, QR), :], sem_o.at[0])

        def o_all():
            return pltpu.make_async_copy(s_ref.at[pl.ds(0, B)], o_hbm, sem_o.at[0])

        def epi_piece(acc_ref, s_prev, cb, ri, state, marker):
            p = divT(s_prev)
            t = modT(s_prev)
            cs = slice(cb * PW, (cb + 1) * PW)
            r0 = mult(t * TM + ri * ER, ER)
            a = acc_ref[ri * ER:(ri + 1) * ER, cs]
            if marker is not None:
                a = (a.reshape(ER // 8, 8, PW) + marker[None]).reshape(ER, PW)
            if isinstance(s_prev, int):
                is2 = p >= 2
                dst = p - 2 if is2 else p + 2
                res = a + s_ref[dst, pl.ds(r0, ER), cs].astype(f32) if is2 else a
                sq = None if is2 else p + 2
            else:
                is2 = p >= 2
                dst = jnp.where(is2, p - 2, p + 2)
                xr = s_ref[dst, pl.ds(r0, ER), cs].astype(f32)
                res = a + jnp.where(is2, xr, 0.0)
                sq = jnp.where(is2, 0, p + 2)
            if sq is not None:
                state = stat_acc(res, state)
            s_ref[dst, pl.ds(r0, ER), cs] = res.astype(bf16)
            if sq is not None and ri == NER - 1:
                store_stats(st_ref, sq, t, cs, state)
                state = None
            return state

        def xstat_piece(q, tile, cs, ri, state, marker):
            r0 = mult(tile * TM + ri * XR, XR)
            v = s_ref[q, pl.ds(r0, XR), cs].astype(f32)
            state = stat_acc(v, state, marker)
            if ri == NXR - 1:
                store_stats(st_ref, q, tile, cs, state)
                state = None
            return state

        def wsel(is_c2, tap):
            if opts.get('w32'):
                return pltpu.bitcast(jnp.where(is_c2, w32_ref[9 + tap], w32_ref[tap]), bf16)
            return pltpu.bitcast(jnp.where(is_c2, pltpu.bitcast(w_ref[9 + tap], u32),
                                           pltpu.bitcast(w_ref[tap], u32)), bf16)

        def half(s, zc_ref, zn_ref, accc_ref, accp_ref, kind):
            is_c2 = s >= 2 * T
            sn = s + 1
            pn = jnp.minimum(divT(sn), 3)
            tn = modT(sn)
            lists = [[('p', k, cb, part) for k in range(NCH) for cb in range(NPW) for part in range(2)],
                     [('e', cb, ri) for ri in range(NER) for cb in range(NPW)]]
            if not opts.get('nox'):
                lists.append([('x', tl, cb, ri) for tl in range(XT) for cb in range(NPW) for ri in range(NXR)])
            pieces = merge(lists)
            npc = len(pieces)
            if kind == 0:
                q = jnp.minimum(divT(s) + 1, 3)
                cv = lax.shift_right_logical(q, 1)
                for g in range(G):
                    finalize_group(st_ref, p_ref, gb_ref, e_ref, q, cv, slice(g * 128, (g + 1) * 128))
            if opts.get('pstat'):
                pc_ref = pca_ref if kind == 0 else pcb_ref
                pc_ref[...] = p_ref[pn]
                pv = tuple(pc_ref[k] for k in range(3))
            else:
                pv = tuple(p_ref[pn, k] for k in range(3))
            xj = jnp.clip(s - 2, 0, T // XT - 1) * XT
            done = 0
            acc = None
            est = [None] * NPW
            xst = None
            pcar = None
            order = (1, 2, 0) if kind == 0 else (0, 1, 2)
            total = 6 * TM + 3 * (TM - W)
            lim = total * last_slot // 36
            pos = 0
            for i in order:
                for j in range(3):
                    tap = i * 3 + j
                    skip = i == order[2]
                    if not skip:
                        lhs = zload(zc_ref, j, i)
                    elif kind == 0:
                        lhs = pltpu.bitcast(zc_ref[j, HR:TM // 2, :], bf16)
                    else:
                        lhs = pltpu.bitcast(zc_ref[j, 2 * HR:2 * HR + (TM - W) // 2, :], bf16)
                    if opts.get('fdyn') and acc is None and (kind == 0 or opts.get('fdyn') == 2):
                        wv = w_ref[jnp.where(is_c2, 9, 0) + tap]
                    else:
                        wv = wsel(is_c2, tap)
                    d = lax.dot_general(lhs, wv, NT, preferred_element_type=f32)
                    rows = d.shape[0]
                    for nn in range(4 * SUB):
                        n, sub = nn // SUB, nn % SUB
                        hi_ = min(npc, ((pos + (rows * (nn + 1)) // (4 * SUB)) * npc) // lim)
                        while done < hi_:
                            pc = pieces[done]
                            marker = marker_of(d, n, sub, PW)
                            if pc[0] == 'p':
                                pcar = produce_sub(s_ref, pv, zn_ref, pn, tn * TM - W, pc[1], pc[2], pc[3], pcar,
                                                   marker)
                            elif pc[0] == 'e':
                                est[pc[1]] = epi_piece(accp_ref, s - 1, pc[1], pc[2], est[pc[1]], marker)
                                if pc[1] == NPW - 1 and ((pc[2] + 1) * ER) % QR == 0:
                                    qi = ((pc[2] + 1) * ER) // QR - 1

                                    @pl.when(s - 1 >= 2 * T)
                                    def _():
                                        o_copy(s - 1, qi).start()
                            else:
                                xst = xstat_piece(1, xj + pc[1], slice(pc[2] * PW, (pc[2] + 1) * PW), pc[3],
                                                  xst, marker)
                            done += 1
                    pos += rows
                    if not skip:
                        acc = d if acc is None else acc + d
                    elif kind == 0:
                        acc = jnp.concatenate([acc[0:W], acc[W:] + d], axis=0)
                    else:
                        acc = jnp.concatenate([acc[0:TM - W] + d, acc[TM - W:]], axis=0)
            if kind == 0:
                top = jnp.where(modT(s) == 0, 0.0, xa_ref[...])
                acc = jnp.concatenate([acc[0:W] + top, acc[W:]], axis=0)
            accc_ref[...] = acc

        def halo_top(wget):
            d = None
            for j in range(3):
                dj = lax.dot_general(pltpu.bitcast(za_ref[j, 0:HR, :], bf16), wget(j), NT,
                                     preferred_element_type=f32)
                d = dj if d is None else d + dj
            xa_ref[...] = d

        def halo_bot(wget):
            d = None
            for j in range(3):
                dj = lax.dot_general(pltpu.bitcast(zb_ref[j, TM // 2 + HR:TM // 2 + 2 * HR, :], bf16), wget(6 + j),
                                     NT, preferred_element_type=f32)
                d = dj if d is None else d + dj
            accb_ref[TM - W:TM, :] = accb_ref[TM - W:TM, :] + d

        def load_pg(cs):
            return tuple(p_ref[0, k, :, cs] for k in range(3))

        def chunk_dots(y_ref, acc_ref, g, first, top, pieces, run, hook=None):
            cs = gcols(g)
            npc = len(pieces)
            KC = opts.get('kc', 1)
            ASUB = opts.get('asub', SUB * KC)
            ndot = 9 // KC
            nslots = (opts.get('a_last', 34) * ndot * 4 * ASUB) // 36
            done = 0
            acc = None
            di = 0
            for ti, i in enumerate((1, 2, 0)):
                if ti == 1 and hook is not None:
                    hook()
                skip = top and i == 0
                for j0 in range(0, 3, KC):
                    js = range(j0, j0 + KC)
                    if skip:
                        lhs = [pltpu.bitcast(y_ref[j, HR:TM // 2, :], bf16) for j in js]
                    else:
                        lhs = [zload(y_ref, j, i) for j in js]
                    rhs = [w_ref[i * 3 + j, :, cs] for j in js]
                    if top and opts.get('w32'):
                        for j, r in zip(js, rhs):
                            w32_ref[i * 3 + j, :, cs] = pltpu.bitcast(r, u32)
                    lhs = lhs[0] if KC == 1 else jnp.concatenate(lhs, axis=1)
                    rhs = rhs[0] if KC == 1 else jnp.concatenate(rhs, axis=1)
                    d = lax.dot_general(lhs, rhs, NT, preferred_element_type=f32)
                    for nn in range(4 * ASUB):
                        n, sub = nn // ASUB, nn % ASUB
                        slot = di * 4 * ASUB + nn
                        hi_ = min(npc, ((slot + 1) * npc) // nslots)
                        while done < hi_:
                            run(pieces[done], marker_of(d, n, sub, 128, ASUB))
                            done += 1
                    di += 1
                    if skip:
                        acc = jnp.concatenate([acc[0:W], acc[W:] + d], axis=0)
                    else:
                        acc = d if acc is None else acc + d
            if first:
                acc_ref[...] = jnp.where(g == 0, 0.0, acc_ref[...]) + acc
            else:
                acc_ref[...] = acc_ref[...] + acc

        with scope('prologue'):
            if opts.get('smallfirst', 1):
                for c in small_copies():
                    c.start()
            lax.fori_loop(0, NXP, lambda k, _: (x00_copy(k).start(), 0)[1], 0)
            if not opts.get('smallfirst', 1):
                def smalls(k, _):
                    for c in small_copies():
                        c.start()
                    return 0
                lax.fori_loop(0, 1, smalls, 0)

            def issue(g, _):
                @pl.when(g > 0)
                def _():
                    x0_copy(g).start()

                def wi(i, _):
                    w1_copy(g, jnp.where(i == 2, 0, i + 1)).start()
                    return 0
                lax.fori_loop(0, 3, wi, 0)
                return 0
            lax.fori_loop(0, G, issue, 0)

            for c in small_copies():
                c.wait()
            for cv in range(2):
                for k in range(2):
                    v = gsm_ref[2 * cv + k].astype(f32)
                    for g in range(G):
                        gb_ref[cv, k, :, g * 128:(g + 1) * 128] = jnp.broadcast_to(v[g:g + 1, :], (8, 128))
            e_ref[...] = jnp.zeros(e_ref.shape, f32)
            st_ref[...] = jnp.zeros(st_ref.shape, f32)
            acca_ref[...] = jnp.zeros(acca_ref.shape, f32)
            accb_ref[...] = jnp.zeros(accb_ref.shape, f32)
            accc_ref[...] = jnp.zeros(accc_ref.shape, f32)

            c0 = slice(0, 128)

            def xs0(k, _):
                x00_copy(k).wait()
                for tt in range(T // NXP):
                    st = None
                    for ri in range(NXR):
                        st = xstat_piece(0, k * (T // NXP) + tt, c0, ri, st, None)
                return 0
            lax.fori_loop(0, NXP, xs0, 0)
            finalize_group(st_ref, p_ref, gb_ref, None, 0, 0, c0)
            pv0 = load_pg(c0)
            for k in range(NCH):
                produce_row(s_ref, pv0, y00_ref, -W, k, c0, c0, None)
                produce_row(s_ref, pv0, y01_ref, TM - W, k, c0, c0, None)

        def chunk(g, c, h):
            ycur = (y00_ref, y01_ref) if c == 0 else (y10_ref, y11_ref)
            ynxt = (y10_ref, y11_ref) if c == 0 else (y00_ref, y01_ref)
            gn = jnp.minimum(g + 1, G - 1)
            cs = gcols(g)
            csn = gcols(gn)
            c0 = slice(0, 128)
            pvc = load_pg(cs)
            state = {'e': [None] * NPW, 'x': None, 'pv': None}
            zs = [('z', k) for k in range(NCH)]
            xs = [('x', t, ri) for t in range(T) for ri in range(NXR)]
            ps = [('p', tl, k) for k in range(NCH) for tl in range(2)]
            es = [('e', cb, ri) for cb in range(NPW) for ri in range(NER)]
            nz = opts.get('nz', 4)
            RP = opts.get('rp', 1)
            rs = [('r', tap, cb, rr) for tap in range(9) for cb in range(4) for rr in range(RP)]
            if c == 0:
                part0 = zs[:nz]
                part1 = merge([xs + [('f',)] + zs[nz:] + ps, rs])
            else:
                part0 = merge([xs, zs[:nz]]) + [('f',)] + zs[nz:]
                part1 = merge([ps, es])

            def run(pc, mk):
                if pc[0] == 'z':
                    produce_row(s_ref, pvc, za_ref, 2 * TM - W, pc[1], cs, cs, mk)
                elif pc[0] == 'e':
                    mw = jnp.concatenate([mk] * (PW // 128), axis=1)
                    state['e'][pc[1]] = epi_piece(accc_ref, 0, pc[1], pc[2], state['e'][pc[1]], mw)
                elif pc[0] == 'r':
                    rsl = slice(pc[2] * 128, (pc[2] + 1) * 128)
                    nr = C // RP
                    v = pltpu.bitcast(w_ref[9 + pc[1], pc[3] * nr:(pc[3] + 1) * nr, rsl], u32)
                    m = pltpu.bitcast(mk, u32)
                    v = (v.reshape(nr // 16, 8, 128) | m[None]).reshape(nr // 2, 128)
                    w32_ref[9 + pc[1], pc[3] * nr // 2:(pc[3] + 1) * nr // 2, rsl] = v
                elif pc[0] == 'x':
                    state['x'] = xstat_piece(0, pc[1], csn, pc[2], state['x'], mk)
                elif pc[0] == 'f':
                    finalize_group(st_ref, p_ref, gb_ref, None, 0, 0, csn)
                    state['pv'] = load_pg(csn)
                else:
                    produce_row(s_ref, state['pv'], ynxt[pc[1]], pc[1] * TM - W, pc[2], csn, c0, mk)
            def hook():
                w1_copy(g, 2).wait()
                w1_copy(g, 0).wait()
            chunk_dots(ycur[0], accc_ref, g, c == 0, True, part0, run, hook if c == 0 else None)
            if c == 0:
                x0_copy(g + 1).wait()

                @pl.when(h == 1)
                def _():
                    w2_copy().wait()
            chunk_dots(ycur[1], accb_ref, g, c == 0, False, part1, run)

        def phase_a(h, _):
            g0 = 2 * h
            w1_copy(g0, 1).wait()
            chunk(g0, 0, h)
            for i in range(3):
                w1_copy(g0 + 1, i).wait()

            @pl.when(h == 0)
            def _():
                x0_copy(2).wait()

                def rest(c, _):
                    @pl.when(c == 0)
                    def _():
                        w2_copy().start()

                    @pl.when(c == 1)
                    def _():
                        x1_copy().start()

                    @pl.when(c == 2)
                    def _():
                        we_copy().start()
                    return 0
                lax.fori_loop(0, 3, rest, 0)
            chunk(g0 + 1, 1, h)
            return 0

        with scope('first'):
            lax.fori_loop(0, 2, phase_a, 0)

        with scope('mid'):
            x1_copy().wait()
            we_copy().wait()
            te = te_ref[...].astype(f32)
            sl = te * jax.nn.sigmoid(te)
            emb = jnp.dot(sl.astype(bf16), we_ref[...], preferred_element_type=f32)
            e_ref[2] = jnp.broadcast_to(emb[0:1, :], (8, C))
            e_ref[3] = jnp.broadcast_to(emb[1:2, :], (8, C))
            halo_top(lambda tap: w_ref[tap])

        NIT = (NSTEP - 2) // 2

        def body(it, carry):
            s0 = 2 * it + 2
            s1 = s0 + 1
            with scope('iter'):
                half(s0, za_ref, zb_ref, acca_ref, accb_ref, 0)
                half(s1, zb_ref, za_ref, accb_ref, acca_ref, 1)

            @pl.when(modT(s1) != T - 1)
            def _():
                if opts.get('hdyn') == 1:
                    wb = jnp.where(s1 >= 2 * T, 9, 0)
                    wget = lambda tap: w_ref[wb + tap]
                elif opts.get('hdyn') == 2:
                    wb = jnp.where(s1 >= 2 * T, 9, 0)
                    wget = lambda tap: w_ref[wb + tap] if tap == 6 else wsel(s1 >= 2 * T, tap)
                else:
                    wget = lambda tap: wsel(s1 >= 2 * T, tap)
                with scope('halo'):
                    halo_bot(wget)
                    halo_top(wget)
            return carry

        with scope('main'):
            lax.fori_loop(0, NIT, body, 0)

        sl_ = NSTEP - 1
        with scope('final'):
            st = [None] * NPW
            for ri in range(NER):
                for cb in range(NPW):
                    st[cb] = epi_piece(accb_ref, sl_, cb, ri, st[cb], None)
                if ((ri + 1) * ER) % QR == 0:
                    o_copy(sl_, ((ri + 1) * ER) // QR - 1).start()
        with scope('owait'):
            o_all().wait()

    def fn(x, t_emb, g1, be1, w1, w_emb, g2, be2, w2):
        xn = jnp.transpose(x, (0, 2, 3, 1)).reshape(B, HW, C)
        w1t = jnp.transpose(w1, (2, 3, 0, 1)).reshape(9, C, C)
        w2t = jnp.transpose(w2, (2, 3, 0, 1)).reshape(9, C, C)
        any_spec = pl.BlockSpec(memory_space=pl.ANY)
        zbuf = pltpu.VMEM((3, R // 2, C), u32)
        ybuf = pltpu.VMEM((3, R // 2, 128), u32)
        abuf = pltpu.VMEM((TM, C), f32)
        out = pl.pallas_call(
            kern,
            in_specs=[any_spec] * 9,
            out_specs=any_spec,
            out_shape=jax.ShapeDtypeStruct((B, HW, C), bf16),
            scratch_shapes=[
                pltpu.VMEM((4, HW, C), bf16),
                pltpu.VMEM((18, C, C), bf16),
                pltpu.VMEM((18, C // 2, C), u32),
                zbuf, zbuf, ybuf, ybuf, ybuf, ybuf,
                abuf, abuf, abuf,
                pltpu.VMEM((W, C), f32),
                pltpu.VMEM((3, 8, C), f32),
                pltpu.VMEM((3, 8, C), f32),
                pltpu.VMEM((4, T, 3, 8, C), f32),
                pltpu.VMEM((4, 3, 8, C), f32),
                pltpu.VMEM((2, 2, 8, C), f32),
                pltpu.VMEM((4, 8, C), f32),
                pltpu.VMEM((B, E), bf16),
                pltpu.VMEM((E, C), bf16),
                pltpu.VMEM((4, G, 128), bf16),
                pltpu.SemaphoreType.DMA((G + 4,)),
                pltpu.SemaphoreType.DMA((G, 3)),
                pltpu.SemaphoreType.DMA((8,)),
                pltpu.SemaphoreType.DMA((1,)),
            ],
            compiler_params=pltpu.CompilerParams(vmem_limit_bytes=100 * 1024 * 1024,
                                                 disable_bounds_checks=True),
        )(xn, t_emb, g1.reshape(G, 128), be1.reshape(G, 128), w1t, w_emb,
          g2.reshape(G, 128), be2.reshape(G, 128), w2t)
        return jnp.transpose(out.reshape(B, H, W, C), (0, 3, 1, 2))
    return fn


_OPTS = {'sub': 8, 'kc': 3, 'w32': 1, 'rp': 8}


@jax.jit
def pallas_standalone__adm_resblock__diffusion_kernel(x, t_emb, g1, be1, w1, w_emb, g2, be2, w2):
    B, C, H, W = x.shape
    E = t_emb.shape[1]
    return build(B, C, H, W, E, TM=512, opts=_OPTS)(x, t_emb, g1, be1, w1, w_emb, g2, be2, w2)
```

```python
import jax
import jax.numpy as jnp
from jax import lax
from jax.experimental import pallas as pl
from jax.experimental.pallas import tpu as pltpu

f32 = jnp.float32
bf16 = jnp.bfloat16
u32 = jnp.uint32
NT = (((1,), (1,)), ((), ()))


def build(B, C, H, W, E, TM=1024, opts=None):
    opts = opts or {}
    HW = H * W
    G = 4
    CG = C // G
    EPS = 1e-5
    T = HW // TM
    assert CG == 128 and B == 2 and T == 4 and W == 64 and H == 64
    TR = TM // W
    NP = TR // 2
    HP = W // 2
    M = NP * HP
    NSTEP = 4 * T
    scope = jax.named_scope

    PW = opts.get('pw', 256)
    NPW = C // PW
    SUB = opts.get('sub', 8)
    XR = opts.get('xr', 64)
    NXR = TM // XR
    last_slot = opts.get('last_slot', 61)
    NQ = opts.get('nq', 4)
    QR = TM // NQ
    UB = 16
    NUB = (C // UB) * G

    def mult(v, m):
        return v if isinstance(v, int) else pl.multiple_of(v, m)

    def divT(v):
        return v // T if isinstance(v, int) else lax.shift_right_logical(v, 2)

    def modT(v):
        return v % T if isinstance(v, int) else jnp.bitwise_and(v, T - 1)

    def marker_of(d, n, sub, width):
        rp = sub * (d.shape[0] // SUB) // 8 * 8
        m = d[rp:rp + 8, n * 128:(n + 1) * 128]
        b = pltpu.bitcast(m, u32)
        z = pltpu.bitcast((b >> 16) >> 16, f32)
        if width > 128:
            z = jnp.concatenate([z] * (width // 128), axis=1)
        return z

    def pack_rows(t):
        return pltpu.bitcast(t.astype(bf16), u32)

    def split_eo(v):
        w = pltpu.bitcast(v, u32)
        return (pltpu.unpack_elementwise(w, index=0, packed_dtype=bf16, unpacked_dtype=f32),
                pltpu.unpack_elementwise(w, index=1, packed_dtype=bf16, unpacked_dtype=f32))

    def join_eo(e, o):
        return pltpu.bitcast(pltpu.pack_elementwise([e, o], packed_dtype=bf16), bf16)

    def act(v, pv, marker):
        n, wd = v.shape
        mu, sc, bt = pv
        if marker is not None:
            mu = mu + marker
        v3 = v.reshape(n // 8, 8, wd)
        hz = ((v3 - mu[None]) * sc[None] + bt[None]).reshape(n, wd)
        return hz * jnp.tanh(hz) + hz

    def act_row(s_ref, pv, q, y, cs, marker, edge):
        yc = y if not edge else jnp.clip(y, 0, H - 1)
        e, o = split_eo(s_ref[q, pl.ds(mult(yc * W, W), W), cs])
        e = act(e, pv, marker)
        o = act(o, pv, marker)
        if edge:
            valid = jnp.logical_and(y >= 0, y < H)
            e = jnp.where(valid, e, 0.0)
            o = jnp.where(valid, o, 0.0)
        return e, o

    def prod_prime(s_ref, pv, q, y0, cs, marker):
        return act_row(s_ref, pv, q, y0 - 1, cs, marker, True) + act_row(s_ref, pv, q, y0, cs, marker, False)

    def prod_pair(s_ref, pv, v_ref, q, y0, j, cs, carry, marker):
        e0, o0, e1, o1 = carry
        e2, o2 = act_row(s_ref, pv, q, y0 + 2 * j + 1, cs, marker, False)
        e3, o3 = act_row(s_ref, pv, q, y0 + 2 * j + 2, cs, marker, j == NP - 1)
        row = lax.broadcasted_iota(jnp.int32, (HP, 128), 0)
        rs = pl.ds(mult(j * (HP // 2), HP // 2), HP // 2)
        for a in range(4):
            if a == 0:
                te, to = e0 - e2, o0 - o2
            elif a == 1:
                te, to = e1 + e2, o1 + o2
            elif a == 2:
                te, to = e2 - e1, o2 - o1
            else:
                te, to = e1 - e3, o1 - o3
            om = jnp.where(row == 0, 0.0, pltpu.roll(to, 1, 0))
            ep = jnp.where(row == HP - 1, 0.0, pltpu.roll(te, HP - 1, 0))
            v_ref[4 * a + 0, rs, cs] = pack_rows(om - to)
            v_ref[4 * a + 1, rs, cs] = pack_rows(te + to)
            v_ref[4 * a + 2, rs, cs] = pack_rows(to - te)
            v_ref[4 * a + 3, rs, cs] = pack_rows(te - ep)
        return e2, o2, e3, o3

    def u_piece(w_ref, u_ref, base, k, marker):
        rb = lax.shift_right_logical(k, 2) if not isinstance(k, int) else k // 4
        cb = jnp.bitwise_and(k, 3) if not isinstance(k, int) else k % 4
        rows = pl.ds(mult(rb * UB, UB), UB)
        orow = pl.ds(mult(rb * (UB // 2), UB // 2), UB // 2)
        cs = pl.ds(mult(cb * 128, 128), 128)
        hs = []
        for i in range(3):
            g0, g1, g2 = (w_ref[base + 3 * i + j, rows, cs].astype(f32) for j in range(3))
            if marker is not None:
                g1 = (g1.reshape(UB // 8, 8, 128) + marker[None]).reshape(UB, 128)
            sm = g0 + g2
            hs.append((g0, (sm + g1) * 0.5, (sm - g1) * 0.5, g2))
        for b in range(4):
            g0, g1, g2 = hs[0][b], hs[1][b], hs[2][b]
            sm = g0 + g2
            for a, val in enumerate((g0, (sm + g1) * 0.5, (sm - g1) * 0.5, g2)):
                u_ref[4 * a + b, orow, cs] = pack_rows(val)

    def stat_acc(v, state, marker=None):
        n = v.shape[0] // 8
        wd = v.shape[1]
        if state is None:
            K = v[0:1, :]
            if marker is not None:
                K = K + marker[0:1, :]
            d = v - K
            return (K, d.reshape(n, 8, wd).sum(axis=0), (d * d).reshape(n, 8, wd).sum(axis=0))
        K, s1, s2 = state
        Kd = K if marker is None else K + marker[0:1, :]
        d = v - Kd
        return (K, s1 + d.reshape(n, 8, wd).sum(axis=0), s2 + (d * d).reshape(n, 8, wd).sum(axis=0))

    def store_stats(st_ref, q, t, cs, state):
        K, s1, s2 = state
        wd = K.shape[1]
        st_ref[q, t, 0, :, cs] = jnp.broadcast_to(K, (8, wd))
        st_ref[q, t, 1, :, cs] = jnp.broadcast_to(s1.sum(axis=0, keepdims=True), (8, wd))
        st_ref[q, t, 2, :, cs] = jnp.broadcast_to(s2.sum(axis=0, keepdims=True), (8, wd))

    def finalize(st_ref, p_ref, gb_ref, e_ref, q):
        cv = q // 2 if isinstance(q, int) else lax.shift_right_logical(q, 1)
        for g in range(G):
            cs = slice(g * 128, (g + 1) * 128)
            K = st_ref[q, :, 0, :, cs]
            s1 = st_ref[q, :, 1, :, cs]
            s2 = st_ref[q, :, 2, :, cs]
            e = e_ref[q, :, cs]
            mean_t = K + s1 * (1.0 / TM) + e[None]
            m2_t = s2 - s1 * s1 * (1.0 / TM)
            mu = jnp.sum(jnp.sum(mean_t, axis=0), axis=1, keepdims=True) * (1.0 / (T * 128))
            dev = mean_t - mu[None]
            tot = m2_t + dev * dev * float(TM)
            var = jnp.sum(jnp.sum(tot, axis=0), axis=1, keepdims=True) * (1.0 / (HW * 128))
            rstd = lax.rsqrt(var + EPS)
            p_ref[q, 0, :, cs] = mu - e
            p_ref[q, 1, :, cs] = gb_ref[cv, 0, :, cs] * (rstd * 0.5)
            p_ref[q, 2, :, cs] = gb_ref[cv, 1, :, cs] * 0.5

    def merge(lists):
        items = []
        for li, l in enumerate(lists):
            for i, it in enumerate(l):
                items.append(((i + 0.5) / len(l), li, it))
        items.sort(key=lambda z: (z[0], z[1]))
        return [it for _, _, it in items]

    def kern(x_hbm, te_hbm, g1_hbm, b1_hbm, w1_hbm, we_hbm, g2_hbm, b2_hbm, w2_hbm, o_hbm,
             s_ref, w_ref, u1_ref, u2_ref, va_ref, vb_ref, ya_ref, yb_ref,
             st_ref, p_ref, gb_ref, e_ref, te_ref, we_ref, gsm_ref, sem_x, sem_w, sem_s, sem_o):

        def gcols(g):
            return pl.ds(mult(g * 128, 128), 128)

        def x0_copy(c):
            rows = pl.ds(mult(c * TM, TM), TM)
            return pltpu.make_async_copy(x_hbm.at[0, rows, :], s_ref.at[0, rows, :], sem_x.at[c])

        def w1_copy(g):
            return pltpu.make_async_copy(w1_hbm.at[:, :, gcols(g)], w_ref.at[pl.ds(0, 9), :, gcols(g)], sem_w.at[g])

        def x1_copy():
            return pltpu.make_async_copy(x_hbm.at[1], s_ref.at[1], sem_s.at[6])

        def w2_copy():
            return pltpu.make_async_copy(w2_hbm, w_ref.at[pl.ds(9, 9)], sem_s.at[7])

        def small_copies():
            return [pltpu.make_async_copy(g1_hbm, gsm_ref.at[0], sem_s.at[0]),
                    pltpu.make_async_copy(b1_hbm, gsm_ref.at[1], sem_s.at[1]),
                    pltpu.make_async_copy(g2_hbm, gsm_ref.at[2], sem_s.at[2]),
                    pltpu.make_async_copy(b2_hbm, gsm_ref.at[3], sem_s.at[3]),
                    pltpu.make_async_copy(te_hbm, te_ref, sem_s.at[4])]

        def we_copy():
            return pltpu.make_async_copy(we_hbm, we_ref, sem_s.at[5])

        def o_copy(s, qi):
            b = divT(s) - 2
            r0 = mult(modT(s) * TM + qi * QR, QR)
            return pltpu.make_async_copy(s_ref.at[b, pl.ds(r0, QR), :], o_hbm.at[b, pl.ds(r0, QR), :], sem_o.at[0])

        def o_all():
            return pltpu.make_async_copy(s_ref.at[pl.ds(0, B)], o_hbm, sem_o.at[0])

        def epi_piece(y_ref, s_prev, kind, r, cb, state, marker):
            p = divT(s_prev)
            t = modT(s_prev)
            cs = slice(cb * PW, (cb + 1) * PW)
            j, par = r // 2, r % 2
            r0 = mult(t * TM + r * W, W)
            ve = y_ref[2 * par, j * HP:(j + 1) * HP, cs]
            vo = y_ref[2 * par + 1, j * HP:(j + 1) * HP, cs]
            if marker is not None:
                ve = (ve.reshape(HP // 8, 8, PW) + marker[None]).reshape(HP, PW)
            if kind == 1:
                dst, sq = p + 2, p + 2
            elif kind == 2:
                dst, sq = p - 2, None
                xe, xo = split_eo(s_ref[dst, pl.ds(r0, W), cs])
                ve, vo = ve + xe, vo + xo
            else:
                is2 = p >= 2
                dst = jnp.where(is2, p - 2, p + 2)
                sq = jnp.where(is2, 0, p + 2)
                xe, xo = split_eo(s_ref[dst, pl.ds(r0, W), cs])
                ve, vo = ve + jnp.where(is2, xe, 0.0), vo + jnp.where(is2, xo, 0.0)
            if sq is not None:
                state = stat_acc(vo, stat_acc(ve, state))
            s_ref[dst, pl.ds(r0, W), cs] = join_eo(ve, vo)
            if sq is not None and r == TR - 1:
                store_stats(st_ref, sq, t, cs, state)
                state = None
            return state

        def xstat_piece(q, tile, cs, ri, state, marker):
            r0 = mult(tile * TM + ri * XR, XR)
            v = s_ref[q, pl.ds(r0, XR), cs].astype(f32)
            state = stat_acc(v, state, marker)
            if ri == NXR - 1:
                store_stats(st_ref, q, tile, cs, state)
                state = None
            return state

        def half(conv, it, second, u_ref, vc_ref, vn_ref, yc_ref, yp_ref):
            s = conv * 2 * T + 2 * it + second
            sn = s + 1
            pn = jnp.minimum(divT(sn), 3)
            y0 = modT(sn) * TR
            lists = [[('p', cb, j) for cb in range(G) for j in range(-1, NP)],
                     [('e', r, cb) for r in range(TR) for cb in range(NPW)]]
            if conv == 0 and second == 0 and not opts.get('nox'):
                lists.append([('x', t, cb, ri) for t in range(T) for cb in range(NPW) for ri in range(NXR)])
            NU = -(-NUB // (T - 1))
            if conv == 0 and second == 1 and not opts.get('nou'):
                lists.append([('u', k) for k in range(NU)])
            pieces = merge(lists)
            npc = len(pieces)
            if second == 1:
                finalize(st_ref, p_ref, gb_ref, e_ref, jnp.minimum(divT(s - 1) + 1, 3))
            pv = tuple(p_ref[pn, k] for k in range(3))
            sp = jnp.maximum(s - 1, 0)
            ekind = 1 if conv == 0 else (0 if second == 0 else 2)
            done = 0
            est = [None] * NPW
            xst = None
            pcar = None
            ys = [None] * 4
            for a in range(4):
                rr = [None, None]
                for b in range(4):
                    k = 4 * a + b
                    d = lax.dot_general(pltpu.bitcast(vc_ref[k], bf16), pltpu.bitcast(u_ref[k], bf16), NT,
                                        preferred_element_type=f32)
                    for nn in range(4 * SUB):
                        n, sub = nn // SUB, nn % SUB
                        hi_ = min(npc, (((k * 4 * SUB + nn) + 1) * npc) // (last_slot * SUB))
                        while done < hi_:
                            pc = pieces[done]
                            if pc[0] == 'p':
                                cs = slice(pc[1] * 128, (pc[1] + 1) * 128)
                                pvc = tuple(t[:, cs] for t in pv)
                                mk = marker_of(d, n, sub, 128)
                                if pc[2] < 0:
                                    pcar = prod_prime(s_ref, pvc, pn, y0, cs, mk)
                                else:
                                    pcar = prod_pair(s_ref, pvc, vn_ref, pn, y0, pc[2], cs, pcar, mk)
                            elif pc[0] == 'e':
                                est[pc[2]] = epi_piece(yp_ref, sp, ekind, pc[1], pc[2], est[pc[2]],
                                                       marker_of(d, n, sub, PW))
                                if conv == 1 and pc[2] == NPW - 1 and ((pc[1] + 1) * W) % QR == 0:
                                    qi = ((pc[1] + 1) * W) // QR - 1
                                    if second == 1:
                                        o_copy(sp, qi).start()
                                    else:
                                        @pl.when(it > 0)
                                        def _():
                                            o_copy(sp, qi).start()
                            elif pc[0] == 'x':
                                xst = xstat_piece(jnp.where(it == 0, 0, 1), pc[1],
                                                  slice(pc[2] * PW, (pc[2] + 1) * PW), pc[3], xst,
                                                  marker_of(d, n, sub, PW))
                            else:
                                ku = jnp.clip((it - 1) * NU + pc[1], 0, NUB - 1)
                                u_piece(w_ref, u2_ref, jnp.where(it == 0, 0, 9), ku, marker_of(d, n, sub, 128))
                            done += 1
                    if b == 0:
                        rr[0] = d
                    elif b == 1:
                        rr[0] = rr[0] + d
                        rr[1] = d
                    elif b == 2:
                        rr[0] = rr[0] + d
                        rr[1] = rr[1] - d
                    else:
                        rr[1] = rr[1] - d
                for c in range(2):
                    if a == 0:
                        ys[c] = rr[c]
                    elif a == 1:
                        ys[c] = ys[c] + rr[c]
                        ys[2 + c] = rr[c]
                    elif a == 2:
                        yc_ref[c] = ys[c] + rr[c]
                        ys[2 + c] = ys[2 + c] - rr[c]
                    else:
                        yc_ref[2 + c] = ys[2 + c] - rr[c]

        with scope('prologue'):
            for c in small_copies():
                c.start()
            lax.fori_loop(0, T, lambda c, _: (x0_copy(c).start(), 0)[1], 0)
            lax.fori_loop(0, G, lambda g, _: (w1_copy(g).start(), 0)[1], 0)

            def rest(c, _):
                @pl.when(c == 0)
                def _():
                    x1_copy().start()

                @pl.when(c == 1)
                def _():
                    w2_copy().start()

                @pl.when(c == 2)
                def _():
                    we_copy().start()
                return 0
            lax.fori_loop(0, 3, rest, 0)

            for c in small_copies():
                c.wait()
            for cv in range(2):
                for k in range(2):
                    v = gsm_ref[2 * cv + k].astype(f32)
                    for g in range(G):
                        gb_ref[cv, k, :, g * 128:(g + 1) * 128] = jnp.broadcast_to(v[g:g + 1, :], (8, 128))
            e_ref[...] = jnp.zeros(e_ref.shape, f32)
            st_ref[...] = jnp.zeros(st_ref.shape, f32)
            yb_ref[...] = jnp.zeros(yb_ref.shape, f32)

            def xs0(c, _):
                x0_copy(c).wait()

                for cb in range(NPW):
                    def rows(ri, st):
                        r0 = pl.multiple_of(c * TM + ri * XR, XR)
                        v = s_ref[0, pl.ds(r0, XR), cb * PW:(cb + 1) * PW].astype(f32)
                        return stat_acc(v, st)
                    v0 = s_ref[0, pl.ds(pl.multiple_of(c * TM, XR), XR), cb * PW:(cb + 1) * PW].astype(f32)
                    st = lax.fori_loop(1, NXR, rows, stat_acc(v0, None))
                    store_stats(st_ref, 0, c, slice(cb * PW, (cb + 1) * PW), st)
                return 0
            lax.fori_loop(0, T, xs0, 0)
            finalize(st_ref, p_ref, gb_ref, e_ref, 0)

            def prod0(cb, _):
                cs = gcols(cb)
                pvc = tuple(p_ref[0, k, :, cs] for k in range(3))
                car = prod_prime(s_ref, pvc, 0, 0, cs, None)

                def pair(j, car):
                    return prod_pair_dyn(j, car, cs, pvc)
                lax.fori_loop(0, NP, pair, car)
                return 0

            def prod_pair_dyn(j, carry, cs, pvc):
                e0, o0, e1, o1 = carry
                e2, o2 = act_row(s_ref, pvc, 0, 2 * j + 1, cs, None, False)
                e3, o3 = act_row(s_ref, pvc, 0, 2 * j + 2, cs, None, False)
                row = lax.broadcasted_iota(jnp.int32, (HP, 128), 0)
                rs = pl.ds(pl.multiple_of(j * (HP // 2), HP // 2), HP // 2)
                for a in range(4):
                    if a == 0:
                        te, to = e0 - e2, o0 - o2
                    elif a == 1:
                        te, to = e1 + e2, o1 + o2
                    elif a == 2:
                        te, to = e2 - e1, o2 - o1
                    else:
                        te, to = e1 - e3, o1 - o3
                    om = jnp.where(row == 0, 0.0, pltpu.roll(to, 1, 0))
                    ep = jnp.where(row == HP - 1, 0.0, pltpu.roll(te, HP - 1, 0))
                    va_ref[4 * a + 0, rs, cs] = pack_rows(om - to)
                    va_ref[4 * a + 1, rs, cs] = pack_rows(te + to)
                    va_ref[4 * a + 2, rs, cs] = pack_rows(to - te)
                    va_ref[4 * a + 3, rs, cs] = pack_rows(te - ep)
                return e2, o2, e3, o3
            lax.fori_loop(0, G, prod0, 0)

            def u1g(g, _):
                w1_copy(g).wait()
                lax.fori_loop(0, C // UB, lambda rb, _: (u_piece(w_ref, u1_ref, 0, rb * 4 + g, None), 0)[1], 0)
                return 0
            lax.fori_loop(0, G, u1g, 0)

        def body1(it, carry):
            @pl.when(it == 1)
            def _():
                x1_copy().wait()
                w2_copy().wait()
                we_copy().wait()
                te = te_ref[...].astype(f32)
                sl = te * jax.nn.sigmoid(te)
                emb = jnp.dot(sl.astype(bf16), we_ref[...], preferred_element_type=f32)
                e_ref[2] = jnp.broadcast_to(emb[0:1, :], (8, C))
                e_ref[3] = jnp.broadcast_to(emb[1:2, :], (8, C))
            with scope('iter1'):
                half(0, it, 0, u1_ref, va_ref, vb_ref, ya_ref, yb_ref)
                half(0, it, 1, u1_ref, vb_ref, va_ref, yb_ref, ya_ref)
            return carry

        with scope('conv1'):
            lax.fori_loop(0, T, body1, 0)

        def body2(it, carry):
            with scope('iter2'):
                half(1, it, 0, u2_ref, va_ref, vb_ref, ya_ref, yb_ref)
                half(1, it, 1, u2_ref, vb_ref, va_ref, yb_ref, ya_ref)
            return carry

        with scope('conv2'):
            lax.fori_loop(0, T, body2, 0)

        sl_ = NSTEP - 1
        with scope('final'):
            st = [None] * NPW
            for r in range(TR):
                for cb in range(NPW):
                    st[cb] = epi_piece(yb_ref, sl_, 2, r, cb, st[cb], None)
                if ((r + 1) * W) % QR == 0:
                    o_copy(sl_, ((r + 1) * W) // QR - 1).start()
        with scope('owait'):
            o_all().wait()

    def fn(x, t_emb, g1, be1, w1, w_emb, g2, be2, w2):
        xn = jnp.transpose(x, (0, 2, 3, 1)).reshape(B, HW, C)
        w1t = jnp.transpose(w1, (2, 3, 0, 1)).reshape(9, C, C)
        w2t = jnp.transpose(w2, (2, 3, 0, 1)).reshape(9, C, C)
        any_spec = pl.BlockSpec(memory_space=pl.ANY)
        ubuf = pltpu.VMEM((16, C // 2, C), u32)
        vbuf = pltpu.VMEM((16, M // 2, C), u32)
        ybuf = pltpu.VMEM((4, M, C), f32)
        out = pl.pallas_call(
            kern,
            in_specs=[any_spec] * 9,
            out_specs=any_spec,
            out_shape=jax.ShapeDtypeStruct((B, HW, C), bf16),
            scratch_shapes=[
                pltpu.VMEM((4, HW, C), bf16),
                pltpu.VMEM((18, C, C), bf16),
                ubuf, ubuf, vbuf, vbuf, ybuf, ybuf,
                pltpu.VMEM((4, T, 3, 8, C), f32),
                pltpu.VMEM((4, 3, 8, C), f32),
                pltpu.VMEM((2, 2, 8, C), f32),
                pltpu.VMEM((4, 8, C), f32),
                pltpu.VMEM((B, E), bf16),
                pltpu.VMEM((E, C), bf16),
                pltpu.VMEM((4, G, 128), bf16),
                pltpu.SemaphoreType.DMA((T,)),
                pltpu.SemaphoreType.DMA((G,)),
                pltpu.SemaphoreType.DMA((8,)),
                pltpu.SemaphoreType.DMA((1,)),
            ],
            compiler_params=pltpu.CompilerParams(vmem_limit_bytes=100 * 1024 * 1024,
                                                 disable_bounds_checks=True),
        )(xn, t_emb, g1.reshape(G, 128), be1.reshape(G, 128), w1t, w_emb,
          g2.reshape(G, 128), be2.reshape(G, 128), w2t)
        return jnp.transpose(out.reshape(B, H, W, C), (0, 3, 1, 2))
    return fn


_OPTS = {}


@jax.jit
def pallas_standalone__adm_resblock__diffusion_kernel(x, t_emb, g1, be1, w1, w_emb, g2, be2, w2):
    B, C, H, W = x.shape
    E = t_emb.shape[1]
    return build(B, C, H, W, E, TM=1024, opts=_OPTS)(x, t_emb, g1, be1, w1, w_emb, g2, be2, w2)
```

```python
import jax
import jax.numpy as jnp
from jax import lax
from jax.experimental import pallas as pl
from jax.experimental.pallas import tpu as pltpu

f32 = jnp.float32
bf16 = jnp.bfloat16
u32 = jnp.uint32
NT = (((1,), (1,)), ((), ()))


def build(B, C, H, W, E, TM=1024, opts=None):
    opts = opts or {}
    HW = H * W
    G = 4
    CG = C // G
    EPS = 1e-5
    T = HW // TM
    assert CG == 128 and B == 2 and T == 4 and W == 64 and H == 64
    TR = TM // W
    NP = TR // 2
    HP = W // 2
    M = NP * HP
    NSTEP = 4 * T
    scope = jax.named_scope

    PW = opts.get('pw', 256)
    NPW = C // PW
    SUB = opts.get('sub', 8)
    XR = opts.get('xr', 64)
    NXR = TM // XR
    last_slot = opts.get('last_slot', 61)
    NQ = opts.get('nq', 4)
    QR = TM // NQ
    UMODE = opts.get('umode', 0)
    XMODE = opts.get('xmode', 0)
    PMODE = opts.get('pmode', 1)
    UB = 16
    NUB = (C // UB) * G

    def mult(v, m):
        return v if isinstance(v, int) else pl.multiple_of(v, m)

    def divT(v):
        return v // T if isinstance(v, int) else lax.shift_right_logical(v, 2)

    def modT(v):
        return v % T if isinstance(v, int) else jnp.bitwise_and(v, T - 1)

    def marker_of(d, n, sub, width):
        rp = sub * (d.shape[0] // SUB) // 8 * 8
        m = d[rp:rp + 8, n * 128:(n + 1) * 128]
        b = pltpu.bitcast(m, u32)
        z = pltpu.bitcast((b >> 16) >> 16, f32)
        if width > 128:
            z = jnp.concatenate([z] * (width // 128), axis=1)
        return z

    def pack_rows(t):
        return pltpu.bitcast(t.astype(bf16), u32)

    def pack2(t):
        n = t.shape[0] // 2
        return pltpu.pack_elementwise([t[:n], t[n:]], packed_dtype=bf16)

    def load_y(y_ref, c, j, cb0, ncb):
        parts = []
        for n in range(cb0, cb0 + ncb):
            lo = y_ref[c, n, pl.ds(j * HP, HP // 2, stride=2), :]
            hi = y_ref[c, n, pl.ds(j * HP + 1, HP // 2, stride=2), :]
            parts.append(jnp.concatenate([lo, hi], axis=0))
        return parts[0] if ncb == 1 else jnp.concatenate(parts, axis=1)

    def store_y(y_ref, c, val):
        for n in range(G):
            y_ref[c, n] = val[:, n * 128:(n + 1) * 128]

    def split_eo(v):
        w = pltpu.bitcast(v, u32)
        return (pltpu.unpack_elementwise(w, index=0, packed_dtype=bf16, unpacked_dtype=f32),
                pltpu.unpack_elementwise(w, index=1, packed_dtype=bf16, unpacked_dtype=f32))

    def join_eo(e, o):
        return pltpu.bitcast(pltpu.pack_elementwise([e, o], packed_dtype=bf16), bf16)

    def act(v, pv, marker):
        n, wd = v.shape
        mu, sc, bt = pv
        if marker is not None:
            mu = mu + marker
        v3 = v.reshape(n // 8, 8, wd)
        hz = ((v3 - mu[None]) * sc[None] + bt[None]).reshape(n, wd)
        return hz * jnp.tanh(hz) + hz

    def act_row(s_ref, pv, q, y, cs, marker, edge):
        yc = y if not edge else jnp.clip(y, 0, H - 1)
        e, o = split_eo(s_ref[q, pl.ds(mult(yc * W, W), W), cs])
        e = act(e, pv, marker)
        o = act(o, pv, marker)
        if edge:
            valid = jnp.logical_and(y >= 0, y < H)
            e = jnp.where(valid, e, 0.0)
            o = jnp.where(valid, o, 0.0)
        return e, o

    def prod_prime(s_ref, pv, q, y0, cs, marker):
        return act_row(s_ref, pv, q, y0 - 1, cs, marker, True) + act_row(s_ref, pv, q, y0, cs, marker, False)

    def prod_pair(s_ref, pv, v_ref, q, y0, j, cs, carry, marker):
        e0, o0, e1, o1 = carry
        e2, o2 = act_row(s_ref, pv, q, y0 + 2 * j + 1, cs, marker, False)
        e3, o3 = act_row(s_ref, pv, q, y0 + 2 * j + 2, cs, marker, j == NP - 1)
        row = lax.broadcasted_iota(jnp.int32, (HP, 128), 0)
        rs = pl.ds(mult(j * (HP // 2), HP // 2), HP // 2)
        for a in range(4):
            if a == 0:
                te, to = e0 - e2, o0 - o2
            elif a == 1:
                te, to = e1 + e2, o1 + o2
            elif a == 2:
                te, to = e2 - e1, o2 - o1
            else:
                te, to = e1 - e3, o1 - o3
            om = jnp.where(row == 0, 0.0, pltpu.roll(to, 1, 0))
            ep = jnp.where(row == HP - 1, 0.0, pltpu.roll(te, HP - 1, 0))
            v_ref[4 * a + 0, rs, cs] = pack2(om - to)
            v_ref[4 * a + 1, rs, cs] = pack2(te + to)
            v_ref[4 * a + 2, rs, cs] = pack2(to - te)
            v_ref[4 * a + 3, rs, cs] = pack2(te - ep)
        return e2, o2, e3, o3

    def prod_a(s_ref, pv, xr_ref, q, y0, cb, i, marker):
        cs = slice(cb * 128, (cb + 1) * 128)
        e, o = act_row(s_ref, pv, q, y0 - 1 + i, cs, marker, i == 0 or i == TR + 1)
        row = lax.broadcasted_iota(jnp.int32, (HP, 128), 0)
        om = jnp.where(row == 0, 0.0, pltpu.roll(o, 1, 0))
        ep = jnp.where(row == HP - 1, 0.0, pltpu.roll(e, HP - 1, 0))
        xr_ref[cb, i, 0] = om - o
        xr_ref[cb, i, 1] = e + o
        xr_ref[cb, i, 2] = o - e
        xr_ref[cb, i, 3] = e - ep

    def prod_b(xr_ref, v_ref, cb, j, b, marker):
        cs = slice(cb * 128, (cb + 1) * 128)
        rs = pl.ds(j * (HP // 2), HP // 2)
        r0, r1, r2, r3 = (xr_ref[cb, 2 * j + i, b] for i in range(4))
        if marker is not None:
            r2 = (r2.reshape(HP // 8, 8, 128) + marker[None]).reshape(HP, 128)
        v_ref[0 + b, rs, cs] = pack2(r0 - r2)
        v_ref[4 + b, rs, cs] = pack2(r1 + r2)
        v_ref[8 + b, rs, cs] = pack2(r2 - r1)
        v_ref[12 + b, rs, cs] = pack2(r1 - r3)

    def u_piece(w_ref, u_ref, base, k, marker, ok=None):
        rb = lax.shift_right_logical(k, 2) if not isinstance(k, int) else k // 4
        cb = jnp.bitwise_and(k, 3) if not isinstance(k, int) else k % 4
        rows = pl.ds(mult(rb * UB, UB), UB)
        ob = rb if ok is None else jnp.where(ok, rb, C // UB)
        orow = pl.ds(mult(ob * (UB // 2), UB // 2), UB // 2)
        cs = pl.ds(mult(cb * 128, 128), 128)
        res = []
        raw = [[split_eo(w_ref[base + 3 * i + j, rows, cs]) for j in range(3)] for i in range(3)]
        for par in range(2):
            hs = []
            for i in range(3):
                g0, g1, g2 = (raw[i][j][par] for j in range(3))
                if marker is not None:
                    g1 = g1 + marker
                sm = g0 + g2
                hs.append((g0, (sm + g1) * 0.5, (sm - g1) * 0.5, g2))
            out = [None] * 16
            for b in range(4):
                g0, g1, g2 = hs[0][b], hs[1][b], hs[2][b]
                sm = g0 + g2
                for a, val in enumerate((g0, (sm + g1) * 0.5, (sm - g1) * 0.5, g2)):
                    out[4 * a + b] = val
            res.append(out)
        for k2 in range(16):
            val = pltpu.pack_elementwise([res[0][k2], res[1][k2]], packed_dtype=bf16)
            if isinstance(u_ref, (list, tuple)):
                u_ref[k2][orow, cs] = val
            else:
                u_ref[k2, orow, cs] = val

    def stat_acc(v, state, marker=None):
        n = v.shape[0] // 8
        wd = v.shape[1]
        if state is None:
            K = v[0:1, :]
            if marker is not None:
                K = K + marker[0:1, :]
            d = v - K
            return (K, d.reshape(n, 8, wd).sum(axis=0), (d * d).reshape(n, 8, wd).sum(axis=0))
        K, s1, s2 = state
        Kd = K if marker is None else K + marker[0:1, :]
        d = v - Kd
        return (K, s1 + d.reshape(n, 8, wd).sum(axis=0), s2 + (d * d).reshape(n, 8, wd).sum(axis=0))

    def store_stats(st_ref, q, t, cs, state):
        K, s1, s2 = state
        wd = K.shape[1]
        st_ref[q, t, 0, :, cs] = jnp.broadcast_to(K, (8, wd))
        st_ref[q, t, 1, :, cs] = jnp.broadcast_to(s1.sum(axis=0, keepdims=True), (8, wd))
        st_ref[q, t, 2, :, cs] = jnp.broadcast_to(s2.sum(axis=0, keepdims=True), (8, wd))

    def finalize(st_ref, p_ref, gb_ref, e_ref, q):
        cv = q // 2 if isinstance(q, int) else lax.shift_right_logical(q, 1)
        for g in range(G):
            cs = slice(g * 128, (g + 1) * 128)
            K = st_ref[q, :, 0, :, cs]
            s1 = st_ref[q, :, 1, :, cs]
            s2 = st_ref[q, :, 2, :, cs]
            e = e_ref[q, :, cs]
            mean_t = K + s1 * (1.0 / TM) + e[None]
            m2_t = s2 - s1 * s1 * (1.0 / TM)
            mu = jnp.sum(jnp.sum(mean_t, axis=0), axis=1, keepdims=True) * (1.0 / (T * 128))
            dev = mean_t - mu[None]
            tot = m2_t + dev * dev * float(TM)
            var = jnp.sum(jnp.sum(tot, axis=0), axis=1, keepdims=True) * (1.0 / (HW * 128))
            rstd = lax.rsqrt(var + EPS)
            p_ref[q, 0, :, cs] = mu - e
            p_ref[q, 1, :, cs] = gb_ref[cv, 0, :, cs] * (rstd * 0.5)
            p_ref[q, 2, :, cs] = gb_ref[cv, 1, :, cs] * 0.5

    def merge(lists):
        items = []
        for li, l in enumerate(lists):
            for i, it in enumerate(l):
                items.append(((i + 0.5) / len(l), li, it))
        items.sort(key=lambda z: (z[0], z[1]))
        return [it for _, _, it in items]

    def kern(x_hbm, te_hbm, g1_hbm, b1_hbm, w1_hbm, we_hbm, g2_hbm, b2_hbm, w2_hbm, o_hbm,
             s_ref, w_ref, u2_ref, xr_ref, va_ref, vb_ref, ya_ref, yb_ref,
             st_ref, p_ref, gb_ref, e_ref, te_ref, we_ref, gsm_ref, sem_x, sem_w, sem_s, sem_o, *u1_ref):

        def gcols(g):
            return pl.ds(mult(g * 128, 128), 128)

        def x0_copy(c):
            rows = pl.ds(mult(c * TM, TM), TM)
            return pltpu.make_async_copy(x_hbm.at[0, rows, :], s_ref.at[0, rows, :], sem_x.at[c])

        def w1_copy(g):
            return pltpu.make_async_copy(w1_hbm.at[:, :, gcols(g)], w_ref.at[pl.ds(0, 9), :, gcols(g)], sem_w.at[g])

        def x1_copy():
            return pltpu.make_async_copy(x_hbm.at[1], s_ref.at[1], sem_s.at[6])

        def w2_copy():
            return pltpu.make_async_copy(w2_hbm, w_ref.at[pl.ds(9, 9)], sem_s.at[7])

        def small_copies():
            return [pltpu.make_async_copy(g1_hbm, gsm_ref.at[0], sem_s.at[0]),
                    pltpu.make_async_copy(b1_hbm, gsm_ref.at[1], sem_s.at[1]),
                    pltpu.make_async_copy(g2_hbm, gsm_ref.at[2], sem_s.at[2]),
                    pltpu.make_async_copy(b2_hbm, gsm_ref.at[3], sem_s.at[3]),
                    pltpu.make_async_copy(te_hbm, te_ref, sem_s.at[4])]

        def we_copy():
            return pltpu.make_async_copy(we_hbm, we_ref, sem_s.at[5])

        def o_copy(s, qi):
            b = divT(s) - 2
            r0 = mult(modT(s) * TM + qi * QR, QR)
            return pltpu.make_async_copy(s_ref.at[b, pl.ds(r0, QR), :], o_hbm.at[b, pl.ds(r0, QR), :], sem_o.at[0])

        def o_all():
            return pltpu.make_async_copy(s_ref.at[pl.ds(0, B)], o_hbm, sem_o.at[0])

        def epi_piece(y_ref, s_prev, kind, r, cb, state, marker):
            p = divT(s_prev)
            t = modT(s_prev)
            cs = slice(cb * PW, (cb + 1) * PW)
            j, par = r // 2, r % 2
            r0 = mult(t * TM + r * W, W)
            ve = load_y(y_ref, 2 * par, j, cb * (PW // 128), PW // 128)
            vo = load_y(y_ref, 2 * par + 1, j, cb * (PW // 128), PW // 128)
            if marker is not None:
                ve = (ve.reshape(HP // 8, 8, PW) + marker[None]).reshape(HP, PW)
            if kind == 1:
                dst, sq = p + 2, p + 2
            elif kind == 2:
                dst, sq = p - 2, None
                xe, xo = split_eo(s_ref[dst, pl.ds(r0, W), cs])
                ve, vo = ve + xe, vo + xo
            else:
                is2 = p >= 2
                dst = jnp.where(is2, p - 2, p + 2)
                sq = jnp.where(is2, 0, p + 2)
                xe, xo = split_eo(s_ref[dst, pl.ds(r0, W), cs])
                ve, vo = ve + jnp.where(is2, xe, 0.0), vo + jnp.where(is2, xo, 0.0)
            if sq is not None:
                state = stat_acc(vo, stat_acc(ve, state))
            s_ref[dst, pl.ds(r0, W), cs] = join_eo(ve, vo)
            if sq is not None and r == TR - 1:
                store_stats(st_ref, sq, t, cs, state)
                state = None
            return state

        def xstat_piece(q, tile, cs, ri, state, marker):
            r0 = mult(tile * TM + ri * XR, XR)
            v = s_ref[q, pl.ds(r0, XR), cs].astype(f32)
            state = stat_acc(v, state, marker)
            if ri == NXR - 1:
                store_stats(st_ref, q, tile, cs, state)
                state = None
            return state

        def half(it, second, u_ref, vc_ref, vn_ref, yc_ref, yp_ref):
            s = 2 * it + second
            sn = s + 1
            pn = jnp.minimum(divT(sn), 3)
            y0 = modT(sn) * TR
            if PMODE == 0:
                plist = [('p', cb, j) for cb in range(G) for j in range(-1, NP)]
            else:
                plist = []
                for cb in range(G):
                    plist += [('a', cb, 0), ('a', cb, 1)]
                    for j in range(NP):
                        plist += [('a', cb, 2 * j + 2), ('a', cb, 2 * j + 3)] + [('b', cb, j, b) for b in range(4)]
            lists = [plist,
                     [('e', r, cb) for r in range(TR) for cb in range(NPW)]]
            if second == 0 and XMODE == 0:
                lists.append([('x', t, cb, ri) for t in range(T) for cb in range(NPW) for ri in range(NXR)])
            NU = -(-NUB // 5)
            if UMODE == 0:
                lists.append([('u', k) for k in range(NU)])
            pieces = merge(lists)
            npc = len(pieces)
            if second == 1:
                finalize(st_ref, p_ref, gb_ref, e_ref, jnp.minimum(divT(s - 1) + 1, 3))
            pv = tuple(p_ref[pn, k] for k in range(3))
            sp = jnp.maximum(s - 1, 0)
            ekind = 0
            done = 0
            est = [None] * NPW
            xst = None
            pcar = None
            ys = [None] * 4
            for a in range(4):
                rr = [None, None]
                for b in range(4):
                    k = 4 * a + b
                    d = lax.dot_general(pltpu.bitcast(vc_ref[k], bf16), pltpu.bitcast(u_ref[k][...], bf16), NT,
                                        preferred_element_type=f32)
                    for nn in range(4 * SUB):
                        n, sub = nn // SUB, nn % SUB
                        hi_ = min(npc, (((k * 4 * SUB + nn) + 1) * npc) // (last_slot * SUB))
                        while done < hi_:
                            pc = pieces[done]
                            if pc[0] == 'p':
                                cs = slice(pc[1] * 128, (pc[1] + 1) * 128)
                                pvc = tuple(t[:, cs] for t in pv)
                                mk = marker_of(d, n, sub, 128)
                                if pc[2] < 0:
                                    pcar = prod_prime(s_ref, pvc, pn, y0, cs, mk)
                                else:
                                    pcar = prod_pair(s_ref, pvc, vn_ref, pn, y0, pc[2], cs, pcar, mk)
                            elif pc[0] == 'a':
                                cs = slice(pc[1] * 128, (pc[1] + 1) * 128)
                                prod_a(s_ref, tuple(t[:, cs] for t in pv), xr_ref, pn, y0, pc[1], pc[2],
                                       marker_of(d, n, sub, 128))
                            elif pc[0] == 'b':
                                prod_b(xr_ref, vn_ref, pc[1], pc[2], pc[3], marker_of(d, n, sub, 128))
                            elif pc[0] == 'e':
                                est[pc[2]] = epi_piece(yp_ref, sp, ekind, pc[1], pc[2], est[pc[2]],
                                                       marker_of(d, n, sub, PW))
                                if pc[2] == NPW - 1 and ((pc[1] + 1) * W) % QR == 0:
                                    qi = ((pc[1] + 1) * W) // QR - 1

                                    @pl.when(sp >= 2 * T)
                                    def _():
                                        o_copy(sp, qi).start()
                            elif pc[0] == 'x':
                                xst = xstat_piece(jnp.where(it == 0, 0, 1), pc[1],
                                                  slice(pc[2] * PW, (pc[2] + 1) * PW), pc[3], xst,
                                                  marker_of(d, n, sub, PW))
                            else:
                                kk = (s - 2) * NU + pc[1]
                                ok = jnp.logical_and(kk >= 0, kk < NUB)
                                u_piece(w_ref, u2_ref, jnp.where(it == 0, 0, 9), jnp.clip(kk, 0, NUB - 1),
                                        marker_of(d, n, sub, 128), ok)
                            done += 1
                    if b == 0:
                        rr[0] = d
                    elif b == 1:
                        rr[0] = rr[0] + d
                        rr[1] = d
                    elif b == 2:
                        rr[0] = rr[0] + d
                        rr[1] = rr[1] - d
                    else:
                        rr[1] = rr[1] - d
                for c in range(2):
                    if a == 0:
                        ys[c] = rr[c]
                    elif a == 1:
                        ys[c] = ys[c] + rr[c]
                        ys[2 + c] = rr[c]
                    elif a == 2:
                        store_y(yc_ref, c, ys[c] + rr[c])
                        ys[2 + c] = ys[2 + c] - rr[c]
                    else:
                        store_y(yc_ref, 2 + c, ys[2 + c] - rr[c])

        def xstat_tile(q, c):
            for cb in range(NPW):
                def rows(ri, st):
                    r0 = pl.multiple_of(c * TM + ri * XR, XR)
                    v = s_ref[q, pl.ds(r0, XR), cb * PW:(cb + 1) * PW].astype(f32)
                    return stat_acc(v, st)
                v0 = s_ref[q, pl.ds(pl.multiple_of(c * TM, XR), XR), cb * PW:(cb + 1) * PW].astype(f32)
                st = lax.fori_loop(1, NXR, rows, stat_acc(v0, None))
                store_stats(st_ref, q, c, slice(cb * PW, (cb + 1) * PW), st)
            return 0

        with scope('prologue'):
            for c in small_copies():
                c.start()
            lax.fori_loop(0, T, lambda c, _: (x0_copy(c).start(), 0)[1], 0)
            lax.fori_loop(0, G, lambda g, _: (w1_copy(g).start(), 0)[1], 0)

            def rest(c, _):
                @pl.when(c == 0)
                def _():
                    x1_copy().start()

                @pl.when(c == 1)
                def _():
                    w2_copy().start()

                @pl.when(c == 2)
                def _():
                    we_copy().start()
                return 0
            lax.fori_loop(0, 3, rest, 0)

            for c in small_copies():
                c.wait()
            for cv in range(2):
                for k in range(2):
                    v = gsm_ref[2 * cv + k].astype(f32)
                    for g in range(G):
                        gb_ref[cv, k, :, g * 128:(g + 1) * 128] = jnp.broadcast_to(v[g:g + 1, :], (8, 128))
            e_ref[...] = jnp.zeros(e_ref.shape, f32)
            st_ref[...] = jnp.zeros(st_ref.shape, f32)
            yb_ref[...] = jnp.zeros(yb_ref.shape, f32)

            def xs0(c, _):
                x0_copy(c).wait()
                return xstat_tile(0, c)
            lax.fori_loop(0, T, xs0, 0)
            finalize(st_ref, p_ref, gb_ref, e_ref, 0)

            def prod0(cb, _):
                cs = gcols(cb)
                pvc = tuple(p_ref[0, k, :, cs] for k in range(3))
                car = prod_prime(s_ref, pvc, 0, 0, cs, None)

                def pair(j, car):
                    return prod_pair_dyn(j, car, cs, pvc)
                lax.fori_loop(0, NP, pair, car)
                return 0

            def prod_pair_dyn(j, carry, cs, pvc):
                e0, o0, e1, o1 = carry
                e2, o2 = act_row(s_ref, pvc, 0, 2 * j + 1, cs, None, False)
                e3, o3 = act_row(s_ref, pvc, 0, 2 * j + 2, cs, None, False)
                row = lax.broadcasted_iota(jnp.int32, (HP, 128), 0)
                rs = pl.ds(pl.multiple_of(j * (HP // 2), HP // 2), HP // 2)
                for a in range(4):
                    if a == 0:
                        te, to = e0 - e2, o0 - o2
                    elif a == 1:
                        te, to = e1 + e2, o1 + o2
                    elif a == 2:
                        te, to = e2 - e1, o2 - o1
                    else:
                        te, to = e1 - e3, o1 - o3
                    om = jnp.where(row == 0, 0.0, pltpu.roll(to, 1, 0))
                    ep = jnp.where(row == HP - 1, 0.0, pltpu.roll(te, HP - 1, 0))
                    va_ref[4 * a + 0, rs, cs] = pack2(om - to)
                    va_ref[4 * a + 1, rs, cs] = pack2(te + to)
                    va_ref[4 * a + 2, rs, cs] = pack2(to - te)
                    va_ref[4 * a + 3, rs, cs] = pack2(te - ep)
                return e2, o2, e3, o3
            lax.fori_loop(0, G, prod0, 0)

            def u1g(g, _):
                w1_copy(g).wait()
                lax.fori_loop(0, C // UB, lambda rb, _: (u_piece(w_ref, u1_ref, 0, rb * 4 + g, None), 0)[1], 0)
                return 0
            lax.fori_loop(0, G, u1g, 0)

        def body(it, carry):
            @pl.when(it == 1)
            def _():
                x1_copy().wait()
                w2_copy().wait()
                we_copy().wait()
                te = te_ref[...].astype(f32)
                sl = te * jax.nn.sigmoid(te)
                emb = jnp.dot(sl.astype(bf16), we_ref[...], preferred_element_type=f32)
                e_ref[2] = jnp.broadcast_to(emb[0:1, :], (8, C))
                e_ref[3] = jnp.broadcast_to(emb[1:2, :], (8, C))
                if XMODE == 1:
                    lax.fori_loop(0, T, lambda c, _: xstat_tile(1, c), 0)

            @pl.when(it == T)
            def _():
                if UMODE == 0:
                    def cp(rb, _):
                        rows = pl.ds(pl.multiple_of(rb * 32, 32), 32)
                        for k in range(16):
                            u1_ref[k][rows, :] = u2_ref[k, rows, :]
                        return 0
                    lax.fori_loop(0, C // 2 // 32, cp, 0)
                else:
                    lax.fori_loop(0, NUB, lambda k, _: (u_piece(w_ref, u1_ref, 9, k, None), 0)[1], 0)
            with scope('iter'):
                half(it, 0, u1_ref, va_ref, vb_ref, ya_ref, yb_ref)
                half(it, 1, u1_ref, vb_ref, va_ref, yb_ref, ya_ref)
            return carry

        with scope('main'):
            lax.fori_loop(0, 2 * T, body, 0)

        sl_ = NSTEP - 1
        with scope('final'):
            st = [None] * NPW
            for r in range(TR):
                for cb in range(NPW):
                    st[cb] = epi_piece(yb_ref, sl_, 2, r, cb, st[cb], None)
                if ((r + 1) * W) % QR == 0:
                    o_copy(sl_, ((r + 1) * W) // QR - 1).start()
        with scope('owait'):
            o_all().wait()

    def fn(x, t_emb, g1, be1, w1, w_emb, g2, be2, w2):
        xn = jnp.transpose(x, (0, 2, 3, 1)).reshape(B, HW, C)
        w1t = jnp.transpose(w1, (2, 3, 0, 1)).reshape(9, C, C)
        w2t = jnp.transpose(w2, (2, 3, 0, 1)).reshape(9, C, C)
        any_spec = pl.BlockSpec(memory_space=pl.ANY)
        ubuf = pltpu.VMEM((C // 2, C), u32)
        vbuf = pltpu.VMEM((16, M // 2, C), u32)
        ybuf = pltpu.VMEM((4, G, M, 128), f32)
        out = pl.pallas_call(
            kern,
            in_specs=[any_spec] * 9,
            out_specs=any_spec,
            out_shape=jax.ShapeDtypeStruct((B, HW, C), bf16),
            scratch_shapes=[
                pltpu.VMEM((4, HW, C), bf16),
                pltpu.VMEM((18, C, C), bf16),
                pltpu.VMEM((16, (C // 2 + UB // 2) if UMODE == 0 else 8, C), u32),
                pltpu.VMEM((G, TR + 2, 4, HP, 128), f32),
                vbuf, vbuf, ybuf, ybuf,
                pltpu.VMEM((4, T, 3, 8, C), f32),
                pltpu.VMEM((4, 3, 8, C), f32),
                pltpu.VMEM((2, 2, 8, C), f32),
                pltpu.VMEM((4, 8, C), f32),
                pltpu.VMEM((B, E), bf16),
                pltpu.VMEM((E, C), bf16),
                pltpu.VMEM((4, G, 128), bf16),
                pltpu.SemaphoreType.DMA((T,)),
                pltpu.SemaphoreType.DMA((G,)),
                pltpu.SemaphoreType.DMA((8,)),
                pltpu.SemaphoreType.DMA((1,)),
            ] + [ubuf] * 16,
            compiler_params=pltpu.CompilerParams(vmem_limit_bytes=100 * 1024 * 1024,
                                                 disable_bounds_checks=True),
        )(xn, t_emb, g1.reshape(G, 128), be1.reshape(G, 128), w1t, w_emb,
          g2.reshape(G, 128), be2.reshape(G, 128), w2t)
        return jnp.transpose(out.reshape(B, H, W, C), (0, 3, 1, 2))
    return fn


_OPTS = {'xmode': 1, 'xr': 256, 'sub': 4}


@jax.jit
def pallas_standalone__adm_resblock__diffusion_kernel(x, t_emb, g1, be1, w1, w_emb, g2, be2, w2):
    B, C, H, W = x.shape
    E = t_emb.shape[1]
    return build(B, C, H, W, E, TM=1024, opts=_OPTS)(x, t_emb, g1, be1, w1, w_emb, g2, be2, w2)
```

```python
import jax
import jax.numpy as jnp
from jax import lax
from jax.experimental import pallas as pl
from jax.experimental.pallas import tpu as pltpu

f32 = jnp.float32
bf16 = jnp.bfloat16
u32 = jnp.uint32
NT = (((1,), (1,)), ((), ()))


def build(B, C, H, W, E, TM=1024, opts=None):
    opts = opts or {}
    HW = H * W
    G = 4
    CG = C // G
    EPS = 1e-5
    T = HW // TM
    assert CG == 128 and B == 2 and T == 4 and W == 64 and H == 64
    TR = TM // W
    NP = TR // 2
    HP = W // 2
    M = NP * HP
    NSTEP = 4 * T
    scope = jax.named_scope

    PW = opts.get('pw', 256)
    NPW = C // PW
    SUB = opts.get('sub', 4)
    XR = opts.get('xr', 256)
    NXR = TM // XR
    last_slot = opts.get('last_slot', 61)
    NQ = opts.get('nq', 4)
    QR = TM // NQ
    UMODE = opts.get('umode', 0)
    XMODE = opts.get('xmode', 0)
    PMODE = opts.get('pmode', 1)
    NSUB = opts.get('nsub', 4)
    XR1 = opts.get('xr1', 32)
    UB = 16
    NUB = (C // UB) * G

    def mult(v, m):
        return v if isinstance(v, int) else pl.multiple_of(v, m)

    def divT(v):
        return v // T if isinstance(v, int) else lax.shift_right_logical(v, 2)

    def modT(v):
        return v % T if isinstance(v, int) else jnp.bitwise_and(v, T - 1)

    def marker_of(d, n, sub, width):
        rp = sub * (d.shape[0] // SUB) // 8 * 8
        m = d[rp:rp + 8, n * 128:(n + 1) * 128]
        b = pltpu.bitcast(m, u32)
        z = pltpu.bitcast((b >> 16) >> 16, f32)
        if width > 128:
            z = jnp.concatenate([z] * (width // 128), axis=1)
        return z

    def pack_rows(t):
        return pltpu.bitcast(t.astype(bf16), u32)

    def pack2(t):
        n = t.shape[0] // 2
        return pltpu.pack_elementwise([t[:n], t[n:]], packed_dtype=bf16)

    def lanes(cb, width=128):
        if isinstance(cb, int):
            return slice(cb * width, (cb + 1) * width)
        return pl.ds(pl.multiple_of(cb * width, width), width)

    def load_y(y_ref, c, j, cb0, ncb):
        parts = []
        for i in range(ncb):
            n = cb0 + i
            lo = y_ref[c, n, pl.ds(j * HP, HP // 2, stride=2), :]
            hi = y_ref[c, n, pl.ds(j * HP + 1, HP // 2, stride=2), :]
            parts.append(jnp.concatenate([lo, hi], axis=0))
        return parts[0] if ncb == 1 else jnp.concatenate(parts, axis=1)

    def store_y(y_ref, c, val):
        for n in range(G):
            y_ref[c, n] = val[:, n * 128:(n + 1) * 128]

    def split_eo(v):
        w = pltpu.bitcast(v, u32)
        return (pltpu.unpack_elementwise(w, index=0, packed_dtype=bf16, unpacked_dtype=f32),
                pltpu.unpack_elementwise(w, index=1, packed_dtype=bf16, unpacked_dtype=f32))

    def join_eo(e, o):
        return pltpu.bitcast(pltpu.pack_elementwise([e, o], packed_dtype=bf16), bf16)

    def act(v, pv, marker):
        n, wd = v.shape
        mu, sc, bt = pv
        if marker is not None:
            mu = mu + marker
        v3 = v.reshape(n // 8, 8, wd)
        hz = ((v3 - mu[None]) * sc[None] + bt[None]).reshape(n, wd)
        return hz * jnp.tanh(hz) + hz

    def act_row(s_ref, pv, q, y, cs, marker, edge):
        yc = y if not edge else jnp.clip(y, 0, H - 1)
        e, o = split_eo(s_ref[q, pl.ds(mult(yc * W, W), W), cs])
        e = act(e, pv, marker)
        o = act(o, pv, marker)
        if edge:
            valid = jnp.logical_and(y >= 0, y < H)
            e = jnp.where(valid, e, 0.0)
            o = jnp.where(valid, o, 0.0)
        return e, o

    def prod_prime(s_ref, pv, q, y0, cs, marker):
        return act_row(s_ref, pv, q, y0 - 1, cs, marker, True) + act_row(s_ref, pv, q, y0, cs, marker, False)

    def prod_pair(s_ref, pv, v_ref, q, y0, j, cs, carry, marker):
        e0, o0, e1, o1 = carry
        e2, o2 = act_row(s_ref, pv, q, y0 + 2 * j + 1, cs, marker, False)
        e3, o3 = act_row(s_ref, pv, q, y0 + 2 * j + 2, cs, marker, j == NP - 1)
        row = lax.broadcasted_iota(jnp.int32, (HP, 128), 0)
        rs = pl.ds(mult(j * (HP // 2), HP // 2), HP // 2)
        for a in range(4):
            if a == 0:
                te, to = e0 - e2, o0 - o2
            elif a == 1:
                te, to = e1 + e2, o1 + o2
            elif a == 2:
                te, to = e2 - e1, o2 - o1
            else:
                te, to = e1 - e3, o1 - o3
            om = jnp.where(row == 0, 0.0, pltpu.roll(to, 1, 0))
            ep = jnp.where(row == HP - 1, 0.0, pltpu.roll(te, HP - 1, 0))
            v_ref[4 * a + 0, rs, cs] = pack2(om - to)
            v_ref[4 * a + 1, rs, cs] = pack2(te + to)
            v_ref[4 * a + 2, rs, cs] = pack2(to - te)
            v_ref[4 * a + 3, rs, cs] = pack2(te - ep)
        return e2, o2, e3, o3

    def prod_a(s_ref, pv, xr_ref, q, y0, cb, i, marker):
        cs = lanes(cb)
        cb = cb if isinstance(cb, int) else 0
        e, o = act_row(s_ref, pv, q, y0 - 1 + i, cs, marker, i == 0 or i == TR + 1)
        row = lax.broadcasted_iota(jnp.int32, (HP, 128), 0)
        om = jnp.where(row == 0, 0.0, pltpu.roll(o, 1, 0))
        ep = jnp.where(row == HP - 1, 0.0, pltpu.roll(e, HP - 1, 0))
        xr_ref[cb, i, 0] = om - o
        xr_ref[cb, i, 1] = e + o
        xr_ref[cb, i, 2] = o - e
        xr_ref[cb, i, 3] = e - ep

    def prod_b(xr_ref, v_ref, cb, j, b, marker):
        cs = lanes(cb)
        cb = cb if isinstance(cb, int) else 0
        rs = pl.ds(j * (HP // 2), HP // 2)
        r0, r1, r2, r3 = (xr_ref[cb, 2 * j + i, b] for i in range(4))
        if marker is not None:
            r2 = (r2.reshape(HP // 8, 8, 128) + marker[None]).reshape(HP, 128)
        v_ref[0 + b, rs, cs] = pack2(r0 - r2)
        v_ref[4 + b, rs, cs] = pack2(r1 + r2)
        v_ref[8 + b, rs, cs] = pack2(r2 - r1)
        v_ref[12 + b, rs, cs] = pack2(r1 - r3)

    def u_piece(w_ref, u_ref, base, k, marker, ok=None):
        rb = lax.shift_right_logical(k, 2) if not isinstance(k, int) else k // 4
        cb = jnp.bitwise_and(k, 3) if not isinstance(k, int) else k % 4
        rows = pl.ds(mult(rb * UB, UB), UB)
        ob = rb if ok is None else jnp.where(ok, rb, C // UB)
        orow = pl.ds(mult(ob * (UB // 2), UB // 2), UB // 2)
        cs = pl.ds(mult(cb * 128, 128), 128)
        res = []
        raw = [[split_eo(w_ref[base + 3 * i + j, rows, cs]) for j in range(3)] for i in range(3)]
        for par in range(2):
            hs = []
            for i in range(3):
                g0, g1, g2 = (raw[i][j][par] for j in range(3))
                if marker is not None:
                    g1 = g1 + marker
                sm = g0 + g2
                hs.append((g0, (sm + g1) * 0.5, (sm - g1) * 0.5, g2))
            out = [None] * 16
            for b in range(4):
                g0, g1, g2 = hs[0][b], hs[1][b], hs[2][b]
                sm = g0 + g2
                for a, val in enumerate((g0, (sm + g1) * 0.5, (sm - g1) * 0.5, g2)):
                    out[4 * a + b] = val
            res.append(out)
        for k2 in range(16):
            val = pltpu.pack_elementwise([res[0][k2], res[1][k2]], packed_dtype=bf16)
            if isinstance(u_ref, (list, tuple)):
                u_ref[k2][orow, cs] = val
            else:
                u_ref[k2, orow, cs] = val

    def stat_acc(v, state, marker=None):
        n = v.shape[0] // 8
        wd = v.shape[1]
        if state is None:
            K = v[0:1, :]
            if marker is not None:
                K = K + marker[0:1, :]
            d = v - K
            return (K, d.reshape(n, 8, wd).sum(axis=0), (d * d).reshape(n, 8, wd).sum(axis=0))
        K, s1, s2 = state
        Kd = K if marker is None else K + marker[0:1, :]
        d = v - Kd
        return (K, s1 + d.reshape(n, 8, wd).sum(axis=0), s2 + (d * d).reshape(n, 8, wd).sum(axis=0))

    def store_stats(st_ref, q, t, cs, state):
        K, s1, s2 = state
        wd = K.shape[1]
        st_ref[q, t, 0, :, cs] = jnp.broadcast_to(K, (8, wd))
        st_ref[q, t, 1, :, cs] = jnp.broadcast_to(s1.sum(axis=0, keepdims=True), (8, wd))
        st_ref[q, t, 2, :, cs] = jnp.broadcast_to(s2.sum(axis=0, keepdims=True), (8, wd))

    def finalize(st_ref, p_ref, gb_ref, e_ref, q):
        cv = q // 2 if isinstance(q, int) else lax.shift_right_logical(q, 1)
        for g in range(G):
            cs = slice(g * 128, (g + 1) * 128)
            K = st_ref[q, :, 0, :, cs]
            s1 = st_ref[q, :, 1, :, cs]
            s2 = st_ref[q, :, 2, :, cs]
            e = e_ref[q, :, cs]
            mean_t = K + s1 * (1.0 / TM) + e[None]
            m2_t = s2 - s1 * s1 * (1.0 / TM)
            mu = jnp.sum(jnp.sum(mean_t, axis=0), axis=1, keepdims=True) * (1.0 / (T * 128))
            dev = mean_t - mu[None]
            tot = m2_t + dev * dev * float(TM)
            var = jnp.sum(jnp.sum(tot, axis=0), axis=1, keepdims=True) * (1.0 / (HW * 128))
            rstd = lax.rsqrt(var + EPS)
            p_ref[q, 0, :, cs] = mu - e
            p_ref[q, 1, :, cs] = gb_ref[cv, 0, :, cs] * (rstd * 0.5)
            p_ref[q, 2, :, cs] = gb_ref[cv, 1, :, cs] * 0.5

    def merge(lists):
        items = []
        for li, l in enumerate(lists):
            for i, it in enumerate(l):
                items.append(((i + 0.5) / len(l), li, it))
        items.sort(key=lambda z: (z[0], z[1]))
        return [it for _, _, it in items]

    def kern(x_hbm, te_hbm, g1_hbm, b1_hbm, w1_hbm, we_hbm, g2_hbm, b2_hbm, w2_hbm, o_hbm,
             s_ref, w_ref, u2_ref, xr_ref, va_ref, vb_ref, ya_ref, yb_ref,
             st_ref, p_ref, gb_ref, e_ref, te_ref, we_ref, gsm_ref, sem_x, sem_w, sem_s, sem_o, *u1_ref):

        def gcols(g):
            return pl.ds(mult(g * 128, 128), 128)

        def x0_copy(c):
            rows = pl.ds(mult(c * TM, TM), TM)
            return pltpu.make_async_copy(x_hbm.at[0, rows, :], s_ref.at[0, rows, :], sem_x.at[c])

        def w1_copy(g):
            return pltpu.make_async_copy(w1_hbm.at[:, gcols(g), :], w_ref.at[pl.ds(0, 9), gcols(g), :], sem_w.at[g])

        def x1_copy():
            return pltpu.make_async_copy(x_hbm.at[1], s_ref.at[1], sem_s.at[6])

        def w2_copy():
            return pltpu.make_async_copy(w2_hbm, w_ref.at[pl.ds(9, 9)], sem_s.at[7])

        def small_copies():
            return [pltpu.make_async_copy(g1_hbm, gsm_ref.at[0], sem_s.at[0]),
                    pltpu.make_async_copy(b1_hbm, gsm_ref.at[1], sem_s.at[1]),
                    pltpu.make_async_copy(g2_hbm, gsm_ref.at[2], sem_s.at[2]),
                    pltpu.make_async_copy(b2_hbm, gsm_ref.at[3], sem_s.at[3]),
                    pltpu.make_async_copy(te_hbm, te_ref, sem_s.at[4])]

        def we_copy():
            return pltpu.make_async_copy(we_hbm, we_ref, sem_s.at[5])

        def o_copy(s, qi):
            b = divT(s) - 2
            r0 = mult(modT(s) * TM + qi * QR, QR)
            return pltpu.make_async_copy(s_ref.at[b, pl.ds(r0, QR), :], o_hbm.at[b, pl.ds(r0, QR), :], sem_o.at[0])

        def o_all():
            return pltpu.make_async_copy(s_ref.at[pl.ds(0, B)], o_hbm, sem_o.at[0])

        def epi_piece(y_ref, s_prev, kind, r, cb, state, marker, PW=PW):
            p = divT(s_prev)
            t = modT(s_prev)
            cs = lanes(cb, PW)
            j, par = r // 2, r % 2
            r0 = mult(t * TM + r * W, W)
            ve = load_y(y_ref, 2 * par, j, cb * (PW // 128), PW // 128)
            vo = load_y(y_ref, 2 * par + 1, j, cb * (PW // 128), PW // 128)
            if marker is not None:
                ve = (ve.reshape(HP // 8, 8, PW) + marker[None]).reshape(HP, PW)
            if kind == 1:
                dst, sq = p + 2, p + 2
            elif kind == 2:
                dst, sq = p - 2, None
                xe, xo = split_eo(s_ref[dst, pl.ds(r0, W), cs])
                ve, vo = ve + xe, vo + xo
            else:
                is2 = p >= 2
                dst = jnp.where(is2, p - 2, p + 2)
                sq = jnp.where(is2, 0, p + 2)
                xe, xo = split_eo(s_ref[dst, pl.ds(r0, W), cs])
                ve, vo = ve + jnp.where(is2, xe, 0.0), vo + jnp.where(is2, xo, 0.0)
            if sq is not None:
                state = stat_acc(vo, stat_acc(ve, state))
            s_ref[dst, pl.ds(r0, W), cs] = join_eo(ve, vo)
            if sq is not None and r == TR - 1:
                store_stats(st_ref, sq, t, cs, state)
                state = None
            return state

        def xstat_piece(q, tile, cs, ri, state, marker):
            r0 = mult(tile * TM + ri * XR1, XR1)
            v = s_ref[q, pl.ds(r0, XR1), cs].astype(f32)
            state = stat_acc(v, state, marker)
            if ri == TM // XR1 - 1:
                store_stats(st_ref, q, tile, cs, state)
                state = None
            return state

        def half(it, second, u_ref, vc_ref, vn_ref, yc_ref, yp_ref):
            s = 2 * it + second
            sn = s + 1
            pn = jnp.minimum(divT(sn), 3)
            y0 = modT(sn) * TR
            if PMODE == 0:
                plist = [('p', cb, j) for cb in range(G) for j in range(-1, NP)]
            else:
                plist = []
                for cb in range(G):
                    plist += [('a', cb, 0), ('a', cb, 1)]
                    for j in range(NP):
                        plist += [('a', cb, 2 * j + 2), ('a', cb, 2 * j + 3)] + [('b', cb, j, b) for b in range(4)]
            lists = [plist,
                     [('e', r, cb) for r in range(TR) for cb in range(NPW)]]
            NU = -(-NUB // 5)
            if UMODE == 0:
                lists.append([('u', k) for k in range(NU)])
            pieces = merge(lists)
            npc = len(pieces)
            if second == 1:
                finalize(st_ref, p_ref, gb_ref, e_ref, jnp.minimum(divT(s - 1) + 1, 3))
            pv = tuple(p_ref[pn, k] for k in range(3))
            sp = s - 1
            ekind = 0
            done = 0
            est = [None] * NPW
            xst = None
            pcar = None
            ys = [None] * 4
            for a in range(4):
                rr = [None, None]
                for b in range(4):
                    k = 4 * a + b
                    d = lax.dot_general(pltpu.bitcast(vc_ref[k], bf16), pltpu.bitcast(u_ref[k][...], bf16), NT,
                                        preferred_element_type=f32)
                    for nn in range(4 * SUB):
                        n, sub = nn // SUB, nn % SUB
                        hi_ = min(npc, (((k * 4 * SUB + nn) + 1) * npc) // (last_slot * SUB))
                        while done < hi_:
                            pc = pieces[done]
                            if pc[0] == 'p':
                                cs = slice(pc[1] * 128, (pc[1] + 1) * 128)
                                pvc = tuple(t[:, cs] for t in pv)
                                mk = marker_of(d, n, sub, 128)
                                if pc[2] < 0:
                                    pcar = prod_prime(s_ref, pvc, pn, y0, cs, mk)
                                else:
                                    pcar = prod_pair(s_ref, pvc, vn_ref, pn, y0, pc[2], cs, pcar, mk)
                            elif pc[0] == 'a':
                                cs = slice(pc[1] * 128, (pc[1] + 1) * 128)
                                prod_a(s_ref, tuple(t[:, cs] for t in pv), xr_ref, pn, y0, pc[1], pc[2],
                                       marker_of(d, n, sub, 128))
                            elif pc[0] == 'b':
                                prod_b(xr_ref, vn_ref, pc[1], pc[2], pc[3], marker_of(d, n, sub, 128))
                            elif pc[0] == 'e':
                                est[pc[2]] = epi_piece(yp_ref, sp, ekind, pc[1], pc[2], est[pc[2]],
                                                       marker_of(d, n, sub, PW))
                                if pc[2] == NPW - 1 and ((pc[1] + 1) * W) % QR == 0:
                                    qi = ((pc[1] + 1) * W) // QR - 1

                                    @pl.when(sp >= 2 * T)
                                    def _():
                                        o_copy(sp, qi).start()
                            elif pc[0] == 'x':
                                xst = xstat_piece(jnp.where(it == 0, 0, 1), pc[1],
                                                  slice(pc[2] * PW, (pc[2] + 1) * PW), pc[3], xst,
                                                  marker_of(d, n, sub, PW))
                            else:
                                kk = (s - 2) * NU + pc[1]
                                ok = jnp.logical_and(kk >= 0, kk < NUB)
                                u_piece(w_ref, u2_ref, 9, jnp.clip(kk, 0, NUB - 1),
                                        marker_of(d, n, sub, 128), ok)
                            done += 1
                    if b == 0:
                        rr[0] = d
                    elif b == 1:
                        rr[0] = rr[0] + d
                        rr[1] = d
                    elif b == 2:
                        rr[0] = rr[0] + d
                        rr[1] = rr[1] - d
                    else:
                        rr[1] = rr[1] - d
                for c in range(2):
                    if a == 0:
                        ys[c] = rr[c]
                    elif a == 1:
                        ys[c] = ys[c] + rr[c]
                        ys[2 + c] = rr[c]
                    elif a == 2:
                        store_y(yc_ref, c, ys[c] + rr[c])
                        ys[2 + c] = ys[2 + c] - rr[c]
                    else:
                        store_y(yc_ref, 2 + c, ys[2 + c] - rr[c])

        def nhalf(step, n, vc_ref, vn_ref, yc_ref, yp_ref):
            y0 = (step + 1) * TR
            plist = [('a', 0), ('a', 1)]
            for j in range(NP):
                plist += [('a', 2 * j + 2), ('a', 2 * j + 3)] + [('b', j, b) for b in range(4)]
            lists = [plist]
            if step == 0:
                lists.append([('u', k) for k in range(NUB // G)])
            else:
                lists.append([('e', r) for r in range(TR)])
                lists.append([('x', cb, ri) for cb in range(NPW) for ri in range(TM // XR1)])
            pieces = merge(lists)
            npc = len(pieces)
            cs = lanes(n)
            pvc = tuple(p_ref[0, k, :, cs] for k in range(3))
            urows = pl.ds(pl.multiple_of(n * (128 // 2), 128 // 2), 128 // 2)
            gn = jnp.minimum(n + 1, G - 1)
            NS = NSUB
            done = 0
            est = xst = None
            ys = [None] * 4
            dprev = None
            for a in range(4):
                rr = [None, None]
                for b in range(4):
                    k = 4 * a + b
                    d = lax.dot_general(pltpu.bitcast(vc_ref[k], bf16), pltpu.bitcast(u1_ref[k][urows, :], bf16), NT,
                                        preferred_element_type=f32)
                    for sub in range(NS):
                        hi_ = npc if k == 15 and sub == NS - 1 else ((k * NS + sub) * npc) // (15 * NS)
                        while done < min(hi_, npc) and dprev is not None:
                            pc = pieces[done]
                            rp = sub * (M // NS) // 8 * 8
                            bits = pltpu.bitcast(dprev[rp:rp + 8, :], u32)
                            mk = pltpu.bitcast((bits >> 16) >> 16, f32)
                            if pc[0] == 'a':
                                prod_a(s_ref, pvc, xr_ref, 0, y0, n, pc[1], mk)
                            elif pc[0] == 'b':
                                prod_b(xr_ref, vn_ref, n, pc[1], pc[2], mk)
                            elif pc[0] == 'u':
                                u_piece(w_ref, u1_ref, 0, gn * (NUB // G) + pc[1], mk)
                            elif pc[0] == 'e':
                                est = epi_piece(yp_ref, 0, 1, pc[1], n, est, mk, PW=128)
                            else:
                                mkx = mk if PW == 128 else jnp.concatenate([mk] * (PW // 128), axis=1)
                                xst = xstat_piece(1, n, slice(pc[1] * PW, (pc[1] + 1) * PW), pc[2], xst, mkx)
                            done += 1
                    dprev = d
                    if b == 0:
                        rr[0] = d
                    elif b == 1:
                        rr[0] = rr[0] + d
                        rr[1] = d
                    elif b == 2:
                        rr[0] = rr[0] + d
                        rr[1] = rr[1] - d
                    else:
                        rr[1] = rr[1] - d
                for c in range(2):
                    if a == 0:
                        ys[c] = rr[c]
                    elif a == 1:
                        ys[c] = ys[c] + rr[c]
                        ys[2 + c] = rr[c]
                    elif a == 2:
                        yc_ref[c, n] = ys[c] + rr[c]
                        ys[2 + c] = ys[2 + c] - rr[c]
                    else:
                        yc_ref[2 + c, n] = ys[2 + c] - rr[c]
            assert done == npc

        def xstat_tile(q, c):
            for cb in range(NPW):
                def rows(ri, st):
                    r0 = pl.multiple_of(c * TM + ri * XR, XR)
                    v = s_ref[q, pl.ds(r0, XR), cb * PW:(cb + 1) * PW].astype(f32)
                    return stat_acc(v, st)
                v0 = s_ref[q, pl.ds(pl.multiple_of(c * TM, XR), XR), cb * PW:(cb + 1) * PW].astype(f32)
                st = lax.fori_loop(1, NXR, rows, stat_acc(v0, None))
                store_stats(st_ref, q, c, slice(cb * PW, (cb + 1) * PW), st)
            return 0

        with scope('prologue'):
            for c in small_copies():
                c.start()
            lax.fori_loop(0, T, lambda c, _: (x0_copy(c).start(), 0)[1], 0)
            lax.fori_loop(0, G, lambda g, _: (w1_copy(g).start(), 0)[1], 0)

            def rest(c, _):
                @pl.when(c == 0)
                def _():
                    x1_copy().start()

                @pl.when(c == 1)
                def _():
                    w2_copy().start()

                @pl.when(c == 2)
                def _():
                    we_copy().start()
                return 0
            lax.fori_loop(0, 3, rest, 0)

            for c in small_copies():
                c.wait()
            for cv in range(2):
                for k in range(2):
                    v = gsm_ref[2 * cv + k].astype(f32)
                    for g in range(G):
                        gb_ref[cv, k, :, g * 128:(g + 1) * 128] = jnp.broadcast_to(v[g:g + 1, :], (8, 128))
            e_ref[...] = jnp.zeros(e_ref.shape, f32)
            st_ref[...] = jnp.zeros(st_ref.shape, f32)

            def xs0(c, _):
                x0_copy(c).wait()
                return xstat_tile(0, c)
            lax.fori_loop(0, T, xs0, 0)
            finalize(st_ref, p_ref, gb_ref, e_ref, 0)

            def prod0(cb, _):
                cs = gcols(cb)
                pvc = tuple(p_ref[0, k, :, cs] for k in range(3))
                car = prod_prime(s_ref, pvc, 0, 0, cs, None)

                def pair(j, car):
                    return prod_pair_dyn(j, car, cs, pvc)
                lax.fori_loop(0, NP, pair, car)
                return 0

            def prod_pair_dyn(j, carry, cs, pvc):
                e0, o0, e1, o1 = carry
                e2, o2 = act_row(s_ref, pvc, 0, 2 * j + 1, cs, None, False)
                e3, o3 = act_row(s_ref, pvc, 0, 2 * j + 2, cs, None, False)
                row = lax.broadcasted_iota(jnp.int32, (HP, 128), 0)
                rs = pl.ds(pl.multiple_of(j * (HP // 2), HP // 2), HP // 2)
                for a in range(4):
                    if a == 0:
                        te, to = e0 - e2, o0 - o2
                    elif a == 1:
                        te, to = e1 + e2, o1 + o2
                    elif a == 2:
                        te, to = e2 - e1, o2 - o1
                    else:
                        te, to = e1 - e3, o1 - o3
                    om = jnp.where(row == 0, 0.0, pltpu.roll(to, 1, 0))
                    ep = jnp.where(row == HP - 1, 0.0, pltpu.roll(te, HP - 1, 0))
                    va_ref[4 * a + 0, rs, cs] = pack2(om - to)
                    va_ref[4 * a + 1, rs, cs] = pack2(te + to)
                    va_ref[4 * a + 2, rs, cs] = pack2(to - te)
                    va_ref[4 * a + 3, rs, cs] = pack2(te - ep)
                return e2, o2, e3, o3
            lax.fori_loop(0, G, prod0, 0)

            w1_copy(0).wait()
            lax.fori_loop(0, NUB // G, lambda k, _: (u_piece(w_ref, u1_ref, 0, k, None), 0)[1], 0)

        def step0(n, _):
            @pl.when(n < G - 1)
            def _():
                w1_copy(n + 1).wait()
            nhalf(0, n, va_ref, vb_ref, ya_ref, yb_ref)
            return 0

        def step1(n, _):
            nhalf(1, n, vb_ref, va_ref, yb_ref, ya_ref)
            return 0

        with scope('step0'):
            lax.fori_loop(0, G, step0, 0)
        with scope('step1'):
            x1_copy().wait()
            lax.fori_loop(0, G, step1, 0)

        def body(it, carry):
            @pl.when(it == 1)
            def _():
                w2_copy().wait()
                we_copy().wait()
                te = te_ref[...].astype(f32)
                sl = te * jax.nn.sigmoid(te)
                emb = jnp.dot(sl.astype(bf16), we_ref[...], preferred_element_type=f32)
                e_ref[2] = jnp.broadcast_to(emb[0:1, :], (8, C))
                e_ref[3] = jnp.broadcast_to(emb[1:2, :], (8, C))

            @pl.when(it == T)
            def _():
                if UMODE == 0:
                    def cp(rb, _):
                        rows = pl.ds(pl.multiple_of(rb * 32, 32), 32)
                        for k in range(16):
                            u1_ref[k][rows, :] = u2_ref[k, rows, :]
                        return 0
                    lax.fori_loop(0, C // 2 // 32, cp, 0)
                else:
                    lax.fori_loop(0, NUB, lambda k, _: (u_piece(w_ref, u1_ref, 9, k, None), 0)[1], 0)
            with scope('iter'):
                half(it, 0, u1_ref, va_ref, vb_ref, ya_ref, yb_ref)
                half(it, 1, u1_ref, vb_ref, va_ref, yb_ref, ya_ref)
            return carry

        with scope('main'):
            lax.fori_loop(1, 2 * T, body, 0)

        sl_ = NSTEP - 1
        with scope('final'):
            st = [None] * NPW
            for r in range(TR):
                for cb in range(NPW):
                    st[cb] = epi_piece(yb_ref, sl_, 2, r, cb, st[cb], None)
                if ((r + 1) * W) % QR == 0:
                    o_copy(sl_, ((r + 1) * W) // QR - 1).start()
        with scope('owait'):
            o_all().wait()

    def fn(x, t_emb, g1, be1, w1, w_emb, g2, be2, w2):
        xn = jnp.transpose(x, (0, 2, 3, 1)).reshape(B, HW, C)
        w1t = jnp.transpose(w1, (2, 3, 0, 1)).reshape(9, C, C)
        w2t = jnp.transpose(w2, (2, 3, 0, 1)).reshape(9, C, C)
        any_spec = pl.BlockSpec(memory_space=pl.ANY)
        ubuf = pltpu.VMEM((C // 2, C), u32)
        vbuf = pltpu.VMEM((16, M // 2, C), u32)
        ybuf = pltpu.VMEM((4, G, M, 128), f32)
        out = pl.pallas_call(
            kern,
            in_specs=[any_spec] * 9,
            out_specs=any_spec,
            out_shape=jax.ShapeDtypeStruct((B, HW, C), bf16),
            scratch_shapes=[
                pltpu.VMEM((4, HW, C), bf16),
                pltpu.VMEM((18, C, C), bf16),
                pltpu.VMEM((16, (C // 2 + UB // 2) if UMODE == 0 else 8, C), u32),
                pltpu.VMEM((G, TR + 2, 4, HP, 128), f32),
                vbuf, vbuf, ybuf, ybuf,
                pltpu.VMEM((4, T, 3, 8, C), f32),
                pltpu.VMEM((4, 3, 8, C), f32),
                pltpu.VMEM((2, 2, 8, C), f32),
                pltpu.VMEM((4, 8, C), f32),
                pltpu.VMEM((B, E), bf16),
                pltpu.VMEM((E, C), bf16),
                pltpu.VMEM((4, G, 128), bf16),
                pltpu.SemaphoreType.DMA((T,)),
                pltpu.SemaphoreType.DMA((G,)),
                pltpu.SemaphoreType.DMA((8,)),
                pltpu.SemaphoreType.DMA((1,)),
            ] + [ubuf] * 16,
            compiler_params=pltpu.CompilerParams(vmem_limit_bytes=100 * 1024 * 1024,
                                                 disable_bounds_checks=True),
        )(xn, t_emb, g1.reshape(G, 128), be1.reshape(G, 128), w1t, w_emb,
          g2.reshape(G, 128), be2.reshape(G, 128), w2t)
        return jnp.transpose(out.reshape(B, H, W, C), (0, 3, 1, 2))
    return fn


_OPTS = {'nsub': 8}


@jax.jit
def pallas_standalone__adm_resblock__diffusion_kernel(x, t_emb, g1, be1, w1, w_emb, g2, be2, w2):
    B, C, H, W = x.shape
    E = t_emb.shape[1]
    return build(B, C, H, W, E, TM=1024, opts=_OPTS)(x, t_emb, g1, be1, w1, w_emb, g2, be2, w2)
```

```python
import jax
import jax.numpy as jnp
from jax import lax
from jax.experimental import pallas as pl
from jax.experimental.pallas import tpu as pltpu

f32 = jnp.float32
bf16 = jnp.bfloat16
u32 = jnp.uint32
NT = (((1,), (1,)), ((), ()))


def build(B, C, H, W, E, TM=1024, opts=None):
    opts = opts or {}
    HW = H * W
    G = 4
    CG = C // G
    EPS = 1e-5
    T = HW // TM
    assert CG == 128 and B == 2 and T == 4 and W == 64 and H == 64
    TR = TM // W
    NP = TR // 2
    HP = W // 2
    NQ4 = W // 4
    M = NP * NQ4
    NB = 6
    NPT = 4 * NB
    NSTEP = 4 * T
    scope = jax.named_scope

    PW = opts.get('pw', 256)
    NPW = C // PW
    SUB = opts.get('sub', 4)
    XR = opts.get('xr', 256)
    NXR = TM // XR
    last_slot = opts.get('last_slot', 61)
    NQ = opts.get('nq', 4)
    QR = TM // NQ
    UMODE = opts.get('umode', 0)
    XMODE = opts.get('xmode', 0)
    NAR = opts.get('nar', 2)
    BG = opts.get('bg', 2)
    NSUB = opts.get('nsub', 4)
    XR1 = opts.get('xr1', 32)
    UB = 16
    NUB = (C // UB) * G

    def mult(v, m):
        return v if isinstance(v, int) else pl.multiple_of(v, m)

    def divT(v):
        return v // T if isinstance(v, int) else lax.shift_right_logical(v, 2)

    def modT(v):
        return v % T if isinstance(v, int) else jnp.bitwise_and(v, T - 1)

    def marker_of(d, n, sub, width):
        rp = sub * (d.shape[0] // SUB) // 8 * 8
        m = d[rp:rp + 8, n * 128:(n + 1) * 128]
        b = pltpu.bitcast(m, u32)
        z = pltpu.bitcast((b >> 16) >> 16, f32)
        if width > 128:
            z = jnp.concatenate([z] * (width // 128), axis=1)
        return z

    def pack2(t):
        n = t.shape[0] // 2
        return pltpu.pack_elementwise([t[:n], t[n:]], packed_dtype=bf16)

    def lanes(cb, width=128):
        if isinstance(cb, int):
            return slice(cb * width, (cb + 1) * width)
        return pl.ds(pl.multiple_of(cb * width, width), width)

    def load_y(y_ref, par, eo, j, cb0, ncb):
        parts = [y_ref[par, eo, cb0 + i, j * HP:(j + 1) * HP, :] for i in range(ncb)]
        return parts[0] if ncb == 1 else jnp.concatenate(parts, axis=1)

    def store_y(y_ref, par, q, n, val):
        y_ref[par, q % 2, n, pl.ds(q // 2, M, stride=2), :] = val

    def split_eo(v):
        w = pltpu.bitcast(v, u32)
        return (pltpu.unpack_elementwise(w, index=0, packed_dtype=bf16, unpacked_dtype=f32),
                pltpu.unpack_elementwise(w, index=1, packed_dtype=bf16, unpacked_dtype=f32))

    def join_eo(e, o):
        return pltpu.bitcast(pltpu.pack_elementwise([e, o], packed_dtype=bf16), bf16)

    def act(v, pv, marker):
        n, wd = v.shape
        mu, sc, bt = pv
        if marker is not None:
            mu = mu + marker
        v3 = v.reshape(n // 8, 8, wd)
        hz = ((v3 - mu[None]) * sc[None] + bt[None]).reshape(n, wd)
        return hz * jnp.tanh(hz) + hz

    def act_row(s_ref, pv, q, y, cs, marker, edge):
        yc = y if not edge else jnp.clip(y, 0, H - 1)
        e, o = split_eo(s_ref[q, pl.ds(mult(yc * W, W), W), cs])
        e = act(e, pv, marker)
        o = act(o, pv, marker)
        if edge:
            valid = jnp.logical_and(y >= 0, y < H)
            e = jnp.where(valid, e, 0.0)
            o = jnp.where(valid, o, 0.0)
        return e, o

    def prod_a(s_ref, pv, ar_ref, xr_ref, q, y0, cb, i, marker):
        cs = lanes(cb)
        cb = cb if isinstance(cb, int) else 0
        e, o = act_row(s_ref, pv, q, y0 - 1 + i, cs, marker, i == 0 or i == TR + 1)
        sl = i % NAR
        ar_ref[cb, sl, 0, 8:8 + HP, :] = e
        ar_ref[cb, sl, 1, 8:8 + HP, :] = o

        def col(eo, r):
            return jnp.concatenate([ar_ref[cb, sl, eo, pl.ds(r + 2 * u, NQ4 // 2, stride=4), :] for u in range(2)], axis=0)
        d0, d1, d2, d3, d4, d5 = col(1, 7), col(0, 8), col(1, 8), col(0, 9), col(1, 9), col(0, 10)
        c = d4 - d2
        e2 = (d3 - d1) * 2.0
        a_ = d4 - d2 * 4.0
        b_ = d3 - d1 * 4.0
        xr_ref[cb, i, 0] = (d0 - d2) * 4.0 + c
        xr_ref[cb, i, 1] = a_ + b_
        xr_ref[cb, i, 2] = a_ - b_
        xr_ref[cb, i, 3] = c + e2
        xr_ref[cb, i, 4] = c - e2
        xr_ref[cb, i, 5] = (d5 - d3) - e2 * 2.0

    def prod_b(xr_ref, v_ref, cb, j, bs, marker):
        cs = lanes(cb)
        cb = cb if isinstance(cb, int) else 0
        rs = pl.ds(j * (NQ4 // 2), NQ4 // 2)
        for b in bs:
            r0, r1, r2, r3 = (xr_ref[cb, 2 * j + i, b] for i in range(4))
            if marker is not None:
                r2 = (r2.reshape(NQ4 // 8, 8, 128) + marker[None]).reshape(NQ4, 128)
            v_ref[b, rs, cs] = pack2(r0 - r2)
            v_ref[NB + b, rs, cs] = pack2(r1 + r2)
            v_ref[2 * NB + b, rs, cs] = pack2(r2 - r1)
            v_ref[3 * NB + b, rs, cs] = pack2(r1 - r3)

    def prod_list(cb):
        pl_ = [('a', cb, 0), ('a', cb, 1)]
        for j in range(NP):
            pl_ += [('a', cb, 2 * j + 2), ('a', cb, 2 * j + 3)]
            pl_ += [('b', cb, j, tuple(range(b, b + BG))) for b in range(0, NB, BG)]
        return pl_

    def out_x(st, b, d):
        if b == 0:
            st['r0'] = d
        elif b in (1, 3):
            st['p'] = d
        elif b == 2:
            st['s12'], st['d12'] = st['p'] + d, st['p'] - d
            st['r0'] = st['r0'] + st['s12']
        elif b == 4:
            s34, d34 = st['p'] + d, st['p'] - d
            st['r0'] = st['r0'] + s34
            st['r1'] = st['d12'] + d34 * 2.0
            st['r2'] = st['s12'] + s34 * 4.0
            st['r3'] = st['d12'] + d34 * 8.0
        else:
            return [st['r0'], st['r1'], st['r2'], st['r3'] + d]
        return None

    def out_y(ys, a, rr, store):
        for q in range(4):
            if a == 0:
                ys[q] = rr[q]
            elif a == 1:
                ys[q] = ys[q] + rr[q]
                ys[4 + q] = rr[q]
            elif a == 2:
                store(0, q, ys[q] + rr[q])
                ys[4 + q] = ys[4 + q] - rr[q]
            else:
                store(1, q, ys[4 + q] - rr[q])

    def u_piece(w_ref, u_ref, base, k, marker, ok=None):
        rb = lax.shift_right_logical(k, 2) if not isinstance(k, int) else k // 4
        cb = jnp.bitwise_and(k, 3) if not isinstance(k, int) else k % 4
        rows = pl.ds(mult(rb * UB, UB), UB)
        ob = rb if ok is None else jnp.where(ok, rb, C // UB)
        orow = pl.ds(mult(ob * (UB // 2), UB // 2), UB // 2)
        cs = pl.ds(mult(cb * 128, 128), 128)
        res = []
        raw = [[split_eo(w_ref[base + 3 * i + j, rows, cs]) for j in range(3)] for i in range(3)]
        for par in range(2):
            hs = []
            for j in range(3):
                g0, g1, g2 = (raw[i][j][par] for i in range(3))
                if marker is not None:
                    g1 = g1 + marker
                sm = g0 + g2
                hs.append((g0, (sm + g1) * 0.5, (sm - g1) * 0.5, g2))
            out = [None] * NPT
            for a in range(4):
                h0, h1, h2 = (hs[j][a] for j in range(3))
                sm = h0 + h2
                pp = h0 * (1.0 / 24.0) + h2 * (1.0 / 6.0)
                qq = h1 * (1.0 / 12.0)
                for b, val in enumerate((h0 * 0.25, (sm + h1) * (-1.0 / 6.0), (sm - h1) * (-1.0 / 6.0),
                                         pp + qq, pp - qq, h2)):
                    out[NB * a + b] = val
            res.append(out)
        for k2 in range(NPT):
            val = pltpu.pack_elementwise([res[0][k2], res[1][k2]], packed_dtype=bf16)
            if isinstance(u_ref, (list, tuple)):
                u_ref[k2][orow, cs] = val
            else:
                u_ref[k2, orow, cs] = val

    def stat_acc(v, state, marker=None):
        n = v.shape[0] // 8
        wd = v.shape[1]
        if state is None:
            K = v[0:1, :]
            if marker is not None:
                K = K + marker[0:1, :]
            d = v - K
            return (K, d.reshape(n, 8, wd).sum(axis=0), (d * d).reshape(n, 8, wd).sum(axis=0))
        K, s1, s2 = state
        Kd = K if marker is None else K + marker[0:1, :]
        d = v - Kd
        return (K, s1 + d.reshape(n, 8, wd).sum(axis=0), s2 + (d * d).reshape(n, 8, wd).sum(axis=0))

    def store_stats(st_ref, q, t, cs, state):
        K, s1, s2 = state
        wd = K.shape[1]
        st_ref[q, t, 0, :, cs] = jnp.broadcast_to(K, (8, wd))
        st_ref[q, t, 1, :, cs] = jnp.broadcast_to(s1.sum(axis=0, keepdims=True), (8, wd))
        st_ref[q, t, 2, :, cs] = jnp.broadcast_to(s2.sum(axis=0, keepdims=True), (8, wd))

    def finalize(st_ref, p_ref, gb_ref, e_ref, q):
        cv = q // 2 if isinstance(q, int) else lax.shift_right_logical(q, 1)
        for g in range(G):
            cs = slice(g * 128, (g + 1) * 128)
            K = st_ref[q, :, 0, :, cs]
            s1 = st_ref[q, :, 1, :, cs]
            s2 = st_ref[q, :, 2, :, cs]
            e = e_ref[q, :, cs]
            mean_t = K + s1 * (1.0 / TM) + e[None]
            m2_t = s2 - s1 * s1 * (1.0 / TM)
            mu = jnp.sum(jnp.sum(mean_t, axis=0), axis=1, keepdims=True) * (1.0 / (T * 128))
            dev = mean_t - mu[None]
            tot = m2_t + dev * dev * float(TM)
            var = jnp.sum(jnp.sum(tot, axis=0), axis=1, keepdims=True) * (1.0 / (HW * 128))
            rstd = lax.rsqrt(var + EPS)
            p_ref[q, 0, :, cs] = mu - e
            p_ref[q, 1, :, cs] = gb_ref[cv, 0, :, cs] * (rstd * 0.5)
            p_ref[q, 2, :, cs] = gb_ref[cv, 1, :, cs] * 0.5

    def merge(lists):
        items = []
        for li, l in enumerate(lists):
            for i, it in enumerate(l):
                items.append(((i + 0.5) / len(l), li, it))
        items.sort(key=lambda z: (z[0], z[1]))
        return [it for _, _, it in items]

    def kern(x_hbm, te_hbm, g1_hbm, b1_hbm, w1_hbm, we_hbm, g2_hbm, b2_hbm, w2_hbm, o_hbm,
             s_ref, w_ref, u2_ref, ar_ref, xr_ref, va_ref, vb_ref, ya_ref, yb_ref,
             st_ref, p_ref, gb_ref, e_ref, te_ref, we_ref, gsm_ref, sem_x, sem_w, sem_s, sem_o, *u1_ref):

        def gcols(g):
            return pl.ds(mult(g * 128, 128), 128)

        def x0_copy(c):
            rows = pl.ds(mult(c * TM, TM), TM)
            return pltpu.make_async_copy(x_hbm.at[0, rows, :], s_ref.at[0, rows, :], sem_x.at[c])

        def w1_copy(g):
            return pltpu.make_async_copy(w1_hbm.at[:, gcols(g), :], w_ref.at[pl.ds(0, 9), gcols(g), :], sem_w.at[g])

        def x1_copy():
            return pltpu.make_async_copy(x_hbm.at[1], s_ref.at[1], sem_s.at[6])

        def w2_copy():
            return pltpu.make_async_copy(w2_hbm, w_ref.at[pl.ds(9, 9)], sem_s.at[7])

        def small_copies():
            return [pltpu.make_async_copy(g1_hbm, gsm_ref.at[0], sem_s.at[0]),
                    pltpu.make_async_copy(b1_hbm, gsm_ref.at[1], sem_s.at[1]),
                    pltpu.make_async_copy(g2_hbm, gsm_ref.at[2], sem_s.at[2]),
                    pltpu.make_async_copy(b2_hbm, gsm_ref.at[3], sem_s.at[3]),
                    pltpu.make_async_copy(te_hbm, te_ref, sem_s.at[4])]

        def we_copy():
            return pltpu.make_async_copy(we_hbm, we_ref, sem_s.at[5])

        def o_copy(s, qi):
            b = divT(s) - 2
            r0 = mult(modT(s) * TM + qi * QR, QR)
            return pltpu.make_async_copy(s_ref.at[b, pl.ds(r0, QR), :], o_hbm.at[b, pl.ds(r0, QR), :], sem_o.at[0])

        def o_all():
            return pltpu.make_async_copy(s_ref.at[pl.ds(0, B)], o_hbm, sem_o.at[0])

        def epi_piece(y_ref, s_prev, kind, r, cb, state, marker, PW=PW):
            p = divT(s_prev)
            t = modT(s_prev)
            cs = lanes(cb, PW)
            j, par = r // 2, r % 2
            r0 = mult(t * TM + r * W, W)
            ve = load_y(y_ref, par, 0, j, cb * (PW // 128), PW // 128)
            vo = load_y(y_ref, par, 1, j, cb * (PW // 128), PW // 128)
            if marker is not None:
                ve = (ve.reshape(HP // 8, 8, PW) + marker[None]).reshape(HP, PW)
            if kind == 1:
                dst, sq = p + 2, p + 2
            elif kind == 2:
                dst, sq = p - 2, None
                xe, xo = split_eo(s_ref[dst, pl.ds(r0, W), cs])
                ve, vo = ve + xe, vo + xo
            else:
                is2 = p >= 2
                dst = jnp.where(is2, p - 2, p + 2)
                sq = jnp.where(is2, 0, p + 2)
                xe, xo = split_eo(s_ref[dst, pl.ds(r0, W), cs])
                ve, vo = ve + jnp.where(is2, xe, 0.0), vo + jnp.where(is2, xo, 0.0)
            if sq is not None:
                state = stat_acc(vo, stat_acc(ve, state))
            s_ref[dst, pl.ds(r0, W), cs] = join_eo(ve, vo)
            if sq is not None and r == TR - 1:
                store_stats(st_ref, sq, t, cs, state)
                state = None
            return state

        def xstat_piece(q, tile, cs, ri, state, marker):
            r0 = mult(tile * TM + ri * XR1, XR1)
            v = s_ref[q, pl.ds(r0, XR1), cs].astype(f32)
            state = stat_acc(v, state, marker)
            if ri == TM // XR1 - 1:
                store_stats(st_ref, q, tile, cs, state)
                state = None
            return state

        def half(it, second, u_ref, vc_ref, vn_ref, yc_ref, yp_ref):
            s = 2 * it + second
            sn = s + 1
            pn = jnp.minimum(divT(sn), 3)
            y0 = modT(sn) * TR
            plist = [pc for cb in range(G) for pc in prod_list(cb)]
            lists = [plist,
                     [('e', r, cb) for r in range(TR) for cb in range(NPW)]]
            NU = -(-NUB // 5)
            if UMODE == 0:
                lists.append([('u', k) for k in range(NU)])
            pieces = merge(lists)
            npc = len(pieces)
            if second == 1:
                finalize(st_ref, p_ref, gb_ref, e_ref, jnp.minimum(divT(s - 1) + 1, 3))
            pv = tuple(p_ref[pn, k] for k in range(3))
            sp = s - 1
            ekind = 0
            done = 0
            est = [None] * NPW
            xst = None
            pcar = None
            ys = [None] * 8
            for a in range(4):
                st = {}
                for b in range(NB):
                    k = NB * a + b
                    d = lax.dot_general(pltpu.bitcast(vc_ref[k], bf16), pltpu.bitcast(u_ref[k][...], bf16), NT,
                                        preferred_element_type=f32)
                    for nn in range(4 * SUB):
                        n, sub = nn // SUB, nn % SUB
                        hi_ = min(npc, (((k * 4 * SUB + nn) + 1) * npc * 64) // (last_slot * NPT * 4 * SUB))
                        while done < hi_:
                            pc = pieces[done]
                            if pc[0] == 'a':
                                cs = slice(pc[1] * 128, (pc[1] + 1) * 128)
                                prod_a(s_ref, tuple(t[:, cs] for t in pv), ar_ref, xr_ref, pn, y0, pc[1], pc[2],
                                       marker_of(d, n, sub, 128))
                            elif pc[0] == 'b':
                                prod_b(xr_ref, vn_ref, pc[1], pc[2], pc[3], marker_of(d, n, sub, 128))
                            elif pc[0] == 'e':
                                est[pc[2]] = epi_piece(yp_ref, sp, ekind, pc[1], pc[2], est[pc[2]],
                                                       marker_of(d, n, sub, PW))
                                if pc[2] == NPW - 1 and ((pc[1] + 1) * W) % QR == 0:
                                    qi = ((pc[1] + 1) * W) // QR - 1

                                    @pl.when(sp >= 2 * T)
                                    def _():
                                        o_copy(sp, qi).start()
                            elif pc[0] == 'x':
                                xst = xstat_piece(jnp.where(it == 0, 0, 1), pc[1],
                                                  slice(pc[2] * PW, (pc[2] + 1) * PW), pc[3], xst,
                                                  marker_of(d, n, sub, PW))
                            else:
                                kk = (s - 2) * NU + pc[1]
                                ok = jnp.logical_and(kk >= 0, kk < NUB)
                                u_piece(w_ref, u2_ref, 9, jnp.clip(kk, 0, NUB - 1),
                                        marker_of(d, n, sub, 128), ok)
                            done += 1
                    rr = out_x(st, b, d)

                def store(par, q, val):
                    for n in range(G):
                        store_y(yc_ref, par, q, n, val[:, n * 128:(n + 1) * 128])
                out_y(ys, a, rr, store)

        def nhalf(step, n, vc_ref, vn_ref, yc_ref, yp_ref):
            y0 = (step + 1) * TR
            plist = prod_list(0)
            lists = [plist]
            if step == 0:
                lists.append([('u', k) for k in range(NUB // G)])
            else:
                lists.append([('e', r) for r in range(TR)])
                lists.append([('x', cb, ri) for cb in range(NPW) for ri in range(TM // XR1)])
            pieces = merge(lists)
            npc = len(pieces)
            cs = lanes(n)
            pvc = tuple(p_ref[0, k, :, cs] for k in range(3))
            urows = pl.ds(pl.multiple_of(n * (128 // 2), 128 // 2), 128 // 2)
            gn = jnp.minimum(n + 1, G - 1)
            NS = NSUB
            done = 0
            est = xst = None
            ys = [None] * 8
            dprev = None
            for a in range(4):
                st = {}
                for b in range(NB):
                    k = NB * a + b
                    d = lax.dot_general(pltpu.bitcast(vc_ref[k], bf16), pltpu.bitcast(u1_ref[k][urows, :], bf16), NT,
                                        preferred_element_type=f32)
                    for sub in range(NS):
                        hi_ = npc if k == NPT - 1 and sub == NS - 1 else ((k * NS + sub) * npc) // ((NPT - 1) * NS)
                        while done < min(hi_, npc) and dprev is not None:
                            pc = pieces[done]
                            rp = sub * (M // NS) // 8 * 8
                            bits = pltpu.bitcast(dprev[rp:rp + 8, :], u32)
                            mk = pltpu.bitcast((bits >> 16) >> 16, f32)
                            if pc[0] == 'a':
                                prod_a(s_ref, pvc, ar_ref, xr_ref, 0, y0, n, pc[2], mk)
                            elif pc[0] == 'b':
                                prod_b(xr_ref, vn_ref, n, pc[2], pc[3], mk)
                            elif pc[0] == 'u':
                                u_piece(w_ref, u1_ref, 0, gn * (NUB // G) + pc[1], mk)
                            elif pc[0] == 'e':
                                est = epi_piece(yp_ref, 0, 1, pc[1], n, est, mk, PW=128)
                            else:
                                mkx = mk if PW == 128 else jnp.concatenate([mk] * (PW // 128), axis=1)
                                xst = xstat_piece(1, n, slice(pc[1] * PW, (pc[1] + 1) * PW), pc[2], xst, mkx)
                            done += 1
                    dprev = d
                    rr = out_x(st, b, d)
                out_y(ys, a, rr, lambda par, q, val: store_y(yc_ref, par, q, n, val))
            assert done == npc

        def xstat_tile(q, c):
            for cb in range(NPW):
                def rows(ri, st):
                    r0 = pl.multiple_of(c * TM + ri * XR, XR)
                    v = s_ref[q, pl.ds(r0, XR), cb * PW:(cb + 1) * PW].astype(f32)
                    return stat_acc(v, st)
                v0 = s_ref[q, pl.ds(pl.multiple_of(c * TM, XR), XR), cb * PW:(cb + 1) * PW].astype(f32)
                st = lax.fori_loop(1, NXR, rows, stat_acc(v0, None))
                store_stats(st_ref, q, c, slice(cb * PW, (cb + 1) * PW), st)
            return 0

        with scope('prologue'):
            for c in small_copies():
                c.start()
            lax.fori_loop(0, T, lambda c, _: (x0_copy(c).start(), 0)[1], 0)
            lax.fori_loop(0, G, lambda g, _: (w1_copy(g).start(), 0)[1], 0)

            def rest(c, _):
                @pl.when(c == 0)
                def _():
                    x1_copy().start()

                @pl.when(c == 1)
                def _():
                    w2_copy().start()

                @pl.when(c == 2)
                def _():
                    we_copy().start()
                return 0
            lax.fori_loop(0, 3, rest, 0)

            for c in small_copies():
                c.wait()
            for cv in range(2):
                for k in range(2):
                    v = gsm_ref[2 * cv + k].astype(f32)
                    for g in range(G):
                        gb_ref[cv, k, :, g * 128:(g + 1) * 128] = jnp.broadcast_to(v[g:g + 1, :], (8, 128))
            e_ref[...] = jnp.zeros(e_ref.shape, f32)
            st_ref[...] = jnp.zeros(st_ref.shape, f32)
            ar_ref[...] = jnp.zeros(ar_ref.shape, f32)

            def xs0(c, _):
                x0_copy(c).wait()
                return xstat_tile(0, c)
            lax.fori_loop(0, T, xs0, 0)
            finalize(st_ref, p_ref, gb_ref, e_ref, 0)

            def prod0(cb, _):
                pvc = tuple(p_ref[0, k, :, gcols(cb)] for k in range(3))
                for pc in prod_list(cb):
                    if pc[0] == 'a':
                        prod_a(s_ref, pvc, ar_ref, xr_ref, 0, 0, cb, pc[2], None)
                    else:
                        prod_b(xr_ref, va_ref, cb, pc[2], pc[3], None)
                return 0
            lax.fori_loop(0, G, prod0, 0)

            w1_copy(0).wait()
            lax.fori_loop(0, NUB // G, lambda k, _: (u_piece(w_ref, u1_ref, 0, k, None), 0)[1], 0)

        def step0(n, _):
            @pl.when(n < G - 1)
            def _():
                w1_copy(n + 1).wait()
            nhalf(0, n, va_ref, vb_ref, ya_ref, yb_ref)
            return 0

        def step1(n, _):
            nhalf(1, n, vb_ref, va_ref, yb_ref, ya_ref)
            return 0

        with scope('step0'):
            lax.fori_loop(0, G, step0, 0)
        with scope('step1'):
            x1_copy().wait()
            lax.fori_loop(0, G, step1, 0)

        def body(it, carry):
            @pl.when(it == 1)
            def _():
                w2_copy().wait()
                we_copy().wait()
                te = te_ref[...].astype(f32)
                sl = te * jax.nn.sigmoid(te)
                emb = jnp.dot(sl.astype(bf16), we_ref[...], preferred_element_type=f32)
                e_ref[2] = jnp.broadcast_to(emb[0:1, :], (8, C))
                e_ref[3] = jnp.broadcast_to(emb[1:2, :], (8, C))

            @pl.when(it == T)
            def _():
                if UMODE == 0:
                    def cp(rb, _):
                        rows = pl.ds(pl.multiple_of(rb * 32, 32), 32)
                        for k in range(NPT):
                            u1_ref[k][rows, :] = u2_ref[k, rows, :]
                        return 0
                    lax.fori_loop(0, C // 2 // 32, cp, 0)
                else:
                    lax.fori_loop(0, NUB, lambda k, _: (u_piece(w_ref, u1_ref, 9, k, None), 0)[1], 0)
            with scope('iter'):
                half(it, 0, u1_ref, va_ref, vb_ref, ya_ref, yb_ref)
                half(it, 1, u1_ref, vb_ref, va_ref, yb_ref, ya_ref)
            return carry

        with scope('main'):
            lax.fori_loop(1, 2 * T, body, 0)

        sl_ = NSTEP - 1
        with scope('final'):
            st = [None] * NPW
            for r in range(TR):
                for cb in range(NPW):
                    st[cb] = epi_piece(yb_ref, sl_, 2, r, cb, st[cb], None)
                if ((r + 1) * W) % QR == 0:
                    o_copy(sl_, ((r + 1) * W) // QR - 1).start()
        with scope('owait'):
            o_all().wait()

    def fn(x, t_emb, g1, be1, w1, w_emb, g2, be2, w2):
        xn = jnp.transpose(x, (0, 2, 3, 1)).reshape(B, HW, C)
        w1t = jnp.transpose(w1, (2, 3, 0, 1)).reshape(9, C, C)
        w2t = jnp.transpose(w2, (2, 3, 0, 1)).reshape(9, C, C)
        any_spec = pl.BlockSpec(memory_space=pl.ANY)
        ubuf = pltpu.VMEM((C // 2, C), u32)
        vbuf = pltpu.VMEM((NPT, M // 2, C), u32)
        ybuf = pltpu.VMEM((2, 2, G, 2 * M, 128), f32)
        out = pl.pallas_call(
            kern,
            in_specs=[any_spec] * 9,
            out_specs=any_spec,
            out_shape=jax.ShapeDtypeStruct((B, HW, C), bf16),
            scratch_shapes=[
                pltpu.VMEM((4, HW, C), bf16),
                pltpu.VMEM((18, C, C), bf16),
                pltpu.VMEM((NPT, (C // 2 + UB // 2) if UMODE == 0 else 8, C), u32),
                pltpu.VMEM((G, NAR, 2, HP + 16, 128), f32),
                pltpu.VMEM((G, TR + 2, NB, NQ4, 128), f32),
                vbuf, vbuf, ybuf, ybuf,
                pltpu.VMEM((4, T, 3, 8, C), f32),
                pltpu.VMEM((4, 3, 8, C), f32),
                pltpu.VMEM((2, 2, 8, C), f32),
                pltpu.VMEM((4, 8, C), f32),
                pltpu.VMEM((B, E), bf16),
                pltpu.VMEM((E, C), bf16),
                pltpu.VMEM((4, G, 128), bf16),
                pltpu.SemaphoreType.DMA((T,)),
                pltpu.SemaphoreType.DMA((G,)),
                pltpu.SemaphoreType.DMA((8,)),
                pltpu.SemaphoreType.DMA((1,)),
            ] + [ubuf] * NPT,
            compiler_params=pltpu.CompilerParams(vmem_limit_bytes=100 * 1024 * 1024,
                                                 disable_bounds_checks=True),
        )(xn, t_emb, g1.reshape(G, 128), be1.reshape(G, 128), w1t, w_emb,
          g2.reshape(G, 128), be2.reshape(G, 128), w2t)
        return jnp.transpose(out.reshape(B, H, W, C), (0, 3, 1, 2))
    return fn


_OPTS = {'nsub': 8}


@jax.jit
def pallas_standalone__adm_resblock__diffusion_kernel(x, t_emb, g1, be1, w1, w_emb, g2, be2, w2):
    B, C, H, W = x.shape
    E = t_emb.shape[1]
    return build(B, C, H, W, E, TM=1024, opts=_OPTS)(x, t_emb, g1, be1, w1, w_emb, g2, be2, w2)
```

```python
import jax
import jax.numpy as jnp
from jax import lax
from jax.experimental import pallas as pl
from jax.experimental.pallas import tpu as pltpu

f32 = jnp.float32
bf16 = jnp.bfloat16
u32 = jnp.uint32
NT = (((1,), (1,)), ((), ()))


def build(B, C, H, W, E, TM=1024, opts=None):
    opts = opts or {}
    HW = H * W
    G = 4
    CG = C // G
    EPS = 1e-5
    T = HW // TM
    assert CG == 128 and B == 2 and T == 4 and W == 64 and H == 64
    TR = TM // W
    NP = TR // 2
    HP = W // 2
    NQ4 = W // 4
    M = NP * NQ4
    NB = 6
    NPT = 4 * NB
    NSTEP = 4 * T
    scope = jax.named_scope

    PW = opts.get('pw', 256)
    NPW = C // PW
    SUB = opts.get('sub', 4)
    XR = opts.get('xr', 256)
    NXR = TM // XR
    last_slot = opts.get('last_slot', 61)
    NQ = opts.get('nq', 4)
    QR = TM // NQ
    UMODE = opts.get('umode', 0)
    XMODE = opts.get('xmode', 0)
    NAR = opts.get('nar', 2)
    SPLIT = opts.get('split', 2)
    PEEL0 = opts.get('peel0', 1)
    WH, W4, W5A, W5B = (opts.get(k_, v_) for k_, v_ in (('wh', 130), ('w4', 40), ('w5a', 80), ('w5b', 30)))
    BG = opts.get('bg', 3)
    NSUB = opts.get('nsub', 8)
    XR1 = opts.get('xr1', 32)
    UB = 16
    NUB = (C // UB) * G

    def mult(v, m):
        return v if isinstance(v, int) else pl.multiple_of(v, m)

    def divT(v):
        return v // T if isinstance(v, int) else lax.shift_right_logical(v, 2)

    def modT(v):
        return v % T if isinstance(v, int) else jnp.bitwise_and(v, T - 1)

    def marker_of(d, n, sub, width):
        rp = sub * (d.shape[0] // SUB) // 8 * 8
        m = d[rp:rp + 8, n * 128:(n + 1) * 128]
        b = pltpu.bitcast(m, u32)
        z = pltpu.bitcast((b >> 16) >> 16, f32)
        if width > 128:
            z = jnp.concatenate([z] * (width // 128), axis=1)
        return z

    def pack2(t):
        n = t.shape[0] // 2
        return pltpu.pack_elementwise([t[:n], t[n:]], packed_dtype=bf16)

    def lanes(cb, width=128):
        if isinstance(cb, int):
            return slice(cb * width, (cb + 1) * width)
        return pl.ds(pl.multiple_of(cb * width, width), width)

    def load_y(y_ref, par, eo, j, cb0, ncb):
        parts = [y_ref[par, eo, cb0 + i, j * HP:(j + 1) * HP, :] for i in range(ncb)]
        return parts[0] if ncb == 1 else jnp.concatenate(parts, axis=1)

    def store_y(y_ref, par, q, n, val):
        if opts.get('nost'):
            y_ref[par, q % 2, n, pl.ds((q // 2) * M, M), :] = val
        else:
            y_ref[par, q % 2, n, pl.ds(q // 2, M, stride=2), :] = val

    def split_eo(v):
        w = pltpu.bitcast(v, u32)
        return (pltpu.unpack_elementwise(w, index=0, packed_dtype=bf16, unpacked_dtype=f32),
                pltpu.unpack_elementwise(w, index=1, packed_dtype=bf16, unpacked_dtype=f32))

    def join_eo(e, o):
        return pltpu.bitcast(pltpu.pack_elementwise([e, o], packed_dtype=bf16), bf16)

    def act(v, pv, marker):
        n, wd = v.shape
        mu, sc, bt = pv
        if marker is not None:
            mu = mu + marker
        v3 = v.reshape(n // 8, 8, wd)
        hz = ((v3 - mu[None]) * sc[None] + bt[None]).reshape(n, wd)
        return hz * jnp.tanh(hz) + hz

    def act_row(s_ref, pv, q, y, cs, marker, edge):
        yc = y if not edge else jnp.clip(y, 0, H - 1)
        e, o = split_eo(s_ref[q, pl.ds(mult(yc * W, W), W), cs])
        e = act(e, pv, marker)
        o = act(o, pv, marker)
        if edge:
            valid = jnp.logical_and(y >= 0, y < H)
            e = jnp.where(valid, e, 0.0)
            o = jnp.where(valid, o, 0.0)
        return e, o

    def prod_a(s_ref, pv, ar_ref, xr_ref, q, y0, cb, i, marker):
        cs = lanes(cb)
        cb = cb if isinstance(cb, int) else 0
        e, o = act_row(s_ref, pv, q, y0 - 1 + i, cs, marker, i == 0 or i == TR + 1)
        sl = i % NAR
        ar_ref[cb, sl, 0, 8:8 + HP, :] = e
        ar_ref[cb, sl, 1, 8:8 + HP, :] = o

        def col(eo, r):
            if opts.get('nold'):
                return ar_ref[cb, sl, eo, pl.ds((r % 3) * 16, 16), :]
            return jnp.concatenate([ar_ref[cb, sl, eo, pl.ds(r + 2 * u, NQ4 // 2, stride=4), :] for u in range(2)], axis=0)
        d0, d1, d2, d3, d4, d5 = col(1, 7), col(0, 8), col(1, 8), col(0, 9), col(1, 9), col(0, 10)
        c = d4 - d2
        e2 = (d3 - d1) * 2.0
        a_ = d4 - d2 * 4.0
        b_ = d3 - d1 * 4.0
        xr_ref[cb, i, 0] = (d0 - d2) * 4.0 + c
        xr_ref[cb, i, 1] = a_ + b_
        xr_ref[cb, i, 2] = a_ - b_
        xr_ref[cb, i, 3] = c + e2
        xr_ref[cb, i, 4] = c - e2
        xr_ref[cb, i, 5] = (d5 - d3) - e2 * 2.0

    def prod_b(xr_ref, v_ref, cb, j, bs, marker):
        cs = lanes(cb)
        cb = cb if isinstance(cb, int) else 0
        rs = pl.ds(j * (NQ4 // 2), NQ4 // 2)
        for b in bs:
            r0, r1, r2, r3 = (xr_ref[cb, 2 * j + i, b] for i in range(4))
            if marker is not None:
                r2 = (r2.reshape(NQ4 // 8, 8, 128) + marker[None]).reshape(NQ4, 128)
            v_ref[b, rs, cs] = pack2(r0 - r2)
            v_ref[NB + b, rs, cs] = pack2(r1 + r2)
            v_ref[2 * NB + b, rs, cs] = pack2(r2 - r1)
            v_ref[3 * NB + b, rs, cs] = pack2(r1 - r3)

    def prod_list(cb):
        pl_ = [('a', cb, 0), ('a', cb, 1)]
        for j in range(NP):
            pl_ += [('a', cb, 2 * j + 2), ('a', cb, 2 * j + 3)]
            pl_ += [('b', cb, j, tuple(range(b, b + BG))) for b in range(0, NB, BG)]
        return pl_

    def out_x(st, b, d):
        if b == 0:
            st['r0'] = d
        elif b in (1, 3):
            st['p'] = d
        elif b == 2:
            st['s12'], st['d12'] = st['p'] + d, st['p'] - d
            st['r0'] = st['r0'] + st['s12']
        elif b == 4:
            s34, d34 = st['p'] + d, st['p'] - d
            st['r0'] = st['r0'] + s34
            st['r1'] = st['d12'] + d34 * 2.0
            st['r2'] = st['s12'] + s34 * 4.0
            st['r3'] = st['d12'] + d34 * 8.0
        else:
            return [st['r0'], st['r1'], st['r2'], st['r3'] + d]
        return None

    def out_y(ys, a, rr, store):
        for q in range(4):
            if a == 0:
                ys[q] = rr[q]
            elif a == 1:
                ys[q] = ys[q] + rr[q]
                ys[4 + q] = rr[q]
            elif a == 2:
                store(0, q, ys[q] + rr[q])
                ys[4 + q] = ys[4 + q] - rr[q]
            else:
                store(1, q, ys[4 + q] - rr[q])

    def u_piece(w_ref, u_ref, base, k, marker, ok=None):
        rb = lax.shift_right_logical(k, 2) if not isinstance(k, int) else k // 4
        cb = jnp.bitwise_and(k, 3) if not isinstance(k, int) else k % 4
        rows = pl.ds(mult(rb * UB, UB), UB)
        ob = rb if ok is None else jnp.where(ok, rb, C // UB)
        orow = pl.ds(mult(ob * (UB // 2), UB // 2), UB // 2)
        cs = pl.ds(mult(cb * 128, 128), 128)
        res = []
        raw = [[split_eo(w_ref[base + 3 * i + j, rows, cs]) for j in range(3)] for i in range(3)]
        for par in range(2):
            hs = []
            for j in range(3):
                g0, g1, g2 = (raw[i][j][par] for i in range(3))
                if marker is not None:
                    g1 = g1 + marker
                sm = g0 + g2
                hs.append((g0, (sm + g1) * 0.5, (sm - g1) * 0.5, g2))
            out = [None] * NPT
            for a in range(4):
                h0, h1, h2 = (hs[j][a] for j in range(3))
                sm = h0 + h2
                pp = h0 * (1.0 / 24.0) + h2 * (1.0 / 6.0)
                qq = h1 * (1.0 / 12.0)
                for b, val in enumerate((h0 * 0.25, (sm + h1) * (-1.0 / 6.0), (sm - h1) * (-1.0 / 6.0),
                                         pp + qq, pp - qq, h2)):
                    out[NB * a + b] = val
            res.append(out)
        for k2 in range(NPT):
            val = pltpu.pack_elementwise([res[0][k2], res[1][k2]], packed_dtype=bf16)
            if isinstance(u_ref, (list, tuple)):
                u_ref[k2][orow, cs] = val
            else:
                u_ref[k2, orow, cs] = val

    def stat_acc(v, state, marker=None):
        n = v.shape[0] // 8
        wd = v.shape[1]
        if state is None:
            K = v[0:1, :]
            if marker is not None:
                K = K + marker[0:1, :]
            d = v - K
            return (K, d.reshape(n, 8, wd).sum(axis=0), (d * d).reshape(n, 8, wd).sum(axis=0))
        K, s1, s2 = state
        Kd = K if marker is None else K + marker[0:1, :]
        d = v - Kd
        return (K, s1 + d.reshape(n, 8, wd).sum(axis=0), s2 + (d * d).reshape(n, 8, wd).sum(axis=0))

    def store_stats(st_ref, q, t, cs, state):
        K, s1, s2 = state
        wd = K.shape[1]
        st_ref[q, t, 0, :, cs] = jnp.broadcast_to(K, (8, wd))
        st_ref[q, t, 1, :, cs] = jnp.broadcast_to(s1.sum(axis=0, keepdims=True), (8, wd))
        st_ref[q, t, 2, :, cs] = jnp.broadcast_to(s2.sum(axis=0, keepdims=True), (8, wd))

    def finalize(st_ref, p_ref, gb_ref, e_ref, q):
        cv = q // 2 if isinstance(q, int) else lax.shift_right_logical(q, 1)
        for g in range(G):
            cs = slice(g * 128, (g + 1) * 128)
            K = st_ref[q, :, 0, :, cs]
            s1 = st_ref[q, :, 1, :, cs]
            s2 = st_ref[q, :, 2, :, cs]
            e = e_ref[q, :, cs]
            mean_t = K + s1 * (1.0 / TM) + e[None]
            m2_t = s2 - s1 * s1 * (1.0 / TM)
            mu = jnp.sum(jnp.sum(mean_t, axis=0), axis=1, keepdims=True) * (1.0 / (T * 128))
            dev = mean_t - mu[None]
            tot = m2_t + dev * dev * float(TM)
            var = jnp.sum(jnp.sum(tot, axis=0), axis=1, keepdims=True) * (1.0 / (HW * 128))
            rstd = lax.rsqrt(var + EPS)
            p_ref[q, 0, :, cs] = mu - e
            p_ref[q, 1, :, cs] = gb_ref[cv, 0, :, cs] * (rstd * 0.5)
            p_ref[q, 2, :, cs] = gb_ref[cv, 1, :, cs] * 0.5

    def merge(lists):
        items = []
        for li, l in enumerate(lists):
            for i, it in enumerate(l):
                items.append(((i + 0.5) / len(l), li, it))
        items.sort(key=lambda z: (z[0], z[1]))
        return [it for _, _, it in items]

    def kern(x_hbm, te_hbm, g1_hbm, b1_hbm, w1_hbm, we_hbm, g2_hbm, b2_hbm, w2_hbm, o_hbm,
             s_ref, w_ref, u2_ref, ar_ref, xr_ref, va_ref, vb_ref, ya_ref, yb_ref,
             st_ref, p_ref, gb_ref, e_ref, te_ref, we_ref, gsm_ref, sem_x, sem_w, sem_s, sem_o, *u1_ref):

        def gcols(g):
            return pl.ds(mult(g * 128, 128), 128)

        def x0_copy(c):
            rows = pl.ds(mult(c * TM, TM), TM)
            return pltpu.make_async_copy(x_hbm.at[0, rows, :], s_ref.at[0, rows, :], sem_x.at[c])

        def w1_copy(g):
            return pltpu.make_async_copy(w1_hbm.at[:, gcols(g), :], w_ref.at[pl.ds(0, 9), gcols(g), :], sem_w.at[g])

        def x1_copy():
            return pltpu.make_async_copy(x_hbm.at[1], s_ref.at[1], sem_s.at[6])

        def w2_copy():
            return pltpu.make_async_copy(w2_hbm, w_ref.at[pl.ds(9, 9)], sem_s.at[7])

        def small_copies():
            return [pltpu.make_async_copy(g1_hbm, gsm_ref.at[0], sem_s.at[0]),
                    pltpu.make_async_copy(b1_hbm, gsm_ref.at[1], sem_s.at[1]),
                    pltpu.make_async_copy(g2_hbm, gsm_ref.at[2], sem_s.at[2]),
                    pltpu.make_async_copy(b2_hbm, gsm_ref.at[3], sem_s.at[3]),
                    pltpu.make_async_copy(te_hbm, te_ref, sem_s.at[4])]

        def we_copy():
            return pltpu.make_async_copy(we_hbm, we_ref, sem_s.at[5])

        def o_copy(s, qi):
            b = divT(s) - 2
            r0 = mult(modT(s) * TM + qi * QR, QR)
            return pltpu.make_async_copy(s_ref.at[b, pl.ds(r0, QR), :], o_hbm.at[b, pl.ds(r0, QR), :], sem_o.at[0])

        def o_all():
            return pltpu.make_async_copy(s_ref.at[pl.ds(0, B)], o_hbm, sem_o.at[0])

        def epi_piece(y_ref, s_prev, kind, r, cb, state, marker, PW=PW):
            p = divT(s_prev)
            t = modT(s_prev)
            cs = lanes(cb, PW)
            j, par = r // 2, r % 2
            r0 = mult(t * TM + r * W, W)
            ve = load_y(y_ref, par, 0, j, cb * (PW // 128), PW // 128)
            vo = load_y(y_ref, par, 1, j, cb * (PW // 128), PW // 128)
            if marker is not None:
                ve = (ve.reshape(HP // 8, 8, PW) + marker[None]).reshape(HP, PW)
            if kind == 1:
                dst, sq = p + 2, p + 2
            elif kind == 2:
                dst, sq = p - 2, None
                xe, xo = split_eo(s_ref[dst, pl.ds(r0, W), cs])
                ve, vo = ve + xe, vo + xo
            else:
                is2 = p >= 2
                dst = jnp.where(is2, p - 2, p + 2)
                sq = jnp.where(is2, 0, p + 2)
                xe, xo = split_eo(s_ref[dst, pl.ds(r0, W), cs])
                ve, vo = ve + jnp.where(is2, xe, 0.0), vo + jnp.where(is2, xo, 0.0)
            if sq is not None:
                state = stat_acc(vo, stat_acc(ve, state))
            s_ref[dst, pl.ds(r0, W), cs] = join_eo(ve, vo)
            if sq is not None and r == TR - 1:
                store_stats(st_ref, sq, t, cs, state)
                state = None
            return state

        def xstat_piece(q, tile, cs, ri, state, marker):
            r0 = mult(tile * TM + ri * XR1, XR1)
            v = s_ref[q, pl.ds(r0, XR1), cs].astype(f32)
            state = stat_acc(v, state, marker)
            if ri == TM // XR1 - 1:
                store_stats(st_ref, q, tile, cs, state)
                state = None
            return state

        def half(it, second, u_ref, vc_ref, vn_ref, yc_ref, yp_ref, conv=None):
            s = 2 * it + second
            sn = s + 1
            pn = jnp.minimum(divT(sn), 3)
            y0 = modT(sn) * TR
            plist = [pc for cb in range(G) for pc in prod_list(cb)]
            lists = [plist,
                     [('e', r, cb) for r in range(TR) for cb in range(NPW)]]
            NU = -(-NUB // (5 if conv is None else 6))
            if UMODE == 0 and conv != 1:
                lists.append([('u', k) for k in range(NU)])
            pieces = merge(lists)
            npc = len(pieces)
            if second == 1:
                finalize(st_ref, p_ref, gb_ref, e_ref, jnp.minimum(divT(s - 1) + 1, 3))
            pv = tuple(p_ref[pn, k] for k in range(3))
            sp = s - 1
            ekind = 0 if conv is None else (1 if conv in (0, 2) else (0 if second == 0 else 2))
            wts = [{0: WH, 1: WH, 2: 100, 3: WH, 4: W4, 5: W5A if k // NB < 2 else W5B}[k % NB] for k in range(NPT)]
            cum = [sum(wts[:k]) for k in range(NPT + 1)]
            done = 0
            est = [None] * NPW
            xst = None
            pcar = None
            ys = [None] * 8
            for a in range(4):
                st = {}
                for b in range(NB):
                    k = NB * a + b
                    d = lax.dot_general(pltpu.bitcast(vc_ref[k], bf16), pltpu.bitcast(u_ref[k][...] if conv != 1 else u_ref[k, 0:C // 2, :], bf16), NT,
                                        preferred_element_type=f32)
                    for nn in range(4 * SUB):
                        n, sub = nn // SUB, nn % SUB
                        hi_ = min(npc, ((cum[k] * 4 * SUB + wts[k] * (nn + 1)) * npc * 64) // (last_slot * cum[NPT] * 4 * SUB))
                        while done < hi_:
                            pc = pieces[done]
                            if pc[0] == 'a':
                                cs = slice(pc[1] * 128, (pc[1] + 1) * 128)
                                prod_a(s_ref, tuple(t[:, cs] for t in pv), ar_ref, xr_ref, pn, y0, pc[1], pc[2],
                                       marker_of(d, n, sub, 128))
                            elif pc[0] == 'b':
                                prod_b(xr_ref, vn_ref, pc[1], pc[2], pc[3], marker_of(d, n, sub, 128))
                            elif pc[0] == 'e':
                                est[pc[2]] = epi_piece(yp_ref, sp, ekind, pc[1], pc[2], est[pc[2]],
                                                       marker_of(d, n, sub, PW))
                                if pc[2] == NPW - 1 and ((pc[1] + 1) * W) % QR == 0 and conv not in (0, 2):
                                    qi = ((pc[1] + 1) * W) // QR - 1

                                    @pl.when(sp >= 2 * T)
                                    def _():
                                        o_copy(sp, qi).start()
                            elif pc[0] == 'x':
                                xst = xstat_piece(jnp.where(it == 0, 0, 1), pc[1],
                                                  slice(pc[2] * PW, (pc[2] + 1) * PW), pc[3], xst,
                                                  marker_of(d, n, sub, PW))
                            else:
                                kk = (s - 2) * NU + pc[1]
                                ok = jnp.logical_and(kk >= 0, kk < NUB)
                                u_piece(w_ref, u2_ref, 9, jnp.clip(kk, 0, NUB - 1),
                                        marker_of(d, n, sub, 128), ok)
                            done += 1
                    rr = out_x(st, b, d)

                def store(par, q, val):
                    for n in range(G):
                        store_y(yc_ref, par, q, n, val[:, n * 128:(n + 1) * 128])
                out_y(ys, a, rr, store)

        def nhalf(step, n, vc_ref, vn_ref, yc_ref, yp_ref, with_u=True):
            y0 = (step + 1) * TR
            plist = prod_list(0)
            lists = [plist]
            if step == 0:
                if with_u:
                    lists.append([('u', k) for k in range(NUB // G)])
            else:
                lists.append([('e', r) for r in range(TR)])
                lists.append([('x', cb, ri) for cb in range(NPW) for ri in range(TM // XR1)])
            pieces = merge(lists)
            npc = len(pieces)
            cs = lanes(n)
            pvc = tuple(p_ref[0, k, :, cs] for k in range(3))
            urows = pl.ds(pl.multiple_of(n * (128 // 2), 128 // 2), 128 // 2)
            gn = jnp.minimum(n + 1, G - 1)
            NS = NSUB
            done = 0
            est = xst = None
            ys = [None] * 8
            dprev = None
            for a in range(4):
                st = {}
                for b in range(NB):
                    k = NB * a + b
                    d = lax.dot_general(pltpu.bitcast(vc_ref[k], bf16), pltpu.bitcast(u1_ref[k][urows, :], bf16), NT,
                                        preferred_element_type=f32)
                    for sub in range(NS):
                        hi_ = npc if k == NPT - 1 and sub == NS - 1 else ((k * NS + sub) * npc) // ((NPT - 1) * NS)
                        while done < min(hi_, npc) and dprev is not None:
                            pc = pieces[done]
                            rp = sub * (M // NS) // 8 * 8
                            bits = pltpu.bitcast(dprev[rp:rp + 8, :], u32)
                            mk = pltpu.bitcast((bits >> 16) >> 16, f32)
                            if pc[0] == 'a':
                                prod_a(s_ref, pvc, ar_ref, xr_ref, 0, y0, n, pc[2], mk)
                            elif pc[0] == 'b':
                                prod_b(xr_ref, vn_ref, n, pc[2], pc[3], mk)
                            elif pc[0] == 'u':
                                u_piece(w_ref, u1_ref, 0, gn * (NUB // G) + pc[1], mk)
                            elif pc[0] == 'e':
                                est = epi_piece(yp_ref, 0, 1, pc[1], n, est, mk, PW=128)
                            else:
                                mkx = mk if PW == 128 else jnp.concatenate([mk] * (PW // 128), axis=1)
                                xst = xstat_piece(1, n, slice(pc[1] * PW, (pc[1] + 1) * PW), pc[2], xst, mkx)
                            done += 1
                    dprev = d
                    rr = out_x(st, b, d)
                out_y(ys, a, rr, lambda par, q, val: store_y(yc_ref, par, q, n, val))
            assert done == npc

        def xstat_tile(q, c):
            for cb in range(NPW):
                def rows(ri, st):
                    r0 = pl.multiple_of(c * TM + ri * XR, XR)
                    v = s_ref[q, pl.ds(r0, XR), cb * PW:(cb + 1) * PW].astype(f32)
                    return stat_acc(v, st)
                v0 = s_ref[q, pl.ds(pl.multiple_of(c * TM, XR), XR), cb * PW:(cb + 1) * PW].astype(f32)
                st = lax.fori_loop(1, NXR, rows, stat_acc(v0, None))
                store_stats(st_ref, q, c, slice(cb * PW, (cb + 1) * PW), st)
            return 0

        with scope('prologue'):
            for c in small_copies():
                c.start()
            lax.fori_loop(0, T, lambda c, _: (x0_copy(c).start(), 0)[1], 0)
            lax.fori_loop(0, G, lambda g, _: (w1_copy(g).start(), 0)[1], 0)

            def rest(c, _):
                @pl.when(c == 0)
                def _():
                    x1_copy().start()

                @pl.when(c == 1)
                def _():
                    w2_copy().start()

                @pl.when(c == 2)
                def _():
                    we_copy().start()
                return 0
            lax.fori_loop(0, 3, rest, 0)

            for c in small_copies():
                c.wait()
            for cv in range(2):
                for k in range(2):
                    v = gsm_ref[2 * cv + k].astype(f32)
                    for g in range(G):
                        gb_ref[cv, k, :, g * 128:(g + 1) * 128] = jnp.broadcast_to(v[g:g + 1, :], (8, 128))
            e_ref[...] = jnp.zeros(e_ref.shape, f32)
            st_ref[...] = jnp.zeros(st_ref.shape, f32)
            ar_ref[...] = jnp.zeros(ar_ref.shape, f32)

            def xs0(c, _):
                x0_copy(c).wait()
                return xstat_tile(0, c)
            lax.fori_loop(0, T, xs0, 0)
            finalize(st_ref, p_ref, gb_ref, e_ref, 0)

            def prod0(cb, _):
                pvc = tuple(p_ref[0, k, :, gcols(cb)] for k in range(3))
                for pc in prod_list(cb):
                    if pc[0] == 'a':
                        prod_a(s_ref, pvc, ar_ref, xr_ref, 0, 0, cb, pc[2], None)
                    else:
                        prod_b(xr_ref, va_ref, cb, pc[2], pc[3], None)
                return 0
            lax.fori_loop(0, G, prod0, 0)

            w1_copy(0).wait()
            lax.fori_loop(0, NUB // G, lambda k, _: (u_piece(w_ref, u1_ref, 0, k, None), 0)[1], 0)

        def step0(n, _):
            if PEEL0:
                w1_copy(n + 1).wait()
            else:
                @pl.when(n < G - 1)
                def _():
                    w1_copy(n + 1).wait()
            nhalf(0, n, va_ref, vb_ref, ya_ref, yb_ref)
            return 0

        def step1(n, _):
            nhalf(1, n, vb_ref, va_ref, yb_ref, ya_ref)
            return 0

        with scope('step0'):
            if PEEL0:
                lax.fori_loop(0, G - 1, step0, 0)
                lax.fori_loop(G - 1, G, lambda n, _: (nhalf(0, n, va_ref, vb_ref, ya_ref, yb_ref, False), 0)[1], 0)
            else:
                lax.fori_loop(0, G, step0, 0)
        with scope('step1'):
            x1_copy().wait()
            lax.fori_loop(0, G, step1, 0)

        def emb_block():
            w2_copy().wait()
            we_copy().wait()
            te = te_ref[...].astype(f32)
            sl = te * jax.nn.sigmoid(te)
            emb = jnp.dot(sl.astype(bf16), we_ref[...], preferred_element_type=f32)
            e_ref[2] = jnp.broadcast_to(emb[0:1, :], (8, C))
            e_ref[3] = jnp.broadcast_to(emb[1:2, :], (8, C))

        def body(it, carry):
            @pl.when(it == 1)
            def _():
                emb_block()

            @pl.when(it == T)
            def _():
                if UMODE == 0:
                    def cp(rb, _):
                        rows = pl.ds(pl.multiple_of(rb * 32, 32), 32)
                        for k in range(NPT):
                            u1_ref[k][rows, :] = u2_ref[k, rows, :]
                        return 0
                    lax.fori_loop(0, C // 2 // 32, cp, 0)
                else:
                    lax.fori_loop(0, NUB, lambda k, _: (u_piece(w_ref, u1_ref, 9, k, None), 0)[1], 0)
            with scope('iter'):
                half(it, 0, u1_ref, va_ref, vb_ref, ya_ref, yb_ref)
                half(it, 1, u1_ref, vb_ref, va_ref, yb_ref, ya_ref)
            return carry

        def body_c(conv):
            def f(it, carry):
                if conv == 0:
                    @pl.when(it == 1)
                    def _():
                        emb_block()
                ur = u2_ref if conv == 1 else u1_ref
                with scope('iter'):
                    half(it, 0, ur, va_ref, vb_ref, ya_ref, yb_ref, conv)
                    half(it, 1, ur, vb_ref, va_ref, yb_ref, ya_ref, conv)
                return carry
            return f

        with scope('main'):
            if SPLIT:
                if SPLIT == 2:
                    emb_block()
                lax.fori_loop(1, T, body_c(0 if SPLIT == 1 else 2), 0)
                lax.fori_loop(T, 2 * T, body_c(1), 0)
            else:
                lax.fori_loop(1, 2 * T, body, 0)

        sl_ = NSTEP - 1
        with scope('final'):
            st = [None] * NPW
            for r in range(TR):
                for cb in range(NPW):
                    st[cb] = epi_piece(yb_ref, sl_, 2, r, cb, st[cb], None)
                if ((r + 1) * W) % QR == 0:
                    o_copy(sl_, ((r + 1) * W) // QR - 1).start()
        with scope('owait'):
            o_all().wait()

    def fn(x, t_emb, g1, be1, w1, w_emb, g2, be2, w2):
        xn = jnp.transpose(x, (0, 2, 3, 1)).reshape(B, HW, C)
        w1t = jnp.transpose(w1, (2, 3, 0, 1)).reshape(9, C, C)
        w2t = jnp.transpose(w2, (2, 3, 0, 1)).reshape(9, C, C)
        any_spec = pl.BlockSpec(memory_space=pl.ANY)
        ubuf = pltpu.VMEM((C // 2, C), u32)
        vbuf = pltpu.VMEM((NPT, M // 2, C), u32)
        ybuf = pltpu.VMEM((2, 2, G, 2 * M, 128), f32)
        out = pl.pallas_call(
            kern,
            in_specs=[any_spec] * 9,
            out_specs=any_spec,
            out_shape=jax.ShapeDtypeStruct((B, HW, C), bf16),
            scratch_shapes=[
                pltpu.VMEM((4, HW, C), bf16),
                pltpu.VMEM((18, C, C), bf16),
                pltpu.VMEM((NPT, (C // 2 + UB // 2) if UMODE == 0 else 8, C), u32),
                pltpu.VMEM((G, NAR, 2, HP + 16, 128), f32),
                pltpu.VMEM((G, TR + 2, NB, NQ4, 128), f32),
                vbuf, vbuf, ybuf, ybuf,
                pltpu.VMEM((4, T, 3, 8, C), f32),
                pltpu.VMEM((4, 3, 8, C), f32),
                pltpu.VMEM((2, 2, 8, C), f32),
                pltpu.VMEM((4, 8, C), f32),
                pltpu.VMEM((B, E), bf16),
                pltpu.VMEM((E, C), bf16),
                pltpu.VMEM((4, G, 128), bf16),
                pltpu.SemaphoreType.DMA((T,)),
                pltpu.SemaphoreType.DMA((G,)),
                pltpu.SemaphoreType.DMA((8,)),
                pltpu.SemaphoreType.DMA((1,)),
            ] + [ubuf] * NPT,
            compiler_params=pltpu.CompilerParams(vmem_limit_bytes=100 * 1024 * 1024,
                                                 disable_bounds_checks=True),
        )(xn, t_emb, g1.reshape(G, 128), be1.reshape(G, 128), w1t, w_emb,
          g2.reshape(G, 128), be2.reshape(G, 128), w2t)
        return jnp.transpose(out.reshape(B, H, W, C), (0, 3, 1, 2))
    return fn


_OPTS = {}


@jax.jit
def pallas_standalone__adm_resblock__diffusion_kernel(x, t_emb, g1, be1, w1, w_emb, g2, be2, w2):
    B, C, H, W = x.shape
    E = t_emb.shape[1]
    return build(B, C, H, W, E, TM=1024, opts=_OPTS)(x, t_emb, g1, be1, w1, w_emb, g2, be2, w2)
```

```python
import jax
import jax.numpy as jnp
from jax import lax
from jax.experimental import pallas as pl
from jax.experimental.pallas import tpu as pltpu

f32 = jnp.float32
bf16 = jnp.bfloat16
u32 = jnp.uint32
NT = (((1,), (1,)), ((), ()))


def build(B, C, H, W, E, TM=1024, opts=None):
    opts = opts or {}
    HW = H * W
    G = 4
    CG = C // G
    EPS = 1e-5
    T = HW // TM
    assert CG == 128 and B == 2 and T == 4 and W == 64 and H == 64
    TR = TM // W
    NP = TR // 2
    HP = W // 2
    NQ4 = W // 4
    M = NP * NQ4
    NB = 6
    NPT = 4 * NB
    NSTEP = 4 * T
    scope = jax.named_scope

    PW = opts.get('pw', 256)
    NPW = C // PW
    SUB = opts.get('sub', 8)
    XR = opts.get('xr', 256)
    NXR = TM // XR
    last_slot = opts.get('last_slot', 61)
    NQ = opts.get('nq', 4)
    QR = TM // NQ
    UMODE = opts.get('umode', 0)
    XMODE = opts.get('xmode', 0)
    NAR = opts.get('nar', 2)
    LAG = opts.get('lag', 2)
    P0 = opts.get('p0', 1)
    EMB0 = opts.get('emb0', 1)
    SPLIT = opts.get('split', 2)
    PEEL0 = opts.get('peel0', 1)
    WH, W4, W5A, W5B = (opts.get(k_, v_) for k_, v_ in (('wh', 130), ('w4', 40), ('w5a', 80), ('w5b', 30)))
    BG = opts.get('bg', 3)
    NSUB = opts.get('nsub', 8)
    XR1 = opts.get('xr1', 32)
    UB = 16
    NUB = (C // UB) * G

    def mult(v, m):
        return v if isinstance(v, int) else pl.multiple_of(v, m)

    def divT(v):
        return v // T if isinstance(v, int) else lax.shift_right_logical(v, 2)

    def modT(v):
        return v % T if isinstance(v, int) else jnp.bitwise_and(v, T - 1)

    def marker_of(d, n, sub, width):
        rp = sub * (d.shape[0] // SUB) // 8 * 8
        m = d[rp:rp + 8, n * 128:(n + 1) * 128]
        b = pltpu.bitcast(m, u32)
        z = pltpu.bitcast((b >> 16) >> 16, f32)
        if width > 128:
            z = jnp.concatenate([z] * (width // 128), axis=1)
        return z

    def pack2(t):
        n = t.shape[0] // 2
        return pltpu.pack_elementwise([t[:n], t[n:]], packed_dtype=bf16)

    def lanes(cb, width=128):
        if isinstance(cb, int):
            return slice(cb * width, (cb + 1) * width)
        return pl.ds(pl.multiple_of(cb * width, width), width)

    def load_y(y_ref, par, eo, j, cb0, ncb):
        parts = [y_ref[par, eo, cb0 + i, j * HP:(j + 1) * HP, :] for i in range(ncb)]
        return parts[0] if ncb == 1 else jnp.concatenate(parts, axis=1)

    def store_y(y_ref, par, q, n, val):
        if opts.get('nost'):
            y_ref[par, q % 2, n, pl.ds((q // 2) * M, M), :] = val
        else:
            y_ref[par, q % 2, n, pl.ds(q // 2, M, stride=2), :] = val

    def split_eo(v):
        w = pltpu.bitcast(v, u32)
        return (pltpu.unpack_elementwise(w, index=0, packed_dtype=bf16, unpacked_dtype=f32),
                pltpu.unpack_elementwise(w, index=1, packed_dtype=bf16, unpacked_dtype=f32))

    def join_eo(e, o):
        return pltpu.bitcast(pltpu.pack_elementwise([e, o], packed_dtype=bf16), bf16)

    def act(v, pv, marker):
        n, wd = v.shape
        sc, bt = pv
        if marker is not None:
            bt = bt + marker
        v3 = v.reshape(n // 8, 8, wd)
        hz = (v3 * sc[None] + bt[None]).reshape(n, wd)
        return hz * jnp.tanh(hz) + hz

    def act_row(s_ref, pv, q, y, cs, marker, edge):
        yc = y if not edge else jnp.clip(y, 0, H - 1)
        e, o = split_eo(s_ref[q, pl.ds(mult(yc * W, W), W), cs])
        e = act(e, pv, marker)
        o = act(o, pv, marker)
        if edge:
            valid = jnp.logical_and(y >= 0, y < H)
            e = jnp.where(valid, e, 0.0)
            o = jnp.where(valid, o, 0.0)
        return e, o

    def prod_a(s_ref, pv, ar_ref, xr_ref, q, y0, cb, i, marker, slot=0):
        cs = lanes(cb)
        cb = cb if isinstance(cb, int) else slot
        e, o = act_row(s_ref, pv, q, y0 - 1 + i, cs, marker, i == 0 or i == TR + 1)
        sl = i % NAR
        ar_ref[cb, sl, 0, 8:8 + HP, :] = e
        ar_ref[cb, sl, 1, 8:8 + HP, :] = o

        def col(eo, r):
            if opts.get('nold'):
                return ar_ref[cb, sl, eo, pl.ds((r % 3) * 16, 16), :]
            return jnp.concatenate([ar_ref[cb, sl, eo, pl.ds(r + 2 * u, NQ4 // 2, stride=4), :] for u in range(2)], axis=0)
        d0, d1, d2, d3, d4, d5 = col(1, 7), col(0, 8), col(1, 8), col(0, 9), col(1, 9), col(0, 10)
        c = d4 - d2
        e2 = (d3 - d1) * 2.0
        a_ = d4 - d2 * 4.0
        b_ = d3 - d1 * 4.0
        xr_ref[cb, i, 0] = (d0 - d2) * 4.0 + c
        xr_ref[cb, i, 1] = a_ + b_
        xr_ref[cb, i, 2] = a_ - b_
        xr_ref[cb, i, 3] = c + e2
        xr_ref[cb, i, 4] = c - e2
        xr_ref[cb, i, 5] = (d5 - d3) - e2 * 2.0

    def prod_b(xr_ref, v_ref, cb, j, bs, marker, slot=0):
        cs = lanes(cb)
        cb = cb if isinstance(cb, int) else slot
        rs = pl.ds(j * (NQ4 // 2), NQ4 // 2)
        for b in bs:
            r0, r1, r2, r3 = (xr_ref[cb, 2 * j + i, b] for i in range(4))
            if marker is not None and (b == bs[0] or not opts.get('mk1')):
                r2 = (r2.reshape(NQ4 // 8, 8, 128) + marker[None]).reshape(NQ4, 128)
            v_ref[b, rs, cs] = pack2(r0 - r2)
            v_ref[NB + b, rs, cs] = pack2(r1 + r2)
            v_ref[2 * NB + b, rs, cs] = pack2(r2 - r1)
            v_ref[3 * NB + b, rs, cs] = pack2(r1 - r3)

    def prod_list(cb):
        pl_ = [('a', cb, 0), ('a', cb, 1)]
        for j in range(NP):
            pl_ += [('a', cb, 2 * j + 2), ('a', cb, 2 * j + 3)]
            pl_ += [('b', cb, j, tuple(range(b, b + BG))) for b in range(0, NB, BG)]
        return pl_

    def out_x(st, b, d):
        if b == 0:
            st['r0'] = d
        elif b in (1, 3):
            st['p'] = d
        elif b == 2:
            st['s12'], st['d12'] = st['p'] + d, st['p'] - d
            st['r0'] = st['r0'] + st['s12']
        elif b == 4:
            s34, d34 = st['p'] + d, st['p'] - d
            st['r0'] = st['r0'] + s34
            st['r1'] = st['d12'] + d34 * 2.0
            st['r2'] = st['s12'] + s34 * 4.0
            st['r3'] = st['d12'] + d34 * 8.0
        else:
            return [st['r0'], st['r1'], st['r2'], st['r3'] + d]
        return None

    def out_y(ys, a, rr, store):
        for q in range(4):
            if a == 0:
                ys[q] = rr[q]
            elif a == 1:
                ys[q] = ys[q] + rr[q]
                ys[4 + q] = rr[q]
            elif a == 2:
                store(0, q, ys[q] + rr[q])
                ys[4 + q] = ys[4 + q] - rr[q]
            else:
                store(1, q, ys[4 + q] - rr[q])

    def u_piece(w_ref, u_ref, base, k, marker, ok=None):
        rb = lax.shift_right_logical(k, 2) if not isinstance(k, int) else k // 4
        cb = jnp.bitwise_and(k, 3) if not isinstance(k, int) else k % 4
        rows = pl.ds(mult(rb * UB, UB), UB)
        ob = rb if ok is None else jnp.where(ok, rb, C // UB)
        orow = pl.ds(mult(ob * (UB // 2), UB // 2), UB // 2)
        cs = pl.ds(mult(cb * 128, 128), 128)
        res = []
        raw = [[split_eo(w_ref[base + 3 * i + j, rows, cs]) for j in range(3)] for i in range(3)]
        for par in range(2):
            hs = []
            for j in range(3):
                g0, g1, g2 = (raw[i][j][par] for i in range(3))
                if marker is not None:
                    g1 = g1 + marker
                sm = g0 + g2
                hs.append((g0, (sm + g1) * 0.5, (sm - g1) * 0.5, g2))
            out = [None] * NPT
            for a in range(4):
                h0, h1, h2 = (hs[j][a] for j in range(3))
                sm = h0 + h2
                pp = h0 * (1.0 / 24.0) + h2 * (1.0 / 6.0)
                qq = h1 * (1.0 / 12.0)
                for b, val in enumerate((h0 * 0.25, (sm + h1) * (-1.0 / 6.0), (sm - h1) * (-1.0 / 6.0),
                                         pp + qq, pp - qq, h2)):
                    out[NB * a + b] = val
            res.append(out)
        for k2 in range(NPT):
            val = pltpu.pack_elementwise([res[0][k2], res[1][k2]], packed_dtype=bf16)
            if isinstance(u_ref, (list, tuple)):
                u_ref[k2][orow, cs] = val
            else:
                u_ref[k2, orow, cs] = val

    def stat_acc(v, state, marker=None):
        n = v.shape[0] // 8
        wd = v.shape[1]
        if state is None:
            K = v[0:1, :]
            if marker is not None:
                K = K + marker[0:1, :]
            d = v - K
            return (K, d.reshape(n, 8, wd).sum(axis=0), (d * d).reshape(n, 8, wd).sum(axis=0))
        K, s1, s2 = state
        Kd = K if marker is None else K + marker[0:1, :]
        d = v - Kd
        return (K, s1 + d.reshape(n, 8, wd).sum(axis=0), s2 + (d * d).reshape(n, 8, wd).sum(axis=0))

    def store_stats(st_ref, q, t, cs, state):
        K, s1, s2 = state
        wd = K.shape[1]
        st_ref[q, t, 0, :, cs] = jnp.broadcast_to(K, (8, wd))
        st_ref[q, t, 1, :, cs] = jnp.broadcast_to(s1.sum(axis=0, keepdims=True), (8, wd))
        st_ref[q, t, 2, :, cs] = jnp.broadcast_to(s2.sum(axis=0, keepdims=True), (8, wd))

    def finalize(st_ref, p_ref, gb_ref, e_ref, q):
        cv = q // 2 if isinstance(q, int) else lax.shift_right_logical(q, 1)
        for g in range(G):
            cs = slice(g * 128, (g + 1) * 128)
            K = st_ref[q, :, 0, :, cs]
            s1 = st_ref[q, :, 1, :, cs]
            s2 = st_ref[q, :, 2, :, cs]
            e = e_ref[q, :, cs]
            mean_t = K + s1 * (1.0 / TM) + e[None]
            m2_t = s2 - s1 * s1 * (1.0 / TM)
            mu = jnp.sum(jnp.sum(mean_t, axis=0), axis=1, keepdims=True) * (1.0 / (T * 128))
            dev = mean_t - mu[None]
            tot = m2_t + dev * dev * float(TM)
            var = jnp.sum(jnp.sum(tot, axis=0), axis=1, keepdims=True) * (1.0 / (HW * 128))
            rstd = lax.rsqrt(var + EPS)
            sc = gb_ref[cv, 0, :, cs] * (rstd * 0.5)
            p_ref[q, 0, :, cs] = sc
            p_ref[q, 1, :, cs] = gb_ref[cv, 1, :, cs] * 0.5 - (mu - e) * sc

    def merge(lists):
        items = []
        for li, l in enumerate(lists):
            for i, it in enumerate(l):
                items.append(((i + 0.5) / len(l), li, it))
        items.sort(key=lambda z: (z[0], z[1]))
        return [it for _, _, it in items]

    def kern(x_hbm, te_hbm, g1_hbm, b1_hbm, w1_hbm, we_hbm, g2_hbm, b2_hbm, w2_hbm, o_hbm,
             s_ref, w_ref, u2_ref, ar_ref, xr_ref, va_ref, vb_ref, ya_ref, yb_ref,
             st_ref, p_ref, gb_ref, e_ref, te_ref, we_ref, gsm_ref, sem_x, sem_w, sem_s, sem_o, *u1_ref):

        def gcols(g):
            return pl.ds(mult(g * 128, 128), 128)

        def x0_copy(c):
            rows = pl.ds(mult(c * TM, TM), TM)
            return pltpu.make_async_copy(x_hbm.at[0, rows, :], s_ref.at[0, rows, :], sem_x.at[c])

        def w1_copy(g):
            return pltpu.make_async_copy(w1_hbm.at[:, gcols(g), :], w_ref.at[pl.ds(0, 9), gcols(g), :], sem_w.at[g])

        def x1_copy():
            return pltpu.make_async_copy(x_hbm.at[1], s_ref.at[1], sem_s.at[6])

        def w2_copy():
            return pltpu.make_async_copy(w2_hbm, w_ref.at[pl.ds(9, 9)], sem_s.at[7])

        def small_copies():
            return [pltpu.make_async_copy(g1_hbm, gsm_ref.at[0], sem_s.at[0]),
                    pltpu.make_async_copy(b1_hbm, gsm_ref.at[1], sem_s.at[1]),
                    pltpu.make_async_copy(g2_hbm, gsm_ref.at[2], sem_s.at[2]),
                    pltpu.make_async_copy(b2_hbm, gsm_ref.at[3], sem_s.at[3]),
                    pltpu.make_async_copy(te_hbm, te_ref, sem_s.at[4])]

        def we_copy():
            return pltpu.make_async_copy(we_hbm, we_ref, sem_s.at[5])

        def o_copy(s, qi):
            b = divT(s) - 2
            r0 = mult(modT(s) * TM + qi * QR, QR)
            return pltpu.make_async_copy(s_ref.at[b, pl.ds(r0, QR), :], o_hbm.at[b, pl.ds(r0, QR), :], sem_o.at[0])

        def o_all():
            return pltpu.make_async_copy(s_ref.at[pl.ds(0, B)], o_hbm, sem_o.at[0])

        def epi_piece(y_ref, s_prev, kind, r, cb, state, marker, PW=PW):
            p = divT(s_prev)
            t = modT(s_prev)
            cs = lanes(cb, PW)
            j, par = r // 2, r % 2
            r0 = mult(t * TM + r * W, W)
            ve = load_y(y_ref, par, 0, j, cb * (PW // 128), PW // 128)
            vo = load_y(y_ref, par, 1, j, cb * (PW // 128), PW // 128)
            if marker is not None:
                ve = (ve.reshape(HP // 8, 8, PW) + marker[None]).reshape(HP, PW)
            if kind == 1:
                dst, sq = p + 2, p + 2
            elif kind == 2:
                dst, sq = p - 2, None
                xe, xo = split_eo(s_ref[dst, pl.ds(r0, W), cs])
                ve, vo = ve + xe, vo + xo
            else:
                is2 = p >= 2
                dst = jnp.where(is2, p - 2, p + 2)
                sq = jnp.where(is2, 0, p + 2)
                xe, xo = split_eo(s_ref[dst, pl.ds(r0, W), cs])
                ve, vo = ve + jnp.where(is2, xe, 0.0), vo + jnp.where(is2, xo, 0.0)
            if sq is not None:
                state = stat_acc(vo, stat_acc(ve, state))
            s_ref[dst, pl.ds(r0, W), cs] = join_eo(ve, vo)
            if sq is not None and r == TR - 1:
                store_stats(st_ref, sq, t, cs, state)
                state = None
            return state

        def xstat_piece(q, tile, cs, ri, state, marker):
            r0 = mult(tile * TM + ri * XR1, XR1)
            v = s_ref[q, pl.ds(r0, XR1), cs].astype(f32)
            state = stat_acc(v, state, marker)
            if ri == TM // XR1 - 1:
                store_stats(st_ref, q, tile, cs, state)
                state = None
            return state

        def half(it, second, u_ref, vc_ref, vn_ref, yc_ref, yp_ref, conv=None):
            s = 2 * it + second
            sn = s + 1
            pn = jnp.minimum(divT(sn), 3)
            y0 = modT(sn) * TR
            plist = [pc for cb in range(G) for pc in prod_list(cb)]
            lists = [plist,
                     [('e', r, cb) for r in range(TR) for cb in range(NPW)]]
            NU = -(-NUB // (5 if conv is None else 6))
            if UMODE == 0 and conv != 1:
                lists.append([('u', k) for k in range(NU)])
            pieces = merge(lists)
            npc = len(pieces)
            if second == 1:
                finalize(st_ref, p_ref, gb_ref, e_ref, jnp.minimum(divT(s - 1) + 1, 3))
            pv = tuple(p_ref[pn, k] for k in range(2))
            sp = s - 1
            ekind = 0 if conv is None else (1 if conv in (0, 2) else (0 if second == 0 else 2))
            wts = [{0: WH, 1: WH, 2: 100, 3: WH, 4: W4, 5: W5A if k // NB < 2 else W5B}[k % NB] for k in range(NPT)]
            cum = [sum(wts[:k]) for k in range(NPT + 1)]
            done = 0
            est = [None] * NPW
            xst = None
            pcar = None
            ys = [None] * 8
            for a in range(4):
                st = {}
                for b in range(NB):
                    k = NB * a + b
                    d = lax.dot_general(pltpu.bitcast(vc_ref[k], bf16), pltpu.bitcast(u_ref[k][...] if conv != 1 else u_ref[k, 0:C // 2, :], bf16), NT,
                                        preferred_element_type=f32)
                    for nn in range(4 * SUB):
                        n, sub = nn // SUB, nn % SUB
                        hi_ = min(npc, ((cum[k] * 4 * SUB + wts[k] * (nn + 1)) * npc * 64) // (last_slot * cum[NPT] * 4 * SUB))
                        while done < hi_:
                            pc = pieces[done]
                            if pc[0] == 'a':
                                cs = slice(pc[1] * 128, (pc[1] + 1) * 128)
                                prod_a(s_ref, tuple(t[:, cs] for t in pv), ar_ref, xr_ref, pn, y0, pc[1], pc[2],
                                       marker_of(d, n, sub, 128))
                            elif pc[0] == 'b':
                                prod_b(xr_ref, vn_ref, pc[1], pc[2], pc[3], marker_of(d, n, sub, 128))
                            elif pc[0] == 'e':
                                est[pc[2]] = epi_piece(yp_ref, sp, ekind, pc[1], pc[2], est[pc[2]],
                                                       marker_of(d, n, sub, PW))
                                if pc[2] == NPW - 1 and ((pc[1] + 1) * W) % QR == 0 and conv not in (0, 2):
                                    qi = ((pc[1] + 1) * W) // QR - 1

                                    @pl.when(sp >= 2 * T)
                                    def _():
                                        o_copy(sp, qi).start()
                            elif pc[0] == 'x':
                                xst = xstat_piece(jnp.where(it == 0, 0, 1), pc[1],
                                                  slice(pc[2] * PW, (pc[2] + 1) * PW), pc[3], xst,
                                                  marker_of(d, n, sub, PW))
                            else:
                                kk = (s - 2) * NU + pc[1]
                                ok = jnp.logical_and(kk >= 0, kk < NUB)
                                u_piece(w_ref, u2_ref, 9, jnp.clip(kk, 0, NUB - 1),
                                        marker_of(d, n, sub, 128), ok)
                            done += 1
                    rr = out_x(st, b, d)

                def store(par, q, val):
                    for n in range(G):
                        store_y(yc_ref, par, q, n, val[:, n * 128:(n + 1) * 128])
                out_y(ys, a, rr, store)

        def emb_part():
            te = te_ref[...].astype(f32)
            sl = te * jax.nn.sigmoid(te)
            emb = jnp.dot(sl.astype(bf16), we_ref[...], preferred_element_type=f32)
            e_ref[2] = jnp.broadcast_to(emb[0:1, :], (8, C))
            e_ref[3] = jnp.broadcast_to(emb[1:2, :], (8, C))

        def nhalf(step, n, vc_ref, vn_ref, yc_ref, yp_ref, with_u=True):
            y0 = (step + 1) * TR
            if step == 0 and P0 == 1:
                lists = [] if with_u else [[pc for cb in range(G) for pc in prod_list(cb)]]
            else:
                lists = [prod_list(None)]
            if step == 0:
                if with_u:
                    lists.append([('u', k) for k in range(NUB // G)])
            else:
                lists.append([('e', r) for r in range(TR)])
                lists.append([('x', cb, ri) for cb in range(NPW) for ri in range(TM // XR1)])
            pieces = merge(lists)
            npc = len(pieces)
            cs = lanes(n)
            pvc = tuple(p_ref[0, k, :, cs] for k in range(2))
            urows = pl.ds(mult(n * (128 // 2), 128 // 2), 128 // 2)
            gn = n + 1 if PEEL0 else jnp.minimum(n + 1, G - 1)
            NS = NSUB
            done = 0
            est = xst = None
            ys = [None] * 8
            dhist = []
            for a in range(4):
                st = {}
                for b in range(NB):
                    k = NB * a + b
                    d = lax.dot_general(pltpu.bitcast(vc_ref[k], bf16), pltpu.bitcast(u1_ref[k][urows, :], bf16), NT,
                                        preferred_element_type=f32)
                    for sub in range(NS):
                        lag = LAG if with_u and step == 0 else 1
                        hi_ = npc if k == NPT - 1 and sub == NS - 1 else (((k - lag + 1) * NS + sub) * npc) // ((NPT - lag) * NS)
                        dprev = dhist[k - lag] if k >= lag else None
                        while done < min(hi_, npc) and dprev is not None:
                            pc = pieces[done]
                            rp = sub * (M // NS) // 8 * 8
                            bits = pltpu.bitcast(dprev[rp:rp + 8, :], u32)
                            mk = pltpu.bitcast((bits >> 16) >> 16, f32)
                            if pc[0] == 'a':
                                cbp = n if pc[1] is None else pc[1]
                                pvp = pvc if pc[1] is None else tuple(p_ref[0, k_, :, lanes(cbp)] for k_ in range(2))
                                prod_a(s_ref, pvp, ar_ref, xr_ref, 0, y0, cbp, pc[2], mk)
                            elif pc[0] == 'b':
                                prod_b(xr_ref, vn_ref, n if pc[1] is None else pc[1], pc[2], pc[3], mk)
                            elif pc[0] == 'u':
                                u_piece(w_ref, u1_ref, 0, gn * (NUB // G) + pc[1], mk)
                            elif pc[0] == 'e':
                                est = epi_piece(yp_ref, 0, 1, pc[1], n, est, mk, PW=128)
                            else:
                                mkx = mk if PW == 128 else jnp.concatenate([mk] * (PW // 128), axis=1)
                                xst = xstat_piece(1, n, slice(pc[1] * PW, (pc[1] + 1) * PW), pc[2], xst, mkx)
                            done += 1
                    dhist.append(d)
                    rr = out_x(st, b, d)
                out_y(ys, a, rr, lambda par, q, val: store_y(yc_ref, par, q, n, val))
            assert done == npc
            if step == 0 and not with_u and EMB0:
                emb_part()

        def xstat_tile(q, c):
            for cb in range(NPW):
                def rows(ri, st):
                    r0 = pl.multiple_of(c * TM + ri * XR, XR)
                    v = s_ref[q, pl.ds(r0, XR), cb * PW:(cb + 1) * PW].astype(f32)
                    return stat_acc(v, st)
                v0 = s_ref[q, pl.ds(pl.multiple_of(c * TM, XR), XR), cb * PW:(cb + 1) * PW].astype(f32)
                st = lax.fori_loop(1, NXR, rows, stat_acc(v0, None))
                store_stats(st_ref, q, c, slice(cb * PW, (cb + 1) * PW), st)
            return 0

        with scope('prologue'):
            for c in small_copies():
                c.start()
            lax.fori_loop(0, T, lambda c, _: (x0_copy(c).start(), 0)[1], 0)
            lax.fori_loop(0, G, lambda g, _: (w1_copy(g).start(), 0)[1], 0)

            def rest(c, _):
                @pl.when(c == (1 if EMB0 else 0))
                def _():
                    x1_copy().start()

                @pl.when(c == (2 if EMB0 else 1))
                def _():
                    w2_copy().start()

                @pl.when(c == (0 if EMB0 else 2))
                def _():
                    we_copy().start()
                return 0
            lax.fori_loop(0, 3, rest, 0)

            for c in small_copies():
                c.wait()
            for cv in range(2):
                for k in range(2):
                    v = gsm_ref[2 * cv + k].astype(f32)
                    for g in range(G):
                        gb_ref[cv, k, :, g * 128:(g + 1) * 128] = jnp.broadcast_to(v[g:g + 1, :], (8, 128))
            e_ref[...] = jnp.zeros(e_ref.shape, f32)
            st_ref[...] = jnp.zeros(st_ref.shape, f32)
            ar_ref[...] = jnp.zeros(ar_ref.shape, f32)

            def xs0(c, _):
                x0_copy(c).wait()
                return xstat_tile(0, c)
            lax.fori_loop(0, T, xs0, 0)
            finalize(st_ref, p_ref, gb_ref, e_ref, 0)

            PU = opts.get('pu', 4)

            def prod0(c2, _):
                for i in range(PU):
                    cb = c2 * PU + i
                    pvc = tuple(p_ref[0, k, :, gcols(cb)] for k in range(2))
                    for pc in prod_list(cb):
                        if pc[0] == 'a':
                            prod_a(s_ref, pvc, ar_ref, xr_ref, 0, 0, cb, pc[2], None, i)
                        else:
                            prod_b(xr_ref, va_ref, cb, pc[2], pc[3], None, i)
                return 0
            lax.fori_loop(0, G // PU, prod0, 0)

            w1_copy(0).wait()
            lax.fori_loop(0, NUB // G, lambda k, _: (u_piece(w_ref, u1_ref, 0, k, None), 0)[1], 0, unroll=opts.get('uu', 4))

        def step0(n, _):
            if PEEL0:
                w1_copy(n + 1).wait()
            else:
                @pl.when(n < G - 1)
                def _():
                    w1_copy(n + 1).wait()
            nhalf(0, n, va_ref, vb_ref, ya_ref, yb_ref)
            return 0

        def step1(n, _):
            nhalf(1, n, vb_ref, va_ref, yb_ref, ya_ref)
            return 0

        with scope('step0'):
            if PEEL0:
                lax.fori_loop(0, G - 1, step0, 0)
                if EMB0:
                    we_copy().wait()
                nhalf(0, G - 1, va_ref, vb_ref, ya_ref, yb_ref, False)
            else:
                lax.fori_loop(0, G, step0, 0)
        with scope('step1'):
            x1_copy().wait()
            lax.fori_loop(0, G, step1, 0)

        def emb_block():
            w2_copy().wait()
            if not EMB0:
                we_copy().wait()
                emb_part()

        def body(it, carry):
            @pl.when(it == 1)
            def _():
                emb_block()

            @pl.when(it == T)
            def _():
                if UMODE == 0:
                    def cp(rb, _):
                        rows = pl.ds(pl.multiple_of(rb * 32, 32), 32)
                        for k in range(NPT):
                            u1_ref[k][rows, :] = u2_ref[k, rows, :]
                        return 0
                    lax.fori_loop(0, C // 2 // 32, cp, 0)
                else:
                    lax.fori_loop(0, NUB, lambda k, _: (u_piece(w_ref, u1_ref, 9, k, None), 0)[1], 0)
            with scope('iter'):
                half(it, 0, u1_ref, va_ref, vb_ref, ya_ref, yb_ref)
                half(it, 1, u1_ref, vb_ref, va_ref, yb_ref, ya_ref)
            return carry

        def body_c(conv):
            def f(it, carry):
                if conv == 0:
                    @pl.when(it == 1)
                    def _():
                        emb_block()
                ur = u2_ref if conv == 1 else u1_ref
                with scope('iter'):
                    half(it, 0, ur, va_ref, vb_ref, ya_ref, yb_ref, conv)
                    half(it, 1, ur, vb_ref, va_ref, yb_ref, ya_ref, conv)
                return carry
            return f

        with scope('main'):
            if SPLIT:
                if SPLIT == 2:
                    emb_block()
                lax.fori_loop(1, T, body_c(0 if SPLIT == 1 else 2), 0)
                lax.fori_loop(T, 2 * T, body_c(1), 0)
            else:
                lax.fori_loop(1, 2 * T, body, 0)

        sl_ = NSTEP - 1
        with scope('final'):
            st = [None] * NPW
            for r in range(TR):
                for cb in range(NPW):
                    st[cb] = epi_piece(yb_ref, sl_, 2, r, cb, st[cb], None)
                if ((r + 1) * W) % QR == 0:
                    o_copy(sl_, ((r + 1) * W) // QR - 1).start()
        with scope('owait'):
            o_all().wait()

    def fn(x, t_emb, g1, be1, w1, w_emb, g2, be2, w2):
        xn = jnp.transpose(x, (0, 2, 3, 1)).reshape(B, HW, C)
        w1t = jnp.transpose(w1, (2, 3, 0, 1)).reshape(9, C, C)
        w2t = jnp.transpose(w2, (2, 3, 0, 1)).reshape(9, C, C)
        any_spec = pl.BlockSpec(memory_space=pl.ANY)
        ubuf = pltpu.VMEM((C // 2, C), u32)
        vbuf = pltpu.VMEM((NPT, M // 2, C), u32)
        ybuf = pltpu.VMEM((2, 2, G, 2 * M, 128), f32)
        out = pl.pallas_call(
            kern,
            in_specs=[any_spec] * 9,
            out_specs=any_spec,
            out_shape=jax.ShapeDtypeStruct((B, HW, C), bf16),
            scratch_shapes=[
                pltpu.VMEM((4, HW, C), bf16),
                pltpu.VMEM((18, C, C), bf16),
                pltpu.VMEM((NPT, (C // 2 + UB // 2) if UMODE == 0 else 8, C), u32),
                pltpu.VMEM((G, NAR, 2, HP + 16, 128), f32),
                pltpu.VMEM((G, TR + 2, NB, NQ4, 128), f32),
                vbuf, vbuf, ybuf, ybuf,
                pltpu.VMEM((4, T, 3, 8, C), f32),
                pltpu.VMEM((4, 2, 8, C), f32),
                pltpu.VMEM((2, 2, 8, C), f32),
                pltpu.VMEM((4, 8, C), f32),
                pltpu.VMEM((B, E), bf16),
                pltpu.VMEM((E, C), bf16),
                pltpu.VMEM((4, G, 128), bf16),
                pltpu.SemaphoreType.DMA((T,)),
                pltpu.SemaphoreType.DMA((G,)),
                pltpu.SemaphoreType.DMA((8,)),
                pltpu.SemaphoreType.DMA((1,)),
            ] + [ubuf] * NPT,
            compiler_params=pltpu.CompilerParams(vmem_limit_bytes=100 * 1024 * 1024,
                                                 disable_bounds_checks=True),
        )(xn, t_emb, g1.reshape(G, 128), be1.reshape(G, 128), w1t, w_emb,
          g2.reshape(G, 128), be2.reshape(G, 128), w2t)
        return jnp.transpose(out.reshape(B, H, W, C), (0, 3, 1, 2))
    return fn


_OPTS = {}


@jax.jit
def pallas_standalone__adm_resblock__diffusion_kernel(x, t_emb, g1, be1, w1, w_emb, g2, be2, w2):
    B, C, H, W = x.shape
    E = t_emb.shape[1]
    return build(B, C, H, W, E, TM=1024, opts=_OPTS)(x, t_emb, g1, be1, w1, w_emb, g2, be2, w2)
```

```python
import jax
import jax.numpy as jnp
from jax import lax
from jax.experimental import pallas as pl
from jax.experimental.pallas import tpu as pltpu

f32 = jnp.float32
bf16 = jnp.bfloat16
u32 = jnp.uint32
NT = (((1,), (1,)), ((), ()))


def build(B, C, H, W, E, TM=1024, opts=None):
    opts = opts or {}
    HW = H * W
    G = 4
    CG = C // G
    EPS = 1e-5
    T = HW // TM
    assert CG == 128 and B == 2 and T == 4 and W == 64 and H == 64
    TR = TM // W
    NP = TR // 2
    HP = W // 2
    NQ4 = W // 4
    M = NP * NQ4
    NB = 6
    NPT = 4 * NB
    NSTEP = 4 * T
    scope = jax.named_scope

    PW = opts.get('pw', 256)
    NPW = C // PW
    SUB = opts.get('sub', 8)
    XR = opts.get('xr', 256)
    NXR = TM // XR
    last_slot = opts.get('last_slot', 61)
    NQ = opts.get('nq', 4)
    QR = TM // NQ
    UMODE = opts.get('umode', 0)
    XMODE = opts.get('xmode', 0)
    NAR = opts.get('nar', 2)
    LAG = opts.get('lag', 2)
    P0 = opts.get('p0', 1)
    EMB0 = opts.get('emb0', 1)
    SPLIT = opts.get('split', 2)
    PEEL0 = opts.get('peel0', 1)
    WH, W4, W5A, W5B = (opts.get(k_, v_) for k_, v_ in (('wh', 130), ('w4', 40), ('w5a', 80), ('w5b', 30)))
    BG = opts.get('bg', 3)
    NSUB = opts.get('nsub', 8)
    XR1 = opts.get('xr1', 32)
    UB = 16
    NUB = (C // UB) * G

    def mult(v, m):
        return v if isinstance(v, int) else pl.multiple_of(v, m)

    def divT(v):
        return v // T if isinstance(v, int) else lax.shift_right_logical(v, 2)

    def modT(v):
        return v % T if isinstance(v, int) else jnp.bitwise_and(v, T - 1)

    def marker_of(d, n, sub, width):
        rp = sub * (d.shape[0] // SUB) // 8 * 8
        m = d[rp:rp + 8, n * 128:(n + 1) * 128]
        b = pltpu.bitcast(m, u32)
        z = pltpu.bitcast((b >> 16) >> 16, f32)
        if width > 128:
            z = jnp.concatenate([z] * (width // 128), axis=1)
        return z

    def pack2(t):
        n = t.shape[0] // 2
        return pltpu.pack_elementwise([t[:n], t[n:]], packed_dtype=bf16)

    def lanes(cb, width=128):
        if isinstance(cb, int):
            return slice(cb * width, (cb + 1) * width)
        return pl.ds(pl.multiple_of(cb * width, width), width)

    def load_y(y_ref, par, eo, j, cb0, ncb):
        parts = [y_ref[par, eo, cb0 + i, j * HP:(j + 1) * HP, :] for i in range(ncb)]
        return parts[0] if ncb == 1 else jnp.concatenate(parts, axis=1)

    def store_y(y_ref, par, q, n, val):
        y_ref[par, q % 2, n, pl.ds(q // 2, M, stride=2), :] = val

    def split_eo(v):
        w = pltpu.bitcast(v, u32)
        return (pltpu.unpack_elementwise(w, index=0, packed_dtype=bf16, unpacked_dtype=f32),
                pltpu.unpack_elementwise(w, index=1, packed_dtype=bf16, unpacked_dtype=f32))

    def join_eo(e, o):
        return pltpu.bitcast(pltpu.pack_elementwise([e, o], packed_dtype=bf16), bf16)

    def act(v, pv, marker):
        n, wd = v.shape
        sc, bt = pv
        if marker is not None:
            bt = bt + marker
        v3 = v.reshape(n // 8, 8, wd)
        hz = (v3 * sc[None] + bt[None]).reshape(n, wd)
        return hz * jnp.tanh(hz) + hz

    def act_row(s_ref, pv, q, y, cs, marker, edge):
        yc = y if not edge else jnp.clip(y, 0, H - 1)
        e, o = split_eo(s_ref[q, pl.ds(mult(yc * W, W), W), cs])
        e = act(e, pv, marker)
        o = act(o, pv, marker)
        if edge:
            valid = jnp.logical_and(y >= 0, y < H)
            e = jnp.where(valid, e, 0.0)
            o = jnp.where(valid, o, 0.0)
        return e, o

    def prod_a(s_ref, pv, ar_ref, xr_ref, q, y0, cb, i, marker, slot=0):
        cs = lanes(cb)
        cb = cb if isinstance(cb, int) else slot
        e, o = act_row(s_ref, pv, q, y0 - 1 + i, cs, marker, i == 0 or i == TR + 1)
        sl = i % NAR
        ar_ref[cb, sl, 0] = e
        ar_ref[cb, sl, 1] = o

        def col(eo, r):
            return jnp.concatenate([ar_ref[cb, sl, eo, pl.ds(r + 2 * u, NQ4 // 2, stride=4), :] for u in range(2)], axis=0)
        d1, d2, d3, d4 = col(0, 0), col(1, 0), col(0, 1), col(1, 1)
        hq = NQ4 // 2
        row = lax.broadcasted_iota(jnp.int32, (hq, 128), 0)
        d0 = jnp.concatenate([jnp.where(row == 0, 0.0, pltpu.roll(d4[hq:], 1, 0)), d4[:hq]], axis=0)
        d5 = jnp.concatenate([d1[hq:], jnp.where(row == hq - 1, 0.0, pltpu.roll(d1[:hq], hq - 1, 0))], axis=0)
        c = d4 - d2
        e2 = (d3 - d1) * 2.0
        a_ = d4 - d2 * 4.0
        b_ = d3 - d1 * 4.0
        xr_ref[cb, i, 0] = (d0 - d2) * 4.0 + c
        xr_ref[cb, i, 1] = a_ + b_
        xr_ref[cb, i, 2] = a_ - b_
        xr_ref[cb, i, 3] = c + e2
        xr_ref[cb, i, 4] = c - e2
        xr_ref[cb, i, 5] = (d5 - d3) - e2 * 2.0

    def prod_b(xr_ref, v_ref, cb, j, bs, marker, slot=0):
        cs = lanes(cb)
        cb = cb if isinstance(cb, int) else slot
        rs = pl.ds(j * (NQ4 // 2), NQ4 // 2)
        for b in bs:
            r0, r1, r2, r3 = (xr_ref[cb, 2 * j + i, b] for i in range(4))
            if marker is not None and (b == bs[0] or not opts.get('mk1')):
                r2 = (r2.reshape(NQ4 // 8, 8, 128) + marker[None]).reshape(NQ4, 128)
            v_ref[b, rs, cs] = pack2(r0 - r2)
            v_ref[NB + b, rs, cs] = pack2(r1 + r2)
            v_ref[2 * NB + b, rs, cs] = pack2(r2 - r1)
            v_ref[3 * NB + b, rs, cs] = pack2(r1 - r3)

    def prod_list(cb):
        pl_ = [('a', cb, 0), ('a', cb, 1)]
        for j in range(NP):
            pl_ += [('a', cb, 2 * j + 2), ('a', cb, 2 * j + 3)]
            pl_ += [('b', cb, j, tuple(range(b, b + BG))) for b in range(0, NB, BG)]
        return pl_

    def out_x(st, b, d):
        if b == 0:
            st['r0'] = d
        elif b in (1, 3):
            st['p'] = d
        elif b == 2:
            st['s12'], st['d12'] = st['p'] + d, st['p'] - d
            st['r0'] = st['r0'] + st['s12']
        elif b == 4:
            s34, d34 = st['p'] + d, st['p'] - d
            st['r0'] = st['r0'] + s34
            st['r1'] = st['d12'] + d34 * 2.0
            st['r2'] = st['s12'] + s34 * 4.0
            st['r3'] = st['d12'] + d34 * 8.0
        else:
            return [st['r0'], st['r1'], st['r2'], st['r3'] + d]
        return None

    def out_y(ys, a, rr, store):
        for q in range(4):
            if a == 0:
                ys[q] = rr[q]
            elif a == 1:
                ys[q] = ys[q] + rr[q]
                ys[4 + q] = rr[q]
            elif a == 2:
                store(0, q, ys[q] + rr[q])
                ys[4 + q] = ys[4 + q] - rr[q]
            else:
                store(1, q, ys[4 + q] - rr[q])

    def u_piece(w_ref, u_ref, base, k, marker, ok=None):
        rb = lax.shift_right_logical(k, 2) if not isinstance(k, int) else k // 4
        cb = jnp.bitwise_and(k, 3) if not isinstance(k, int) else k % 4
        rows = pl.ds(mult(rb * UB, UB), UB)
        ob = rb if ok is None else jnp.where(ok, rb, C // UB)
        orow = pl.ds(mult(ob * (UB // 2), UB // 2), UB // 2)
        cs = pl.ds(mult(cb * 128, 128), 128)
        res = []
        raw = [[split_eo(w_ref[base + 3 * i + j, rows, cs]) for j in range(3)] for i in range(3)]
        for par in range(2):
            hs = []
            for j in range(3):
                g0, g1, g2 = (raw[i][j][par] for i in range(3))
                if marker is not None:
                    g1 = g1 + marker
                sm = g0 + g2
                hs.append((g0, (sm + g1) * 0.5, (sm - g1) * 0.5, g2))
            out = [None] * NPT
            for a in range(4):
                h0, h1, h2 = (hs[j][a] for j in range(3))
                sm = h0 + h2
                pp = h0 * (1.0 / 24.0) + h2 * (1.0 / 6.0)
                qq = h1 * (1.0 / 12.0)
                for b, val in enumerate((h0 * 0.25, (sm + h1) * (-1.0 / 6.0), (sm - h1) * (-1.0 / 6.0),
                                         pp + qq, pp - qq, h2)):
                    out[NB * a + b] = val
            res.append(out)
        for k2 in range(NPT):
            val = pltpu.pack_elementwise([res[0][k2], res[1][k2]], packed_dtype=bf16)
            if isinstance(u_ref, (list, tuple)):
                u_ref[k2][orow, cs] = val
            else:
                u_ref[k2, orow, cs] = val

    def stat_acc(v, state, marker=None):
        n = v.shape[0] // 8
        wd = v.shape[1]
        if state is None:
            K = v[0:1, :]
            if marker is not None:
                K = K + marker[0:1, :]
            d = v - K
            return (K, d.reshape(n, 8, wd).sum(axis=0), (d * d).reshape(n, 8, wd).sum(axis=0))
        K, s1, s2 = state
        Kd = K if marker is None else K + marker[0:1, :]
        d = v - Kd
        return (K, s1 + d.reshape(n, 8, wd).sum(axis=0), s2 + (d * d).reshape(n, 8, wd).sum(axis=0))

    def store_stats(st_ref, q, t, cs, state):
        K, s1, s2 = state
        wd = K.shape[1]
        st_ref[q, t, 0, :, cs] = jnp.broadcast_to(K, (8, wd))
        st_ref[q, t, 1, :, cs] = jnp.broadcast_to(s1.sum(axis=0, keepdims=True), (8, wd))
        st_ref[q, t, 2, :, cs] = jnp.broadcast_to(s2.sum(axis=0, keepdims=True), (8, wd))

    def finalize(st_ref, p_ref, gb_ref, e_ref, q):
        cv = q // 2 if isinstance(q, int) else lax.shift_right_logical(q, 1)
        for g in range(G):
            cs = slice(g * 128, (g + 1) * 128)
            K = st_ref[q, :, 0, :, cs]
            s1 = st_ref[q, :, 1, :, cs]
            s2 = st_ref[q, :, 2, :, cs]
            e = e_ref[q, :, cs]
            mean_t = K + s1 * (1.0 / TM) + e[None]
            m2_t = s2 - s1 * s1 * (1.0 / TM)
            mu = jnp.sum(jnp.sum(mean_t, axis=0), axis=1, keepdims=True) * (1.0 / (T * 128))
            dev = mean_t - mu[None]
            tot = m2_t + dev * dev * float(TM)
            var = jnp.sum(jnp.sum(tot, axis=0), axis=1, keepdims=True) * (1.0 / (HW * 128))
            rstd = lax.rsqrt(var + EPS)
            sc = gb_ref[cv, 0, :, cs] * (rstd * 0.5)
            p_ref[q, 0, :, cs] = sc
            p_ref[q, 1, :, cs] = gb_ref[cv, 1, :, cs] * 0.5 - (mu - e) * sc

    def merge(lists):
        items = []
        for li, l in enumerate(lists):
            for i, it in enumerate(l):
                items.append(((i + 0.5) / len(l), li, it))
        items.sort(key=lambda z: (z[0], z[1]))
        return [it for _, _, it in items]

    def kern(x_hbm, te_hbm, g1_hbm, b1_hbm, w1_hbm, we_hbm, g2_hbm, b2_hbm, w2_hbm, o_hbm,
             s_ref, w_ref, u2_ref, ar_ref, xr_ref, va_ref, vb_ref, ya_ref, yb_ref,
             st_ref, p_ref, gb_ref, e_ref, te_ref, we_ref, gsm_ref, sem_x, sem_w, sem_s, sem_o, *u1_ref):

        def gcols(g):
            return pl.ds(mult(g * 128, 128), 128)

        def x0_copy(c):
            rows = pl.ds(mult(c * TM, TM), TM)
            return pltpu.make_async_copy(x_hbm.at[0, rows, :], s_ref.at[0, rows, :], sem_x.at[c])

        def w1_copy(g):
            return pltpu.make_async_copy(w1_hbm.at[:, gcols(g), :], w_ref.at[pl.ds(0, 9), gcols(g), :], sem_w.at[g])

        def x1_copy():
            return pltpu.make_async_copy(x_hbm.at[1], s_ref.at[1], sem_s.at[6])

        def w2_copy():
            return pltpu.make_async_copy(w2_hbm, w_ref.at[pl.ds(9, 9)], sem_s.at[7])

        def small_copies():
            return [pltpu.make_async_copy(g1_hbm, gsm_ref.at[0], sem_s.at[0]),
                    pltpu.make_async_copy(b1_hbm, gsm_ref.at[1], sem_s.at[1]),
                    pltpu.make_async_copy(g2_hbm, gsm_ref.at[2], sem_s.at[2]),
                    pltpu.make_async_copy(b2_hbm, gsm_ref.at[3], sem_s.at[3]),
                    pltpu.make_async_copy(te_hbm, te_ref, sem_s.at[4])]

        def we_copy():
            return pltpu.make_async_copy(we_hbm, we_ref, sem_s.at[5])

        def o_copy(s, qi):
            b = divT(s) - 2
            r0 = mult(modT(s) * TM + qi * QR, QR)
            return pltpu.make_async_copy(s_ref.at[b, pl.ds(r0, QR), :], o_hbm.at[b, pl.ds(r0, QR), :], sem_o.at[0])

        def o_all():
            return pltpu.make_async_copy(s_ref.at[pl.ds(0, B)], o_hbm, sem_o.at[0])

        def epi_piece(y_ref, s_prev, kind, r, cb, state, marker, PW=PW):
            p = divT(s_prev)
            t = modT(s_prev)
            cs = lanes(cb, PW)
            j, par = r // 2, r % 2
            r0 = mult(t * TM + r * W, W)
            ve = load_y(y_ref, par, 0, j, cb * (PW // 128), PW // 128)
            vo = load_y(y_ref, par, 1, j, cb * (PW // 128), PW // 128)
            if marker is not None:
                ve = (ve.reshape(HP // 8, 8, PW) + marker[None]).reshape(HP, PW)
            if kind == 1:
                dst, sq = p + 2, p + 2
            elif kind == 2:
                dst, sq = p - 2, None
                xe, xo = split_eo(s_ref[dst, pl.ds(r0, W), cs])
                ve, vo = ve + xe, vo + xo
            else:
                is2 = p >= 2
                dst = jnp.where(is2, p - 2, p + 2)
                sq = jnp.where(is2, 0, p + 2)
                xe, xo = split_eo(s_ref[dst, pl.ds(r0, W), cs])
                ve, vo = ve + jnp.where(is2, xe, 0.0), vo + jnp.where(is2, xo, 0.0)
            if sq is not None:
                state = stat_acc(vo, stat_acc(ve, state))
            s_ref[dst, pl.ds(r0, W), cs] = join_eo(ve, vo)
            if sq is not None and r == TR - 1:
                store_stats(st_ref, sq, t, cs, state)
                state = None
            return state

        def xstat_piece(q, tile, cs, ri, state, marker):
            r0 = mult(tile * TM + ri * XR1, XR1)
            v = s_ref[q, pl.ds(r0, XR1), cs].astype(f32)
            state = stat_acc(v, state, marker)
            if ri == TM // XR1 - 1:
                store_stats(st_ref, q, tile, cs, state)
                state = None
            return state

        def half(it, second, u_ref, vc_ref, vn_ref, yc_ref, yp_ref, conv=None):
            s = 2 * it + second
            sn = s + 1
            pn = jnp.minimum(divT(sn), 3)
            y0 = modT(sn) * TR
            plist = [pc for cb in range(G) for pc in prod_list(cb)]
            lists = [plist,
                     [('e', r, cb) for r in range(TR) for cb in range(NPW)]]
            NU = -(-NUB // (5 if conv is None else 6))
            if UMODE == 0 and conv != 1:
                lists.append([('u', k) for k in range(NU)])
            pieces = merge(lists)
            npc = len(pieces)
            if second == 1:
                finalize(st_ref, p_ref, gb_ref, e_ref, jnp.minimum(divT(s - 1) + 1, 3))
            pv = tuple(p_ref[pn, k] for k in range(2))
            sp = s - 1
            ekind = 0 if conv is None else (1 if conv in (0, 2) else (0 if second == 0 else 2))
            wts = [{0: WH, 1: WH, 2: 100, 3: WH, 4: W4, 5: W5A if k // NB < 2 else W5B}[k % NB] for k in range(NPT)]
            cum = [sum(wts[:k]) for k in range(NPT + 1)]
            done = 0
            est = [None] * NPW
            xst = None
            pcar = None
            ys = [None] * 8
            for a in range(4):
                st = {}
                for b in range(NB):
                    k = NB * a + b
                    d = lax.dot_general(pltpu.bitcast(vc_ref[k], bf16), pltpu.bitcast(u_ref[k][...] if conv != 1 else u_ref[k, 0:C // 2, :], bf16), NT,
                                        preferred_element_type=f32)
                    for nn in range(4 * SUB):
                        n, sub = nn // SUB, nn % SUB
                        hi_ = min(npc, ((cum[k] * 4 * SUB + wts[k] * (nn + 1)) * npc * 64) // (last_slot * cum[NPT] * 4 * SUB))
                        while done < hi_:
                            pc = pieces[done]
                            if pc[0] == 'a':
                                cs = slice(pc[1] * 128, (pc[1] + 1) * 128)
                                prod_a(s_ref, tuple(t[:, cs] for t in pv), ar_ref, xr_ref, pn, y0, pc[1], pc[2],
                                       marker_of(d, n, sub, 128))
                            elif pc[0] == 'b':
                                prod_b(xr_ref, vn_ref, pc[1], pc[2], pc[3], marker_of(d, n, sub, 128))
                            elif pc[0] == 'e':
                                est[pc[2]] = epi_piece(yp_ref, sp, ekind, pc[1], pc[2], est[pc[2]],
                                                       marker_of(d, n, sub, PW))
                                if pc[2] == NPW - 1 and ((pc[1] + 1) * W) % QR == 0 and conv not in (0, 2):
                                    qi = ((pc[1] + 1) * W) // QR - 1

                                    @pl.when(sp >= 2 * T)
                                    def _():
                                        o_copy(sp, qi).start()
                            elif pc[0] == 'x':
                                xst = xstat_piece(jnp.where(it == 0, 0, 1), pc[1],
                                                  slice(pc[2] * PW, (pc[2] + 1) * PW), pc[3], xst,
                                                  marker_of(d, n, sub, PW))
                            else:
                                kk = (s - 2) * NU + pc[1]
                                ok = jnp.logical_and(kk >= 0, kk < NUB)
                                u_piece(w_ref, u2_ref, 9, jnp.clip(kk, 0, NUB - 1),
                                        marker_of(d, n, sub, 128), ok)
                            done += 1
                    rr = out_x(st, b, d)

                def store(par, q, val):
                    for n in range(G):
                        store_y(yc_ref, par, q, n, val[:, n * 128:(n + 1) * 128])
                out_y(ys, a, rr, store)

        def emb_part():
            te = te_ref[...].astype(f32)
            sl = te * jax.nn.sigmoid(te)
            emb = jnp.dot(sl.astype(bf16), we_ref[...], preferred_element_type=f32)
            e_ref[2] = jnp.broadcast_to(emb[0:1, :], (8, C))
            e_ref[3] = jnp.broadcast_to(emb[1:2, :], (8, C))

        def nhalf(step, n, vc_ref, vn_ref, yc_ref, yp_ref, with_u=True):
            y0 = (step + 1) * TR
            if step == 0 and P0 == 1:
                lists = [] if with_u else [[pc for cb in range(G) for pc in prod_list(cb)]]
            else:
                lists = [prod_list(None)]
            if step == 0:
                if with_u:
                    lists.append([('u', k) for k in range(NUB // G)])
            else:
                lists.append([('e', r) for r in range(TR)])
                lists.append([('x', cb, ri) for cb in range(NPW) for ri in range(TM // XR1)])
            pieces = merge(lists)
            npc = len(pieces)
            cs = lanes(n)
            pvc = tuple(p_ref[0, k, :, cs] for k in range(2))
            urows = pl.ds(mult(n * (128 // 2), 128 // 2), 128 // 2)
            gn = n + 1 if PEEL0 else jnp.minimum(n + 1, G - 1)
            NS = NSUB
            done = 0
            est = xst = None
            ys = [None] * 8
            dhist = []
            for a in range(4):
                st = {}
                for b in range(NB):
                    k = NB * a + b
                    d = lax.dot_general(pltpu.bitcast(vc_ref[k], bf16), pltpu.bitcast(u1_ref[k][urows, :], bf16), NT,
                                        preferred_element_type=f32)
                    for sub in range(NS):
                        lag = LAG if with_u and step == 0 else 1
                        hi_ = npc if k == NPT - 1 and sub == NS - 1 else (((k - lag + 1) * NS + sub) * npc) // ((NPT - lag) * NS)
                        dprev = dhist[k - lag] if k >= lag else None
                        while done < min(hi_, npc) and dprev is not None:
                            pc = pieces[done]
                            rp = sub * (M // NS) // 8 * 8
                            bits = pltpu.bitcast(dprev[rp:rp + 8, :], u32)
                            mk = pltpu.bitcast((bits >> 16) >> 16, f32)
                            if pc[0] == 'a':
                                cbp = n if pc[1] is None else pc[1]
                                pvp = pvc if pc[1] is None else tuple(p_ref[0, k_, :, lanes(cbp)] for k_ in range(2))
                                prod_a(s_ref, pvp, ar_ref, xr_ref, 0, y0, cbp, pc[2], mk)
                            elif pc[0] == 'b':
                                prod_b(xr_ref, vn_ref, n if pc[1] is None else pc[1], pc[2], pc[3], mk)
                            elif pc[0] == 'u':
                                u_piece(w_ref, u1_ref, 0, gn * (NUB // G) + pc[1], mk)
                            elif pc[0] == 'e':
                                est = epi_piece(yp_ref, 0, 1, pc[1], n, est, mk, PW=128)
                            else:
                                mkx = mk if PW == 128 else jnp.concatenate([mk] * (PW // 128), axis=1)
                                xst = xstat_piece(1, n, slice(pc[1] * PW, (pc[1] + 1) * PW), pc[2], xst, mkx)
                            done += 1
                    dhist.append(d)
                    rr = out_x(st, b, d)
                out_y(ys, a, rr, lambda par, q, val: store_y(yc_ref, par, q, n, val))
            assert done == npc
            if step == 0 and not with_u and EMB0:
                emb_part()

        def xstat_tile(q, c):
            for cb in range(NPW):
                def rows(ri, st):
                    r0 = pl.multiple_of(c * TM + ri * XR, XR)
                    v = s_ref[q, pl.ds(r0, XR), cb * PW:(cb + 1) * PW].astype(f32)
                    return stat_acc(v, st)
                v0 = s_ref[q, pl.ds(pl.multiple_of(c * TM, XR), XR), cb * PW:(cb + 1) * PW].astype(f32)
                st = lax.fori_loop(1, NXR, rows, stat_acc(v0, None))
                store_stats(st_ref, q, c, slice(cb * PW, (cb + 1) * PW), st)
            return 0

        with scope('prologue'):
            for c in small_copies():
                c.start()
            lax.fori_loop(0, T, lambda c, _: (x0_copy(c).start(), 0)[1], 0)
            lax.fori_loop(0, G, lambda g, _: (w1_copy(g).start(), 0)[1], 0)

            def rest(c, _):
                @pl.when(c == (1 if EMB0 else 0))
                def _():
                    x1_copy().start()

                @pl.when(c == (2 if EMB0 else 1))
                def _():
                    w2_copy().start()

                @pl.when(c == (0 if EMB0 else 2))
                def _():
                    we_copy().start()
                return 0
            lax.fori_loop(0, 3, rest, 0)

            for c in small_copies():
                c.wait()
            for cv in range(2):
                for k in range(2):
                    v = gsm_ref[2 * cv + k].astype(f32)
                    for g in range(G):
                        gb_ref[cv, k, :, g * 128:(g + 1) * 128] = jnp.broadcast_to(v[g:g + 1, :], (8, 128))
            e_ref[...] = jnp.zeros(e_ref.shape, f32)
            st_ref[...] = jnp.zeros(st_ref.shape, f32)

            def xs0(c, _):
                x0_copy(c).wait()
                return xstat_tile(0, c)
            lax.fori_loop(0, T, xs0, 0)
            finalize(st_ref, p_ref, gb_ref, e_ref, 0)

            PU = opts.get('pu', 4)

            def prod0(c2, _):
                for i in range(PU):
                    cb = c2 * PU + i
                    pvc = tuple(p_ref[0, k, :, gcols(cb)] for k in range(2))
                    for pc in prod_list(cb):
                        if pc[0] == 'a':
                            prod_a(s_ref, pvc, ar_ref, xr_ref, 0, 0, cb, pc[2], None, i)
                        else:
                            prod_b(xr_ref, va_ref, cb, pc[2], pc[3], None, i)
                return 0
            lax.fori_loop(0, G // PU, prod0, 0)

            w1_copy(0).wait()
            lax.fori_loop(0, NUB // G, lambda k, _: (u_piece(w_ref, u1_ref, 0, k, None), 0)[1], 0, unroll=opts.get('uu', 4))

        def step0(n, _):
            if PEEL0:
                w1_copy(n + 1).wait()
            else:
                @pl.when(n < G - 1)
                def _():
                    w1_copy(n + 1).wait()
            nhalf(0, n, va_ref, vb_ref, ya_ref, yb_ref)
            return 0

        def step1(n, _):
            nhalf(1, n, vb_ref, va_ref, yb_ref, ya_ref)
            return 0

        with scope('step0'):
            if PEEL0:
                lax.fori_loop(0, G - 1, step0, 0)
                if EMB0:
                    we_copy().wait()
                nhalf(0, G - 1, va_ref, vb_ref, ya_ref, yb_ref, False)
            else:
                lax.fori_loop(0, G, step0, 0)
        with scope('step1'):
            x1_copy().wait()
            lax.fori_loop(0, G, step1, 0)

        def emb_block():
            w2_copy().wait()
            if not EMB0:
                we_copy().wait()
                emb_part()

        def body(it, carry):
            @pl.when(it == 1)
            def _():
                emb_block()

            @pl.when(it == T)
            def _():
                if UMODE == 0:
                    def cp(rb, _):
                        rows = pl.ds(pl.multiple_of(rb * 32, 32), 32)
                        for k in range(NPT):
                            u1_ref[k][rows, :] = u2_ref[k, rows, :]
                        return 0
                    lax.fori_loop(0, C // 2 // 32, cp, 0)
                else:
                    lax.fori_loop(0, NUB, lambda k, _: (u_piece(w_ref, u1_ref, 9, k, None), 0)[1], 0)
            with scope('iter'):
                half(it, 0, u1_ref, va_ref, vb_ref, ya_ref, yb_ref)
                half(it, 1, u1_ref, vb_ref, va_ref, yb_ref, ya_ref)
            return carry

        def body_c(conv):
            def f(it, carry):
                if conv == 0:
                    @pl.when(it == 1)
                    def _():
                        emb_block()
                ur = u2_ref if conv == 1 else u1_ref
                with scope('iter'):
                    half(it, 0, ur, va_ref, vb_ref, ya_ref, yb_ref, conv)
                    half(it, 1, ur, vb_ref, va_ref, yb_ref, ya_ref, conv)
                return carry
            return f

        with scope('main'):
            if SPLIT:
                if SPLIT == 2:
                    emb_block()
                lax.fori_loop(1, T, body_c(0 if SPLIT == 1 else 2), 0)
                lax.fori_loop(T, 2 * T, body_c(1), 0)
            else:
                lax.fori_loop(1, 2 * T, body, 0)

        sl_ = NSTEP - 1
        with scope('final'):
            st = [None] * NPW
            for r in range(TR):
                for cb in range(NPW):
                    st[cb] = epi_piece(yb_ref, sl_, 2, r, cb, st[cb], None)
                if ((r + 1) * W) % QR == 0:
                    o_copy(sl_, ((r + 1) * W) // QR - 1).start()
        with scope('owait'):
            o_all().wait()

    def fn(x, t_emb, g1, be1, w1, w_emb, g2, be2, w2):
        xn = jnp.transpose(x, (0, 2, 3, 1)).reshape(B, HW, C)
        w1t = jnp.transpose(w1, (2, 3, 0, 1)).reshape(9, C, C)
        w2t = jnp.transpose(w2, (2, 3, 0, 1)).reshape(9, C, C)
        any_spec = pl.BlockSpec(memory_space=pl.ANY)
        ubuf = pltpu.VMEM((C // 2, C), u32)
        vbuf = pltpu.VMEM((NPT, M // 2, C), u32)
        ybuf = pltpu.VMEM((2, 2, G, 2 * M, 128), f32)
        out = pl.pallas_call(
            kern,
            in_specs=[any_spec] * 9,
            out_specs=any_spec,
            out_shape=jax.ShapeDtypeStruct((B, HW, C), bf16),
            scratch_shapes=[
                pltpu.VMEM((4, HW, C), bf16),
                pltpu.VMEM((18, C, C), bf16),
                pltpu.VMEM((NPT, (C // 2 + UB // 2) if UMODE == 0 else 8, C), u32),
                pltpu.VMEM((G, NAR, 2, HP, 128), f32),
                pltpu.VMEM((G, TR + 2, NB, NQ4, 128), f32),
                vbuf, vbuf, ybuf, ybuf,
                pltpu.VMEM((4, T, 3, 8, C), f32),
                pltpu.VMEM((4, 2, 8, C), f32),
                pltpu.VMEM((2, 2, 8, C), f32),
                pltpu.VMEM((4, 8, C), f32),
                pltpu.VMEM((B, E), bf16),
                pltpu.VMEM((E, C), bf16),
                pltpu.VMEM((4, G, 128), bf16),
                pltpu.SemaphoreType.DMA((T,)),
                pltpu.SemaphoreType.DMA((G,)),
                pltpu.SemaphoreType.DMA((8,)),
                pltpu.SemaphoreType.DMA((1,)),
            ] + [ubuf] * NPT,
            compiler_params=pltpu.CompilerParams(vmem_limit_bytes=100 * 1024 * 1024,
                                                 disable_bounds_checks=True),
        )(xn, t_emb, g1.reshape(G, 128), be1.reshape(G, 128), w1t, w_emb,
          g2.reshape(G, 128), be2.reshape(G, 128), w2t)
        return jnp.transpose(out.reshape(B, H, W, C), (0, 3, 1, 2))
    return fn


_OPTS = {'last_slot': 62}


@jax.jit
def pallas_standalone__adm_resblock__diffusion_kernel(x, t_emb, g1, be1, w1, w_emb, g2, be2, w2):
    B, C, H, W = x.shape
    E = t_emb.shape[1]
    return build(B, C, H, W, E, TM=1024, opts=_OPTS)(x, t_emb, g1, be1, w1, w_emb, g2, be2, w2)
```

```python
import jax
import jax.numpy as jnp
from jax import lax
from jax.experimental import pallas as pl
from jax.experimental.pallas import tpu as pltpu

f32 = jnp.float32
bf16 = jnp.bfloat16
u32 = jnp.uint32
NT = (((1,), (1,)), ((), ()))


def build(B, C, H, W, E, TM=1024, opts=None):
    opts = opts or {}
    HW = H * W
    G = 4
    CG = C // G
    EPS = 1e-5
    T = HW // TM
    assert CG == 128 and B == 2 and T == 4 and W == 64 and H == 64
    TR = TM // W
    NP = TR // 2
    HP = W // 2
    NQ4 = W // 4
    M = NP * NQ4
    NB = 6
    NPT = 4 * NB
    NSTEP = 4 * T
    scope = jax.named_scope

    PW = opts.get('pw', 256)
    NPW = C // PW
    SUB = opts.get('sub', 8)
    XR = opts.get('xr', 128)
    NXR = TM // XR
    last_slot = opts.get('last_slot', 62)
    NQ = opts.get('nq', 4)
    QR = TM // NQ
    UMODE = opts.get('umode', 0)
    XMODE = opts.get('xmode', 0)
    NAR = opts.get('nar', 2)
    XC = opts.get('xc', 2)
    LAG = opts.get('lag', 2)
    P0 = opts.get('p0', 1)
    EMB0 = opts.get('emb0', 1)
    SPLIT = opts.get('split', 2)
    PEEL0 = opts.get('peel0', 1)
    WH, W4, W5A, W5B = (opts.get(k_, v_) for k_, v_ in (('wh', 130), ('w4', 40), ('w5a', 80), ('w5b', 30)))
    BG = opts.get('bg', 3)
    NSUB = opts.get('nsub', 8)
    XR1 = opts.get('xr1', 32)
    UB = 16
    NUB = (C // UB) * G

    def mult(v, m):
        return v if isinstance(v, int) else pl.multiple_of(v, m)

    def divT(v):
        return v // T if isinstance(v, int) else lax.shift_right_logical(v, 2)

    def modT(v):
        return v % T if isinstance(v, int) else jnp.bitwise_and(v, T - 1)

    def marker_of(d, n, sub, width):
        rp = sub * (d.shape[0] // SUB) // 8 * 8
        m = d[rp:rp + 8, n * 128:(n + 1) * 128]
        b = pltpu.bitcast(m, u32)
        z = pltpu.bitcast((b >> 16) >> 16, f32)
        if width > 128:
            z = jnp.concatenate([z] * (width // 128), axis=1)
        return z

    def pack2(t):
        n = t.shape[0] // 2
        return pltpu.pack_elementwise([t[:n], t[n:]], packed_dtype=bf16)

    def lanes(cb, width=128):
        if isinstance(cb, int):
            return slice(cb * width, (cb + 1) * width)
        return pl.ds(pl.multiple_of(cb * width, width), width)

    def load_y(y_ref, par, eo, j, cb0, ncb):
        parts = [y_ref[par, eo, cb0 + i, j * HP:(j + 1) * HP, :] for i in range(ncb)]
        return parts[0] if ncb == 1 else jnp.concatenate(parts, axis=1)

    def store_y(y_ref, par, q, n, val):
        y_ref[par, q % 2, n, pl.ds(q // 2, M, stride=2), :] = val

    def split_eo(v):
        w = pltpu.bitcast(v, u32)
        return (pltpu.unpack_elementwise(w, index=0, packed_dtype=bf16, unpacked_dtype=f32),
                pltpu.unpack_elementwise(w, index=1, packed_dtype=bf16, unpacked_dtype=f32))

    def join_eo(e, o):
        return pltpu.bitcast(pltpu.pack_elementwise([e, o], packed_dtype=bf16), bf16)

    def act(v, pv, marker):
        n, wd = v.shape
        sc, bt = pv
        if marker is not None:
            bt = bt + marker
        v3 = v.reshape(n // 8, 8, wd)
        hz = (v3 * sc[None] + bt[None]).reshape(n, wd)
        return hz * jnp.tanh(hz) + hz

    def act_row(s_ref, pv, q, y, cs, marker, edge):
        yc = y if not edge else jnp.clip(y, 0, H - 1)
        e, o = split_eo(s_ref[q, pl.ds(mult(yc * W, W), W), cs])
        e = act(e, pv, marker)
        o = act(o, pv, marker)
        if edge:
            valid = jnp.logical_and(y >= 0, y < H)
            e = jnp.where(valid, e, 0.0)
            o = jnp.where(valid, o, 0.0)
        return e, o

    def prod_a(s_ref, pv, ar_ref, xr_ref, q, y0, cb, i, marker, slot=0):
        cs = lanes(cb)
        cb = cb if isinstance(cb, int) else slot
        e, o = act_row(s_ref, pv, q, y0 - 1 + i, cs, marker, i == 0 or i == TR + 1)
        sl = i % NAR
        ar_ref[cb, sl, 0] = e
        ar_ref[cb, sl, 1] = o

        def col(eo, r):
            return jnp.concatenate([ar_ref[cb, sl, eo, pl.ds(r + 2 * u, NQ4 // 2, stride=4), :] for u in range(2)], axis=0)
        d1, d2, d3, d4 = col(0, 0), col(1, 0), col(0, 1), col(1, 1)
        hq = NQ4 // 2
        row = lax.broadcasted_iota(jnp.int32, (hq, 128), 0)
        d0 = jnp.concatenate([jnp.where(row == 0, 0.0, pltpu.roll(d4[hq:], 1, 0)), d4[:hq]], axis=0)
        d5 = jnp.concatenate([d1[hq:], jnp.where(row == hq - 1, 0.0, pltpu.roll(d1[:hq], hq - 1, 0))], axis=0)
        c = d4 - d2
        e2 = (d3 - d1) * 2.0
        a_ = d4 - d2 * 4.0
        b_ = d3 - d1 * 4.0
        xr_ref[cb, i, 0] = (d0 - d2) * 4.0 + c
        xr_ref[cb, i, 1] = a_ + b_
        xr_ref[cb, i, 2] = a_ - b_
        xr_ref[cb, i, 3] = c + e2
        xr_ref[cb, i, 4] = c - e2
        xr_ref[cb, i, 5] = (d5 - d3) - e2 * 2.0

    def prod_b(xr_ref, v_ref, cb, j, bs, marker, slot=0):
        cs = lanes(cb)
        cb = cb if isinstance(cb, int) else slot
        rs = pl.ds(j * (NQ4 // 2), NQ4 // 2)
        for b in bs:
            r0, r1, r2, r3 = (xr_ref[cb, 2 * j + i, b] for i in range(4))
            if marker is not None and (b == bs[0] or not opts.get('mk1')):
                r2 = (r2.reshape(NQ4 // 8, 8, 128) + marker[None]).reshape(NQ4, 128)
            v_ref[b, rs, cs] = pack2(r0 - r2)
            v_ref[NB + b, rs, cs] = pack2(r1 + r2)
            v_ref[2 * NB + b, rs, cs] = pack2(r2 - r1)
            v_ref[3 * NB + b, rs, cs] = pack2(r1 - r3)

    def prod_list(cb):
        pl_ = [('a', cb, 0), ('a', cb, 1)]
        for j in range(NP):
            pl_ += [('a', cb, 2 * j + 2), ('a', cb, 2 * j + 3)]
            pl_ += [('b', cb, j, tuple(range(b, b + BG))) for b in range(0, NB, BG)]
        return pl_

    def out_x(st, b, d):
        if b == 0:
            st['r0'] = d
        elif b in (1, 3):
            st['p'] = d
        elif b == 2:
            st['s12'], st['d12'] = st['p'] + d, st['p'] - d
            st['r0'] = st['r0'] + st['s12']
        elif b == 4:
            s34, d34 = st['p'] + d, st['p'] - d
            st['r0'] = st['r0'] + s34
            st['r1'] = st['d12'] + d34 * 2.0
            st['r2'] = st['s12'] + s34 * 4.0
            st['r3'] = st['d12'] + d34 * 8.0
        else:
            return [st['r0'], st['r1'], st['r2'], st['r3'] + d]
        return None

    def out_y(ys, a, rr, store):
        for q in range(4):
            if a == 0:
                ys[q] = rr[q]
            elif a == 1:
                ys[q] = ys[q] + rr[q]
                ys[4 + q] = rr[q]
            elif a == 2:
                store(0, q, ys[q] + rr[q])
                ys[4 + q] = ys[4 + q] - rr[q]
            else:
                store(1, q, ys[4 + q] - rr[q])

    def u_piece(w_ref, u_ref, base, k, marker, ok=None):
        rb = lax.shift_right_logical(k, 2) if not isinstance(k, int) else k // 4
        cb = jnp.bitwise_and(k, 3) if not isinstance(k, int) else k % 4
        rows = pl.ds(mult(rb * UB, UB), UB)
        ob = rb if ok is None else jnp.where(ok, rb, C // UB)
        orow = pl.ds(mult(ob * (UB // 2), UB // 2), UB // 2)
        cs = pl.ds(mult(cb * 128, 128), 128)
        res = []
        raw = [[split_eo(w_ref[base + 3 * i + j, rows, cs]) for j in range(3)] for i in range(3)]
        for par in range(2):
            hs = []
            for j in range(3):
                g0, g1, g2 = (raw[i][j][par] for i in range(3))
                if marker is not None:
                    g1 = g1 + marker
                sm = g0 + g2
                hs.append((g0, sm + g1, sm - g1, g2))
            out = [None] * NPT
            for a in range(4):
                cy = 0.5 if a in (1, 2) else 1.0
                h0, h1, h2 = (hs[j][a] for j in range(3))
                sm = h0 + h2
                pp = h0 * (cy / 24.0) + h2 * (cy / 6.0)
                qq = h1 * (cy / 12.0)
                for b, val in enumerate((h0 * (cy / 4.0), (sm + h1) * (-cy / 6.0), (sm - h1) * (-cy / 6.0),
                                         pp + qq, pp - qq, h2 if cy == 1.0 else h2 * cy)):
                    out[NB * a + b] = val
            res.append(out)
        for k2 in range(NPT):
            val = pltpu.pack_elementwise([res[0][k2], res[1][k2]], packed_dtype=bf16)
            if isinstance(u_ref, (list, tuple)):
                u_ref[k2][orow, cs] = val
            else:
                u_ref[k2, orow, cs] = val

    def stat_acc(v, state, marker=None):
        n = v.shape[0] // 8
        wd = v.shape[1]
        if state is None:
            K = v[0:1, :]
            if marker is not None:
                K = K + marker[0:1, :]
            d = v - K
            return (K, d.reshape(n, 8, wd).sum(axis=0), (d * d).reshape(n, 8, wd).sum(axis=0))
        K, s1, s2 = state
        Kd = K if marker is None else K + marker[0:1, :]
        d = v - Kd
        return (K, s1 + d.reshape(n, 8, wd).sum(axis=0), s2 + (d * d).reshape(n, 8, wd).sum(axis=0))

    def store_stats(st_ref, q, t, cs, state):
        K, s1, s2 = state
        wd = K.shape[1]
        st_ref[q, t, 0, :, cs] = jnp.broadcast_to(K, (8, wd))
        st_ref[q, t, 1, :, cs] = jnp.broadcast_to(s1.sum(axis=0, keepdims=True), (8, wd))
        st_ref[q, t, 2, :, cs] = jnp.broadcast_to(s2.sum(axis=0, keepdims=True), (8, wd))

    def finalize(st_ref, p_ref, gb_ref, e_ref, q):
        cv = q // 2 if isinstance(q, int) else lax.shift_right_logical(q, 1)
        for g in range(G):
            cs = slice(g * 128, (g + 1) * 128)
            K = st_ref[q, :, 0, :, cs]
            s1 = st_ref[q, :, 1, :, cs]
            s2 = st_ref[q, :, 2, :, cs]
            e = e_ref[q, :, cs]
            mean_t = K + s1 * (1.0 / TM) + e[None]
            m2_t = s2 - s1 * s1 * (1.0 / TM)
            mu = jnp.sum(jnp.sum(mean_t, axis=0), axis=1, keepdims=True) * (1.0 / (T * 128))
            dev = mean_t - mu[None]
            tot = m2_t + dev * dev * float(TM)
            var = jnp.sum(jnp.sum(tot, axis=0), axis=1, keepdims=True) * (1.0 / (HW * 128))
            rstd = lax.rsqrt(var + EPS)
            sc = gb_ref[cv, 0, :, cs] * (rstd * 0.5)
            p_ref[q, 0, :, cs] = sc
            p_ref[q, 1, :, cs] = gb_ref[cv, 1, :, cs] * 0.5 - (mu - e) * sc

    def merge(lists):
        items = []
        for li, l in enumerate(lists):
            for i, it in enumerate(l):
                items.append(((i + 0.5) / len(l), li, it))
        items.sort(key=lambda z: (z[0], z[1]))
        return [it for _, _, it in items]

    def kern(x_hbm, te_hbm, g1_hbm, b1_hbm, w1_hbm, we_hbm, g2_hbm, b2_hbm, w2_hbm, o_hbm,
             s_ref, w_ref, u2_ref, ar_ref, xr_ref, va_ref, vb_ref, ya_ref, yb_ref,
             st_ref, p_ref, gb_ref, e_ref, te_ref, we_ref, gsm_ref, sem_x, sem_w, sem_s, sem_o, *u1_ref):

        def gcols(g):
            return pl.ds(mult(g * 128, 128), 128)

        def x0_copy(c):
            rows = pl.ds(mult(c * (TM // XC), TM // XC), TM // XC)
            return pltpu.make_async_copy(x_hbm.at[0, rows, :], s_ref.at[0, rows, :], sem_x.at[c])

        def w1_copy(g):
            return pltpu.make_async_copy(w1_hbm.at[:, gcols(g), :], w_ref.at[pl.ds(0, 9), gcols(g), :], sem_w.at[g])

        def x1_copy():
            return pltpu.make_async_copy(x_hbm.at[1], s_ref.at[1], sem_s.at[6])

        def w2_copy():
            return pltpu.make_async_copy(w2_hbm, w_ref.at[pl.ds(9, 9)], sem_s.at[7])

        def small_copies():
            return [pltpu.make_async_copy(g1_hbm, gsm_ref.at[0], sem_s.at[0]),
                    pltpu.make_async_copy(b1_hbm, gsm_ref.at[1], sem_s.at[1]),
                    pltpu.make_async_copy(g2_hbm, gsm_ref.at[2], sem_s.at[2]),
                    pltpu.make_async_copy(b2_hbm, gsm_ref.at[3], sem_s.at[3]),
                    pltpu.make_async_copy(te_hbm, te_ref, sem_s.at[4])]

        def we_copy():
            return pltpu.make_async_copy(we_hbm, we_ref, sem_s.at[5])

        def o_copy(s, qi):
            b = divT(s) - 2
            r0 = mult(modT(s) * TM + qi * QR, QR)
            return pltpu.make_async_copy(s_ref.at[b, pl.ds(r0, QR), :], o_hbm.at[b, pl.ds(r0, QR), :], sem_o.at[0])

        def o_all():
            return pltpu.make_async_copy(s_ref.at[pl.ds(0, B)], o_hbm, sem_o.at[0])

        def epi_piece(y_ref, s_prev, kind, r, cb, state, marker, PW=PW):
            p = divT(s_prev)
            t = modT(s_prev)
            cs = lanes(cb, PW)
            j, par = r // 2, r % 2
            r0 = mult(t * TM + r * W, W)
            ve = load_y(y_ref, par, 0, j, cb * (PW // 128), PW // 128)
            vo = load_y(y_ref, par, 1, j, cb * (PW // 128), PW // 128)
            if marker is not None:
                ve = (ve.reshape(HP // 8, 8, PW) + marker[None]).reshape(HP, PW)
            if kind == 1:
                dst, sq = p + 2, p + 2
            elif kind == 2:
                dst, sq = p - 2, None
                xe, xo = split_eo(s_ref[dst, pl.ds(r0, W), cs])
                ve, vo = ve + xe, vo + xo
            else:
                is2 = p >= 2
                dst = jnp.where(is2, p - 2, p + 2)
                sq = jnp.where(is2, 0, p + 2)
                xe, xo = split_eo(s_ref[dst, pl.ds(r0, W), cs])
                ve, vo = ve + jnp.where(is2, xe, 0.0), vo + jnp.where(is2, xo, 0.0)
            if sq is not None:
                state = stat_acc(vo, stat_acc(ve, state))
            s_ref[dst, pl.ds(r0, W), cs] = join_eo(ve, vo)
            if sq is not None and r == TR - 1:
                store_stats(st_ref, sq, t, cs, state)
                state = None
            return state

        def xstat_piece(q, tile, cs, ri, state, marker):
            r0 = mult(tile * TM + ri * XR1, XR1)
            v = s_ref[q, pl.ds(r0, XR1), cs].astype(f32)
            state = stat_acc(v, state, marker)
            if ri == TM // XR1 - 1:
                store_stats(st_ref, q, tile, cs, state)
                state = None
            return state

        def half(it, second, u_ref, vc_ref, vn_ref, yc_ref, yp_ref, conv=None):
            s = 2 * it + second
            sn = s + 1
            pn = jnp.minimum(divT(sn), 3)
            y0 = modT(sn) * TR
            plist = [pc for cb in range(G) for pc in prod_list(cb)]
            lists = [plist,
                     [('e', r, cb) for r in range(TR) for cb in range(NPW)]]
            NU = -(-NUB // (5 if conv is None else 6))
            if UMODE == 0 and conv != 1:
                lists.append([('u', k) for k in range(NU)])
            pieces = merge(lists)
            npc = len(pieces)
            if second == 1:
                finalize(st_ref, p_ref, gb_ref, e_ref, jnp.minimum(divT(s - 1) + 1, 3))
            pv = tuple(p_ref[pn, k] for k in range(2))
            sp = s - 1
            ekind = 0 if conv is None else (1 if conv in (0, 2) else (0 if second == 0 else 2))
            wts = [{0: WH, 1: WH, 2: 100, 3: WH, 4: W4, 5: W5A if k // NB < 2 else W5B}[k % NB] for k in range(NPT)]
            cum = [sum(wts[:k]) for k in range(NPT + 1)]
            done = 0
            est = [None] * NPW
            xst = None
            pcar = None
            ys = [None] * 8
            for a in range(4):
                st = {}
                for b in range(NB):
                    k = NB * a + b
                    d = lax.dot_general(pltpu.bitcast(vc_ref[k], bf16), pltpu.bitcast(u_ref[k][...] if conv != 1 else u_ref[k, 0:C // 2, :], bf16), NT,
                                        preferred_element_type=f32)
                    for nn in range(4 * SUB):
                        n, sub = nn // SUB, nn % SUB
                        hi_ = min(npc, ((cum[k] * 4 * SUB + wts[k] * (nn + 1)) * npc * 64) // (last_slot * cum[NPT] * 4 * SUB))
                        while done < hi_:
                            pc = pieces[done]
                            if pc[0] == 'a':
                                cs = slice(pc[1] * 128, (pc[1] + 1) * 128)
                                prod_a(s_ref, tuple(t[:, cs] for t in pv), ar_ref, xr_ref, pn, y0, pc[1], pc[2],
                                       marker_of(d, n, sub, 128))
                            elif pc[0] == 'b':
                                prod_b(xr_ref, vn_ref, pc[1], pc[2], pc[3], marker_of(d, n, sub, 128))
                            elif pc[0] == 'e':
                                est[pc[2]] = epi_piece(yp_ref, sp, ekind, pc[1], pc[2], est[pc[2]],
                                                       marker_of(d, n, sub, PW))
                                if pc[2] == NPW - 1 and ((pc[1] + 1) * W) % QR == 0 and conv not in (0, 2):
                                    qi = ((pc[1] + 1) * W) // QR - 1

                                    @pl.when(sp >= 2 * T)
                                    def _():
                                        o_copy(sp, qi).start()
                            elif pc[0] == 'x':
                                xst = xstat_piece(jnp.where(it == 0, 0, 1), pc[1],
                                                  slice(pc[2] * PW, (pc[2] + 1) * PW), pc[3], xst,
                                                  marker_of(d, n, sub, PW))
                            else:
                                kk = (s - 2) * NU + pc[1]
                                ok = jnp.logical_and(kk >= 0, kk < NUB)
                                u_piece(w_ref, u2_ref, 9, jnp.clip(kk, 0, NUB - 1),
                                        marker_of(d, n, sub, 128), ok)
                            done += 1
                    rr = out_x(st, b, d)

                def store(par, q, val):
                    for n in range(G):
                        store_y(yc_ref, par, q, n, val[:, n * 128:(n + 1) * 128])
                out_y(ys, a, rr, store)

        def emb_part():
            te = te_ref[...].astype(f32)
            sl = te * jax.nn.sigmoid(te)
            emb = jnp.dot(sl.astype(bf16), we_ref[...], preferred_element_type=f32)
            e_ref[2] = jnp.broadcast_to(emb[0:1, :], (8, C))
            e_ref[3] = jnp.broadcast_to(emb[1:2, :], (8, C))

        def nhalf(step, n, vc_ref, vn_ref, yc_ref, yp_ref, with_u=True):
            y0 = (step + 1) * TR
            if step == 0 and P0 == 1:
                lists = [] if with_u else [[pc for cb in range(G) for pc in prod_list(cb)]]
            else:
                lists = [prod_list(None)]
            if step == 0:
                if with_u:
                    lists.append([('u', k) for k in range(NUB // G)])
            else:
                lists.append([('e', r) for r in range(TR)])
                lists.append([('x', cb, ri) for cb in range(NPW) for ri in range(TM // XR1)])
            pieces = merge(lists)
            npc = len(pieces)
            cs = lanes(n)
            pvc = tuple(p_ref[0, k, :, cs] for k in range(2))
            urows = pl.ds(mult(n * (128 // 2), 128 // 2), 128 // 2)
            gn = n + 1 if PEEL0 else jnp.minimum(n + 1, G - 1)
            NS = NSUB
            done = 0
            est = xst = None
            ys = [None] * 8
            dhist = []
            for a in range(4):
                st = {}
                for b in range(NB):
                    k = NB * a + b
                    d = lax.dot_general(pltpu.bitcast(vc_ref[k], bf16), pltpu.bitcast(u1_ref[k][urows, :], bf16), NT,
                                        preferred_element_type=f32)
                    for sub in range(NS):
                        lag = LAG if with_u and step == 0 else 1
                        hi_ = npc if k == NPT - 1 and sub == NS - 1 else (((k - lag + 1) * NS + sub) * npc) // ((NPT - lag) * NS)
                        dprev = dhist[k - lag] if k >= lag else None
                        while done < min(hi_, npc) and dprev is not None:
                            pc = pieces[done]
                            rp = sub * (M // NS) // 8 * 8
                            bits = pltpu.bitcast(dprev[rp:rp + 8, :], u32)
                            mk = pltpu.bitcast((bits >> 16) >> 16, f32)
                            if pc[0] == 'a':
                                cbp = n if pc[1] is None else pc[1]
                                pvp = pvc if pc[1] is None else tuple(p_ref[0, k_, :, lanes(cbp)] for k_ in range(2))
                                prod_a(s_ref, pvp, ar_ref, xr_ref, 0, y0, cbp, pc[2], mk)
                            elif pc[0] == 'b':
                                prod_b(xr_ref, vn_ref, n if pc[1] is None else pc[1], pc[2], pc[3], mk)
                            elif pc[0] == 'u':
                                u_piece(w_ref, u1_ref, 0, gn * (NUB // G) + pc[1], mk)
                            elif pc[0] == 'e':
                                est = epi_piece(yp_ref, 0, 1, pc[1], n, est, mk, PW=128)
                            else:
                                mkx = mk if PW == 128 else jnp.concatenate([mk] * (PW // 128), axis=1)
                                xst = xstat_piece(1, n, slice(pc[1] * PW, (pc[1] + 1) * PW), pc[2], xst, mkx)
                            done += 1
                    dhist.append(d)
                    rr = out_x(st, b, d)
                out_y(ys, a, rr, lambda par, q, val: store_y(yc_ref, par, q, n, val))
            assert done == npc
            if step == 0 and not with_u and EMB0:
                emb_part()

        def xstat_tile0(c):
            st = [None] * NPW
            rows_per = TM // XC
            for h in range(XC):
                x0_copy(c * XC + h).wait()
                for ri in range(rows_per // XR):
                    r0 = pl.multiple_of(c * TM + h * rows_per + ri * XR, XR)
                    for cb in range(NPW):
                        v = s_ref[0, pl.ds(r0, XR), cb * PW:(cb + 1) * PW].astype(f32)
                        st[cb] = stat_acc(v, st[cb])
            for cb in range(NPW):
                store_stats(st_ref, 0, c, slice(cb * PW, (cb + 1) * PW), st[cb])
            return 0

        with scope('prologue'):
            for c in small_copies():
                c.start()
            lax.fori_loop(0, T * XC, lambda c, _: (x0_copy(c).start(), 0)[1], 0)
            lax.fori_loop(0, G, lambda g, _: (w1_copy(g).start(), 0)[1], 0)

            def rest(c, _):
                @pl.when(c == (1 if EMB0 else 0))
                def _():
                    x1_copy().start()

                @pl.when(c == (2 if EMB0 else 1))
                def _():
                    w2_copy().start()

                @pl.when(c == (0 if EMB0 else 2))
                def _():
                    we_copy().start()
                return 0
            lax.fori_loop(0, 3, rest, 0)

            for c in small_copies():
                c.wait()
            for cv in range(2):
                for k in range(2):
                    v = gsm_ref[2 * cv + k].astype(f32)
                    for g in range(G):
                        gb_ref[cv, k, :, g * 128:(g + 1) * 128] = jnp.broadcast_to(v[g:g + 1, :], (8, 128))
            e_ref[...] = jnp.zeros(e_ref.shape, f32)
            st_ref[...] = jnp.zeros(st_ref.shape, f32)

            lax.fori_loop(0, T, lambda c, _: xstat_tile0(c), 0)
            finalize(st_ref, p_ref, gb_ref, e_ref, 0)

            PU = opts.get('pu', 4)

            def prod0(c2, _):
                for i in range(PU):
                    cb = c2 * PU + i
                    pvc = tuple(p_ref[0, k, :, gcols(cb)] for k in range(2))
                    for pc in prod_list(cb):
                        if pc[0] == 'a':
                            prod_a(s_ref, pvc, ar_ref, xr_ref, 0, 0, cb, pc[2], None, i)
                        else:
                            prod_b(xr_ref, va_ref, cb, pc[2], pc[3], None, i)
                return 0
            lax.fori_loop(0, G // PU, prod0, 0)

            w1_copy(0).wait()
            lax.fori_loop(0, NUB // G, lambda k, _: (u_piece(w_ref, u1_ref, 0, k, None), 0)[1], 0, unroll=opts.get('uu', 4))

        def step0(n, _):
            if PEEL0:
                w1_copy(n + 1).wait()
            else:
                @pl.when(n < G - 1)
                def _():
                    w1_copy(n + 1).wait()
            nhalf(0, n, va_ref, vb_ref, ya_ref, yb_ref)
            return 0

        def step1(n, _):
            nhalf(1, n, vb_ref, va_ref, yb_ref, ya_ref)
            return 0

        with scope('step0'):
            if PEEL0:
                lax.fori_loop(0, G - 1, step0, 0)
                if EMB0:
                    we_copy().wait()
                nhalf(0, G - 1, va_ref, vb_ref, ya_ref, yb_ref, False)
            else:
                lax.fori_loop(0, G, step0, 0)
        with scope('step1'):
            x1_copy().wait()
            lax.fori_loop(0, G, step1, 0)

        def emb_block():
            w2_copy().wait()
            if not EMB0:
                we_copy().wait()
                emb_part()

        def body(it, carry):
            @pl.when(it == 1)
            def _():
                emb_block()

            @pl.when(it == T)
            def _():
                if UMODE == 0:
                    def cp(rb, _):
                        rows = pl.ds(pl.multiple_of(rb * 32, 32), 32)
                        for k in range(NPT):
                            u1_ref[k][rows, :] = u2_ref[k, rows, :]
                        return 0
                    lax.fori_loop(0, C // 2 // 32, cp, 0)
                else:
                    lax.fori_loop(0, NUB, lambda k, _: (u_piece(w_ref, u1_ref, 9, k, None), 0)[1], 0)
            with scope('iter'):
                half(it, 0, u1_ref, va_ref, vb_ref, ya_ref, yb_ref)
                half(it, 1, u1_ref, vb_ref, va_ref, yb_ref, ya_ref)
            return carry

        def body_c(conv):
            def f(it, carry):
                if conv == 0:
                    @pl.when(it == 1)
                    def _():
                        emb_block()
                ur = u2_ref if conv == 1 else u1_ref
                with scope('iter'):
                    half(it, 0, ur, va_ref, vb_ref, ya_ref, yb_ref, conv)
                    half(it, 1, ur, vb_ref, va_ref, yb_ref, ya_ref, conv)
                return carry
            return f

        with scope('main'):
            if SPLIT:
                if SPLIT == 2:
                    emb_block()
                lax.fori_loop(1, T, body_c(0 if SPLIT == 1 else 2), 0)
                lax.fori_loop(T, 2 * T, body_c(1), 0)
            else:
                lax.fori_loop(1, 2 * T, body, 0)

        sl_ = NSTEP - 1
        with scope('final'):
            st = [None] * NPW
            for r in range(TR):
                for cb in range(NPW):
                    st[cb] = epi_piece(yb_ref, sl_, 2, r, cb, st[cb], None)
                if ((r + 1) * W) % QR == 0:
                    o_copy(sl_, ((r + 1) * W) // QR - 1).start()
        with scope('owait'):
            o_all().wait()

    def fn(x, t_emb, g1, be1, w1, w_emb, g2, be2, w2):
        xn = jnp.transpose(x, (0, 2, 3, 1)).reshape(B, HW, C)
        w1t = jnp.transpose(w1, (2, 3, 0, 1)).reshape(9, C, C)
        w2t = jnp.transpose(w2, (2, 3, 0, 1)).reshape(9, C, C)
        any_spec = pl.BlockSpec(memory_space=pl.ANY)
        ubuf = pltpu.VMEM((C // 2, C), u32)
        vbuf = pltpu.VMEM((NPT, M // 2, C), u32)
        ybuf = pltpu.VMEM((2, 2, G, 2 * M, 128), f32)
        out = pl.pallas_call(
            kern,
            in_specs=[any_spec] * 9,
            out_specs=any_spec,
            out_shape=jax.ShapeDtypeStruct((B, HW, C), bf16),
            scratch_shapes=[
                pltpu.VMEM((4, HW, C), bf16),
                pltpu.VMEM((18, C, C), bf16),
                pltpu.VMEM((NPT, (C // 2 + UB // 2) if UMODE == 0 else 8, C), u32),
                pltpu.VMEM((G, NAR, 2, HP, 128), f32),
                pltpu.VMEM((G, TR + 2, NB, NQ4, 128), f32),
                vbuf, vbuf, ybuf, ybuf,
                pltpu.VMEM((4, T, 3, 8, C), f32),
                pltpu.VMEM((4, 2, 8, C), f32),
                pltpu.VMEM((2, 2, 8, C), f32),
                pltpu.VMEM((4, 8, C), f32),
                pltpu.VMEM((B, E), bf16),
                pltpu.VMEM((E, C), bf16),
                pltpu.VMEM((4, G, 128), bf16),
                pltpu.SemaphoreType.DMA((T * XC,)),
                pltpu.SemaphoreType.DMA((G,)),
                pltpu.SemaphoreType.DMA((8,)),
                pltpu.SemaphoreType.DMA((1,)),
            ] + [ubuf] * NPT,
            compiler_params=pltpu.CompilerParams(vmem_limit_bytes=100 * 1024 * 1024,
                                                 disable_bounds_checks=True),
        )(xn, t_emb, g1.reshape(G, 128), be1.reshape(G, 128), w1t, w_emb,
          g2.reshape(G, 128), be2.reshape(G, 128), w2t)
        return jnp.transpose(out.reshape(B, H, W, C), (0, 3, 1, 2))
    return fn


_OPTS = {}


@jax.jit
def pallas_standalone__adm_resblock__diffusion_kernel(x, t_emb, g1, be1, w1, w_emb, g2, be2, w2):
    B, C, H, W = x.shape
    E = t_emb.shape[1]
    return build(B, C, H, W, E, TM=1024, opts=_OPTS)(x, t_emb, g1, be1, w1, w_emb, g2, be2, w2)
```

```python
import jax
import jax.numpy as jnp
from jax import lax
from jax.experimental import pallas as pl
from jax.experimental.pallas import tpu as pltpu

f32 = jnp.float32
bf16 = jnp.bfloat16
u32 = jnp.uint32
NT = (((1,), (1,)), ((), ()))


def build(B, C, H, W, E, TM=1024, opts=None):
    opts = opts or {}
    HW = H * W
    G = 4
    CG = C // G
    EPS = 1e-5
    T = HW // TM
    assert CG == 128 and B == 2 and T == 4 and W == 64 and H == 64
    TR = TM // W
    NP = TR // 2
    HP = W // 2
    NQ4 = W // 4
    M = NP * NQ4
    NB = 6
    NPT = 4 * NB
    NSTEP = 4 * T
    scope = jax.named_scope

    PW = opts.get('pw', 256)
    NPW = C // PW
    SUB = opts.get('sub', 8)
    XR = opts.get('xr', 128)
    NXR = TM // XR
    last_slot = opts.get('last_slot', 62)
    NQ = opts.get('nq', 4)
    QR = TM // NQ
    UMODE = opts.get('umode', 0)
    XMODE = opts.get('xmode', 0)
    NAR = opts.get('nar', 2)
    FROW = opts.get('frow', 1)
    XC = opts.get('xc', 2)
    LAG = opts.get('lag', 2)
    P0 = opts.get('p0', 1)
    EMB0 = opts.get('emb0', 1)
    SPLIT = opts.get('split', 2)
    PEEL0 = opts.get('peel0', 1)
    WH, W4, W5A, W5B = (opts.get(k_, v_) for k_, v_ in (('wh', 130), ('w4', 40), ('w5a', 80), ('w5b', 30)))
    BG = opts.get('bg', 3)
    NSUB = opts.get('nsub', 8)
    XR1 = opts.get('xr1', 32)
    UB = 16
    NUB = (C // UB) * G

    def mult(v, m):
        return v if isinstance(v, int) else pl.multiple_of(v, m)

    def divT(v):
        return v // T if isinstance(v, int) else lax.shift_right_logical(v, 2)

    def modT(v):
        return v % T if isinstance(v, int) else jnp.bitwise_and(v, T - 1)

    def marker_of(d, n, sub, width):
        rp = sub * (d.shape[0] // SUB) // 8 * 8
        m = d[rp:rp + 8, n * 128:(n + 1) * 128]
        b = pltpu.bitcast(m, u32)
        z = pltpu.bitcast((b >> 16) >> 16, f32)
        if width > 128:
            z = jnp.concatenate([z] * (width // 128), axis=1)
        return z

    def pack2(t):
        n = t.shape[0] // 2
        return pltpu.pack_elementwise([t[:n], t[n:]], packed_dtype=bf16)

    def lanes(cb, width=128):
        if isinstance(cb, int):
            return slice(cb * width, (cb + 1) * width)
        return pl.ds(pl.multiple_of(cb * width, width), width)

    def load_y(y_ref, par, eo, j, cb0, ncb):
        parts = [y_ref[par, eo, cb0 + i, j * HP:(j + 1) * HP, :] for i in range(ncb)]
        return parts[0] if ncb == 1 else jnp.concatenate(parts, axis=1)

    def store_y(y_ref, par, q, n, val):
        y_ref[par, q % 2, n, pl.ds(q // 2, M, stride=2), :] = val

    def split_eo(v):
        w = pltpu.bitcast(v, u32)
        return (pltpu.unpack_elementwise(w, index=0, packed_dtype=bf16, unpacked_dtype=f32),
                pltpu.unpack_elementwise(w, index=1, packed_dtype=bf16, unpacked_dtype=f32))

    def join_eo(e, o):
        return pltpu.bitcast(pltpu.pack_elementwise([e, o], packed_dtype=bf16), bf16)

    def act(v, pv, marker):
        n, wd = v.shape
        sc, bt = pv
        if marker is not None:
            bt = bt + marker
        v3 = v.reshape(n // 8, 8, wd)
        hz = (v3 * sc[None] + bt[None]).reshape(n, wd)
        return hz * jnp.tanh(hz) + hz

    def act_row(s_ref, pv, q, y, cs, marker, edge):
        yc = y if not edge else jnp.clip(y, 0, H - 1)
        e, o = split_eo(s_ref[q, pl.ds(mult(yc * W, W), W), cs])
        e = act(e, pv, marker)
        o = act(o, pv, marker)
        if edge:
            valid = jnp.logical_and(y >= 0, y < H)
            e = jnp.where(valid, e, 0.0)
            o = jnp.where(valid, o, 0.0)
        return e, o

    def prod_a(s_ref, pv, ar_ref, xr_ref, q, y0, cb, i, marker, slot=0):
        cs = lanes(cb)
        cb = cb if isinstance(cb, int) else slot
        e, o = act_row(s_ref, pv, q, y0 - 1 + i, cs, marker, i == 0 or i == TR + 1)
        sl = i % NAR
        ar_ref[cb, sl, 0] = e
        ar_ref[cb, sl, 1] = o

        def col(eo, r):
            return jnp.concatenate([ar_ref[cb, sl, eo, pl.ds(r + 2 * u, NQ4 // 2, stride=4), :] for u in range(2)], axis=0)
        d1, d2, d3, d4 = col(0, 0), col(1, 0), col(0, 1), col(1, 1)
        hq = NQ4 // 2
        row = lax.broadcasted_iota(jnp.int32, (hq, 128), 0)
        d0 = jnp.concatenate([jnp.where(row == 0, 0.0, pltpu.roll(d4[hq:], 1, 0)), d4[:hq]], axis=0)
        d5 = jnp.concatenate([d1[hq:], jnp.where(row == hq - 1, 0.0, pltpu.roll(d1[:hq], hq - 1, 0))], axis=0)
        c = d4 - d2
        e2 = (d3 - d1) * 2.0
        a_ = d4 - d2 * 4.0
        b_ = d3 - d1 * 4.0
        xr_ref[cb, i, 0] = (d0 - d2) * 4.0 + c
        xr_ref[cb, i, 1] = a_ + b_
        xr_ref[cb, i, 2] = a_ - b_
        xr_ref[cb, i, 3] = c + e2
        xr_ref[cb, i, 4] = c - e2
        xr_ref[cb, i, 5] = (d5 - d3) - e2 * 2.0

    def prod_b(xr_ref, v_ref, cb, j, bs, marker, slot=0):
        cs = lanes(cb)
        cb = cb if isinstance(cb, int) else slot
        rs = pl.ds(j * (NQ4 // 2), NQ4 // 2)
        for b in bs:
            r0, r1, r2, r3 = (xr_ref[cb, 2 * j + i, b] for i in range(4))
            if marker is not None and (b == bs[0] or not opts.get('mk1')):
                r2 = (r2.reshape(NQ4 // 8, 8, 128) + marker[None]).reshape(NQ4, 128)
            v_ref[b, rs, cs] = pack2(r0 - r2)
            v_ref[NB + b, rs, cs] = pack2(r1 + r2)
            v_ref[2 * NB + b, rs, cs] = pack2(r2 - r1)
            v_ref[3 * NB + b, rs, cs] = pack2(r1 - r3)

    def prod_list(cb):
        pl_ = [('a', cb, 0), ('a', cb, 1)]
        for j in range(NP):
            pl_ += [('a', cb, 2 * j + 2), ('a', cb, 2 * j + 3)]
            pl_ += [('b', cb, j, tuple(range(b, b + BG))) for b in range(0, NB, BG)]
        return pl_

    def out_x(st, b, d):
        if b == 0:
            st['r0'] = d
        elif b in (1, 3):
            st['p'] = d
        elif b == 2:
            st['s12'], st['d12'] = st['p'] + d, st['p'] - d
            st['r0'] = st['r0'] + st['s12']
        elif b == 4:
            s34, d34 = st['p'] + d, st['p'] - d
            st['r0'] = st['r0'] + s34
            st['r1'] = st['d12'] + d34 * 2.0
            st['r2'] = st['s12'] + s34 * 4.0
            st['r3'] = st['d12'] + d34 * 8.0
        else:
            return [st['r0'], st['r1'], st['r2'], st['r3'] + d]
        return None

    def out_y(ys, a, rr, store):
        for q in range(4):
            if a == 0:
                ys[q] = rr[q]
            elif a == 1:
                ys[q] = ys[q] + rr[q]
                ys[4 + q] = rr[q]
            elif a == 2:
                store(0, q, ys[q] + rr[q])
                ys[4 + q] = ys[4 + q] - rr[q]
            else:
                store(1, q, ys[4 + q] - rr[q])

    def u_piece(w_ref, u_ref, base, k, marker, ok=None):
        rb = lax.shift_right_logical(k, 2) if not isinstance(k, int) else k // 4
        cb = jnp.bitwise_and(k, 3) if not isinstance(k, int) else k % 4
        rows = pl.ds(mult(rb * UB, UB), UB)
        ob = rb if ok is None else jnp.where(ok, rb, C // UB)
        orow = pl.ds(mult(ob * (UB // 2), UB // 2), UB // 2)
        cs = pl.ds(mult(cb * 128, 128), 128)
        res = []
        raw = [[split_eo(w_ref[base + 3 * i + j, rows, cs]) for j in range(3)] for i in range(3)]
        for par in range(2):
            hs = []
            for j in range(3):
                g0, g1, g2 = (raw[i][j][par] for i in range(3))
                if marker is not None:
                    g1 = g1 + marker
                sm = g0 + g2
                hs.append((g0, sm + g1, sm - g1, g2))
            out = [None] * NPT
            for a in range(4):
                cy = 0.5 if a in (1, 2) else 1.0
                h0, h1, h2 = (hs[j][a] for j in range(3))
                sm = h0 + h2
                pp = h0 * (cy / 24.0) + h2 * (cy / 6.0)
                qq = h1 * (cy / 12.0)
                for b, val in enumerate((h0 * (cy / 4.0), (sm + h1) * (-cy / 6.0), (sm - h1) * (-cy / 6.0),
                                         pp + qq, pp - qq, h2 if cy == 1.0 else h2 * cy)):
                    out[NB * a + b] = val
            res.append(out)
        for k2 in range(NPT):
            val = pltpu.pack_elementwise([res[0][k2], res[1][k2]], packed_dtype=bf16)
            if isinstance(u_ref, (list, tuple)):
                u_ref[k2][orow, cs] = val
            else:
                u_ref[k2, orow, cs] = val

    def stat_acc(v, state, marker=None):
        n = v.shape[0] // 8
        wd = v.shape[1]
        if state is None:
            K = v[0:1, :]
            if marker is not None:
                K = K + marker[0:1, :]
            d = v - K
            return (K, d.reshape(n, 8, wd).sum(axis=0), (d * d).reshape(n, 8, wd).sum(axis=0))
        K, s1, s2 = state
        Kd = K if marker is None else K + marker[0:1, :]
        d = v - Kd
        return (K, s1 + d.reshape(n, 8, wd).sum(axis=0), s2 + (d * d).reshape(n, 8, wd).sum(axis=0))

    def store_stats(st_ref, q, t, cs, state):
        K, s1, s2 = state
        wd = K.shape[1]
        st_ref[q, t, 0, :, cs] = jnp.broadcast_to(K, (8, wd))
        st_ref[q, t, 1, :, cs] = jnp.broadcast_to(s1.sum(axis=0, keepdims=True), (8, wd))
        st_ref[q, t, 2, :, cs] = jnp.broadcast_to(s2.sum(axis=0, keepdims=True), (8, wd))

    def finalize(st_ref, p_ref, gb_ref, e_ref, q):
        cv = q // 2 if isinstance(q, int) else lax.shift_right_logical(q, 1)
        for g in range(G):
            cs = slice(g * 128, (g + 1) * 128)
            K = st_ref[q, :, 0, :, cs]
            s1 = st_ref[q, :, 1, :, cs]
            s2 = st_ref[q, :, 2, :, cs]
            e = e_ref[q, :, cs]
            mean_t = K + s1 * (1.0 / TM) + e[None]
            m2_t = s2 - s1 * s1 * (1.0 / TM)
            mu = jnp.sum(jnp.sum(mean_t, axis=0), axis=1, keepdims=True) * (1.0 / (T * 128))
            dev = mean_t - mu[None]
            tot = m2_t + dev * dev * float(TM)
            var = jnp.sum(jnp.sum(tot, axis=0), axis=1, keepdims=True) * (1.0 / (HW * 128))
            rstd = lax.rsqrt(var + EPS)
            sc = gb_ref[cv, 0, :, cs] * (rstd * 0.5)
            p_ref[q, 0, :, cs] = sc
            p_ref[q, 1, :, cs] = gb_ref[cv, 1, :, cs] * 0.5 - (mu - e) * sc

    def merge(lists):
        items = []
        for li, l in enumerate(lists):
            for i, it in enumerate(l):
                items.append(((i + 0.5) / len(l), li, it))
        items.sort(key=lambda z: (z[0], z[1]))
        return [it for _, _, it in items]

    def kern(x_hbm, te_hbm, g1_hbm, b1_hbm, w1_hbm, we_hbm, g2_hbm, b2_hbm, w2_hbm, o_hbm,
             s_ref, w_ref, u2_ref, ar_ref, xr_ref, va_ref, vb_ref, ya_ref, yb_ref,
             st_ref, p_ref, gb_ref, e_ref, te_ref, we_ref, gsm_ref, sem_x, sem_w, sem_s, sem_o, sem_x1, *u1_ref):

        def gcols(g):
            return pl.ds(mult(g * 128, 128), 128)

        def x0_copy(c):
            rows = pl.ds(mult(c * (TM // XC), TM // XC), TM // XC)
            return pltpu.make_async_copy(x_hbm.at[0, rows, :], s_ref.at[0, rows, :], sem_x.at[c])

        def w1_copy(g):
            return pltpu.make_async_copy(w1_hbm.at[:, gcols(g), :], w_ref.at[pl.ds(0, 9), gcols(g), :], sem_w.at[g])

        def x1_copy(c):
            rows = pl.ds(mult(c * TM, TM), TM)
            return pltpu.make_async_copy(x_hbm.at[1, rows, :], s_ref.at[1, rows, :], sem_x1.at[c])

        def w2_copy():
            return pltpu.make_async_copy(w2_hbm, w_ref.at[pl.ds(9, 9)], sem_s.at[7])

        def small_copies():
            return [pltpu.make_async_copy(g1_hbm, gsm_ref.at[0], sem_s.at[0]),
                    pltpu.make_async_copy(b1_hbm, gsm_ref.at[1], sem_s.at[1]),
                    pltpu.make_async_copy(g2_hbm, gsm_ref.at[2], sem_s.at[2]),
                    pltpu.make_async_copy(b2_hbm, gsm_ref.at[3], sem_s.at[3]),
                    pltpu.make_async_copy(te_hbm, te_ref, sem_s.at[4])]

        def we_copy():
            return pltpu.make_async_copy(we_hbm, we_ref, sem_s.at[5])

        def o_copy(s, qi):
            b = divT(s) - 2
            r0 = mult(modT(s) * TM + qi * QR, QR)
            return pltpu.make_async_copy(s_ref.at[b, pl.ds(r0, QR), :], o_hbm.at[b, pl.ds(r0, QR), :], sem_o.at[0])

        def o_all():
            return pltpu.make_async_copy(s_ref.at[pl.ds(0, B)], o_hbm, sem_o.at[0])

        def epi_piece(y_ref, s_prev, kind, r, cb, state, marker, PW=PW):
            p = divT(s_prev)
            t = modT(s_prev)
            cs = lanes(cb, PW)
            j, par = r // 2, r % 2
            r0 = mult(t * TM + r * W, W)
            ve = load_y(y_ref, par, 0, j, cb * (PW // 128), PW // 128)
            vo = load_y(y_ref, par, 1, j, cb * (PW // 128), PW // 128)
            if marker is not None:
                ve = (ve.reshape(HP // 8, 8, PW) + marker[None]).reshape(HP, PW)
            if kind == 1:
                dst, sq = p + 2, p + 2
            elif kind == 2:
                dst, sq = p - 2, None
                xe, xo = split_eo(s_ref[dst, pl.ds(r0, W), cs])
                ve, vo = ve + xe, vo + xo
            else:
                is2 = p >= 2
                dst = jnp.where(is2, p - 2, p + 2)
                sq = jnp.where(is2, 0, p + 2)
                xe, xo = split_eo(s_ref[dst, pl.ds(r0, W), cs])
                ve, vo = ve + jnp.where(is2, xe, 0.0), vo + jnp.where(is2, xo, 0.0)
            if sq is not None:
                state = stat_acc(vo, stat_acc(ve, state))
            s_ref[dst, pl.ds(r0, W), cs] = join_eo(ve, vo)
            if sq is not None and r == TR - 1:
                store_stats(st_ref, sq, t, cs, state)
                state = None
            return state

        def xstat_piece(q, tile, cs, ri, state, marker):
            r0 = mult(tile * TM + ri * XR1, XR1)
            v = s_ref[q, pl.ds(r0, XR1), cs].astype(f32)
            state = stat_acc(v, state, marker)
            if ri == TM // XR1 - 1:
                store_stats(st_ref, q, tile, cs, state)
                state = None
            return state

        def half(it, second, u_ref, vc_ref, vn_ref, yc_ref, yp_ref, conv=None):
            s = 2 * it + second
            sn = s + 1
            pn = jnp.minimum(divT(sn), 3)
            y0 = modT(sn) * TR
            plist = [pc for cb in range(G) for pc in prod_list(cb)]
            lists = [plist,
                     [('e', r, cb) for r in range(TR) for cb in range(NPW)]]
            NU = -(-NUB // (5 if conv is None else 6))
            if UMODE == 0 and conv != 1:
                lists.append([('u', k) for k in range(NU)])
            pieces = merge(lists)
            npc = len(pieces)
            if second == 1:
                finalize(st_ref, p_ref, gb_ref, e_ref, jnp.minimum(divT(s - 1) + 1, 3))
            pv = tuple(p_ref[pn, k] for k in range(2))
            sp = s - 1
            ekind = 0 if conv is None else (1 if conv in (0, 2) else (0 if second == 0 else 2))
            wts = [{0: WH, 1: WH, 2: 100, 3: WH, 4: W4, 5: W5A if k // NB < 2 else W5B}[k % NB] for k in range(NPT)]
            cum = [sum(wts[:k]) for k in range(NPT + 1)]
            done = 0
            est = [None] * NPW
            xst = None
            pcar = None
            ys = [None] * 8
            for a in range(4):
                st = {}
                for b in range(NB):
                    k = NB * a + b
                    d = lax.dot_general(pltpu.bitcast(vc_ref[k], bf16), pltpu.bitcast(u_ref[k][...] if conv != 1 else u_ref[k, 0:C // 2, :], bf16), NT,
                                        preferred_element_type=f32)
                    for nn in range(4 * SUB):
                        n, sub = nn // SUB, nn % SUB
                        hi_ = min(npc, ((cum[k] * 4 * SUB + wts[k] * (nn + 1)) * npc * 64) // (last_slot * cum[NPT] * 4 * SUB))
                        while done < hi_:
                            pc = pieces[done]
                            if pc[0] == 'a':
                                cs = slice(pc[1] * 128, (pc[1] + 1) * 128)
                                prod_a(s_ref, tuple(t[:, cs] for t in pv), ar_ref, xr_ref, pn, y0, pc[1], pc[2],
                                       marker_of(d, n, sub, 128))
                            elif pc[0] == 'b':
                                prod_b(xr_ref, vn_ref, pc[1], pc[2], pc[3], marker_of(d, n, sub, 128))
                            elif pc[0] == 'e':
                                est[pc[2]] = epi_piece(yp_ref, sp, ekind, pc[1], pc[2], est[pc[2]],
                                                       marker_of(d, n, sub, PW))
                                if pc[2] == NPW - 1 and ((pc[1] + 1) * W) % QR == 0 and conv not in (0, 2):
                                    qi = ((pc[1] + 1) * W) // QR - 1

                                    @pl.when(sp >= 2 * T)
                                    def _():
                                        o_copy(sp, qi).start()
                            elif pc[0] == 'x':
                                xst = xstat_piece(jnp.where(it == 0, 0, 1), pc[1],
                                                  slice(pc[2] * PW, (pc[2] + 1) * PW), pc[3], xst,
                                                  marker_of(d, n, sub, PW))
                            else:
                                kk = (s - 2) * NU + pc[1]
                                ok = jnp.logical_and(kk >= 0, kk < NUB)
                                u_piece(w_ref, u2_ref, 9, jnp.clip(kk, 0, NUB - 1),
                                        marker_of(d, n, sub, 128), ok)
                            done += 1
                    rr = out_x(st, b, d)

                def store(par, q, val):
                    for n in range(G):
                        store_y(yc_ref, par, q, n, val[:, n * 128:(n + 1) * 128])
                out_y(ys, a, rr, store)

        def emb_part():
            te = te_ref[...].astype(f32)
            sl = te * jax.nn.sigmoid(te)
            emb = jnp.dot(sl.astype(bf16), we_ref[...], preferred_element_type=f32)
            e_ref[2] = jnp.broadcast_to(emb[0:1, :], (8, C))
            e_ref[3] = jnp.broadcast_to(emb[1:2, :], (8, C))

        def nhalf(step, n, vc_ref, vn_ref, yc_ref, yp_ref, with_u=True):
            y0 = (step + 1) * TR
            if step == 0 and P0 == 1:
                lists = [] if with_u else [[pc for cb in range(G) for pc in prod_list(cb)]]
            else:
                lists = [prod_list(None)]
            if step == 0:
                if with_u:
                    lists.append([('u', k) for k in range(NUB // G)])
            else:
                lists.append([('e', r) for r in range(TR)])
                lists.append([('x', cb, ri) for cb in range(NPW) for ri in range(TM // XR1)])
            pieces = merge(lists)
            npc = len(pieces)
            cs = lanes(n)
            pvc = tuple(p_ref[0, k, :, cs] for k in range(2))
            urows = pl.ds(mult(n * (128 // 2), 128 // 2), 128 // 2)
            gn = n + 1 if PEEL0 else jnp.minimum(n + 1, G - 1)
            NS = NSUB
            done = 0
            est = xst = None
            ys = [None] * 8
            dhist = []
            for a in range(4):
                st = {}
                for b in range(NB):
                    k = NB * a + b
                    d = lax.dot_general(pltpu.bitcast(vc_ref[k], bf16), pltpu.bitcast(u1_ref[k][urows, :], bf16), NT,
                                        preferred_element_type=f32)
                    for sub in range(NS):
                        lag = LAG if with_u and step == 0 else 1
                        hi_ = npc if k == NPT - 1 and sub == NS - 1 else (((k - lag + 1) * NS + sub) * npc) // ((NPT - lag) * NS)
                        dprev = dhist[k - lag] if k >= lag else None
                        while done < min(hi_, npc) and dprev is not None:
                            pc = pieces[done]
                            rp = sub * (M // NS) // 8 * 8
                            bits = pltpu.bitcast(dprev[rp:rp + 8, :], u32)
                            mk = pltpu.bitcast((bits >> 16) >> 16, f32)
                            if pc[0] == 'a':
                                cbp = n if pc[1] is None else pc[1]
                                pvp = pvc if pc[1] is None else tuple(p_ref[0, k_, :, lanes(cbp)] for k_ in range(2))
                                prod_a(s_ref, pvp, ar_ref, xr_ref, 0, y0, cbp, pc[2], mk)
                            elif pc[0] == 'b':
                                prod_b(xr_ref, vn_ref, n if pc[1] is None else pc[1], pc[2], pc[3], mk)
                            elif pc[0] == 'u':
                                u_piece(w_ref, u1_ref, 0, gn * (NUB // G) + pc[1], mk)
                            elif pc[0] == 'e':
                                est = epi_piece(yp_ref, 0, 1, pc[1], n, est, mk, PW=128)
                            else:
                                mkx = mk if PW == 128 else jnp.concatenate([mk] * (PW // 128), axis=1)
                                xst = xstat_piece(1, n, slice(pc[1] * PW, (pc[1] + 1) * PW), pc[2], xst, mkx)
                            done += 1
                    dhist.append(d)
                    rr = out_x(st, b, d)
                out_y(ys, a, rr, lambda par, q, val: store_y(yc_ref, par, q, n, val))
            assert done == npc
            if step == 0 and not with_u and EMB0:
                emb_part()

        def xstat_tile0(c):
            st = [None] * NPW
            rows_per = TM // XC
            for h in range(XC):
                x0_copy(c * XC + h).wait()
                for ri in range(rows_per // XR):
                    r0 = pl.multiple_of(c * TM + h * rows_per + ri * XR, XR)
                    for cb in range(NPW):
                        v = s_ref[0, pl.ds(r0, XR), cb * PW:(cb + 1) * PW].astype(f32)
                        st[cb] = stat_acc(v, st[cb])
            for cb in range(NPW):
                store_stats(st_ref, 0, c, slice(cb * PW, (cb + 1) * PW), st[cb])
            return 0

        with scope('prologue'):
            for c in small_copies():
                c.start()
            lax.fori_loop(0, T * XC, lambda c, _: (x0_copy(c).start(), 0)[1], 0)
            lax.fori_loop(0, G, lambda g, _: (w1_copy(g).start(), 0)[1], 0)

            def rest(c, _):
                @pl.when(c == (1 if EMB0 else 0))
                def _():
                    lax.fori_loop(0, T, lambda c_, _: (x1_copy(c_).start(), 0)[1], 0)

                @pl.when(c == (2 if EMB0 else 1))
                def _():
                    w2_copy().start()

                @pl.when(c == (0 if EMB0 else 2))
                def _():
                    we_copy().start()
                return 0
            lax.fori_loop(0, 3, rest, 0)

            for c in small_copies():
                c.wait()
            for cv in range(2):
                for k in range(2):
                    v = gsm_ref[2 * cv + k].astype(f32)
                    for g in range(G):
                        gb_ref[cv, k, :, g * 128:(g + 1) * 128] = jnp.broadcast_to(v[g:g + 1, :], (8, 128))
            e_ref[...] = jnp.zeros(e_ref.shape, f32)
            st_ref[...] = jnp.zeros(st_ref.shape, f32)

            lax.fori_loop(0, T, lambda c, _: xstat_tile0(c), 0)
            finalize(st_ref, p_ref, gb_ref, e_ref, 0)

            PU = opts.get('pu', 4)

            def prod0(c2, _):
                for i in range(PU):
                    cb = c2 * PU + i
                    pvc = tuple(p_ref[0, k, :, gcols(cb)] for k in range(2))
                    for pc in prod_list(cb):
                        if pc[0] == 'a':
                            prod_a(s_ref, pvc, ar_ref, xr_ref, 0, 0, cb, pc[2], None, i)
                        else:
                            prod_b(xr_ref, va_ref, cb, pc[2], pc[3], None, i)
                return 0
            lax.fori_loop(0, G // PU, prod0, 0)

            w1_copy(0).wait()
            lax.fori_loop(0, NUB // G, lambda k, _: (u_piece(w_ref, u1_ref, 0, k, None), 0)[1], 0, unroll=opts.get('uu', 4))

        def step0(n, _):
            if PEEL0:
                w1_copy(n + 1).wait()
            else:
                @pl.when(n < G - 1)
                def _():
                    w1_copy(n + 1).wait()
            nhalf(0, n, va_ref, vb_ref, ya_ref, yb_ref)
            return 0

        def step1(n, _):
            x1_copy(n).wait()
            nhalf(1, n, vb_ref, va_ref, yb_ref, ya_ref)
            return 0

        with scope('step0'):
            if PEEL0:
                lax.fori_loop(0, G - 1, step0, 0)
                if EMB0:
                    we_copy().wait()
                nhalf(0, G - 1, va_ref, vb_ref, ya_ref, yb_ref, False)
            else:
                lax.fori_loop(0, G, step0, 0)
        with scope('step1'):
            lax.fori_loop(0, G, step1, 0)

        def emb_block():
            w2_copy().wait()
            if not EMB0:
                we_copy().wait()
                emb_part()

        def body(it, carry):
            @pl.when(it == 1)
            def _():
                emb_block()

            @pl.when(it == T)
            def _():
                if UMODE == 0:
                    def cp(rb, _):
                        rows = pl.ds(pl.multiple_of(rb * 32, 32), 32)
                        for k in range(NPT):
                            u1_ref[k][rows, :] = u2_ref[k, rows, :]
                        return 0
                    lax.fori_loop(0, C // 2 // 32, cp, 0)
                else:
                    lax.fori_loop(0, NUB, lambda k, _: (u_piece(w_ref, u1_ref, 9, k, None), 0)[1], 0)
            with scope('iter'):
                half(it, 0, u1_ref, va_ref, vb_ref, ya_ref, yb_ref)
                half(it, 1, u1_ref, vb_ref, va_ref, yb_ref, ya_ref)
            return carry

        def body_c(conv):
            def f(it, carry):
                if conv == 0:
                    @pl.when(it == 1)
                    def _():
                        emb_block()
                ur = u2_ref if conv == 1 else u1_ref
                with scope('iter'):
                    half(it, 0, ur, va_ref, vb_ref, ya_ref, yb_ref, conv)
                    half(it, 1, ur, vb_ref, va_ref, yb_ref, ya_ref, conv)
                return carry
            return f

        with scope('main'):
            if SPLIT:
                if SPLIT == 2:
                    emb_block()
                lax.fori_loop(1, T, body_c(0 if SPLIT == 1 else 2), 0)
                lax.fori_loop(T, 2 * T, body_c(1), 0)
            else:
                lax.fori_loop(1, 2 * T, body, 0)

        sl_ = NSTEP - 1
        with scope('final'):
            st = [None] * NPW
            for r in range(TR):
                for cb in range(NPW):
                    st[cb] = epi_piece(yb_ref, sl_, 2, r, cb, st[cb], None)
                if FROW:
                    if (r + 1) % FROW == 0:
                        rows = pl.ds((T - 1) * TM + (r + 1 - FROW) * W, FROW * W)
                        pltpu.make_async_copy(s_ref.at[B - 1, rows, :], o_hbm.at[B - 1, rows, :], sem_o.at[0]).start()
                elif ((r + 1) * W) % QR == 0:
                    o_copy(sl_, ((r + 1) * W) // QR - 1).start()
        with scope('owait'):
            o_all().wait()

    def fn(x, t_emb, g1, be1, w1, w_emb, g2, be2, w2):
        xn = jnp.transpose(x, (0, 2, 3, 1)).reshape(B, HW, C)
        w1t = jnp.transpose(w1, (2, 3, 0, 1)).reshape(9, C, C)
        w2t = jnp.transpose(w2, (2, 3, 0, 1)).reshape(9, C, C)
        any_spec = pl.BlockSpec(memory_space=pl.ANY)
        ubuf = pltpu.VMEM((C // 2, C), u32)
        vbuf = pltpu.VMEM((NPT, M // 2, C), u32)
        ybuf = pltpu.VMEM((2, 2, G, 2 * M, 128), f32)
        out = pl.pallas_call(
            kern,
            in_specs=[any_spec] * 9,
            out_specs=any_spec,
            out_shape=jax.ShapeDtypeStruct((B, HW, C), bf16),
            scratch_shapes=[
                pltpu.VMEM((4, HW, C), bf16),
                pltpu.VMEM((18, C, C), bf16),
                pltpu.VMEM((NPT, (C // 2 + UB // 2) if UMODE == 0 else 8, C), u32),
                pltpu.VMEM((G, NAR, 2, HP, 128), f32),
                pltpu.VMEM((G, TR + 2, NB, NQ4, 128), f32),
                vbuf, vbuf, ybuf, ybuf,
                pltpu.VMEM((4, T, 3, 8, C), f32),
                pltpu.VMEM((4, 2, 8, C), f32),
                pltpu.VMEM((2, 2, 8, C), f32),
                pltpu.VMEM((4, 8, C), f32),
                pltpu.VMEM((B, E), bf16),
                pltpu.VMEM((E, C), bf16),
                pltpu.VMEM((4, G, 128), bf16),
                pltpu.SemaphoreType.DMA((T * XC,)),
                pltpu.SemaphoreType.DMA((G,)),
                pltpu.SemaphoreType.DMA((8,)),
                pltpu.SemaphoreType.DMA((1,)),
                pltpu.SemaphoreType.DMA((T,)),
            ] + [ubuf] * NPT,
            compiler_params=pltpu.CompilerParams(vmem_limit_bytes=100 * 1024 * 1024,
                                                 disable_bounds_checks=True),
        )(xn, t_emb, g1.reshape(G, 128), be1.reshape(G, 128), w1t, w_emb,
          g2.reshape(G, 128), be2.reshape(G, 128), w2t)
        return jnp.transpose(out.reshape(B, H, W, C), (0, 3, 1, 2))
    return fn


_OPTS = {}


@jax.jit
def pallas_standalone__adm_resblock__diffusion_kernel(x, t_emb, g1, be1, w1, w_emb, g2, be2, w2):
    B, C, H, W = x.shape
    E = t_emb.shape[1]
    return build(B, C, H, W, E, TM=1024, opts=_OPTS)(x, t_emb, g1, be1, w1, w_emb, g2, be2, w2)
```
